```python
import jax
import jax.numpy as jnp

def _softmax(x, axis=-1):
    return jax.nn.softmax(x, axis=axis)

def _gelu(x):
    return jax.nn.gelu(x, approximate=True)

def _silu(x):
    return jax.nn.silu(x)

def _sigmoid(x):
    return jax.nn.sigmoid(x)

def _layernorm(x, axis=-1, eps=1e-05):
    m = jnp.mean(x, axis=axis, keepdims=True)
    v = jnp.var(x, axis=axis, keepdims=True)
    return (x - m) / jnp.sqrt(v + eps)

def _scatter_add(tgt, idx, src, axis=0):
    return tgt.at[idx].add(src)

def _segment_sum(src, seg, n):
    return jax.ops.segment_sum(src, seg, n)

class _Rng:

    def __init__(self, key):
        self._k = key

    def _next(self):
        self._k, sub = jax.random.split(self._k)
        return sub

    def normal(self, shape):
        return jax.random.normal(self._next(), shape, dtype=jnp.bfloat16)

    def randint(self, lo, hi, shape):
        return jax.random.randint(self._next(), shape, lo, hi, dtype=jnp.int32)

    def uniform(self, shape, lo=0.0, hi=1.0):
        return jax.random.uniform(self._next(), shape, jnp.bfloat16, lo, hi)

    def permutation(self, n):
        return jax.random.permutation(self._next(), n)
kernel_name = 'adaLN_cond__memory_aug_recurrent_mem_tr__mixer_s_mlp__prompt'

def setup_inputs():
    _rng = _Rng(jax.random.key(int.from_bytes(__import__("os").urandom(4), "little")))
    _w = lambda a: (lambda t: t.astype(jnp.bfloat16) if jnp.issubdtype(t.dtype, jnp.floating) else t)(jnp.asarray(a))

    def _A_setup():
        B, S, Dm = (1, 2048, 1024)
        H, Dh = (32, 128)
        M, seg = (8, 32)
        seg = min(seg, S)
        S = S // seg * seg
        return {'x': _w((lambda *s: _rng.normal(s) * 0.05)(B, S, Dm)), 'mem0': _w((lambda *s: _rng.normal(s) * 0.05)(B, M, Dm)), 'Wq': _w((lambda *s: _rng.normal(s) * 0.05)(Dm, H, Dh) * Dm ** (-0.5)), 'Wk': _w((lambda *s: _rng.normal(s) * 0.05)(Dm, H, Dh) * Dm ** (-0.5)), 'Wv': _w((lambda *s: _rng.normal(s) * 0.05)(Dm, H, Dh) * Dm ** (-0.5)), 'Wo': _w((lambda *s: _rng.normal(s) * 0.05)(H, Dh, Dm) * (H * Dh) ** (-0.5)), 'seg_len': seg}
    _A_in = _A_setup()

    def _B_setup():
        B, S, D, F = (1, 2048, 1024, 3584)
        return {'x': _w((lambda *s: _rng.normal(s) * 0.05)(B, S, D)), 'w1': _w((lambda *s: _rng.normal(s) * 0.05)(D, D) * D ** (-0.5)), 'w2': _w((lambda *s: _rng.normal(s) * 0.05)(D, D) * D ** (-0.5)), 'w3': _w((lambda *s: _rng.normal(s) * 0.05)(D, F) * D ** (-0.5)), 'w4': _w((lambda *s: _rng.normal(s) * 0.05)(F, D) * F ** (-0.5))}
    _B_in = _B_setup()
    return {'A_x': _A_in['x'], 'A_mem0': _A_in['mem0'], 'A_Wq': _A_in['Wq'], 'A_Wk': _A_in['Wk'], 'A_Wv': _A_in['Wv'], 'A_Wo': _A_in['Wo'], 'A_seg_len': _A_in['seg_len'], 'B_x': _B_in['x'], 'B_w1': _B_in['w1'], 'B_w2': _B_in['w2'], 'B_w3': _B_in['w3'], 'B_w4': _B_in['w4'], 'c': _w((lambda *s: _rng.normal(s) * 0.05)(1, 1024)), 'w_mod': _w((lambda *s: _rng.normal(s) * 0.05)(1024, 6 * 1024) * 1024 ** (-0.5))}

def reference(A_x, A_mem0, A_Wq, A_Wk, A_Wv, A_Wo, A_seg_len, B_x, B_w1, B_w2, B_w3, B_w4, c, w_mod):

    def _A_ref(x, mem0, Wq, Wk, Wv, Wo, seg_len):
        B, S, Dm = x.shape
        H, Dh = (Wq.shape[1], Wq.shape[2])
        M = mem0.shape[1]
        scale = Dh ** (-0.5)
        n_seg = S // seg_len
        L = M + seg_len
        idx = jnp.arange(L)
        mask = (idx[:, None] < M) | (idx[:, None] >= idx[None, :])
        mem = mem0
        outs = []
        for s in range(n_seg):
            xs = x[:, s * seg_len:(s + 1) * seg_len, :].copy()
            h = jnp.concatenate([mem, xs], axis=1)
            q = jnp.einsum('btd,dhe->bhte', h, Wq)
            k = jnp.einsum('btd,dhe->bhte', h, Wk)
            v = jnp.einsum('btd,dhe->bhte', h, Wv)
            scores = jnp.einsum('bhqe,bhke->bhqk', q, k) * scale
            scores = jnp.where(mask[None, None], scores, -1000000000.0)
            p = _softmax(scores, axis=-1)
            o = jnp.einsum('bhqk,bhke->bhqe', p, v)
            o = jnp.einsum('bhte,hed->btd', o, Wo)
            mem = o[:, :M, :].copy()
            outs.append(o[:, M:, :])
        return jnp.concatenate(outs, axis=1)

    def _B_ref(x, w1, w2, w3, w4):
        B, S, D = x.shape
        h = _gelu(_layernorm(x, axis=-1) @ w1)
        c = D // 4
        g0 = jnp.pad(h[:, :, 0 * c:1 * c], ((0, 0), (1, 0), (0, 0)))[:, :S, :]
        g1 = jnp.pad(h[:, :, 1 * c:2 * c], ((0, 0), (0, 1), (0, 0)))[:, 1:, :]
        g2 = jnp.pad(h[:, :, 2 * c:3 * c], ((0, 0), (2, 0), (0, 0)))[:, :S, :]
        g3 = jnp.pad(h[:, :, 3 * c:], ((0, 0), (0, 2), (0, 0)))[:, 2:, :]
        hs = jnp.concatenate([g0, g1, g2, g3], axis=-1) @ w2
        x1 = x + hs
        h2 = _gelu(_layernorm(x1, axis=-1) @ w3) @ w4
        return x1 + h2
    x = A_x
    mod = (_silu(c) @ w_mod).reshape(c.shape[0], 6, 1, -1)
    sa, ca, ga, sb, cb, gb = (mod[:, 0].copy(), mod[:, 1].copy(), mod[:, 2].copy(), mod[:, 3].copy(), mod[:, 4].copy(), mod[:, 5].copy())
    h = _layernorm(x, axis=-1) * (1 + ca) + sa
    x = x + ga * _A_ref(h, A_mem0, A_Wq, A_Wk, A_Wv, A_Wo, A_seg_len)
    h = _layernorm(x, axis=-1) * (1 + cb) + sb
    x = x + gb * _B_ref(h, B_w1, B_w2, B_w3, B_w4)
    return x
```

```python
import functools

import jax
import jax.numpy as jnp
from jax import lax
import jax.experimental.pallas as pl
import jax.experimental.pallas.tpu as pltpu

bf16, f32, u32 = jnp.bfloat16, jnp.float32, jnp.uint32

S, D, H, DH, MEM, SEG, F = 2048, 1024, 32, 128, 8, 32, 3584
NSEG = S // SEG
XR = 24
PRE = S - XR * NSEG
RING = 576
QOFF = RING - PRE
OOFF = 192
PITCH = 520
NT = D // 128
NF = F // 128
BM = 128
NB = S // BM
GH = 4
NPAIR = H // 2
EPS = 1e-5
SCALE = DH ** -0.5


def _ln(x):
    m = jnp.mean(x, axis=-1, keepdims=True)
    xc = x - m
    v = jnp.mean(xc * xc, axis=-1, keepdims=True)
    return xc * lax.rsqrt(v + EPS)


def _gelu(x):
    return jax.nn.gelu(x, approximate=True)


def _dot(a, b):
    return jnp.dot(a, b, preferred_element_type=f32)


def _kernel(x_hbm, mem0_hbm, wq_hbm, wk_hbm, wv_hbm, wo_hbm, w1_hbm, w2_hbm, w3_hbm, w4_hbm,
            c_hbm, wmod_hbm, out_hbm,
            x_v, a_v, h0_v, lhs_v, c_v, mem0_v, mod_v, wmod_v, wa_v, wb_v, wo_v,
            w1_v, w2_v, w3_v, w4_v,
            sem_small, sem_x, sem_stage, sem_mod, sem_w, sem_out):
    wqkv_hbm = (wq_hbm, wk_hbm, wv_hbm)

    c_cp = pltpu.make_async_copy(c_hbm, c_v, sem_small.at[0])
    mem0_cp = pltpu.make_async_copy(mem0_hbm, mem0_v, sem_small.at[1])
    X0 = PRE + 128
    x0_cp = pltpu.make_async_copy(x_hbm.at[pl.ds(0, X0)], x_v.at[pl.ds(0, X0)], sem_x.at[0])
    x1_cp = pltpu.make_async_copy(x_hbm.at[pl.ds(X0, S - X0)], x_v.at[pl.ds(X0, S - X0)],
                                  sem_x.at[1])

    def slab_cp(src, dst, n, sem):
        col = n * 128 if isinstance(n, int) else pl.multiple_of(n * 128, 128)
        return pltpu.make_async_copy(src.at[:, pl.ds(col, 128)], dst.at[n], sem)

    def mod_cps(lo, hi, k):
        return [slab_cp(wmod_hbm, wmod_v, n, sem_mod.at[k]) for n in range(lo, hi)]

    def mod_compute(lo, hi):
        cf = c_v[...].astype(f32)
        sc = (cf * jax.nn.sigmoid(cf)).astype(bf16)
        sc = jnp.broadcast_to(sc, (8, D))
        for n in range(lo, hi):
            mod_v[:, n * 128:(n + 1) * 128] = _dot(sc, wmod_v[n])

    def mod(k):
        return mod_v[0:1, k * D:(k + 1) * D]

    def h_rows(r0, n):
        return (_ln(x_v[pl.ds(r0, n), :].astype(f32)) * (1.0 + mod(1)) + mod(0)).astype(bf16)

    def phase_a(stage, *rr):
        rings, orings = rr[:8], rr[8:]

        def stage_cp(t, hh, piece):
            d0 = piece * 256 if isinstance(piece, int) else pl.multiple_of(piece * 256, 256)
            return pltpu.make_async_copy(
                wqkv_hbm[t].at[pl.ds(d0, 256), pl.ds(hh * 16, 16), :],
                stage.at[hh, pl.ds(d0, 256)], sem_stage.at[hh, piece])

        def repack(hh, dst, t, p0, n):
            for u in range(n):
                p = p0 + u
                a = pltpu.bitcast(stage[hh, 2 * p], u32)
                b = pltpu.bitcast(stage[hh, 2 * p + 1], u32)
                ev = (a & jnp.uint32(0xFFFF)) | (b << 16)
                od = (a >> 16) | (b & jnp.uint32(0xFFFF0000))
                dst[pl.ds(t * (16 * PITCH) + p, 8, stride=PITCH), :] = ev
                dst[pl.ds(t * (16 * PITCH) + 8 * PITCH + p, 8, stride=PITCH), :] = od

        def w_slab(t, h):
            src = wa_v if h < 16 else wb_v
            l = h % 16
            slot = (l % 2) * 8 + l // 2
            base = (t * 16 + slot) * PITCH
            if not isinstance(base, int):
                base = pl.multiple_of(base, 8)
            return pltpu.bitcast(src[pl.ds(base, D // 2), :], bf16)

        def ring_of(t, h):
            return rings[(h // 2) % 8], t * 4 + (h // 16) * 2 + h % 2

        c_cp.start()
        mem0_cp.start()
        x0_cp.start()
        for k in range(4):
            stage_cp(0, 0, k).start()
        for cp in mod_cps(0, 16, 0):
            cp.start()
        for k in range(4):
            stage_cp(0, 1, k).start()

        def first_repack(k, c):
            stage_cp(0, 0, k).wait()

            def inner(i, cc):
                repack(0, wa_v, 0, k * 128 + i * 16, 16)
                return cc
            lax.fori_loop(0, 8, inner, 0)
            stage_cp(1, 0, k).start()
            return c
        lax.fori_loop(0, 4, first_repack, 0)

        c_cp.wait()
        mem0_cp.wait()
        x0_cp.wait()
        for cp in mod_cps(0, 16, 0):
            cp.wait()
        mod_compute(0, 16)

        def h0_body(i, c):
            r0 = pl.multiple_of(i * 32, 32)
            for u in range(2):
                h0_v[pl.ds(r0 + 16 * u, 16), :] = h_rows(r0 + 16 * u, 16)
            return c
        lax.fori_loop(0, PRE // 32, h0_body, 0)
        lhs_v[0:XR, :] = h_rows(PRE, XR)
        lhs_v[XR:XR + MEM, :] = mem0_v[...]

        def pre_sub(t, hh):
            nh = 1 - hh
            tn = t if hh == 0 else jnp.minimum(t + 1, 2)
            dst = wb_v if hh == 0 else wa_v

            def body(it, c):
                if hh == 0:
                    stage_cp(0, nh, it).wait()
                else:
                    @pl.when(t < 2)
                    def _():
                        stage_cp(0, nh, it).wait()
                r0 = pl.multiple_of(it * BM, BM)
                for l in range(16):
                    h = hh * 16 + l
                    y = _dot(h0_v[pl.ds(r0, BM), :], w_slab(t, h))
                    rg, ix = ring_of(t, h)
                    rg[ix, pl.ds(QOFF + r0, BM), :] = y.astype(bf16)
                    repack(nh, dst, tn, it * 128 + l * 8, 8)
                for tt in range(1, 3):
                    @pl.when(t + 1 + hh == tt)
                    def _():
                        stage_cp(tt, nh, it).start()
                @pl.when(t == 0)
                def _():
                    slab_cp(wo_hbm, wo_v, hh * 4 + it, sem_w.at[0]).start()
                return c
            lax.fori_loop(0, 4, body, 0)

        def pre_body(t, c):
            pre_sub(t, 0)
            pre_sub(t, 1)

            @pl.when(t == 0)
            def _():
                x1_cp.start()
            return c
        lax.fori_loop(0, 3, pre_body, 0)

        for cp in mod_cps(16, 48, 1):
            cp.start()
        for n in range(NT):
            slab_cp(w1_hbm, w1_v, n, sem_w.at[1]).start()
        for n in range(NT):
            slab_cp(w2_hbm, w2_v, n, sem_w.at[2]).start()
        for n in range(NF):
            slab_cp(w3_hbm, w3_v, n, sem_w.at[3]).start()
        for n in range(NT):
            slab_cp(w4_hbm, w4_v, n, sem_w.at[4]).start()
        x1_cp.wait()
        for n in range(NT):
            slab_cp(wo_hbm, wo_v, n, sem_w.at[0]).wait()

        L2 = 2 * (SEG + MEM)
        r = lax.broadcasted_iota(jnp.int32, (L2, L2), 0)
        c = lax.broadcasted_iota(jnp.int32, (L2, L2), 1)
        r1 = ((r >= SEG) & (r < 2 * SEG)) | (r >= 2 * SEG + MEM)
        c1 = ((c >= SEG) & (c < 2 * SEG)) | (c >= 2 * SEG + MEM)
        same = r1 == c1
        mask = same & ((r >= 2 * SEG) | (c >= 2 * SEG) | (c <= r))
        fill = jnp.where(same, -1e9, -jnp.inf).astype(f32)

        def step(s, carry):
            woff = pl.multiple_of((XR * s) % RING, 8)
            roff = pl.multiple_of((SEG * s + QOFF) % RING, SEG)
            owr = pl.multiple_of((SEG * s + OOFF) % RING, SEG)
            ord_ = pl.multiple_of((XR * s + OOFF) % RING, 8)
            lhs = lhs_v[...]
            nxt = pl.multiple_of(PRE + XR * jnp.minimum(s + 1, NSEG - 1), 8)
            lhs_v[0:XR, :] = h_rows(nxt, XR)
            acc = [None] * NT
            ym, ps, om = {}, {}, {}

            def qkv(h):
                for t in range(3):
                    y = _dot(lhs, w_slab(t, h))
                    rg, ix = ring_of(t, h)
                    rg[ix, pl.ds(woff, XR), :] = y[0:XR].astype(bf16)
                    ym[(t, h)] = y[XR:XR + MEM]

            def get(t, p):
                rg, i0 = ring_of(t, 2 * p)
                _, i1 = ring_of(t, 2 * p + 1)
                mm = jnp.concatenate([ym.pop((t, 2 * p)), ym.pop((t, 2 * p + 1))], axis=0)
                return jnp.concatenate([rg[i0, pl.ds(roff, SEG), :], rg[i1, pl.ds(roff, SEG), :],
                                        mm.astype(bf16)], axis=0)

            def sm(p):
                sc = lax.dot_general(get(0, p), get(1, p), (((1,), (1,)), ((), ())),
                                     preferred_element_type=f32) * SCALE
                sc = jnp.where(mask, sc, fill)
                e = jnp.exp(sc - jnp.max(sc, axis=-1, keepdims=True))
                ps[p] = (e * (1.0 / jnp.sum(e, axis=-1, keepdims=True))).astype(bf16)

            def pv(p):
                o = _dot(ps.pop(p), get(2, p))
                for j in range(2):
                    h = 2 * p + j
                    orings[h // GH][h % GH, pl.ds(owr, SEG), :] = (
                        o[SEG * j:SEG * (j + 1)].astype(bf16))
                    om[h] = o[2 * SEG + MEM * j:2 * SEG + MEM * (j + 1)].astype(bf16)

            def wo(g):
                olg = jnp.concatenate(
                    [jnp.concatenate([orings[g][h % GH, pl.ds(ord_, XR), :], om.pop(h)], axis=0)
                     for h in range(g * GH, (g + 1) * GH)], axis=1)
                for n in range(NT):
                    y = _dot(olg, wo_v[n, g * GH * DH:(g + 1) * GH * DH, :])
                    acc[n] = y if acc[n] is None else acc[n] + y

            gd = [0]

            def big(h):
                if h < H:
                    qkv(h)
                else:
                    wo(gd[0])
                    gd[0] += 1

            for i in range(NPAIR + 3):
                big(2 * i)
                if 0 <= i - 3 < NPAIR:
                    pv(i - 3)
                if i < NPAIR + 2:
                    big(2 * i + 1)
                if 0 <= i - 1 < NPAIR:
                    sm(i - 1)
            while gd[0] < H // GH:
                big(H)
            res = jnp.concatenate(acc, axis=1).astype(bf16)
            a_v[pl.ds(pl.multiple_of(XR * s, 8), XR), :] = res[0:XR]
            lhs_v[XR:XR + MEM, :] = res[XR:XR + MEM]
            return carry
        lax.fori_loop(0, NSEG, step, 0)

        def tail(b, c):
            r0 = pl.multiple_of(b * BM, BM)
            for n in range(NT):
                o = jnp.concatenate([orings[h // GH][h % GH, pl.ds(r0, BM), :] for h in range(H)],
                                    axis=1)
                a_v[pl.ds(S - PRE + r0, BM), n * 128:(n + 1) * 128] = (
                    _dot(o, wo_v[n]).astype(bf16))
            return c
        lax.fori_loop(0, PRE // BM, tail, 0)

    pl.run_scoped(
        phase_a,
        pltpu.VMEM((2, D, 16, DH), bf16),
        *([pltpu.VMEM((12, RING, DH), bf16)] * 8 + [pltpu.VMEM((GH, RING, DH), bf16)] * (H // GH)))

    def phase_b(g_v, xa_v, hb_v, base_v, x1_v, y1_v, z_v, y2_v, u_v):
        for cp in mod_cps(16, 48, 1):
            cp.wait()
        for n in range(NT):
            slab_cp(w1_hbm, w1_v, n, sem_w.at[1]).wait()
        for n in range(NT):
            slab_cp(w2_hbm, w2_v, n, sem_w.at[2]).wait()
        for n in range(NF):
            slab_cp(w3_hbm, w3_v, n, sem_w.at[3]).wait()
        for n in range(NT):
            slab_cp(w4_hbm, w4_v, n, sem_w.at[4]).wait()
        mod_compute(16, 48)
        for n in range(NT):
            g_v[n, 0:8, :] = jnp.zeros((8, 128), f32)
            g_v[n, S + 8:S + 16, :] = jnp.zeros((8, 128), f32)

        RC = 16

        def row0(j):
            return j * BM if isinstance(j, int) else pl.multiple_of(j * BM, BM)

        def s0_pre(j):
            r0, sl = row0(j), j % 2
            for k in range(BM // RC):
                rows = pl.ds(r0 + k * RC, RC)
                xa = x_v[rows, :].astype(f32) + mod(2) * a_v[rows, :].astype(f32)
                hb = _ln(xa) * (1.0 + mod(4)) + mod(3)
                xa_v[sl, k * RC:(k + 1) * RC, :] = xa
                hb_v[sl, k * RC:(k + 1) * RC, :] = hb
                y1_v[k * RC:(k + 1) * RC, :] = _ln(hb).astype(bf16)

        def s0_mm(j):
            r0 = row0(j)
            for n in range(NT):
                g_v[n, pl.ds(8 + r0, BM), :] = _gelu(_dot(y1_v[...], w1_v[n]))

        def s1_mm(j):
            r0, sl = row0(j), j % 2
            shift = (-1, 1, -2, 2)
            for n in range(NT):
                z_v[:, n * 128:(n + 1) * 128] = (
                    g_v[n, pl.ds(8 + r0 + shift[n // 2], BM), :].astype(bf16))
            for n in range(NT):
                x1_v[:, n * 128:(n + 1) * 128] = (
                    hb_v[sl, :, n * 128:(n + 1) * 128] + _dot(z_v[...], w2_v[n]))

        def s1_post(j):
            sl = j % 2
            for k in range(BM // RC):
                x1 = x1_v[k * RC:(k + 1) * RC, :]
                y2_v[k * RC:(k + 1) * RC, :] = _ln(x1).astype(bf16)
                base_v[sl, k * RC:(k + 1) * RC, :] = xa_v[sl, k * RC:(k + 1) * RC, :] + mod(5) * x1

        def s2_w3():
            for f in range(NF):
                u_v[:, f * 128:(f + 1) * 128] = _gelu(_dot(y2_v[...], w3_v[f])).astype(bf16)

        def s2_w4(j, n):
            r0, sl = row0(j), j % 2
            gb = mod_v[0:1, 5 * D + n * 128:5 * D + (n + 1) * 128]
            a_v[pl.ds(r0, BM), n * 128:(n + 1) * 128] = (
                base_v[sl, :, n * 128:(n + 1) * 128] + gb * _dot(u_v[...], w4_v[n])).astype(bf16)

        def out_cp(j):
            r0 = row0(j)
            return pltpu.make_async_copy(a_v.at[pl.ds(r0, BM)], out_hbm.at[pl.ds(r0, BM)],
                                         sem_out.at[j])

        s0_pre(0)
        s0_mm(0)
        s0_pre(1)
        s0_mm(1)
        s1_mm(0)
        s1_post(0)

        def blk(j, c):
            j2 = jnp.minimum(j + 2, NB - 1)
            j1 = jnp.minimum(j + 1, NB - 1)
            s0_pre(j2)
            s2_w3()
            s0_mm(j2)
            for n in range(NT // 2):
                s2_w4(j, n)
            s1_mm(j1)
            for n in range(NT // 2, NT):
                s2_w4(j, n)
            s1_post(j1)
            out_cp(j).start()
            return c
        lax.fori_loop(0, NB, blk, 0)
        for j in range(NB):
            out_cp(j).wait()

    pl.run_scoped(
        phase_b,
        pltpu.VMEM((NT, S + 16, 128), f32),
        pltpu.VMEM((2, BM, D), f32), pltpu.VMEM((2, BM, D), f32), pltpu.VMEM((2, BM, D), f32),
        pltpu.VMEM((BM, D), f32),
        pltpu.VMEM((BM, D), bf16), pltpu.VMEM((BM, D), bf16), pltpu.VMEM((BM, D), bf16),
        pltpu.VMEM((BM, F), bf16))


@functools.partial(jax.jit, static_argnames=("A_seg_len",))
def pallas_adaLN_cond__memory_aug_recurrent_mem_tr__mixer_s_mlp__prompt_kernel(
    A_x: jax.Array,
    A_mem0: jax.Array,
    A_Wq: jax.Array,
    A_Wk: jax.Array,
    A_Wv: jax.Array,
    A_Wo: jax.Array,
    A_seg_len,
    B_x: jax.Array,
    B_w1: jax.Array,
    B_w2: jax.Array,
    B_w3: jax.Array,
    B_w4: jax.Array,
    c: jax.Array,
    w_mod: jax.Array,
):
    assert A_seg_len == SEG and A_x.shape == (1, S, D) and A_Wq.shape == (D, H, DH)
    any_spec = pl.BlockSpec(memory_space=pl.ANY)
    out = pl.pallas_call(
        _kernel,
        out_shape=jax.ShapeDtypeStruct((S, D), bf16),
        in_specs=[any_spec] * 12,
        out_specs=any_spec,
        scratch_shapes=[
            pltpu.VMEM((S, D), bf16),
            pltpu.VMEM((S, D), bf16),
            pltpu.VMEM((PRE, D), bf16),
            pltpu.VMEM((XR + MEM, D), bf16),
            pltpu.VMEM((1, D), bf16),
            pltpu.VMEM((MEM, D), bf16),
            pltpu.VMEM((8, 6 * D), f32),
            pltpu.VMEM((6 * NT, D, 128), bf16),
            pltpu.VMEM((48 * PITCH, 128), u32),
            pltpu.VMEM((48 * PITCH, 128), u32),
            pltpu.VMEM((NT, H * DH, 128), bf16),
            pltpu.VMEM((NT, D, 128), bf16),
            pltpu.VMEM((NT, D, 128), bf16),
            pltpu.VMEM((NF, D, 128), bf16),
            pltpu.VMEM((NT, F, 128), bf16),
            pltpu.SemaphoreType.DMA((2,)),
            pltpu.SemaphoreType.DMA((2,)),
            pltpu.SemaphoreType.DMA((2, 4)),
            pltpu.SemaphoreType.DMA((2,)),
            pltpu.SemaphoreType.DMA((5,)),
            pltpu.SemaphoreType.DMA((NB,)),
        ],
        compiler_params=pltpu.CompilerParams(vmem_limit_bytes=120 * 1024 * 1024),
    )(A_x.reshape(S, D), A_mem0.reshape(MEM, D), A_Wq, A_Wk, A_Wv, A_Wo.reshape(H * DH, D),
      B_w1, B_w2, B_w3, B_w4, c, w_mod)
    return out.reshape(1, S, D)
```

```python
import functools

import jax
import jax.numpy as jnp
from jax import lax
import jax.experimental.pallas as pl
import jax.experimental.pallas.tpu as pltpu

bf16, f32, u32 = jnp.bfloat16, jnp.float32, jnp.uint32

S, D, H, DH, MEM, SEG, F = 2048, 1024, 32, 128, 8, 32, 3584
NSEG = S // SEG
XR = 24
PRE = S - XR * NSEG
RING = 576
QOFF = RING - PRE
OOFF = 192
PITCH = 520
NT = D // 128
NF = F // 128
BM = 128
NB = S // BM
GH = 4
NPAIR = H // 2
PADL = 128
EPS = 1e-5
SCALE = DH ** -0.5


def _ln(x):
    m = jnp.mean(x, axis=-1, keepdims=True)
    xc = x - m
    v = jnp.mean(xc * xc, axis=-1, keepdims=True)
    return xc * lax.rsqrt(v + EPS)


def _gelu(x):
    return jax.nn.gelu(x, approximate=True)


def _dot(a, b):
    return jnp.dot(a, b, preferred_element_type=f32)


def _kernel(x_hbm, mem0_hbm, wq_hbm, wk_hbm, wv_hbm, wo_hbm, w1_hbm, w2_hbm, w3_hbm, w4_hbm,
            c_hbm, wmod_hbm, out_hbm,
            x_v, a_v, h0_v, lhs_v, c_v, mem0_v, mod_v, wmod_v, w_v, wo_v,
            w1_v, w2_v, w3_v, w4_v,
            sem_small, sem_x, sem_stage, sem_mod, sem_w, sem_out):
    wqkv_hbm = (wq_hbm, wk_hbm, wv_hbm)

    c_cp = pltpu.make_async_copy(c_hbm, c_v, sem_small.at[0])
    mem0_cp = pltpu.make_async_copy(mem0_hbm, mem0_v, sem_small.at[1])
    X0 = PRE + 128
    x0_cp = pltpu.make_async_copy(x_hbm.at[pl.ds(0, X0)], x_v.at[pl.ds(0, X0)], sem_x.at[0])
    x1_cp = pltpu.make_async_copy(x_hbm.at[pl.ds(X0, S - X0)], x_v.at[pl.ds(X0, S - X0)],
                                  sem_x.at[1])

    def w_cp(src, dst, k):
        return pltpu.make_async_copy(src, dst.at[:, pl.ds(0, src.shape[1])], sem_w.at[k])

    wo_cp, w1_cp, w2_cp, w3_cp, w4_cp = (
        w_cp(a, b, k) for k, (a, b) in enumerate(
            ((wo_hbm, wo_v), (w1_hbm, w1_v), (w2_hbm, w2_v), (w3_hbm, w3_v), (w4_hbm, w4_v))))

    def mod_cp(lo, hi, k):
        cols = pl.ds(lo * 128, (hi - lo) * 128)
        return pltpu.make_async_copy(wmod_hbm.at[:, cols], wmod_v.at[:, cols], sem_mod.at[k])

    def mod_compute(lo, hi):
        cf = c_v[...].astype(f32)
        sc = (cf * jax.nn.sigmoid(cf)).astype(bf16)
        sc = jnp.broadcast_to(sc, (8, D))
        for n in range(lo, hi):
            mod_v[:, n * 128:(n + 1) * 128] = _dot(sc, wmod_v[:, n * 128:(n + 1) * 128])

    def mod(k):
        return mod_v[0:1, k * D:(k + 1) * D]

    def h_rows(r0, n):
        return (_ln(x_v[pl.ds(r0, n), :].astype(f32)) * (1.0 + mod(1)) + mod(0)).astype(bf16)

    def phase_a(stage, xh_v, *rr):
        rings, orings = rr[:8], rr[8:]

        def stage_cp(t, hh, piece):
            d0 = piece * 256 if isinstance(piece, int) else pl.multiple_of(piece * 256, 256)
            h0 = hh * 16 if isinstance(hh, int) else pl.multiple_of(hh * 16, 16)
            return pltpu.make_async_copy(
                wqkv_hbm[t].at[pl.ds(d0, 256), pl.ds(h0, 16), :],
                stage.at[hh, pl.ds(d0, 256)], sem_stage.at[hh, piece])

        def repack(hh, ch, p0, n):
            for u in range(n):
                p = p0 + u
                a = pltpu.bitcast(stage[hh, 2 * p], u32)
                b = pltpu.bitcast(stage[hh, 2 * p + 1], u32)
                ev = (a & jnp.uint32(0xFFFF)) | (b << 16)
                od = (a >> 16) | (b & jnp.uint32(0xFFFF0000))
                w_v[pl.ds(ch * (16 * PITCH) + p, 8, stride=PITCH), :] = ev
                w_v[pl.ds(ch * (16 * PITCH) + 8 * PITCH + p, 8, stride=PITCH), :] = od

        def w_slab(ch, l):
            base = (ch * 16 + (l % 2) * 8 + l // 2) * PITCH
            if not isinstance(base, int):
                base = pl.multiple_of(base, 8)
            return pltpu.bitcast(w_v[pl.ds(base, D // 2), :], bf16)

        def ring_of(ch, l):
            return rings[l // 2], ch * 2 + l % 2

        c_cp.start()
        mem0_cp.start()
        x0_cp.start()
        mod_cp(0, 8, 0).start()
        mod_cp(8, 16, 1).start()
        x0_cp.wait()
        for k in range(4):
            stage_cp(0, 0, k).start()

        def xhat_body(i, c):
            r0 = pl.multiple_of(i * 32, 32)
            for u in range(2):
                rows = pl.ds(r0 + 16 * u, 16)
                xh_v[rows, :] = _ln(x_v[rows, :].astype(f32))
            return c
        lax.fori_loop(0, PRE // 32, xhat_body, 0)

        c_cp.wait()
        mem0_cp.wait()
        mod_cp(0, 8, 0).wait()
        mod_cp(8, 16, 1).wait()
        mod_compute(0, 16)

        def h0_body(i, c):
            rows = pl.ds(pl.multiple_of(i * 64, 64), 64)
            h0_v[rows, :] = (xh_v[rows, :] * (1.0 + mod(1)) + mod(0)).astype(bf16)
            return c
        lax.fori_loop(0, PRE // 64, h0_body, 0)
        lhs_v[0:XR, :] = h_rows(PRE, XR)
        lhs_v[XR:XR + MEM, :] = mem0_v[...]

        def first_repack(k, c):
            stage_cp(0, 0, k).wait()
            stage_cp(0, 1, k).start()

            def inner(i, cc):
                repack(0, 0, k * 128 + i * 16, 16)
                return cc
            lax.fori_loop(0, 8, inner, 0)
            return c
        lax.fori_loop(0, 4, first_repack, 0)
        for k in range(4):
            stage_cp(1, 0, k).start()

        def pre_body(i, c):
            ch, it = i // 4, i % 4
            nh = (ch + 1) % 2
            cn = jnp.where(ch < 5, ch + 1, 4)

            @pl.when(ch < 5)
            def _():
                stage_cp(0, nh, it).wait()
            r0 = pl.multiple_of(it * BM, BM)
            for l in range(16):
                y = _dot(h0_v[pl.ds(r0, BM), :], w_slab(ch, l))
                rg, ix = ring_of(ch, l)
                rg[ix, pl.ds(QOFF + r0, BM), :] = y.astype(bf16)
                if l < 15:
                    n = 9 if l < 8 else 8
                    repack(nh, cn, it * 128 + (l * 9 if l < 8 else 72 + (l - 8) * 8), n)
            for tt in range(1, 3):
                @pl.when((ch + 3) // 2 == tt)
                def _():
                    stage_cp(tt, nh, it).start()

            @pl.when(i == 8)
            def _():
                wo_cp.start()
                x1_cp.start()
            return c
        lax.fori_loop(0, 24, pre_body, 0)

        mod_cp(16, 48, 2).start()
        for cp in (w1_cp, w2_cp, w3_cp, w4_cp):
            cp.start()
        x1_cp.wait()
        wo_cp.wait()

        L2 = 2 * (SEG + MEM)
        r = lax.broadcasted_iota(jnp.int32, (L2, L2), 0)
        c = lax.broadcasted_iota(jnp.int32, (L2, L2), 1)
        r1 = ((r >= SEG) & (r < 2 * SEG)) | (r >= 2 * SEG + MEM)
        c1 = ((c >= SEG) & (c < 2 * SEG)) | (c >= 2 * SEG + MEM)
        same = r1 == c1
        mask = same & ((r >= 2 * SEG) | (c >= 2 * SEG) | (c <= r))
        fill = jnp.where(same, -1e9, -jnp.inf).astype(f32)

        def step(s, carry):
            woff = pl.multiple_of((XR * s) % RING, 8)
            roff = pl.multiple_of((SEG * s + QOFF) % RING, SEG)
            owr = pl.multiple_of((SEG * s + OOFF) % RING, SEG)
            ord_ = pl.multiple_of((XR * s + OOFF) % RING, 8)
            lhs = lhs_v[...]
            nxt = pl.multiple_of(PRE + XR * jnp.minimum(s + 1, NSEG - 1), 8)
            lhs_v[0:XR, :] = h_rows(nxt, XR)
            acc = [None] * NT
            ym, ps, om = {}, {}, {}

            def qkv(h):
                for t in range(3):
                    y = _dot(lhs, w_slab(2 * t + h // 16, h % 16))
                    rg, ix = ring_of(2 * t + h // 16, h % 16)
                    rg[ix, pl.ds(woff, XR), :] = y[0:XR].astype(bf16)
                    ym[(t, h)] = y[XR:XR + MEM]

            def get(t, p):
                rg, i0 = ring_of(2 * t + p // 8, (2 * p) % 16)
                i1 = i0 + 1
                mm = jnp.concatenate([ym.pop((t, 2 * p)), ym.pop((t, 2 * p + 1))], axis=0)
                return jnp.concatenate([rg[i0, pl.ds(roff, SEG), :], rg[i1, pl.ds(roff, SEG), :],
                                        mm.astype(bf16)], axis=0)

            def sm(p):
                sc = lax.dot_general(get(0, p), get(1, p), (((1,), (1,)), ((), ())),
                                     preferred_element_type=f32) * SCALE
                sc = jnp.where(mask, sc, fill)
                e = jnp.exp(sc - jnp.max(sc, axis=-1, keepdims=True))
                ps[p] = (e * (1.0 / jnp.sum(e, axis=-1, keepdims=True))).astype(bf16)

            def pv(p):
                o = _dot(ps.pop(p), get(2, p))
                for j in range(2):
                    h = 2 * p + j
                    orings[h // GH][h % GH, pl.ds(owr, SEG), :] = (
                        o[SEG * j:SEG * (j + 1)].astype(bf16))
                    om[h] = o[2 * SEG + MEM * j:2 * SEG + MEM * (j + 1)].astype(bf16)

            def wo(g):
                olg = jnp.concatenate(
                    [jnp.concatenate([orings[g][h % GH, pl.ds(ord_, XR), :], om.pop(h)], axis=0)
                     for h in range(g * GH, (g + 1) * GH)], axis=1)
                for n in range(NT):
                    y = _dot(olg, wo_v[g * GH * DH:(g + 1) * GH * DH, n * 128:(n + 1) * 128])
                    acc[n] = y if acc[n] is None else acc[n] + y

            gd = [0]

            def big(h):
                if h < H:
                    qkv(h)
                else:
                    wo(gd[0])
                    gd[0] += 1

            for i in range(NPAIR + 3):
                big(2 * i)
                if 0 <= i - 3 < NPAIR:
                    pv(i - 3)
                if i < NPAIR + 2:
                    big(2 * i + 1)
                if 0 <= i - 1 < NPAIR:
                    sm(i - 1)
            while gd[0] < H // GH:
                big(H)
            res = jnp.concatenate(acc, axis=1).astype(bf16)
            a_v[pl.ds(pl.multiple_of(XR * s, 8), XR), :] = res[0:XR]
            lhs_v[XR:XR + MEM, :] = res[XR:XR + MEM]
            return carry
        lax.fori_loop(0, NSEG, step, 0)

        def tail(b, c):
            r0 = pl.multiple_of(b * BM, BM)
            for n in range(NT):
                o = jnp.concatenate([orings[h // GH][h % GH, pl.ds(r0, BM), :] for h in range(H)],
                                    axis=1)
                a_v[pl.ds(S - PRE + r0, BM), n * 128:(n + 1) * 128] = (
                    _dot(o, wo_v[:, n * 128:(n + 1) * 128]).astype(bf16))
            return c
        lax.fori_loop(0, PRE // BM, tail, 0)

    pl.run_scoped(
        phase_a,
        pltpu.VMEM((2, D, 16, DH), bf16),
        pltpu.VMEM((PRE, D), f32),
        *([pltpu.VMEM((12, RING, DH), bf16)] * 8 + [pltpu.VMEM((GH, RING, DH), bf16)] * (H // GH)))

    def phase_b(g_v, xa_v, hb_v, base_v, x1_v, y1_v, z_v, y2_v, u_v):
        mod_cp(16, 48, 2).wait()
        for cp in (w1_cp, w2_cp, w3_cp, w4_cp):
            cp.wait()
        mod_compute(16, 48)
        for n in range(NT):
            g_v[n, 0:8, :] = jnp.zeros((8, 128), f32)
            g_v[n, S + 8:S + 16, :] = jnp.zeros((8, 128), f32)

        RC = 16

        def row0(j):
            return j * BM if isinstance(j, int) else pl.multiple_of(j * BM, BM)

        def s0_pre(j):
            r0, sl = row0(j), j % 2
            for k in range(BM // RC):
                rows = pl.ds(r0 + k * RC, RC)
                xa = x_v[rows, :].astype(f32) + mod(2) * a_v[rows, :].astype(f32)
                hb = _ln(xa) * (1.0 + mod(4)) + mod(3)
                xa_v[sl, k * RC:(k + 1) * RC, :] = xa
                hb_v[sl, k * RC:(k + 1) * RC, :] = hb
                y1_v[k * RC:(k + 1) * RC, :] = _ln(hb).astype(bf16)

        def s0_mm(j):
            r0 = row0(j)
            for n in range(NT):
                g_v[n, pl.ds(8 + r0, BM), :] = _gelu(_dot(y1_v[...], w1_v[:, n * 128:(n + 1) * 128]))

        def s1_mm(j):
            r0, sl = row0(j), j % 2
            shift = (-1, 1, -2, 2)
            for n in range(NT):
                z_v[:, n * 128:(n + 1) * 128] = (
                    g_v[n, pl.ds(8 + r0 + shift[n // 2], BM), :].astype(bf16))
            for n in range(NT):
                x1_v[:, n * 128:(n + 1) * 128] = (
                    hb_v[sl, :, n * 128:(n + 1) * 128] + _dot(z_v[...], w2_v[:, n * 128:(n + 1) * 128]))

        def s1_post(j):
            sl = j % 2
            for k in range(BM // RC):
                x1 = x1_v[k * RC:(k + 1) * RC, :]
                y2_v[k * RC:(k + 1) * RC, :] = _ln(x1).astype(bf16)
                base_v[sl, k * RC:(k + 1) * RC, :] = xa_v[sl, k * RC:(k + 1) * RC, :] + mod(5) * x1

        def s2_w3():
            for f in range(NF):
                u_v[:, f * 128:(f + 1) * 128] = _gelu(_dot(y2_v[...], w3_v[:, f * 128:(f + 1) * 128])).astype(bf16)

        def s2_w4(j, n):
            r0, sl = row0(j), j % 2
            gb = mod_v[0:1, 5 * D + n * 128:5 * D + (n + 1) * 128]
            a_v[pl.ds(r0, BM), n * 128:(n + 1) * 128] = (
                base_v[sl, :, n * 128:(n + 1) * 128] + gb * _dot(u_v[...], w4_v[:, n * 128:(n + 1) * 128])).astype(bf16)

        def out_cp(j):
            r0 = row0(j)
            return pltpu.make_async_copy(a_v.at[pl.ds(r0, BM)], out_hbm.at[pl.ds(r0, BM)],
                                         sem_out.at[j])

        s0_pre(0)
        s0_mm(0)
        s0_pre(1)
        s0_mm(1)
        s1_mm(0)
        s1_post(0)

        def blk(j, c):
            j2 = jnp.minimum(j + 2, NB - 1)
            j1 = jnp.minimum(j + 1, NB - 1)
            s0_pre(j2)
            s2_w3()
            s0_mm(j2)
            for n in range(NT // 2):
                s2_w4(j, n)
            s1_mm(j1)
            for n in range(NT // 2, NT):
                s2_w4(j, n)
            s1_post(j1)
            out_cp(j).start()
            return c
        lax.fori_loop(0, NB, blk, 0)
        for j in range(NB):
            out_cp(j).wait()

    pl.run_scoped(
        phase_b,
        pltpu.VMEM((NT, S + 16, 128), f32),
        pltpu.VMEM((2, BM, D), f32), pltpu.VMEM((2, BM, D), f32), pltpu.VMEM((2, BM, D), f32),
        pltpu.VMEM((BM, D), f32),
        pltpu.VMEM((BM, D), bf16), pltpu.VMEM((BM, D), bf16), pltpu.VMEM((BM, D), bf16),
        pltpu.VMEM((BM, F), bf16))


@functools.partial(jax.jit, static_argnames=("A_seg_len",))
def pallas_adaLN_cond__memory_aug_recurrent_mem_tr__mixer_s_mlp__prompt_kernel(
    A_x: jax.Array,
    A_mem0: jax.Array,
    A_Wq: jax.Array,
    A_Wk: jax.Array,
    A_Wv: jax.Array,
    A_Wo: jax.Array,
    A_seg_len,
    B_x: jax.Array,
    B_w1: jax.Array,
    B_w2: jax.Array,
    B_w3: jax.Array,
    B_w4: jax.Array,
    c: jax.Array,
    w_mod: jax.Array,
):
    assert A_seg_len == SEG and A_x.shape == (1, S, D) and A_Wq.shape == (D, H, DH)
    any_spec = pl.BlockSpec(memory_space=pl.ANY)
    out = pl.pallas_call(
        _kernel,
        out_shape=jax.ShapeDtypeStruct((S, D), bf16),
        in_specs=[any_spec] * 12,
        out_specs=any_spec,
        scratch_shapes=[
            pltpu.VMEM((S, D), bf16),
            pltpu.VMEM((S, D), bf16),
            pltpu.VMEM((PRE, D), bf16),
            pltpu.VMEM((XR + MEM, D), bf16),
            pltpu.VMEM((1, D), bf16),
            pltpu.VMEM((MEM, D), bf16),
            pltpu.VMEM((8, 6 * D), f32),
            pltpu.VMEM((D, 6 * D + PADL), bf16),
            pltpu.VMEM((96 * PITCH, 128), u32),
            pltpu.VMEM((H * DH, D + PADL), bf16),
            pltpu.VMEM((D, D + PADL), bf16),
            pltpu.VMEM((D, D + PADL), bf16),
            pltpu.VMEM((D, F + PADL), bf16),
            pltpu.VMEM((F, D + PADL), bf16),
            pltpu.SemaphoreType.DMA((2,)),
            pltpu.SemaphoreType.DMA((2,)),
            pltpu.SemaphoreType.DMA((2, 4)),
            pltpu.SemaphoreType.DMA((3,)),
            pltpu.SemaphoreType.DMA((5,)),
            pltpu.SemaphoreType.DMA((NB,)),
        ],
        compiler_params=pltpu.CompilerParams(vmem_limit_bytes=120 * 1024 * 1024),
    )(A_x.reshape(S, D), A_mem0.reshape(MEM, D), A_Wq, A_Wk, A_Wv, A_Wo.reshape(H * DH, D),
      B_w1, B_w2, B_w3, B_w4, c, w_mod)
    return out.reshape(1, S, D)
```

```python
import functools

import jax
import jax.numpy as jnp
from jax import lax
import jax.experimental.pallas as pl
import jax.experimental.pallas.tpu as pltpu

bf16, f32, u32 = jnp.bfloat16, jnp.float32, jnp.uint32

S, D, H, DH, MEM, SEG, F = 2048, 1024, 32, 128, 8, 32, 3584
NSEG = S // SEG
XR = 24
PRE = S - XR * NSEG
RING = 576
QOFF = RING - PRE
OOFF = 192
PITCH = 520
NT = D // 128
NF = F // 128
BM = 128
NB = S // BM
GH = 4
NPAIR = H // 2
HR = (S - PRE) // 2
PADL = 128
SH = 16
RC = 16
EPS = 1e-5
LOG2E = 1.4426950408889634
SCALE = DH ** -0.5
CFG = dict(pre=True, step=True, tail=True, b=True, pre_rb=2, unroll=2, nlo=6, lastg=2, nf=7)


def _ln(x):
    m = jnp.mean(x, axis=-1, keepdims=True)
    xc = x - m
    v = jnp.mean(xc * xc, axis=-1, keepdims=True)
    return xc * lax.rsqrt(v + EPS)


def _gelu(x):
    return jax.nn.gelu(x, approximate=True)


def _dot(a, b):
    return jnp.dot(a, b, preferred_element_type=f32)


def _pk(x):
    return pltpu.bitcast(x.astype(bf16), u32)


def _unpk(x):
    return pltpu.bitcast(x, bf16)


def _tie(w, after, r=0, k=0):
    if after is None:
        return w
    m = functools.reduce(lambda a, b: a & b,
                         [after[:, i * 128:(i + 1) * 128] for i in range(after.shape[1] // 128)])
    mf = pltpu.bitcast(m, f32)
    z = jnp.where(mf * mf < 0.0, jnp.uint32(1), jnp.uint32(0))
    row = w[r:r + 8]
    parts = [row[:, :k * 128], row[:, k * 128:(k + 1) * 128] | z, row[:, (k + 1) * 128:]]
    row = jnp.concatenate([p for p in parts if p.shape[1]], axis=1)
    parts = [w[:r], row, w[r + 8:]]
    return jnp.concatenate([p for p in parts if p.shape[0]], axis=0)


def _kernel(x_hbm, mem0_hbm, wq_hbm, wk_hbm, wv_hbm, wo_hbm, w1_hbm, w2_hbm, w3_hbm, w4_hbm,
            c_hbm, wmod_hbm, out_hbm,
            c_v, x_v, a_v, h0_v, mem_v, mem0_v, mod_v, wmod_v, w_v, wo_v,
            w1_v, w2_v, w3_v, w4_v,
            g_v, xa_v, hb_v, base_v, x1_v, y1_v, z_v, y2_v, u_v,
            stage, xh_v, hx_v,
            r0_, r1_, r2_, r3_, r4_, r5_, r6_, r7_, o0_, o1_, o2_, o3_, o4_, o5_, o6_, o7_,
            zero_s, sem_small, sem_x, sem_stage, sem_mod, sem_w, sem_out):
    wqkv_hbm = (wq_hbm, wk_hbm, wv_hbm)
    rings = (r0_, r1_, r2_, r3_, r4_, r5_, r6_, r7_)
    orings = (o0_, o1_, o2_, o3_, o4_, o5_, o6_, o7_)

    c_cp = pltpu.make_async_copy(c_hbm, c_v, sem_small.at[0])
    mem0_cp = pltpu.make_async_copy(mem0_hbm, mem0_v, sem_small.at[1])
    X0 = PRE + 128
    x0_cp = pltpu.make_async_copy(x_hbm.at[pl.ds(0, X0)], x_v.at[pl.ds(0, X0)], sem_x.at[0])
    x1_cp = pltpu.make_async_copy(x_hbm.at[pl.ds(X0, S - X0)], x_v.at[pl.ds(X0, S - X0)],
                                  sem_x.at[1])

    def w_cp(src, dst, k):
        return pltpu.make_async_copy(src, dst.at[:, pl.ds(0, src.shape[1])], sem_w.at[k])

    wo_cp, w1_cp, w2_cp, w3_cp, w4_cp = (
        w_cp(a, b, k) for k, (a, b) in enumerate(
            ((wo_hbm, wo_v), (w1_hbm, w1_v), (w2_hbm, w2_v), (w3_hbm, w3_v), (w4_hbm, w4_v))))

    def mod_cp(lo, hi, k):
        cols = pl.ds(lo * 128, (hi - lo) * 128)
        return pltpu.make_async_copy(wmod_hbm.at[:, cols], wmod_v.at[:, cols], sem_mod.at[k])

    def stage_cp(t, hh, piece):
        d0 = piece * 256 if isinstance(piece, int) else pl.multiple_of(piece * 256, 256)
        h0 = hh * 16 if isinstance(hh, int) else pl.multiple_of(hh * 16, 16)
        return pltpu.make_async_copy(
            wqkv_hbm[t].at[pl.ds(d0, 256), pl.ds(h0, 16), :],
            stage.at[hh, pl.ds(d0, 256)], sem_stage.at[hh, piece])

    def out_cp(j):
        r0 = j * BM if isinstance(j, int) else pl.multiple_of(j * BM, BM)
        return pltpu.make_async_copy(a_v.at[pl.ds(r0, BM)], out_hbm.at[pl.ds(r0, BM)],
                                     sem_out.at[j])

    def tile(n):
        return slice(n * 128, (n + 1) * 128)

    def mod_compute(lo, hi):
        cf = c_v[...].astype(f32)
        sc = (cf * jax.nn.sigmoid(cf)).astype(bf16)
        sc = jnp.broadcast_to(sc, (8, D))
        for n in range(lo, hi):
            mod_v[:, tile(n)] = _dot(sc, wmod_v[:, tile(n)])

    def mod(k):
        return mod_v[0:1, k * D:(k + 1) * D]

    def repack(hh, ch, p0, n):
        for u in range(n):
            p = p0 + u
            a = pltpu.bitcast(stage[hh, 2 * p], u32)
            b = pltpu.bitcast(stage[hh, 2 * p + 1], u32)
            ev = (a & jnp.uint32(0xFFFF)) | (b << 16)
            od = (a >> 16) | (b & jnp.uint32(0xFFFF0000))
            w_v[pl.ds(ch * (16 * PITCH) + p, 8, stride=PITCH), :] = ev
            w_v[pl.ds(ch * (16 * PITCH) + 8 * PITCH + p, 8, stride=PITCH), :] = od

    def w_slab(ch, l, lo=0, hi=D):
        base = (ch * 16 + (l % 2) * 8 + l // 2) * PITCH + lo // 2
        if not isinstance(base, int):
            base = pl.multiple_of(base, 8)
        return _unpk(w_v[pl.ds(base, (hi - lo) // 2), :])

    def ring_of(ch, l):
        return rings[l // 2], ch * 2 + l % 2

    c_cp.start()
    mem0_cp.start()
    x0_cp.start()
    mod_cp(0, 8, 0).start()
    mod_cp(8, 16, 1).start()
    zero_s[0] = 0
    x_v[S:S + SH, :] = jnp.zeros((SH, D), bf16)
    a_v[S:S + SH, :] = jnp.zeros((SH, D), bf16)
    x0_cp.wait()
    for k in range(4):
        stage_cp(0, 0, k).start()

    def xhat_body(i, c):
        r0 = pl.multiple_of(i * 64, 64)
        for u in range(4):
            rows = pl.ds(r0 + RC * u, RC)
            xh_v[rows, :] = _ln(x_v[rows, :].astype(f32))
        return c
    lax.fori_loop(0, PRE // 64, xhat_body, 0)

    c_cp.wait()
    mem0_cp.wait()
    mod_cp(0, 8, 0).wait()
    mod_cp(8, 16, 1).wait()
    mod_compute(0, 16)

    def h0_body(i, c):
        rows = pl.ds(pl.multiple_of(i * 64, 64), 64)
        h0_v[pl.ds(pl.multiple_of(i * 32, 32), 32), :] = _pk(
            xh_v[rows, :] * (1.0 + mod(1)) + mod(0))
        return c
    lax.fori_loop(0, PRE // 64, h0_body, 0)
    mem_v[...] = pltpu.bitcast(mem0_v[...], u32)

    def first_repack(k, c):
        stage_cp(0, 0, k).wait()
        stage_cp(0, 1, k).start()

        def inner(i, cc):
            repack(0, 0, k * 128 + i * 16, 16)
            return cc
        lax.fori_loop(0, 8, inner, 0)
        return c
    lax.fori_loop(0, 4, first_repack, 0)
    for k in range(4):
        stage_cp(1, 0, k).start()

    def pre_body(i, c):
        RB = CFG['pre_rb']
        ch, it0 = i // (4 // RB), (i % (4 // RB)) * RB
        nh = (ch + 1) % 2
        cn = jnp.where(ch < 5, ch + 1, 4)
        done = {}

        @pl.when(ch < 5)
        def _():
            for rb in range(RB):
                stage_cp(0, nh, it0 + rb).wait()

        for rb in range(RB):
            it = it0 + rb
            r0 = pl.multiple_of(it * (BM // 2), BM // 2)
            for l in range(16):
                lhs = _tie(h0_v[pl.ds(r0, BM // 2), :], done.pop(l, None))
                y = _dot(_unpk(lhs), w_slab(ch, l))
                rg, ix = ring_of(ch, l)
                rg[ix, pl.ds(QOFF // 2 + r0, BM // 2), :] = _pk(y)
                if l < 15:
                    n = 9 if l < 8 else 8
                    repack(nh, cn, it * 128 + (l * 9 if l < 8 else 72 + (l - 8) * 8), n)
                if l % 2 == 1 and l < 12:
                    hr = pl.multiple_of(jnp.maximum(ch * 4 + it - 8, 0) * 96 + (l // 2) * RC, RC)
                    xs = x_v[pl.ds(PRE + hr, RC), :].astype(f32)
                    hx = _pk(_ln(xs) * (1.0 + mod(1)) + mod(0))
                    done[l + 4] = hx
                    for k in range(NT):
                        hx_v[k, pl.ds(pl.multiple_of(hr // 2, 8), 8), :] = hx[:, tile(k)]
        for tt in range(1, 3):
            @pl.when((ch + 3) // 2 == tt)
            def _():
                for rb in range(RB):
                    stage_cp(tt, nh, it0 + rb).start()

        @pl.when(i == 4 // RB - 1)
        def _():
            x1_cp.start()

        @pl.when(i == 8 // RB - 1)
        def _():
            x1_cp.wait()
            wo_cp.start()
        return c
    if CFG['pre']:
        lax.fori_loop(0, 24 // CFG['pre_rb'], pre_body, 0)

    mod_cp(16, 48, 2).start()
    for cp in (w1_cp, w2_cp, w3_cp, w4_cp):
        cp.start()
    wo_cp.wait()

    L2 = 2 * (SEG + MEM)
    r = lax.broadcasted_iota(jnp.int32, (L2, L2), 0)
    c = lax.broadcasted_iota(jnp.int32, (L2, L2), 1)
    r1 = ((r >= SEG) & (r < 2 * SEG)) | (r >= 2 * SEG + MEM)
    c1 = ((c >= SEG) & (c < 2 * SEG)) | (c >= 2 * SEG + MEM)
    same = r1 == c1
    mask = same & ((r >= 2 * SEG) | (c >= 2 * SEG) | (c <= r))
    fill = jnp.where(same, -1e9 / SCALE, -jnp.inf).astype(f32)

    def step(s, mem, zero):
        woff = pl.multiple_of((XR // 2 * s) % (RING // 2), 4)
        roff = pl.multiple_of((SEG // 2 * s + QOFF // 2) % (RING // 2), SEG // 2)
        owr = pl.multiple_of((SEG // 2 * s + OOFF // 2) % (RING // 2), SEG // 2)
        ord_ = pl.multiple_of((XR // 2 * s + OOFF // 2) % (RING // 2), 4)
        arow = pl.multiple_of(XR * s, 8)
        acc = [None] * NT
        ym, ps, om, part = {}, {}, {}, {}
        HK = D // 2
        tiles = [_unpk(jnp.concatenate(
            [hx_v[k, pl.ds(s * (XR // 2), XR // 2), :] | zero, mem[k]], axis=0))
            for k in range(NT)]
        mem_new = []

        def lhs(lo, hi):
            return jnp.concatenate(tiles[lo // 128:hi // 128], axis=1)

        def qkv_lo(h, t):
            part[(t, h)] = _dot(lhs(0, HK), w_slab(2 * t + h // 16, h % 16, 0, HK))

        def qkv(h):
            for t in range(3):
                ch, l = 2 * t + h // 16, h % 16
                if (t, h) in part:
                    y = _dot(lhs(HK, D), w_slab(ch, l, HK, D)) + part.pop((t, h))
                else:
                    y = _dot(lhs(0, D), w_slab(ch, l))
                rg, ix = ring_of(ch, l)
                rg[ix, pl.ds(woff, XR // 2), :] = _pk(y[0:XR])
                ym[(t, h)] = y[XR:XR + MEM]

        def get(t, p):
            rg, i0 = ring_of(2 * t + p // 8, (2 * p) % 16)
            mm = jnp.concatenate([ym.pop((t, 2 * p)), ym.pop((t, 2 * p + 1))], axis=0)
            return _unpk(jnp.concatenate(
                [rg[i0, pl.ds(roff, SEG // 2), :], rg[i0 + 1, pl.ds(roff, SEG // 2), :], _pk(mm)],
                axis=0))

        def sm(p):
            sc = lax.dot_general(get(0, p), get(1, p), (((1,), (1,)), ((), ())),
                                 preferred_element_type=f32)
            sc = jnp.where(mask, sc, fill)
            e = jnp.exp2((sc - jnp.max(sc, axis=-1, keepdims=True)) * (SCALE * LOG2E))
            ps[p] = (e * pl.reciprocal(jnp.sum(e, axis=-1, keepdims=True), approx=True)
                     ).astype(bf16)

        def pv(p):
            o = _dot(ps.pop(p), get(2, p))
            for j in range(2):
                h = 2 * p + j
                orings[h // GH][h % GH, pl.ds(owr, SEG // 2), :] = _pk(o[SEG * j:SEG * (j + 1)])
                om[h] = _pk(o[2 * SEG + MEM * j:2 * SEG + MEM * (j + 1)])

        def wo(g0, g1):
            olg = _unpk(jnp.concatenate(
                [jnp.concatenate([orings[h // GH][h % GH, pl.ds(ord_, XR // 2), :] | zero,
                                  om.pop(h)], axis=0)
                 for h in range(g0 * GH, g1 * GH)], axis=1))
            for n in range(NT):
                y = _dot(olg, wo_v[g0 * GH * DH:g1 * GH * DH, tile(n)])
                acc[n] = y if acc[n] is None else y + acc[n]
                if g1 == H // GH:
                    a_v[pl.ds(arow, XR), tile(n)] = acc[n][0:XR].astype(bf16)
                    mem_new.append(_pk(acc[n][XR:XR + MEM]))

        gd = [0]

        def big(h):
            if h < H:
                qkv(h)
            else:
                wo(gd[0], gd[0] + 1)
                gd[0] += 1

        for i in range(CFG['nlo']):
            qkv_lo(i // 3, i % 3)
        for i in range(NPAIR + 3):
            big(2 * i)
            if 0 <= i - 3 < NPAIR:
                pv(i - 3)
            if i < NPAIR + 2:
                big(2 * i + 1)
            if 0 <= i - 1 < NPAIR:
                sm(i - 1)
        while gd[0] < H // GH - CFG['lastg']:
            big(H)
        wo(gd[0], H // GH)
        return mem_new

    def steps(i, carry):
        zero = zero_s[0].astype(u32)
        mem = [mem_v[:, tile(k)] for k in range(NT)]
        for j in range(CFG['unroll']):
            mem = step(i * CFG['unroll'] + j, mem, zero)
        for k in range(NT):
            mem_v[:, tile(k)] = mem[k]
        return carry
    if CFG['step']:
        lax.fori_loop(0, NSEG // CFG['unroll'], steps, 0)

    def tail(b, c):
        z0 = pl.multiple_of(zero_s[0], 64)
        r0 = pl.multiple_of(b * (BM // 2), BM // 2)
        for n in range(NT):
            o = jnp.concatenate([orings[h // GH][h % GH, pl.ds(r0, BM // 2), :] for h in range(H)],
                                axis=1)
            a_v[pl.ds(S - PRE + 2 * r0, BM), tile(n)] = (
                _dot(_unpk(o), wo_v[pl.ds(z0, H * DH), tile(n)]).astype(bf16))
        return c
    if CFG['tail']:
        lax.fori_loop(0, PRE // BM, tail, 0)

    if not CFG['b']:
        cp = pltpu.make_async_copy(a_v.at[pl.ds(0, S)], out_hbm, sem_out.at[0])
        cp.start()
        cp.wait()
        return

    mod_cp(16, 48, 2).wait()
    for cp in (w1_cp, w2_cp, w3_cp, w4_cp):
        cp.wait()
    mod_compute(16, 48)

    def p0(tok, w):
        rows = pl.ds(tok, RC)
        xa = x_v[rows, :].astype(f32) + mod(2) * a_v[rows, :].astype(f32)
        hb = _ln(xa) * (1.0 + mod(4)) + mod(3)
        xa_v[w:w + RC, :] = xa
        hb_v[w:w + RC, :] = hb
        return _pk(_ln(hb))

    y0 = p0(0, 0)
    for k in range(BM // RC):
        y1_v[k * 8:(k + 1) * 8, :] = p0(SH + k * RC, SH + k * RC)
    for n in range(NT):
        g_v[n, 0:8, :] = jnp.zeros((8, 128), f32)
        g_v[n, 8:8 + SH, :] = _gelu(_dot(_unpk(y0), w1_v[:, tile(n)]))

    HM = BM // 2
    shift = (-1, 1, -2, 2)

    def blk(j, c):
        r0 = pl.multiple_of(j * BM, BM)
        nxt = pl.multiple_of(jnp.minimum(j + 1, NB - 1) * BM + SH, SH)
        more = j < NB - 1

        def w1_half(hf):
            for n in range(NT):
                g = _gelu(_dot(_unpk(y1_v[hf * 32:(hf + 1) * 32, :]), w1_v[:, tile(n)]))
                w0 = 8 + SH + hf * HM
                if hf == 0:
                    g_v[n, w0:w0 + HM, :] = g
                else:
                    g_v[n, w0:w0 + HM - SH, :] = g[0:HM - SH]
                    g_v[n, w0 + HM - SH:w0 + HM, :] = jnp.where(more, g[HM - SH:HM], 0.0)

        def w2_half(hf):
            for n in range(NT):
                w0 = 8 + hf * HM + shift[n // 2]
                z_v[hf * 32:(hf + 1) * 32, tile(n)] = _pk(g_v[n, w0:w0 + HM, :])
            for n in range(NT):
                x1_v[hf * HM:(hf + 1) * HM, tile(n)] = (
                    _dot(_unpk(z_v[hf * 32:(hf + 1) * 32, :]), w2_v[:, tile(n)])
                    + hb_v[hf * HM:(hf + 1) * HM, tile(n)])

        def p1_half(hf):
            for k in range(hf * HM // RC, (hf + 1) * HM // RC):
                x1 = x1_v[k * RC:(k + 1) * RC, :]
                y2_v[k * 8:(k + 1) * 8, :] = _pk(_ln(x1))
                base_v[k * RC:(k + 1) * RC, :] = xa_v[k * RC:(k + 1) * RC, :] + mod(5) * x1

        def w3(f, lo, hi, after=None):
            u_v[lo:hi, tile(f)] = _pk(_gelu(
                _dot(_unpk(_tie(y2_v[lo:hi, :], after)), w3_v[:, tile(f)])))

        w1_half(0)
        w1_half(1)
        w2_half(0)
        w2_half(1)
        p1_half(0)
        for f in range(CFG['nf']):
            w3(f, 0, 32)
        p1_half(1)
        for f in range(CFG['nf']):
            w3(f, 32, 64)
        for n in range(NT):
            g_v[n, 0:8 + SH, :] = g_v[n, BM:BM + 8 + SH, :]
        xa_v[0:SH, :] = xa_v[BM:BM + SH, :]
        hb_v[0:SH, :] = hb_v[BM:BM + SH, :]
        done = {}
        for f in range(CFG['nf'], NF):
            w3(f, 0, 64, done.pop(f, None))
            k = (f - CFG['nf']) // 2
            if (f - CFG['nf']) % 2 == 0 and k < BM // RC:
                y = p0(nxt + k * RC, SH + k * RC)
                y1_v[k * 8:(k + 1) * 8, :] = y
                done[f + 4] = y
        for n in range(NT):
            gb = mod_v[0:1, 5 * D + n * 128:5 * D + (n + 1) * 128]
            a_v[pl.ds(r0, BM), tile(n)] = (
                base_v[:, tile(n)] + gb * _dot(_unpk(u_v[...]), w4_v[:, tile(n)])).astype(bf16)
        out_cp(j).start()
        return c
    lax.fori_loop(0, NB, blk, 0)
    for j in range(NB):
        out_cp(j).wait()


@functools.partial(jax.jit, static_argnames=("A_seg_len",))
def pallas_adaLN_cond__memory_aug_recurrent_mem_tr__mixer_s_mlp__prompt_kernel(
    A_x: jax.Array,
    A_mem0: jax.Array,
    A_Wq: jax.Array,
    A_Wk: jax.Array,
    A_Wv: jax.Array,
    A_Wo: jax.Array,
    A_seg_len,
    B_x: jax.Array,
    B_w1: jax.Array,
    B_w2: jax.Array,
    B_w3: jax.Array,
    B_w4: jax.Array,
    c: jax.Array,
    w_mod: jax.Array,
):
    assert A_seg_len == SEG and A_x.shape == (1, S, D) and A_Wq.shape == (D, H, DH)
    any_spec = pl.BlockSpec(memory_space=pl.ANY)
    out = pl.pallas_call(
        _kernel,
        out_shape=jax.ShapeDtypeStruct((S, D), bf16),
        in_specs=[any_spec] * 12,
        out_specs=any_spec,
        scratch_shapes=[
            pltpu.VMEM((1, D), bf16),
            pltpu.VMEM((S + SH, D), bf16),
            pltpu.VMEM((S + SH, D), bf16),
            pltpu.VMEM((PRE // 2, D), u32),
            pltpu.VMEM((MEM // 2, D), u32),
            pltpu.VMEM((MEM, D), bf16),
            pltpu.VMEM((8, 6 * D), f32),
            pltpu.VMEM((D, 6 * D + PADL), bf16),
            pltpu.VMEM((96 * PITCH, 128), u32),
            pltpu.VMEM((H * DH, D + PADL), bf16),
            pltpu.VMEM((D, D + PADL), bf16),
            pltpu.VMEM((D, D + PADL), bf16),
            pltpu.VMEM((D, F + PADL), bf16),
            pltpu.VMEM((F, D + PADL), bf16),
            pltpu.VMEM((NT, BM + 32, 128), f32),
            pltpu.VMEM((BM + SH, D), f32),
            pltpu.VMEM((BM + SH, D), f32),
            pltpu.VMEM((BM, D), f32),
            pltpu.VMEM((BM, D), f32),
            pltpu.VMEM((BM // 2, D), u32),
            pltpu.VMEM((BM // 2, D), u32),
            pltpu.VMEM((BM // 2, D), u32),
            pltpu.VMEM((BM // 2, F), u32),
            pltpu.VMEM((2, D, 16, DH), bf16),
            pltpu.VMEM((PRE, D), f32),
            pltpu.VMEM((NT, HR, 128), u32),
        ] + [pltpu.VMEM((12, RING // 2, DH), u32)] * 8
          + [pltpu.VMEM((GH, RING // 2, DH), u32)] * (H // GH) + [
            pltpu.SMEM((1,), jnp.int32),
            pltpu.SemaphoreType.DMA((2,)),
            pltpu.SemaphoreType.DMA((2,)),
            pltpu.SemaphoreType.DMA((2, 4)),
            pltpu.SemaphoreType.DMA((3,)),
            pltpu.SemaphoreType.DMA((5,)),
            pltpu.SemaphoreType.DMA((NB,)),
        ],
        compiler_params=pltpu.CompilerParams(vmem_limit_bytes=120 * 1024 * 1024),
    )(A_x.reshape(S, D), A_mem0.reshape(MEM, D), A_Wq, A_Wk, A_Wv, A_Wo.reshape(H * DH, D),
      B_w1, B_w2, B_w3, B_w4, c, w_mod)
    return out.reshape(1, S, D)
```

```python
import functools

import jax
import jax.numpy as jnp
from jax import lax
import jax.experimental.pallas as pl
import jax.experimental.pallas.tpu as pltpu

bf16, f32, u32 = jnp.bfloat16, jnp.float32, jnp.uint32

S, D, H, DH, MEM, SEG, F = 2048, 1024, 32, 128, 8, 32, 3584
NSEG = S // SEG
XR = 24
PRE = S - XR * NSEG
RING = 576
QOFF = RING - PRE
OOFF = 192
PITCH = 520
NT = D // 128
NF = F // 128
BM = 128
NB = S // BM
GH = 4
NPAIR = H // 2
HR = (S - PRE) // 2
PADL = 128
SH = 16
RC = 16
EPS = 1e-5
LOG2E = 1.4426950408889634
SCALE = DH ** -0.5
CFG = dict(pre=True, step=True, tail=True, b=True, pre_rb=2, unroll=2, nlo=6, lastg=2, nf=7, p0k=24)


def _ln(x):
    m = jnp.mean(x, axis=-1, keepdims=True)
    xc = x - m
    v = jnp.mean(xc * xc, axis=-1, keepdims=True)
    return xc * lax.rsqrt(v + EPS)


def _gelu(x):
    return jax.nn.gelu(x, approximate=True)


def _dot(a, b):
    return jnp.dot(a, b, preferred_element_type=f32)


def _pk(x):
    return pltpu.bitcast(x.astype(bf16), u32)


def _unpk(x):
    return pltpu.bitcast(x, bf16)


def _tie(w, after, r=0, k=0):
    if after is None:
        return w
    m = functools.reduce(lambda a, b: a & b,
                         [after[:, i * 128:(i + 1) * 128] for i in range(after.shape[1] // 128)])
    mf = pltpu.bitcast(m, f32)
    z = jnp.where(mf * mf < 0.0, jnp.uint32(1), jnp.uint32(0))
    row = w[r:r + 8]
    parts = [row[:, :k * 128], row[:, k * 128:(k + 1) * 128] | z, row[:, (k + 1) * 128:]]
    row = jnp.concatenate([p for p in parts if p.shape[1]], axis=1)
    parts = [w[:r], row, w[r + 8:]]
    return jnp.concatenate([p for p in parts if p.shape[0]], axis=0)


def _kernel(x_hbm, mem0_hbm, wq_hbm, wk_hbm, wv_hbm, wo_hbm, w1_hbm, w2_hbm, w3_hbm, w4_hbm,
            c_hbm, wmod_hbm, out_hbm,
            c_v, x_v, a_v, h0_v, mem_v, mem0_v, mod_v, wmod_v, w_v, wo_v,
            w1_v, w2_v, w3_v, w4_v,
            g_v, xa_v, hb_v, base_v, x1_v, y1_v, z_v, y2_v, u_v,
            stage, xh_v, hx_v,
            r0_, r1_, r2_, r3_, r4_, r5_, r6_, r7_, o0_, o1_, o2_, o3_, o4_, o5_, o6_, o7_,
            zero_s, sem_small, sem_x, sem_stage, sem_mod, sem_w, sem_out):
    wqkv_hbm = (wq_hbm, wk_hbm, wv_hbm)
    rings = (r0_, r1_, r2_, r3_, r4_, r5_, r6_, r7_)
    orings = (o0_, o1_, o2_, o3_, o4_, o5_, o6_, o7_)

    c_cp = pltpu.make_async_copy(c_hbm, c_v, sem_small.at[0])
    mem0_cp = pltpu.make_async_copy(mem0_hbm, mem0_v, sem_small.at[1])
    X0 = PRE + 128
    x0_cp = pltpu.make_async_copy(x_hbm.at[pl.ds(0, X0)], x_v.at[pl.ds(0, X0)], sem_x.at[0])
    x1_cp = pltpu.make_async_copy(x_hbm.at[pl.ds(X0, S - X0)], x_v.at[pl.ds(X0, S - X0)],
                                  sem_x.at[1])

    def w_cp(src, dst, k):
        return pltpu.make_async_copy(src, dst.at[:, pl.ds(0, src.shape[1])], sem_w.at[k])

    wo_cp, w1_cp, w2_cp, w3_cp, w4_cp = (
        w_cp(a, b, k) for k, (a, b) in enumerate(
            ((wo_hbm, wo_v), (w1_hbm, w1_v), (w2_hbm, w2_v), (w3_hbm, w3_v), (w4_hbm, w4_v))))

    def mod_cp(lo, hi, k):
        cols = pl.ds(lo * 128, (hi - lo) * 128)
        return pltpu.make_async_copy(wmod_hbm.at[:, cols], wmod_v.at[:, cols], sem_mod.at[k])

    def stage_cp(t, hh, piece):
        d0 = piece * 256 if isinstance(piece, int) else pl.multiple_of(piece * 256, 256)
        h0 = hh * 16 if isinstance(hh, int) else pl.multiple_of(hh * 16, 16)
        return pltpu.make_async_copy(
            wqkv_hbm[t].at[pl.ds(d0, 256), pl.ds(h0, 16), :],
            stage.at[hh, pl.ds(d0, 256)], sem_stage.at[hh, piece])

    def out_cp(j):
        r0 = j * BM if isinstance(j, int) else pl.multiple_of(j * BM, BM)
        return pltpu.make_async_copy(a_v.at[pl.ds(r0, BM)], out_hbm.at[pl.ds(r0, BM)],
                                     sem_out.at[j])

    def tile(n):
        return slice(n * 128, (n + 1) * 128)

    def mod_compute(lo, hi):
        cf = c_v[...].astype(f32)
        sc = (cf * jax.nn.sigmoid(cf)).astype(bf16)
        sc = jnp.broadcast_to(sc, (8, D))
        for n in range(lo, hi):
            mod_v[:, tile(n)] = _dot(sc, wmod_v[:, tile(n)])

    def mod(k):
        return mod_v[0:1, k * D:(k + 1) * D]

    def repack(hh, ch, p0, n):
        for u in range(n):
            p = p0 + u
            a = pltpu.bitcast(stage[hh, 2 * p], u32)
            b = pltpu.bitcast(stage[hh, 2 * p + 1], u32)
            ev = (a & jnp.uint32(0xFFFF)) | (b << 16)
            od = (a >> 16) | (b & jnp.uint32(0xFFFF0000))
            w_v[pl.ds(ch * (16 * PITCH) + p, 8, stride=PITCH), :] = ev
            w_v[pl.ds(ch * (16 * PITCH) + 8 * PITCH + p, 8, stride=PITCH), :] = od

    def w_slab(ch, l, lo=0, hi=D):
        base = (ch * 16 + (l % 2) * 8 + l // 2) * PITCH + lo // 2
        if not isinstance(base, int):
            base = pl.multiple_of(base, 8)
        return _unpk(w_v[pl.ds(base, (hi - lo) // 2), :])

    def ring_of(ch, l):
        return rings[l // 2], ch * 2 + l % 2

    c_cp.start()
    mem0_cp.start()
    x0_cp.start()
    mod_cp(0, 8, 0).start()
    mod_cp(8, 16, 1).start()
    zero_s[0] = 0
    x_v[S:S + SH, :] = jnp.zeros((SH, D), bf16)
    a_v[S:S + SH, :] = jnp.zeros((SH, D), bf16)
    x0_cp.wait()
    for k in range(4):
        stage_cp(0, 0, k).start()

    def xhat_body(i, c):
        r0 = pl.multiple_of(i * 64, 64)
        for u in range(4):
            rows = pl.ds(r0 + RC * u, RC)
            xh_v[rows, :] = _ln(x_v[rows, :].astype(f32))
        return c
    lax.fori_loop(0, PRE // 64, xhat_body, 0)

    c_cp.wait()
    mem0_cp.wait()
    mod_cp(0, 8, 0).wait()
    mod_cp(8, 16, 1).wait()
    mod_compute(0, 16)

    def h0_body(i, c):
        rows = pl.ds(pl.multiple_of(i * 64, 64), 64)
        h0_v[pl.ds(pl.multiple_of(i * 32, 32), 32), :] = _pk(
            xh_v[rows, :] * (1.0 + mod(1)) + mod(0))
        return c
    lax.fori_loop(0, PRE // 64, h0_body, 0)
    mem_v[...] = pltpu.bitcast(mem0_v[...], u32)

    def first_repack(k, c):
        stage_cp(0, 0, k).wait()
        stage_cp(0, 1, k).start()

        def inner(i, cc):
            repack(0, 0, k * 128 + i * 16, 16)
            return cc
        lax.fori_loop(0, 8, inner, 0)
        return c
    lax.fori_loop(0, 4, first_repack, 0)
    for k in range(4):
        stage_cp(1, 0, k).start()

    def pre_body(i, c):
        RB = CFG['pre_rb']
        ch, it0 = i // (4 // RB), (i % (4 // RB)) * RB
        nh = (ch + 1) % 2
        cn = jnp.where(ch < 5, ch + 1, 4)
        done = {}

        @pl.when(ch < 5)
        def _():
            for rb in range(RB):
                stage_cp(0, nh, it0 + rb).wait()

        for rb in range(RB):
            it = it0 + rb
            r0 = pl.multiple_of(it * (BM // 2), BM // 2)
            for l in range(16):
                lhs = _tie(h0_v[pl.ds(r0, BM // 2), :], done.pop(l, None))
                y = _dot(_unpk(lhs), w_slab(ch, l))
                rg, ix = ring_of(ch, l)
                rg[ix, pl.ds(QOFF // 2 + r0, BM // 2), :] = _pk(y)
                if l < 15:
                    n = 9 if l < 8 else 8
                    repack(nh, cn, it * 128 + (l * 9 if l < 8 else 72 + (l - 8) * 8), n)
                if l % 2 == 1 and l < 12:
                    hr = pl.multiple_of(jnp.maximum(ch * 4 + it - 8, 0) * 96 + (l // 2) * RC, RC)
                    xs = x_v[pl.ds(PRE + hr, RC), :].astype(f32)
                    hx = _pk(_ln(xs) * (1.0 + mod(1)) + mod(0))
                    done[l + 4] = hx
                    for k in range(NT):
                        hx_v[k, pl.ds(pl.multiple_of(hr // 2, 8), 8), :] = hx[:, tile(k)]
        for tt in range(1, 3):
            @pl.when((ch + 3) // 2 == tt)
            def _():
                for rb in range(RB):
                    stage_cp(tt, nh, it0 + rb).start()

        @pl.when(i == 4 // RB - 1)
        def _():
            x1_cp.start()

        @pl.when(i == 8 // RB - 1)
        def _():
            x1_cp.wait()
            wo_cp.start()
        return c
    if CFG['pre']:
        lax.fori_loop(0, 24 // CFG['pre_rb'], pre_body, 0)

    mod_cp(16, 48, 2).start()
    for cp in (w1_cp, w2_cp, w3_cp, w4_cp):
        cp.start()
    wo_cp.wait()

    L2 = 2 * (SEG + MEM)
    r = lax.broadcasted_iota(jnp.int32, (L2, L2), 0)
    c = lax.broadcasted_iota(jnp.int32, (L2, L2), 1)
    r1 = ((r >= SEG) & (r < 2 * SEG)) | (r >= 2 * SEG + MEM)
    c1 = ((c >= SEG) & (c < 2 * SEG)) | (c >= 2 * SEG + MEM)
    same = r1 == c1
    mask = same & ((r >= 2 * SEG) | (c >= 2 * SEG) | (c <= r))
    fill = jnp.where(same, -1e9 / SCALE, -jnp.inf).astype(f32)

    def step(s, mem, zero):
        woff = pl.multiple_of((XR // 2 * s) % (RING // 2), 4)
        roff = pl.multiple_of((SEG // 2 * s + QOFF // 2) % (RING // 2), SEG // 2)
        owr = pl.multiple_of((SEG // 2 * s + OOFF // 2) % (RING // 2), SEG // 2)
        ord_ = pl.multiple_of((XR // 2 * s + OOFF // 2) % (RING // 2), 4)
        arow = pl.multiple_of(XR * s, 8)
        acc = [None] * NT
        ym, ps, om, part = {}, {}, {}, {}
        HK = D // 2
        tiles = [_unpk(jnp.concatenate(
            [hx_v[k, pl.ds(s * (XR // 2), XR // 2), :] | zero, mem[k]], axis=0))
            for k in range(NT)]
        mem_new = []

        def lhs(lo, hi):
            return jnp.concatenate(tiles[lo // 128:hi // 128], axis=1)

        def qkv_lo(h, t):
            part[(t, h)] = _dot(lhs(0, HK), w_slab(2 * t + h // 16, h % 16, 0, HK))

        def qkv(h):
            for t in range(3):
                ch, l = 2 * t + h // 16, h % 16
                if (t, h) in part:
                    y = _dot(lhs(HK, D), w_slab(ch, l, HK, D)) + part.pop((t, h))
                else:
                    y = _dot(lhs(0, D), w_slab(ch, l))
                rg, ix = ring_of(ch, l)
                rg[ix, pl.ds(woff, XR // 2), :] = _pk(y[0:XR])
                ym[(t, h)] = y[XR:XR + MEM]

        def get(t, p):
            rg, i0 = ring_of(2 * t + p // 8, (2 * p) % 16)
            mm = jnp.concatenate([ym.pop((t, 2 * p)), ym.pop((t, 2 * p + 1))], axis=0)
            return _unpk(jnp.concatenate(
                [rg[i0, pl.ds(roff, SEG // 2), :], rg[i0 + 1, pl.ds(roff, SEG // 2), :], _pk(mm)],
                axis=0))

        def sm(p):
            sc = lax.dot_general(get(0, p), get(1, p), (((1,), (1,)), ((), ())),
                                 preferred_element_type=f32)
            sc = jnp.where(mask, sc, fill)
            e = jnp.exp2((sc - jnp.max(sc, axis=-1, keepdims=True)) * (SCALE * LOG2E))
            ps[p] = (e * pl.reciprocal(jnp.sum(e, axis=-1, keepdims=True), approx=True)
                     ).astype(bf16)

        def pv(p):
            o = _dot(ps.pop(p), get(2, p))
            for j in range(2):
                h = 2 * p + j
                orings[h // GH][h % GH, pl.ds(owr, SEG // 2), :] = _pk(o[SEG * j:SEG * (j + 1)])
                om[h] = _pk(o[2 * SEG + MEM * j:2 * SEG + MEM * (j + 1)])

        def wo(g0, g1):
            olg = _unpk(jnp.concatenate(
                [jnp.concatenate([orings[h // GH][h % GH, pl.ds(ord_, XR // 2), :] | zero,
                                  om.pop(h)], axis=0)
                 for h in range(g0 * GH, g1 * GH)], axis=1))
            for n in range(NT):
                y = _dot(olg, wo_v[g0 * GH * DH:g1 * GH * DH, tile(n)])
                acc[n] = y if acc[n] is None else y + acc[n]
                if g1 == H // GH:
                    a_v[pl.ds(arow, XR), tile(n)] = acc[n][0:XR].astype(bf16)
                    mem_new.append(_pk(acc[n][XR:XR + MEM]))

        gd = [0]

        def big(h):
            if h < H:
                qkv(h)
            else:
                wo(gd[0], gd[0] + 1)
                gd[0] += 1

        for i in range(CFG['nlo']):
            qkv_lo(i // 3, i % 3)
        for i in range(NPAIR + 3):
            big(2 * i)
            if 0 <= i - 3 < NPAIR:
                pv(i - 3)
            if i < NPAIR + 2:
                big(2 * i + 1)
            if 0 <= i - 1 < NPAIR:
                sm(i - 1)
        while gd[0] < H // GH - CFG['lastg']:
            big(H)
        wo(gd[0], H // GH)
        return mem_new

    def steps(i, carry):
        zero = zero_s[0].astype(u32)
        mem = [mem_v[:, tile(k)] for k in range(NT)]
        for j in range(CFG['unroll']):
            mem = step(i * CFG['unroll'] + j, mem, zero)
        for k in range(NT):
            mem_v[:, tile(k)] = mem[k]
        return carry
    if CFG['step']:
        lax.fori_loop(0, NSEG // CFG['unroll'], steps, 0)

    def tail(b, c):
        z0 = pl.multiple_of(zero_s[0], 64)
        r0 = pl.multiple_of(b * (BM // 2), BM // 2)
        for n in range(NT):
            o = jnp.concatenate([orings[h // GH][h % GH, pl.ds(r0, BM // 2), :] for h in range(H)],
                                axis=1)
            a_v[pl.ds(S - PRE + 2 * r0, BM), tile(n)] = (
                _dot(_unpk(o), wo_v[pl.ds(z0, H * DH), tile(n)]).astype(bf16))
        return c
    if CFG['tail']:
        lax.fori_loop(0, PRE // BM, tail, 0)

    if not CFG['b']:
        cp = pltpu.make_async_copy(a_v.at[pl.ds(0, S)], out_hbm, sem_out.at[0])
        cp.start()
        cp.wait()
        return

    mod_cp(16, 48, 2).wait()
    for cp in (w1_cp, w2_cp, w3_cp, w4_cp):
        cp.wait()
    mod_compute(16, 48)

    def p0(tok, w):
        rows = pl.ds(tok, RC)
        xa = x_v[rows, :].astype(f32) + mod(2) * a_v[rows, :].astype(f32)
        hb = _ln(xa) * (1.0 + mod(4)) + mod(3)
        xa_v[w:w + RC, :] = xa
        hb_v[w:w + RC, :] = hb
        return _pk(_ln(hb))

    y0 = p0(0, 0)
    for k in range(BM // RC):
        y1_v[k * 8:(k + 1) * 8, :] = p0(SH + k * RC, SH + k * RC)
    for n in range(NT):
        g_v[n, 0:8, :] = jnp.zeros((8, 128), f32)
        g_v[n, 8:8 + SH, :] = _gelu(_dot(_unpk(y0), w1_v[:, tile(n)]))

    HM = BM // 2
    shift = (-1, 1, -2, 2)

    def blk(j, c):
        r0 = pl.multiple_of(j * BM, BM)
        nxt = pl.multiple_of(jnp.minimum(j + 1, NB - 1) * BM + SH, SH)
        more = j < NB - 1

        def w1_half(hf):
            for n in range(NT):
                g = _gelu(_dot(_unpk(y1_v[hf * 32:(hf + 1) * 32, :]), w1_v[:, tile(n)]))
                w0 = 8 + SH + hf * HM
                if hf == 0:
                    g_v[n, w0:w0 + HM, :] = g
                else:
                    g_v[n, w0:w0 + HM - SH, :] = g[0:HM - SH]
                    g_v[n, w0 + HM - SH:w0 + HM, :] = jnp.where(more, g[HM - SH:HM], 0.0)

        def w2_half(hf):
            for n in range(NT):
                w0 = 8 + hf * HM + shift[n // 2]
                z_v[hf * 32:(hf + 1) * 32, tile(n)] = _pk(g_v[n, w0:w0 + HM, :])
            for n in range(NT):
                x1_v[hf * HM:(hf + 1) * HM, tile(n)] = (
                    _dot(_unpk(z_v[hf * 32:(hf + 1) * 32, :]), w2_v[:, tile(n)])
                    + hb_v[hf * HM:(hf + 1) * HM, tile(n)])

        def p1_half(hf):
            for k in range(hf * HM // RC, (hf + 1) * HM // RC):
                x1 = x1_v[k * RC:(k + 1) * RC, :]
                y2_v[k * 8:(k + 1) * 8, :] = _pk(_ln(x1))
                base_v[k * RC:(k + 1) * RC, :] = xa_v[k * RC:(k + 1) * RC, :] + mod(5) * x1

        def w3(f, lo, hi, after=None):
            u_v[lo:hi, tile(f)] = _pk(_gelu(
                _dot(_unpk(_tie(y2_v[lo:hi, :], after)), w3_v[:, tile(f)])))

        w1_half(0)
        w1_half(1)
        w2_half(0)
        w2_half(1)
        p1_half(0)
        for f in range(CFG['nf']):
            w3(f, 0, 32)
        p1_half(1)
        for f in range(CFG['nf']):
            w3(f, 32, 64)
        for n in range(NT):
            g_v[n, 0:8 + SH, :] = g_v[n, BM:BM + 8 + SH, :]
        xa_v[0:SH, :] = xa_v[BM:BM + SH, :]
        hb_v[0:SH, :] = hb_v[BM:BM + SH, :]
        for f in range(CFG['nf'], NF):
            w3(f, 0, 64)
        for n in range(NT):
            y = p0(nxt + n * RC, SH + n * RC)
            y1_v[n * 8:(n + 1) * 8, :] = y
            gb = mod_v[0:1, 5 * D + n * 128:5 * D + (n + 1) * 128]
            u = _unpk(_tie(u_v[...], y, 0, CFG['p0k']))
            a_v[pl.ds(r0, BM), tile(n)] = (
                base_v[:, tile(n)] + gb * _dot(u, w4_v[:, tile(n)])).astype(bf16)
        out_cp(j).start()
        return c
    lax.fori_loop(0, NB, blk, 0)
    for j in range(NB):
        out_cp(j).wait()


@functools.partial(jax.jit, static_argnames=("A_seg_len",))
def pallas_adaLN_cond__memory_aug_recurrent_mem_tr__mixer_s_mlp__prompt_kernel(
    A_x: jax.Array,
    A_mem0: jax.Array,
    A_Wq: jax.Array,
    A_Wk: jax.Array,
    A_Wv: jax.Array,
    A_Wo: jax.Array,
    A_seg_len,
    B_x: jax.Array,
    B_w1: jax.Array,
    B_w2: jax.Array,
    B_w3: jax.Array,
    B_w4: jax.Array,
    c: jax.Array,
    w_mod: jax.Array,
):
    assert A_seg_len == SEG and A_x.shape == (1, S, D) and A_Wq.shape == (D, H, DH)
    any_spec = pl.BlockSpec(memory_space=pl.ANY)
    out = pl.pallas_call(
        _kernel,
        out_shape=jax.ShapeDtypeStruct((S, D), bf16),
        in_specs=[any_spec] * 12,
        out_specs=any_spec,
        scratch_shapes=[
            pltpu.VMEM((1, D), bf16),
            pltpu.VMEM((S + SH, D), bf16),
            pltpu.VMEM((S + SH, D), bf16),
            pltpu.VMEM((PRE // 2, D), u32),
            pltpu.VMEM((MEM // 2, D), u32),
            pltpu.VMEM((MEM, D), bf16),
            pltpu.VMEM((8, 6 * D), f32),
            pltpu.VMEM((D, 6 * D + PADL), bf16),
            pltpu.VMEM((96 * PITCH, 128), u32),
            pltpu.VMEM((H * DH, D + PADL), bf16),
            pltpu.VMEM((D, D + PADL), bf16),
            pltpu.VMEM((D, D + PADL), bf16),
            pltpu.VMEM((D, F + PADL), bf16),
            pltpu.VMEM((F, D + PADL), bf16),
            pltpu.VMEM((NT, BM + 32, 128), f32),
            pltpu.VMEM((BM + SH, D), f32),
            pltpu.VMEM((BM + SH, D), f32),
            pltpu.VMEM((BM, D), f32),
            pltpu.VMEM((BM, D), f32),
            pltpu.VMEM((BM // 2, D), u32),
            pltpu.VMEM((BM // 2, D), u32),
            pltpu.VMEM((BM // 2, D), u32),
            pltpu.VMEM((BM // 2, F), u32),
            pltpu.VMEM((2, D, 16, DH), bf16),
            pltpu.VMEM((PRE, D), f32),
            pltpu.VMEM((NT, HR, 128), u32),
        ] + [pltpu.VMEM((12, RING // 2, DH), u32)] * 8
          + [pltpu.VMEM((GH, RING // 2, DH), u32)] * (H // GH) + [
            pltpu.SMEM((1,), jnp.int32),
            pltpu.SemaphoreType.DMA((2,)),
            pltpu.SemaphoreType.DMA((2,)),
            pltpu.SemaphoreType.DMA((2, 4)),
            pltpu.SemaphoreType.DMA((3,)),
            pltpu.SemaphoreType.DMA((5,)),
            pltpu.SemaphoreType.DMA((NB,)),
        ],
        compiler_params=pltpu.CompilerParams(vmem_limit_bytes=120 * 1024 * 1024),
    )(A_x.reshape(S, D), A_mem0.reshape(MEM, D), A_Wq, A_Wk, A_Wv, A_Wo.reshape(H * DH, D),
      B_w1, B_w2, B_w3, B_w4, c, w_mod)
    return out.reshape(1, S, D)
```

```python
import functools

import jax
import jax.numpy as jnp
from jax import lax
import jax.experimental.pallas as pl
import jax.experimental.pallas.tpu as pltpu

bf16, f32, u32 = jnp.bfloat16, jnp.float32, jnp.uint32

S, D, H, DH, MEM, SEG, F = 2048, 1024, 32, 128, 8, 32, 3584
NSEG = S // SEG
XR = 24
PRE = S - XR * NSEG
RING = 576
QOFF = RING - PRE
OOFF = 192
PITCH = 520
NT = D // 128
NF = F // 128
BM = 128
NB = S // BM
GH = 4
NPAIR = H // 2
HR = (S - PRE) // 2
PADL = 128
SH = 16
KP = 256
RC = 16
EPS = 1e-5
LOG2E = 1.4426950408889634
SCALE = DH ** -0.5
CFG = dict(pre=True, step=True, tail=True, b=True, pre_rb=2, unroll=2, nlo=6, lastg=2, nf=7, p0k=24)


def _ln(x):
    m = jnp.mean(x, axis=-1, keepdims=True)
    xc = x - m
    v = jnp.mean(xc * xc, axis=-1, keepdims=True)
    return xc * lax.rsqrt(v + EPS)


def _gelu(x):
    return jax.nn.gelu(x, approximate=True)


def _dot(a, b):
    return jnp.dot(a, b, preferred_element_type=f32)


def _pk(x):
    return pltpu.bitcast(x.astype(bf16), u32)


def _unpk(x):
    return pltpu.bitcast(x, bf16)


def _tie(w, after, r=0, k=0):
    if after is None:
        return w
    m = functools.reduce(lambda a, b: a & b,
                         [after[:, i * 128:(i + 1) * 128] for i in range(after.shape[1] // 128)])
    mf = pltpu.bitcast(m, f32)
    z = jnp.where(mf * mf < 0.0, jnp.uint32(1), jnp.uint32(0))
    row = w[r:r + 8]
    parts = [row[:, :k * 128], row[:, k * 128:(k + 1) * 128] | z, row[:, (k + 1) * 128:]]
    row = jnp.concatenate([p for p in parts if p.shape[1]], axis=1)
    parts = [w[:r], row, w[r + 8:]]
    return jnp.concatenate([p for p in parts if p.shape[0]], axis=0)


def _kernel(x_hbm, mem0_hbm, wq_hbm, wk_hbm, wv_hbm, wo_hbm, w1_hbm, w2_hbm, w3_hbm, w4_hbm,
            c_hbm, wmod_hbm, out_hbm,
            c_v, x_v, a_v, h0_v, mem_v, mem0_v, mod_v, wmod_v, w_v, wo_v,
            w1_v, w2_v, w3_v, w4_v,
            g_v, xa_v, hb_v, base_v, x1_v, y1_v, z_v, y2_v, u_v,
            stage, xh_v, hx_v, acc_v,
            r0_, r1_, r2_, r3_, r4_, r5_, r6_, r7_, o0_, o1_, o2_, o3_, o4_, o5_, o6_, o7_,
            zero_s, sem_small, sem_x, sem_stage, sem_mod, sem_w, sem_out):
    wqkv_hbm = (wq_hbm, wk_hbm, wv_hbm)
    rings = (r0_, r1_, r2_, r3_, r4_, r5_, r6_, r7_)
    orings = (o0_, o1_, o2_, o3_, o4_, o5_, o6_, o7_)

    c_cp = pltpu.make_async_copy(c_hbm, c_v, sem_small.at[0])
    mem0_cp = pltpu.make_async_copy(mem0_hbm, mem0_v, sem_small.at[1])

    def x_cp(q):
        rows = pl.ds(q * PRE, PRE)
        return pltpu.make_async_copy(x_hbm.at[rows], x_v.at[rows], sem_x.at[q])

    def w_cp(src, dst, k):
        return pltpu.make_async_copy(src, dst.at[:, pl.ds(0, src.shape[1])], sem_w.at[k])

    wo_cp, w1_cp, w2_cp, w3_cp, w4_cp = (
        w_cp(a, b, k) for k, (a, b) in enumerate(
            ((wo_hbm, wo_v), (w1_hbm, w1_v), (w2_hbm, w2_v), (w3_hbm, w3_v), (w4_hbm, w4_v))))

    def mod0_cp(j, k):
        cols = pl.ds(j * D + k * KP, KP)
        return pltpu.make_async_copy(wmod_hbm.at[:, cols], w3_v.at[:, cols], sem_mod.at[j, k])

    mod1_cp = pltpu.make_async_copy(wmod_hbm.at[:, pl.ds(2 * D, 4 * D)],
                                    wmod_v.at[:, pl.ds(0, 4 * D)], sem_w.at[5])

    def stage_cp(t, hh, piece):
        d0 = piece * KP if isinstance(piece, int) else pl.multiple_of(piece * KP, KP)
        return pltpu.make_async_copy(
            wqkv_hbm[t].at[pl.ds(d0, KP), pl.ds(hh * 16, 16), :],
            stage.at[hh, pl.ds(d0, KP)], sem_stage.at[hh, piece])

    def out_cp(j):
        r0 = j * BM if isinstance(j, int) else pl.multiple_of(j * BM, BM)
        return pltpu.make_async_copy(a_v.at[pl.ds(r0, BM)], out_hbm.at[pl.ds(r0, BM)],
                                     sem_out.at[j])

    def tile(n):
        return slice(n * 128, (n + 1) * 128)

    def mod_compute(src, tiles, off):
        cf = c_v[...].astype(f32)
        sc = (cf * jax.nn.sigmoid(cf)).astype(bf16)
        sc = jnp.broadcast_to(sc, (8, D))
        for n in tiles:
            mod_v[:, tile(n + off)] = _dot(sc, src[:, tile(n)])

    def mod(k):
        return mod_v[0:1, k * D:(k + 1) * D]

    def repack(hh, ch, p0, n):
        for u in range(n):
            p = p0 + u
            a = pltpu.bitcast(stage[hh, 2 * p], u32)
            b = pltpu.bitcast(stage[hh, 2 * p + 1], u32)
            ev = (a & jnp.uint32(0xFFFF)) | (b << 16)
            od = (a >> 16) | (b & jnp.uint32(0xFFFF0000))
            w_v[pl.ds(ch * (16 * PITCH) + p, 8, stride=PITCH), :] = ev
            w_v[pl.ds(ch * (16 * PITCH) + 8 * PITCH + p, 8, stride=PITCH), :] = od

    def w_slab(ch, l, lo=0, hi=D):
        base = (ch * 16 + (l % 2) * 8 + l // 2) * PITCH + lo // 2
        return _unpk(w_v[base:base + (hi - lo) // 2, :])

    def ring_of(ch, l):
        return rings[l // 2], ch * 2 + l % 2

    c_cp.start()
    mem0_cp.start()
    x_cp(0).start()
    stage_cp(0, 0, 0).start()
    zero_s[0] = 0
    x_v[S:S + SH, :] = jnp.zeros((SH, D), bf16)
    a_v[S:S + SH, :] = jnp.zeros((SH, D), bf16)
    mod_v[...] = jnp.zeros(mod_v.shape, f32)
    mod0_cp(0, 0).start()
    mod0_cp(1, 0).start()
    x_cp(0).wait()
    stage_cp(0, 1, 0).start()
    stage_cp(0, 0, 1).start()

    def xhat_body(i, c):
        r0 = pl.multiple_of(i * 64, 64)
        for u in range(4):
            rows = pl.ds(r0 + RC * u, RC)
            xh_v[rows, :] = _ln(x_v[rows, :].astype(f32))
        return c
    lax.fori_loop(0, PRE // 64, xhat_body, 0)

    c_cp.wait()
    mem0_cp.wait()
    mem_v[...] = pltpu.bitcast(mem0_v[...], u32)
    stage_cp(0, 0, 0).wait()

    def first_repack(i, c):
        repack(0, 0, i * 16, 16)
        return c
    lax.fori_loop(0, KP // 32, first_repack, 0)

    NPC = D // KP
    assert NPC == 4

    def pre_body(i, c):
        t, k = i >> 2, i & 3
        i1 = jnp.minimum(i + 1, 3 * NPC - 1)
        t1, k1 = i1 >> 2, i1 & 3

        for kk in range(NPC):
            @pl.when(i == kk)
            def _():
                mod0_cp(0, kk).wait()
                mod0_cp(1, kk).wait()
                tl = range(kk * KP // 128, (kk + 1) * KP // 128)
                mod_compute(w3_v, list(tl) + [NT + n for n in tl], 0)
                cols = slice(kk * KP, (kk + 1) * KP)
                sa = mod_v[0:1, kk * KP:(kk + 1) * KP]
                ca = mod_v[0:1, D + kk * KP:D + (kk + 1) * KP]
                for q in range(PRE // 64):
                    h0_v[kk, q * 32:(q + 1) * 32, :] = _pk(
                        xh_v[q * 64:(q + 1) * 64, cols] * (1.0 + ca) + sa)
                if kk + 1 < NPC:
                    mod0_cp(0, kk + 1).start()
                    mod0_cp(1, kk + 1).start()
                stage_cp((kk + 1) // NPC, 1, (kk + 1) % NPC).start()
                stage_cp((kk + 2) // NPC, 0, (kk + 2) % NPC).start()
                if kk in (1, 2):
                    x_cp(kk).start()

        stage_cp(0, 1, k).wait()

        @pl.when(i < 3 * NPC - 1)
        def _():
            stage_cp(0, 0, k1).wait()

        z0 = pl.multiple_of(zero_s[0], 64)
        w0 = pl.multiple_of(t * (32 * PITCH) + k * (KP // 2), 32)
        xrow = jnp.where(i >= NPC, PRE + (i - NPC) * 192, 0)
        hrow = jnp.maximum(i - NPC, 0) * 96
        done = {}
        nd = 0
        for h in range(H):
            hh, l = h // 16, h % 16
            w = _unpk(w_v[pl.ds(w0 + (hh * 16 + (l % 2) * 8 + l // 2) * PITCH, KP // 2), :])
            for rb in range(PRE // BM):
                lhs = _tie(h0_v[k, rb * 64:(rb + 1) * 64, :], done.pop(nd, None))
                rows = pl.ds(z0 + rb * BM, BM)
                y = _dot(_unpk(lhs), w) + jnp.where(k > 0, acc_v[h, rows, :], 0.0)
                acc_v[h, rows, :] = y
                rings[l // 2][t * 4 + hh * 2 + l % 2,
                              QOFF // 2 + rb * 64:QOFF // 2 + (rb + 1) * 64, :] = _pk(y)
                nd += 1
            if l < 15:
                n = 9 if l < 8 else 8
                p0_ = l * 9 if l < 8 else 72 + (l - 8) * 8
                if hh == 0:
                    repack(1, 2 * t + 1 + zero_s[0], k * (KP // 2) + p0_, n)
                else:
                    repack(0, 2 * t1, k1 * (KP // 2) + p0_, n)
            if h % 2 == 1 and h < 24:
                q = h // 2
                xs = x_v[pl.ds(pl.multiple_of(xrow + q * RC, RC), RC), :].astype(f32)
                hx = _pk(_ln(xs) * (1.0 + mod(1)) + mod(0))
                done[nd + 12] = hx
                for n in range(NT):
                    hx_v[n, pl.ds(pl.multiple_of(hrow + q * 8, 8), 8), :] = hx[:, tile(n)]
        for tt in range(1, 3):
            @pl.when(jnp.logical_and(i >= NPC - 2, (i + 3) >> 2 == tt))
            def _():
                stage_cp(tt, 1, (i + 3) & 3).start()

            @pl.when(jnp.logical_and(i >= NPC - 2, t + 1 == tt))
            def _():
                stage_cp(tt, 0, k).start()

        @pl.when(i == NPC - 1)
        def _():
            x_cp(1).wait()
            x_cp(2).wait()
            x_cp(3).start()

        @pl.when(i == NPC)
        def _():
            wo_cp.start()

        @pl.when(i == NPC + 1)
        def _():
            x_cp(3).wait()
        return c
    if CFG['pre']:
        lax.fori_loop(0, 3 * NPC, pre_body, 0)

    mod1_cp.start()
    for cp in (w1_cp, w2_cp, w3_cp, w4_cp):
        cp.start()
    wo_cp.wait()

    L2 = 2 * (SEG + MEM)
    r = lax.broadcasted_iota(jnp.int32, (L2, L2), 0)
    c = lax.broadcasted_iota(jnp.int32, (L2, L2), 1)
    r1 = ((r >= SEG) & (r < 2 * SEG)) | (r >= 2 * SEG + MEM)
    c1 = ((c >= SEG) & (c < 2 * SEG)) | (c >= 2 * SEG + MEM)
    same = r1 == c1
    mask = same & ((r >= 2 * SEG) | (c >= 2 * SEG) | (c <= r))
    fill = jnp.where(same, -1e9 / SCALE, -jnp.inf).astype(f32)

    def step(s, mem, zero):
        woff = pl.multiple_of((XR // 2 * s) % (RING // 2), 4)
        roff = pl.multiple_of((SEG // 2 * s + QOFF // 2) % (RING // 2), SEG // 2)
        owr = pl.multiple_of((SEG // 2 * s + OOFF // 2) % (RING // 2), SEG // 2)
        ord_ = pl.multiple_of((XR // 2 * s + OOFF // 2) % (RING // 2), 4)
        arow = pl.multiple_of(XR * s, 8)
        acc = [None] * NT
        ym, ps, om, part = {}, {}, {}, {}
        HK = D // 2
        tiles = [_unpk(jnp.concatenate(
            [hx_v[k, pl.ds(s * (XR // 2), XR // 2), :] | zero, mem[k]], axis=0))
            for k in range(NT)]
        mem_new = []

        def lhs(lo, hi):
            return jnp.concatenate(tiles[lo // 128:hi // 128], axis=1)

        def qkv_lo(h, t):
            part[(t, h)] = _dot(lhs(0, HK), w_slab(2 * t + h // 16, h % 16, 0, HK))

        def qkv(h):
            for t in range(3):
                ch, l = 2 * t + h // 16, h % 16
                if (t, h) in part:
                    y = _dot(lhs(HK, D), w_slab(ch, l, HK, D)) + part.pop((t, h))
                else:
                    y = _dot(lhs(0, D), w_slab(ch, l))
                rg, ix = ring_of(ch, l)
                rg[ix, pl.ds(woff, XR // 2), :] = _pk(y[0:XR])
                ym[(t, h)] = y[XR:XR + MEM]

        def get(t, p):
            rg, i0 = ring_of(2 * t + p // 8, (2 * p) % 16)
            mm = jnp.concatenate([ym.pop((t, 2 * p)), ym.pop((t, 2 * p + 1))], axis=0)
            return _unpk(jnp.concatenate(
                [rg[i0, pl.ds(roff, SEG // 2), :], rg[i0 + 1, pl.ds(roff, SEG // 2), :], _pk(mm)],
                axis=0))

        def sm(p):
            sc = lax.dot_general(get(0, p), get(1, p), (((1,), (1,)), ((), ())),
                                 preferred_element_type=f32)
            sc = jnp.where(mask, sc, fill)
            e = jnp.exp2((sc - jnp.max(sc, axis=-1, keepdims=True)) * (SCALE * LOG2E))
            ps[p] = (e * pl.reciprocal(jnp.sum(e, axis=-1, keepdims=True), approx=True)
                     ).astype(bf16)

        def pv(p):
            o = _dot(ps.pop(p), get(2, p))
            for j in range(2):
                h = 2 * p + j
                orings[h // GH][h % GH, pl.ds(owr, SEG // 2), :] = _pk(o[SEG * j:SEG * (j + 1)])
                om[h] = _pk(o[2 * SEG + MEM * j:2 * SEG + MEM * (j + 1)])

        def wo(g0, g1):
            olg = _unpk(jnp.concatenate(
                [jnp.concatenate([orings[h // GH][h % GH, pl.ds(ord_, XR // 2), :] | zero,
                                  om.pop(h)], axis=0)
                 for h in range(g0 * GH, g1 * GH)], axis=1))
            for n in range(NT):
                y = _dot(olg, wo_v[g0 * GH * DH:g1 * GH * DH, tile(n)])
                acc[n] = y if acc[n] is None else y + acc[n]
                if g1 == H // GH:
                    a_v[pl.ds(arow, XR), tile(n)] = acc[n][0:XR].astype(bf16)
                    mem_new.append(_pk(acc[n][XR:XR + MEM]))

        gd = [0]

        def big(h):
            if h < H:
                qkv(h)
            else:
                wo(gd[0], gd[0] + 1)
                gd[0] += 1

        for i in range(CFG['nlo']):
            qkv_lo(i // 3, i % 3)
        for i in range(NPAIR + 3):
            big(2 * i)
            if 0 <= i - 3 < NPAIR:
                pv(i - 3)
            if i < NPAIR + 2:
                big(2 * i + 1)
            if 0 <= i - 1 < NPAIR:
                sm(i - 1)
        while gd[0] < H // GH - CFG['lastg']:
            big(H)
        wo(gd[0], H // GH)
        return mem_new

    def steps(i, carry):
        zero = zero_s[0].astype(u32)
        mem = [mem_v[:, tile(k)] for k in range(NT)]
        for j in range(CFG['unroll']):
            mem = step(i * CFG['unroll'] + j, mem, zero)
        for k in range(NT):
            mem_v[:, tile(k)] = mem[k]
        return carry
    if CFG['step']:
        lax.fori_loop(0, NSEG // CFG['unroll'], steps, 0)

    def tail(b, c):
        z0 = pl.multiple_of(zero_s[0], 64)
        r0 = pl.multiple_of(b * (BM // 2), BM // 2)
        for n in range(NT):
            o = jnp.concatenate([orings[h // GH][h % GH, pl.ds(r0, BM // 2), :] for h in range(H)],
                                axis=1)
            a_v[pl.ds(S - PRE + 2 * r0, BM), tile(n)] = (
                _dot(_unpk(o), wo_v[pl.ds(z0, H * DH), tile(n)]).astype(bf16))
        return c
    if CFG['tail']:
        lax.fori_loop(0, PRE // BM, tail, 0)

    if not CFG['b']:
        cp = pltpu.make_async_copy(a_v.at[pl.ds(0, S)], out_hbm, sem_out.at[0])
        cp.start()
        cp.wait()
        return

    mod1_cp.wait()
    for cp in (w1_cp, w2_cp, w3_cp, w4_cp):
        cp.wait()
    mod_compute(wmod_v, range(4 * NT), 2 * NT)

    def p0(tok, w):
        rows = pl.ds(tok, RC)
        xa = x_v[rows, :].astype(f32) + mod(2) * a_v[rows, :].astype(f32)
        hb = _ln(xa) * (1.0 + mod(4)) + mod(3)
        xa_v[w:w + RC, :] = xa
        hb_v[w:w + RC, :] = hb
        return _pk(_ln(hb))

    y0 = p0(0, 0)
    for k in range(BM // RC):
        y1_v[k * 8:(k + 1) * 8, :] = p0(SH + k * RC, SH + k * RC)
    for n in range(NT):
        g_v[n, 0:8, :] = jnp.zeros((8, 128), f32)
        g_v[n, 8:8 + SH, :] = _gelu(_dot(_unpk(y0), w1_v[:, tile(n)]))

    HM = BM // 2
    shift = (-1, 1, -2, 2)

    def blk(j, c):
        r0 = pl.multiple_of(j * BM, BM)
        nxt = pl.multiple_of(jnp.minimum(j + 1, NB - 1) * BM + SH, SH)
        more = j < NB - 1

        def w1_half(hf):
            for n in range(NT):
                g = _gelu(_dot(_unpk(y1_v[hf * 32:(hf + 1) * 32, :]), w1_v[:, tile(n)]))
                w0 = 8 + SH + hf * HM
                if hf == 0:
                    g_v[n, w0:w0 + HM, :] = g
                else:
                    g_v[n, w0:w0 + HM - SH, :] = g[0:HM - SH]
                    g_v[n, w0 + HM - SH:w0 + HM, :] = jnp.where(more, g[HM - SH:HM], 0.0)

        def w2_half(hf):
            for n in range(NT):
                w0 = 8 + hf * HM + shift[n // 2]
                z_v[hf * 32:(hf + 1) * 32, tile(n)] = _pk(g_v[n, w0:w0 + HM, :])
            for n in range(NT):
                x1_v[hf * HM:(hf + 1) * HM, tile(n)] = (
                    _dot(_unpk(z_v[hf * 32:(hf + 1) * 32, :]), w2_v[:, tile(n)])
                    + hb_v[hf * HM:(hf + 1) * HM, tile(n)])

        def p1_half(hf):
            for k in range(hf * HM // RC, (hf + 1) * HM // RC):
                x1 = x1_v[k * RC:(k + 1) * RC, :]
                y2_v[k * 8:(k + 1) * 8, :] = _pk(_ln(x1))
                base_v[k * RC:(k + 1) * RC, :] = xa_v[k * RC:(k + 1) * RC, :] + mod(5) * x1

        def w3(f, lo, hi, after=None):
            u_v[lo:hi, tile(f)] = _pk(_gelu(
                _dot(_unpk(_tie(y2_v[lo:hi, :], after)), w3_v[:, tile(f)])))

        w1_half(0)
        w1_half(1)
        w2_half(0)
        w2_half(1)
        p1_half(0)
        for f in range(CFG['nf']):
            w3(f, 0, 32)
        p1_half(1)
        for f in range(CFG['nf']):
            w3(f, 32, 64)
        for n in range(NT):
            g_v[n, 0:8 + SH, :] = g_v[n, BM:BM + 8 + SH, :]
        xa_v[0:SH, :] = xa_v[BM:BM + SH, :]
        hb_v[0:SH, :] = hb_v[BM:BM + SH, :]
        for f in range(CFG['nf'], NF):
            w3(f, 0, 64)
        for n in range(NT):
            y = p0(nxt + n * RC, SH + n * RC)
            y1_v[n * 8:(n + 1) * 8, :] = y
            gb = mod_v[0:1, 5 * D + n * 128:5 * D + (n + 1) * 128]
            u = _unpk(_tie(u_v[...], y, 0, CFG['p0k']))
            a_v[pl.ds(r0, BM), tile(n)] = (
                base_v[:, tile(n)] + gb * _dot(u, w4_v[:, tile(n)])).astype(bf16)
        out_cp(j).start()
        return c
    lax.fori_loop(0, NB, blk, 0)
    for j in range(NB):
        out_cp(j).wait()


@functools.partial(jax.jit, static_argnames=("A_seg_len",))
def pallas_adaLN_cond__memory_aug_recurrent_mem_tr__mixer_s_mlp__prompt_kernel(
    A_x: jax.Array,
    A_mem0: jax.Array,
    A_Wq: jax.Array,
    A_Wk: jax.Array,
    A_Wv: jax.Array,
    A_Wo: jax.Array,
    A_seg_len,
    B_x: jax.Array,
    B_w1: jax.Array,
    B_w2: jax.Array,
    B_w3: jax.Array,
    B_w4: jax.Array,
    c: jax.Array,
    w_mod: jax.Array,
):
    assert A_seg_len == SEG and A_x.shape == (1, S, D) and A_Wq.shape == (D, H, DH)
    any_spec = pl.BlockSpec(memory_space=pl.ANY)
    out = pl.pallas_call(
        _kernel,
        out_shape=jax.ShapeDtypeStruct((S, D), bf16),
        in_specs=[any_spec] * 12,
        out_specs=any_spec,
        scratch_shapes=[
            pltpu.VMEM((1, D), bf16),
            pltpu.VMEM((S + SH, D), bf16),
            pltpu.VMEM((S + SH, D), bf16),
            pltpu.VMEM((D // KP, PRE // 2, KP), u32),
            pltpu.VMEM((MEM // 2, D), u32),
            pltpu.VMEM((MEM, D), bf16),
            pltpu.VMEM((8, 6 * D), f32),
            pltpu.VMEM((D, 4 * D + PADL), bf16),
            pltpu.VMEM((96 * PITCH, 128), u32),
            pltpu.VMEM((H * DH, D + PADL), bf16),
            pltpu.VMEM((D, D + PADL), bf16),
            pltpu.VMEM((D, D + PADL), bf16),
            pltpu.VMEM((D, F + PADL), bf16),
            pltpu.VMEM((F, D + PADL), bf16),
            pltpu.VMEM((NT, BM + 32, 128), f32),
            pltpu.VMEM((BM + SH, D), f32),
            pltpu.VMEM((BM + SH, D), f32),
            pltpu.VMEM((BM, D), f32),
            pltpu.VMEM((BM, D), f32),
            pltpu.VMEM((BM // 2, D), u32),
            pltpu.VMEM((BM // 2, D), u32),
            pltpu.VMEM((BM // 2, D), u32),
            pltpu.VMEM((BM // 2, F), u32),
            pltpu.VMEM((2, D, 16, DH), bf16),
            pltpu.VMEM((PRE, D), f32),
            pltpu.VMEM((NT, HR, 128), u32),
            pltpu.VMEM((H, PRE, DH), f32),
        ] + [pltpu.VMEM((12, RING // 2, DH), u32)] * 8
          + [pltpu.VMEM((GH, RING // 2, DH), u32)] * (H // GH) + [
            pltpu.SMEM((1,), jnp.int32),
            pltpu.SemaphoreType.DMA((2,)),
            pltpu.SemaphoreType.DMA((4,)),
            pltpu.SemaphoreType.DMA((2, 4)),
            pltpu.SemaphoreType.DMA((2, 4)),
            pltpu.SemaphoreType.DMA((6,)),
            pltpu.SemaphoreType.DMA((NB,)),
        ],
        compiler_params=pltpu.CompilerParams(vmem_limit_bytes=120 * 1024 * 1024),
    )(A_x.reshape(S, D), A_mem0.reshape(MEM, D), A_Wq, A_Wk, A_Wv, A_Wo.reshape(H * DH, D),
      B_w1, B_w2, B_w3, B_w4, c, w_mod)
    return out.reshape(1, S, D)
```

```python
import functools

import jax
import jax.numpy as jnp
from jax import lax
import jax.experimental.pallas as pl
import jax.experimental.pallas.tpu as pltpu

bf16, f32, u32 = jnp.bfloat16, jnp.float32, jnp.uint32

S, D, H, DH, MEM, SEG, F = 2048, 1024, 32, 128, 8, 32, 3584
NSEG = S // SEG
XR = 24
PRE = S - XR * NSEG
RING = 576
QOFF = RING - PRE
PITCH = 520
NT = D // 128
NF = F // 128
BM = 128
NB = S // BM
NPAIR = H // 2
HR = (S - PRE) // 2
PADL = 128
SH = 16
KP = 256
RC = 16
EPS = 1e-5
LOG2E = 1.4426950408889634
SCALE = DH ** -0.5
CFG = dict(pre=True, step=True, b=True, nlo=6, he=24, nf=7, p0k=24)


def _ln(x):
    m = jnp.mean(x, axis=-1, keepdims=True)
    xc = x - m
    v = jnp.mean(xc * xc, axis=-1, keepdims=True)
    return xc * lax.rsqrt(v + EPS)


def _gelu(x):
    return jax.nn.gelu(x, approximate=True)


def _dot(a, b):
    return jnp.dot(a, b, preferred_element_type=f32)


def _pk(x):
    return pltpu.bitcast(x.astype(bf16), u32)


def _unpk(x):
    return pltpu.bitcast(x, bf16)


def _tie(w, after, r=0, k=0):
    if after is None:
        return w
    m = functools.reduce(lambda a, b: a & b,
                         [after[:, i * 128:(i + 1) * 128] for i in range(after.shape[1] // 128)])
    mf = pltpu.bitcast(m, f32)
    z = jnp.where(mf * mf < 0.0, jnp.uint32(1), jnp.uint32(0))
    row = w[r:r + 8]
    parts = [row[:, :k * 128], row[:, k * 128:(k + 1) * 128] | z, row[:, (k + 1) * 128:]]
    row = jnp.concatenate([p for p in parts if p.shape[1]], axis=1)
    parts = [w[:r], row, w[r + 8:]]
    return jnp.concatenate([p for p in parts if p.shape[0]], axis=0)


def _kernel(x_hbm, mem0_hbm, wq_hbm, wk_hbm, wv_hbm, wo_hbm, w1_hbm, w2_hbm, w3_hbm, w4_hbm,
            c_hbm, wmod_hbm, out_hbm,
            c_v, x_v, a_v, h0_v, mem_v, mem0_v, mod_v, wmod_v, w_v, wo_v,
            w1_v, w2_v, w3_v, w4_v,
            g_v, xa_v, hb_v, base_v, x1_v, y1_v, z_v, y2_v, u_v,
            stage, xh_v, hx_v, acc_v,
            r0_, r1_, r2_, r3_, r4_, r5_, r6_, r7_,
            zero_s, sem_small, sem_x, sem_stage, sem_mod, sem_w, sem_out):
    wqkv_hbm = (wq_hbm, wk_hbm, wv_hbm)
    rings = (r0_, r1_, r2_, r3_, r4_, r5_, r6_, r7_)

    c_cp = pltpu.make_async_copy(c_hbm, c_v, sem_small.at[0])
    mem0_cp = pltpu.make_async_copy(mem0_hbm, mem0_v, sem_small.at[1])

    def x_cp(q):
        rows = pl.ds(q * PRE, PRE)
        return pltpu.make_async_copy(x_hbm.at[rows], x_v.at[rows], sem_x.at[q])

    def w_cp(src, dst, k):
        return pltpu.make_async_copy(src, dst.at[:, pl.ds(0, src.shape[1])], sem_w.at[k])

    wo_cp, w1_cp, w2_cp, w3_cp, w4_cp = (
        w_cp(a, b, k) for k, (a, b) in enumerate(
            ((wo_hbm, wo_v), (w1_hbm, w1_v), (w2_hbm, w2_v), (w3_hbm, w3_v), (w4_hbm, w4_v))))

    def mod0_cp(j, k):
        cols = pl.ds(j * D + k * KP, KP)
        return pltpu.make_async_copy(wmod_hbm.at[:, cols], w3_v.at[:, cols], sem_mod.at[j, k])

    mod1_cp = pltpu.make_async_copy(wmod_hbm.at[:, pl.ds(2 * D, 4 * D)],
                                    wmod_v.at[:, pl.ds(0, 4 * D)], sem_w.at[5])

    def stage_cp(t, hh, piece):
        d0 = piece * KP if isinstance(piece, int) else pl.multiple_of(piece * KP, KP)
        return pltpu.make_async_copy(
            wqkv_hbm[t].at[pl.ds(d0, KP), pl.ds(hh * 16, 16), :],
            stage.at[hh, pl.ds(d0, KP)], sem_stage.at[hh, piece])

    def out_cp(j):
        r0 = j * BM if isinstance(j, int) else pl.multiple_of(j * BM, BM)
        return pltpu.make_async_copy(a_v.at[pl.ds(r0, BM)], out_hbm.at[pl.ds(r0, BM)],
                                     sem_out.at[j])

    def tile(n):
        return slice(n * 128, (n + 1) * 128)

    def mod_compute(src, tiles, off):
        cf = c_v[...].astype(f32)
        sc = (cf * jax.nn.sigmoid(cf)).astype(bf16)
        sc = jnp.broadcast_to(sc, (8, D))
        for n in tiles:
            mod_v[:, tile(n + off)] = _dot(sc, src[:, tile(n)])

    def mod(k):
        return mod_v[0:1, k * D:(k + 1) * D]

    def repack(hh, ch, p0, n):
        for u in range(n):
            p = p0 + u
            a = pltpu.bitcast(stage[hh, 2 * p], u32)
            b = pltpu.bitcast(stage[hh, 2 * p + 1], u32)
            ev = (a & jnp.uint32(0xFFFF)) | (b << 16)
            od = (a >> 16) | (b & jnp.uint32(0xFFFF0000))
            w_v[pl.ds(ch * (16 * PITCH) + p, 8, stride=PITCH), :] = ev
            w_v[pl.ds(ch * (16 * PITCH) + 8 * PITCH + p, 8, stride=PITCH), :] = od

    def w_slab(ch, l, lo=0, hi=D):
        base = (ch * 16 + (l % 2) * 8 + l // 2) * PITCH + lo // 2
        return _unpk(w_v[base:base + (hi - lo) // 2, :])

    def ring_of(ch, l):
        return rings[l // 2], ch * 2 + l % 2

    c_cp.start()
    mem0_cp.start()
    x_cp(0).start()
    stage_cp(0, 0, 0).start()
    zero_s[0] = 0
    x_v[S:S + SH, :] = jnp.zeros((SH, D), bf16)
    a_v[S:S + SH, :] = jnp.zeros((SH, D), bf16)
    mod_v[...] = jnp.zeros(mod_v.shape, f32)
    mod0_cp(0, 0).start()
    mod0_cp(1, 0).start()
    x_cp(0).wait()
    stage_cp(0, 1, 0).start()
    stage_cp(0, 0, 1).start()

    def xhat_body(i, c):
        r0 = pl.multiple_of(i * 64, 64)
        for u in range(4):
            rows = pl.ds(r0 + RC * u, RC)
            xh_v[rows, :] = _ln(x_v[rows, :].astype(f32))
        return c
    lax.fori_loop(0, PRE // 64, xhat_body, 0)

    c_cp.wait()
    mem0_cp.wait()
    mem_v[...] = pltpu.bitcast(mem0_v[...], u32)
    stage_cp(0, 0, 0).wait()

    def first_repack(i, c):
        repack(0, 0, i * 16, 16)
        return c
    lax.fori_loop(0, KP // 32, first_repack, 0)

    NPC = D // KP
    assert NPC == 4

    def pre_body(i, c):
        t, k = i >> 2, i & 3
        i1 = jnp.minimum(i + 1, 3 * NPC - 1)
        t1, k1 = i1 >> 2, i1 & 3

        for kk in range(NPC):
            @pl.when(i == kk)
            def _():
                mod0_cp(0, kk).wait()
                mod0_cp(1, kk).wait()
                tl = range(kk * KP // 128, (kk + 1) * KP // 128)
                mod_compute(w3_v, list(tl) + [NT + n for n in tl], 0)
                cols = slice(kk * KP, (kk + 1) * KP)
                sa = mod_v[0:1, kk * KP:(kk + 1) * KP]
                ca = mod_v[0:1, D + kk * KP:D + (kk + 1) * KP]
                for q in range(PRE // 64):
                    h0_v[kk, q * 32:(q + 1) * 32, :] = _pk(
                        xh_v[q * 64:(q + 1) * 64, cols] * (1.0 + ca) + sa)
                if kk + 1 < NPC:
                    mod0_cp(0, kk + 1).start()
                    mod0_cp(1, kk + 1).start()
                stage_cp((kk + 1) // NPC, 1, (kk + 1) % NPC).start()
                stage_cp((kk + 2) // NPC, 0, (kk + 2) % NPC).start()
                if kk in (1, 2):
                    x_cp(kk).start()

        stage_cp(0, 1, k).wait()

        @pl.when(i < 3 * NPC - 1)
        def _():
            stage_cp(0, 0, k1).wait()

        z0 = pl.multiple_of(zero_s[0], 64)
        w0 = pl.multiple_of(t * (32 * PITCH) + k * (KP // 2), 32)
        xrow = jnp.where(i >= NPC, PRE + (i - NPC) * 192, 0)
        hrow = jnp.maximum(i - NPC, 0) * 96
        done = {}
        nd = 0
        for h in range(H):
            hh, l = h // 16, h % 16
            w = _unpk(w_v[pl.ds(w0 + (hh * 16 + (l % 2) * 8 + l // 2) * PITCH, KP // 2), :])
            for rb in range(PRE // BM):
                lhs = _tie(h0_v[k, rb * 64:(rb + 1) * 64, :], done.pop(nd, None))
                rows = pl.ds(z0 + rb * BM, BM)
                y = _dot(_unpk(lhs), w) + jnp.where(k > 0, acc_v[h, rows, :], 0.0)
                acc_v[h, rows, :] = y
                rings[l // 2][t * 4 + hh * 2 + l % 2,
                              QOFF // 2 + rb * 64:QOFF // 2 + (rb + 1) * 64, :] = _pk(y)
                nd += 1
            if l < 15:
                n = 9 if l < 8 else 8
                p0_ = l * 9 if l < 8 else 72 + (l - 8) * 8
                if hh == 0:
                    repack(1, 2 * t + 1 + zero_s[0], k * (KP // 2) + p0_, n)
                else:
                    repack(0, 2 * t1, k1 * (KP // 2) + p0_, n)
            if h % 2 == 1 and h < 24:
                q = h // 2
                xs = x_v[pl.ds(pl.multiple_of(xrow + q * RC, RC), RC), :].astype(f32)
                hx = _pk(_ln(xs) * (1.0 + mod(1)) + mod(0))
                done[nd + 12] = hx
                for n in range(NT):
                    hx_v[n, pl.ds(pl.multiple_of(hrow + q * 8, 8), 8), :] = hx[:, tile(n)]
        for tt in range(1, 3):
            @pl.when(jnp.logical_and(i >= NPC - 2, (i + 3) >> 2 == tt))
            def _():
                stage_cp(tt, 1, (i + 3) & 3).start()

            @pl.when(jnp.logical_and(i >= NPC - 2, t + 1 == tt))
            def _():
                stage_cp(tt, 0, k).start()

        @pl.when(i == NPC - 1)
        def _():
            x_cp(1).wait()
            x_cp(2).wait()
            x_cp(3).start()

        @pl.when(i == NPC)
        def _():
            wo_cp.start()

        @pl.when(i == NPC + 1)
        def _():
            x_cp(3).wait()
        return c
    if CFG['pre']:
        lax.fori_loop(0, 3 * NPC, pre_body, 0)

    mod1_cp.start()
    for cp in (w1_cp, w2_cp, w3_cp, w4_cp):
        cp.start()
    wo_cp.wait()

    L2 = 2 * (SEG + MEM)
    r = lax.broadcasted_iota(jnp.int32, (L2, L2), 0)
    c = lax.broadcasted_iota(jnp.int32, (L2, L2), 1)
    r1 = ((r >= SEG) & (r < 2 * SEG)) | (r >= 2 * SEG + MEM)
    c1 = ((c >= SEG) & (c < 2 * SEG)) | (c >= 2 * SEG + MEM)
    same = r1 == c1
    mask = same & ((r >= 2 * SEG) | (c >= 2 * SEG) | (c <= r))
    fill = jnp.where(same, -1e9 / SCALE, -jnp.inf).astype(f32)

    def step(s, mem, zero, left):
        woff = pl.multiple_of((XR // 2 * s) % (RING // 2), 4)
        roff = pl.multiple_of((SEG // 2 * s + QOFF // 2) % (RING // 2), SEG // 2)
        arow = pl.multiple_of(SEG * s, SEG)
        acc = [None] * NT
        ym, ps, ol, part, rest = {}, {}, {}, {}, {}
        HK = D // 2
        tiles = [_unpk(jnp.concatenate(
            [hx_v[k, pl.ds(s * (XR // 2), XR // 2), :] | zero, mem[k]], axis=0))
            for k in range(NT)]
        mem_new = []

        def lhs(lo, hi):
            return jnp.concatenate(tiles[lo // 128:hi // 128], axis=1)

        def qkv_lo(h, t):
            part[(t, h)] = _dot(lhs(0, HK), w_slab(2 * t + h // 16, h % 16, 0, HK))

        def qkv(h):
            for t in range(3):
                ch, l = 2 * t + h // 16, h % 16
                if (t, h) in part:
                    y = _dot(lhs(HK, D), w_slab(ch, l, HK, D)) + part.pop((t, h))
                else:
                    y = _dot(lhs(0, D), w_slab(ch, l))
                rg, ix = ring_of(ch, l)
                rg[ix, pl.ds(woff, XR // 2), :] = _pk(y[0:XR])
                ym[(t, h)] = y[XR:XR + MEM]

        def get(t, p):
            rg, i0 = ring_of(2 * t + p // 8, (2 * p) % 16)
            mm = jnp.concatenate([ym.pop((t, 2 * p)), ym.pop((t, 2 * p + 1))], axis=0)
            return _unpk(jnp.concatenate(
                [rg[i0, pl.ds(roff, SEG // 2), :], rg[i0 + 1, pl.ds(roff, SEG // 2), :], _pk(mm)],
                axis=0))

        def sm(p):
            sc = lax.dot_general(get(0, p), get(1, p), (((1,), (1,)), ((), ())),
                                 preferred_element_type=f32)
            sc = jnp.where(mask, sc, fill)
            e = jnp.exp2((sc - jnp.max(sc, axis=-1, keepdims=True)) * (SCALE * LOG2E))
            ps[p] = (e * pl.reciprocal(jnp.sum(e, axis=-1, keepdims=True), approx=True)
                     ).astype(bf16)

        def pv(p):
            o = _dot(ps.pop(p), get(2, p))
            for j in range(2):
                h = 2 * p + j
                ox = o[SEG * j:SEG * (j + 1)]
                om = o[2 * SEG + MEM * j:2 * SEG + MEM * (j + 1)]
                if left is None:
                    ol[h] = jnp.concatenate([ox[0:XR], om], axis=0).astype(bf16)
                    rest[h] = ox[XR:SEG]
                else:
                    ol[h] = jnp.concatenate([ox, left[h], om], axis=0).astype(bf16)

        def wo(n, h0, h1):
            for h in range(h0, h1):
                y = _dot(ol[h], wo_v[h * DH:(h + 1) * DH, tile(n)])
                acc[n] = y if acc[n] is None else y + acc[n]
            if h1 == H:
                if left is None:
                    a_v[pl.ds(arow, XR), tile(n)] = acc[n][0:XR].astype(bf16)
                else:
                    a_v[pl.ds(arow, SEG), tile(n)] = acc[n][0:SEG].astype(bf16)
                    a_v[pl.ds(arow - (SEG - XR), SEG - XR), tile(n)] = (
                        acc[n][SEG:2 * SEG - XR].astype(bf16))
                mem_new.append(_pk(acc[n][-MEM:]))

        HE = CFG['he']
        nd = [0]

        def big(h):
            if h < H:
                qkv(h)
            else:
                wo(nd[0], 0, HE)
                nd[0] += 1

        for i in range(CFG['nlo']):
            qkv_lo(i // 3, i % 3)
        for i in range(NPAIR + 3):
            big(2 * i)
            if 0 <= i - 3 < NPAIR:
                pv(i - 3)
            if i < NPAIR + 2:
                big(2 * i + 1)
            if 0 <= i - 1 < NPAIR:
                sm(i - 1)
        while nd[0] < NT:
            big(H)
        for n in range(NT):
            wo(n, HE, H)
        return mem_new, rest

    def steps(i, carry):
        zero = zero_s[0].astype(u32)
        mem = [mem_v[:, tile(k)] for k in range(NT)]
        mem, rest = step(2 * i, mem, zero, None)
        mem, _ = step(2 * i + 1, mem, zero, rest)
        for k in range(NT):
            mem_v[:, tile(k)] = mem[k]
        return carry
    if CFG['step']:
        lax.fori_loop(0, NSEG // 2, steps, 0)

    if not CFG['b']:
        cp = pltpu.make_async_copy(a_v.at[pl.ds(0, S)], out_hbm, sem_out.at[0])
        cp.start()
        cp.wait()
        return

    mod1_cp.wait()
    for cp in (w1_cp, w2_cp, w3_cp, w4_cp):
        cp.wait()
    mod_compute(wmod_v, range(4 * NT), 2 * NT)

    def p0(tok, w):
        rows = pl.ds(tok, RC)
        xa = x_v[rows, :].astype(f32) + mod(2) * a_v[rows, :].astype(f32)
        hb = _ln(xa) * (1.0 + mod(4)) + mod(3)
        xa_v[w:w + RC, :] = xa
        hb_v[w:w + RC, :] = hb
        return _pk(_ln(hb))

    y0 = p0(0, 0)
    for k in range(BM // RC):
        y1_v[k * 8:(k + 1) * 8, :] = p0(SH + k * RC, SH + k * RC)
    for n in range(NT):
        g_v[n, 0:8, :] = jnp.zeros((8, 128), f32)
        g_v[n, 8:8 + SH, :] = _gelu(_dot(_unpk(y0), w1_v[:, tile(n)]))

    HM = BM // 2
    shift = (-1, 1, -2, 2)

    def blk(j, c):
        r0 = pl.multiple_of(j * BM, BM)
        nxt = pl.multiple_of(jnp.minimum(j + 1, NB - 1) * BM + SH, SH)
        more = j < NB - 1

        def w1_half(hf):
            for n in range(NT):
                g = _gelu(_dot(_unpk(y1_v[hf * 32:(hf + 1) * 32, :]), w1_v[:, tile(n)]))
                w0 = 8 + SH + hf * HM
                if hf == 0:
                    g_v[n, w0:w0 + HM, :] = g
                else:
                    g_v[n, w0:w0 + HM - SH, :] = g[0:HM - SH]
                    g_v[n, w0 + HM - SH:w0 + HM, :] = jnp.where(more, g[HM - SH:HM], 0.0)

        def w2_half(hf):
            for n in range(NT):
                w0 = 8 + hf * HM + shift[n // 2]
                z_v[hf * 32:(hf + 1) * 32, tile(n)] = _pk(g_v[n, w0:w0 + HM, :])
            for n in range(NT):
                x1_v[hf * HM:(hf + 1) * HM, tile(n)] = (
                    _dot(_unpk(z_v[hf * 32:(hf + 1) * 32, :]), w2_v[:, tile(n)])
                    + hb_v[hf * HM:(hf + 1) * HM, tile(n)])

        def p1_half(hf):
            for k in range(hf * HM // RC, (hf + 1) * HM // RC):
                x1 = x1_v[k * RC:(k + 1) * RC, :]
                y2_v[k * 8:(k + 1) * 8, :] = _pk(_ln(x1))
                base_v[k * RC:(k + 1) * RC, :] = xa_v[k * RC:(k + 1) * RC, :] + mod(5) * x1

        def w3(f, lo, hi, after=None):
            u_v[lo:hi, tile(f)] = _pk(_gelu(
                _dot(_unpk(_tie(y2_v[lo:hi, :], after)), w3_v[:, tile(f)])))

        w1_half(0)
        w1_half(1)
        w2_half(0)
        w2_half(1)
        p1_half(0)
        for f in range(CFG['nf']):
            w3(f, 0, 32)
        p1_half(1)
        for f in range(CFG['nf']):
            w3(f, 32, 64)
        for n in range(NT):
            g_v[n, 0:8 + SH, :] = g_v[n, BM:BM + 8 + SH, :]
        xa_v[0:SH, :] = xa_v[BM:BM + SH, :]
        hb_v[0:SH, :] = hb_v[BM:BM + SH, :]
        for f in range(CFG['nf'], NF):
            w3(f, 0, 64)
        for n in range(NT):
            y = p0(nxt + n * RC, SH + n * RC)
            y1_v[n * 8:(n + 1) * 8, :] = y
            gb = mod_v[0:1, 5 * D + n * 128:5 * D + (n + 1) * 128]
            u = _unpk(_tie(u_v[...], y, 0, CFG['p0k']))
            a_v[pl.ds(r0, BM), tile(n)] = (
                base_v[:, tile(n)] + gb * _dot(u, w4_v[:, tile(n)])).astype(bf16)
        out_cp(j).start()
        return c
    lax.fori_loop(0, NB, blk, 0)
    for j in range(NB):
        out_cp(j).wait()


@functools.partial(jax.jit, static_argnames=("A_seg_len",))
def pallas_adaLN_cond__memory_aug_recurrent_mem_tr__mixer_s_mlp__prompt_kernel(
    A_x: jax.Array,
    A_mem0: jax.Array,
    A_Wq: jax.Array,
    A_Wk: jax.Array,
    A_Wv: jax.Array,
    A_Wo: jax.Array,
    A_seg_len,
    B_x: jax.Array,
    B_w1: jax.Array,
    B_w2: jax.Array,
    B_w3: jax.Array,
    B_w4: jax.Array,
    c: jax.Array,
    w_mod: jax.Array,
):
    assert A_seg_len == SEG and A_x.shape == (1, S, D) and A_Wq.shape == (D, H, DH)
    any_spec = pl.BlockSpec(memory_space=pl.ANY)
    out = pl.pallas_call(
        _kernel,
        out_shape=jax.ShapeDtypeStruct((S, D), bf16),
        in_specs=[any_spec] * 12,
        out_specs=any_spec,
        scratch_shapes=[
            pltpu.VMEM((1, D), bf16),
            pltpu.VMEM((S + SH, D), bf16),
            pltpu.VMEM((S + SH, D), bf16),
            pltpu.VMEM((D // KP, PRE // 2, KP), u32),
            pltpu.VMEM((MEM // 2, D), u32),
            pltpu.VMEM((MEM, D), bf16),
            pltpu.VMEM((8, 6 * D), f32),
            pltpu.VMEM((D, 4 * D + PADL), bf16),
            pltpu.VMEM((96 * PITCH, 128), u32),
            pltpu.VMEM((H * DH, D + PADL), bf16),
            pltpu.VMEM((D, D + PADL), bf16),
            pltpu.VMEM((D, D + PADL), bf16),
            pltpu.VMEM((D, F + PADL), bf16),
            pltpu.VMEM((F, D + PADL), bf16),
            pltpu.VMEM((NT, BM + 32, 128), f32),
            pltpu.VMEM((BM + SH, D), f32),
            pltpu.VMEM((BM + SH, D), f32),
            pltpu.VMEM((BM, D), f32),
            pltpu.VMEM((BM, D), f32),
            pltpu.VMEM((BM // 2, D), u32),
            pltpu.VMEM((BM // 2, D), u32),
            pltpu.VMEM((BM // 2, D), u32),
            pltpu.VMEM((BM // 2, F), u32),
            pltpu.VMEM((2, D, 16, DH), bf16),
            pltpu.VMEM((PRE, D), f32),
            pltpu.VMEM((NT, HR, 128), u32),
            pltpu.VMEM((H, PRE, DH), f32),
        ] + [pltpu.VMEM((12, RING // 2, DH), u32)] * 8 + [
            pltpu.SMEM((1,), jnp.int32),
            pltpu.SemaphoreType.DMA((2,)),
            pltpu.SemaphoreType.DMA((4,)),
            pltpu.SemaphoreType.DMA((2, 4)),
            pltpu.SemaphoreType.DMA((2, 4)),
            pltpu.SemaphoreType.DMA((6,)),
            pltpu.SemaphoreType.DMA((NB,)),
        ],
        compiler_params=pltpu.CompilerParams(vmem_limit_bytes=120 * 1024 * 1024),
    )(A_x.reshape(S, D), A_mem0.reshape(MEM, D), A_Wq, A_Wk, A_Wv, A_Wo.reshape(H * DH, D),
      B_w1, B_w2, B_w3, B_w4, c, w_mod)
    return out.reshape(1, S, D)
```

```python
import functools

import jax
import jax.numpy as jnp
from jax import lax
import jax.experimental.pallas as pl
import jax.experimental.pallas.tpu as pltpu

bf16, f32, u32 = jnp.bfloat16, jnp.float32, jnp.uint32

S, D, H, DH, MEM, SEG, F = 2048, 1024, 32, 128, 8, 32, 3584
NSEG = S // SEG
XR = 24
PRE = S - XR * NSEG
RING = 576
QOFF = RING - PRE
PITCH = 520
NT = D // 128
NF = F // 128
BM = 128
NB = S // BM
NPAIR = H // 2
HR = (S - PRE) // 2
PADL = 128
SH = 16
KP = 256
RC = 16
EPS = 1e-5
LOG2E = 1.4426950408889634
SCALE = DH ** -0.5
CFG = dict(pre=True, step=True, b=True, nlo=6, he=24, ds=5, dp=10, dv=0, qk=((0, 0), (1, 0), (0, 1), (1, 1)), ow=(0, 7, 8), nf=7, p0k=24)


def _ln(x):
    m = jnp.mean(x, axis=-1, keepdims=True)
    xc = x - m
    v = jnp.mean(xc * xc, axis=-1, keepdims=True)
    return xc * lax.rsqrt(v + EPS)


def _gelu(x):
    return jax.nn.gelu(x, approximate=True)


def _dot(a, b):
    return jnp.dot(a, b, preferred_element_type=f32)


def _pk(x):
    return pltpu.bitcast(x.astype(bf16), u32)


def _unpk(x):
    return pltpu.bitcast(x, bf16)


def _tie(w, after, r=0, k=0):
    if after is None:
        return w
    m = functools.reduce(lambda a, b: a & b,
                         [after[:, i * 128:(i + 1) * 128] for i in range(after.shape[1] // 128)])
    mf = pltpu.bitcast(m, f32)
    z = jnp.where(mf * mf < 0.0, jnp.uint32(1), jnp.uint32(0))
    row = w[r:r + 8]
    parts = [row[:, :k * 128], row[:, k * 128:(k + 1) * 128] | z, row[:, (k + 1) * 128:]]
    row = jnp.concatenate([p for p in parts if p.shape[1]], axis=1)
    parts = [w[:r], row, w[r + 8:]]
    return jnp.concatenate([p for p in parts if p.shape[0]], axis=0)


def _kernel(x_hbm, mem0_hbm, wq_hbm, wk_hbm, wv_hbm, wo_hbm, w1_hbm, w2_hbm, w3_hbm, w4_hbm,
            c_hbm, wmod_hbm, out_hbm,
            c_v, x_v, a_v, h0_v, mem_v, mem0_v, mod_v, wmod_v, w_v, wo_v,
            w1_v, w2_v, w3_v, w4_v,
            g_v, xa_v, hb_v, base_v, x1_v, y1_v, z_v, y2_v, u_v,
            stage, xh_v, hx_v, acc_v,
            r0_, r1_, r2_, r3_, r4_, r5_, r6_, r7_,
            zero_s, sem_small, sem_x, sem_stage, sem_mod, sem_w, sem_out):
    wqkv_hbm = (wq_hbm, wk_hbm, wv_hbm)
    rings = (r0_, r1_, r2_, r3_, r4_, r5_, r6_, r7_)

    c_cp = pltpu.make_async_copy(c_hbm, c_v, sem_small.at[0])
    mem0_cp = pltpu.make_async_copy(mem0_hbm, mem0_v, sem_small.at[1])

    def x_cp(q):
        rows = pl.ds(q * PRE, PRE)
        return pltpu.make_async_copy(x_hbm.at[rows], x_v.at[rows], sem_x.at[q])

    def w_cp(src, dst, k):
        return pltpu.make_async_copy(src, dst.at[:, pl.ds(0, src.shape[1])], sem_w.at[k])

    wo_cp, w1_cp, w2_cp, w3_cp, w4_cp = (
        w_cp(a, b, k) for k, (a, b) in enumerate(
            ((wo_hbm, wo_v), (w1_hbm, w1_v), (w2_hbm, w2_v), (w3_hbm, w3_v), (w4_hbm, w4_v))))

    def mod0_cp(j, k):
        cols = pl.ds(j * D + k * KP, KP)
        return pltpu.make_async_copy(wmod_hbm.at[:, cols], w3_v.at[:, cols], sem_mod.at[j, k])

    mod1_cp = pltpu.make_async_copy(wmod_hbm.at[:, pl.ds(2 * D, 4 * D)],
                                    wmod_v.at[:, pl.ds(0, 4 * D)], sem_w.at[5])

    def stage_cp(t, hh, piece):
        d0 = piece * KP if isinstance(piece, int) else pl.multiple_of(piece * KP, KP)
        return pltpu.make_async_copy(
            wqkv_hbm[t].at[pl.ds(d0, KP), pl.ds(hh * 16, 16), :],
            stage.at[hh, pl.ds(d0, KP)], sem_stage.at[hh, piece])

    def tile(n):
        return slice(n * 128, (n + 1) * 128)

    def mod_compute(src, tiles, off):
        cf = c_v[...].astype(f32)
        sc = (cf * jax.nn.sigmoid(cf)).astype(bf16)
        sc = jnp.broadcast_to(sc, (8, D))
        for n in tiles:
            mod_v[:, tile(n + off)] = _dot(sc, src[:, tile(n)])

    def mod(k):
        return mod_v[0:1, k * D:(k + 1) * D]

    def repack(hh, ch, p0, n):
        for u in range(n):
            p = p0 + u
            a = pltpu.bitcast(stage[hh, 2 * p], u32)
            b = pltpu.bitcast(stage[hh, 2 * p + 1], u32)
            ev = (a & jnp.uint32(0xFFFF)) | (b << 16)
            od = (a >> 16) | (b & jnp.uint32(0xFFFF0000))
            w_v[pl.ds(ch * (16 * PITCH) + p, 8, stride=PITCH), :] = ev
            w_v[pl.ds(ch * (16 * PITCH) + 8 * PITCH + p, 8, stride=PITCH), :] = od

    def w_slab(ch, l, lo=0, hi=D):
        base = (ch * 16 + (l % 2) * 8 + l // 2) * PITCH + lo // 2
        return _unpk(w_v[base:base + (hi - lo) // 2, :])

    def ring_of(ch, l):
        return rings[l // 2], ch * 2 + l % 2

    c_cp.start()
    mem0_cp.start()
    x_cp(0).start()
    stage_cp(0, 0, 0).start()
    zero_s[0] = 0
    x_v[S:S + SH, :] = jnp.zeros((SH, D), bf16)
    a_v[S:S + SH, :] = jnp.zeros((SH, D), bf16)
    mod_v[...] = jnp.zeros(mod_v.shape, f32)
    mod0_cp(0, 0).start()
    mod0_cp(1, 0).start()
    x_cp(0).wait()
    stage_cp(0, 1, 0).start()

    def xhat_body(i, c):
        r0 = pl.multiple_of(i * 64, 64)
        for u in range(4):
            rows = pl.ds(r0 + RC * u, RC)
            xh_v[rows, :] = _ln(x_v[rows, :].astype(f32))
        return c
    lax.fori_loop(0, PRE // 64, xhat_body, 0)

    c_cp.wait()
    mem0_cp.wait()
    mem_v[...] = pltpu.bitcast(mem0_v[...], u32)
    stage_cp(0, 0, 0).wait()

    def first_repack(i, c):
        repack(0, 0, i * 16, 16)
        return c
    lax.fori_loop(0, KP // 32, first_repack, 0)

    NPC = D // KP
    assert NPC == 4

    def pre_body(i, c):
        t, k = i >> 2, i & 3
        fresh = jnp.logical_and(i > 0, i < 3 * NPC - 1)
        i1 = jnp.where(fresh, i + 1, i)
        t1, k1 = i1 >> 2, i1 & 3

        for kk in range(NPC):
            @pl.when(i == kk)
            def _():
                mod0_cp(0, kk).wait()
                mod0_cp(1, kk).wait()
                if kk == 1:
                    stage_cp(0, 0, 1).wait()
                    repack(0, 0, KP // 2, KP // 2)
                tl = range(kk * KP // 128, (kk + 1) * KP // 128)
                mod_compute(w3_v, list(tl) + [NT + n for n in tl], 0)
                cols = slice(kk * KP, (kk + 1) * KP)
                sa = mod_v[0:1, kk * KP:(kk + 1) * KP]
                ca = mod_v[0:1, D + kk * KP:D + (kk + 1) * KP]
                for q in range(PRE // 64):
                    h0_v[kk, q * 32:(q + 1) * 32, :] = _pk(
                        xh_v[q * 64:(q + 1) * 64, cols] * (1.0 + ca) + sa)
                if kk == 0:
                    stage_cp(0, 0, 1).start()
                if kk + 1 < NPC:
                    mod0_cp(0, kk + 1).start()
                    mod0_cp(1, kk + 1).start()
                stage_cp((kk + 1) // NPC, 1, (kk + 1) % NPC).start()
                stage_cp((kk + 2) // NPC, 0, (kk + 2) % NPC).start()
                if kk in (1, 2):
                    x_cp(kk).start()

        stage_cp(0, 1, k).wait()

        @pl.when(fresh)
        def _():
            stage_cp(0, 0, k1).wait()

        z0 = pl.multiple_of(zero_s[0], 64)
        w0 = pl.multiple_of(t * (32 * PITCH) + k * (KP // 2), 32)
        xrow = jnp.where(i >= NPC, PRE + (i - NPC) * 192, 0)
        hrow = jnp.maximum(i - NPC, 0) * 96
        done = {}
        nd = 0
        for h in range(H):
            hh, l = h // 16, h % 16
            w = _unpk(w_v[pl.ds(w0 + (hh * 16 + (l % 2) * 8 + l // 2) * PITCH, KP // 2), :])
            for rb in range(PRE // BM):
                lhs = _tie(h0_v[k, rb * 64:(rb + 1) * 64, :], done.pop(nd, None))
                rows = pl.ds(z0 + rb * BM, BM)
                y = _dot(_unpk(lhs), w) + jnp.where(k > 0, acc_v[h, rows, :], 0.0)
                acc_v[h, rows, :] = y
                rings[l // 2][t * 4 + hh * 2 + l % 2,
                              QOFF // 2 + rb * 64:QOFF // 2 + (rb + 1) * 64, :] = _pk(y)
                nd += 1
            if l < 15:
                n = 9 if l < 8 else 8
                p0_ = l * 9 if l < 8 else 72 + (l - 8) * 8
                if hh == 0:
                    repack(1, 2 * t + 1 + zero_s[0], k * (KP // 2) + p0_, n)
                else:
                    repack(0, 2 * t1, k1 * (KP // 2) + p0_, n)
            if h % 2 == 1 and h < 24:
                q = h // 2
                xs = x_v[pl.ds(pl.multiple_of(xrow + q * RC, RC), RC), :].astype(f32)
                hx = _pk(_ln(xs) * (1.0 + mod(1)) + mod(0))
                done[nd + 12] = hx
                for n in range(NT):
                    hx_v[n, pl.ds(pl.multiple_of(hrow + q * 8, 8), 8), :] = hx[:, tile(n)]
        for tt in range(1, 3):
            @pl.when(jnp.logical_and(i >= NPC - 2, (i + 3) >> 2 == tt))
            def _():
                stage_cp(tt, 1, (i + 3) & 3).start()

            @pl.when(jnp.logical_and(i >= NPC - 2, t + 1 == tt))
            def _():
                stage_cp(tt, 0, k).start()

        @pl.when(i == NPC - 1)
        def _():
            x_cp(1).wait()
            x_cp(2).wait()
            x_cp(3).start()

        @pl.when(i == NPC)
        def _():
            wo_cp.start()

        @pl.when(i == NPC + 1)
        def _():
            x_cp(3).wait()
        return c
    if CFG['pre']:
        lax.fori_loop(0, 3 * NPC, pre_body, 0)

    mod1_cp.start()
    for cp in (w1_cp, w2_cp, w3_cp, w4_cp):
        cp.start()
    wo_cp.wait()

    L2 = 2 * (SEG + MEM)
    r = lax.broadcasted_iota(jnp.int32, (L2, L2), 0)
    c = lax.broadcasted_iota(jnp.int32, (L2, L2), 1)
    r1 = ((r >= SEG) & (r < 2 * SEG)) | (r >= 2 * SEG + MEM)
    c1 = ((c >= SEG) & (c < 2 * SEG)) | (c >= 2 * SEG + MEM)
    same = r1 == c1
    mask = same & ((r >= 2 * SEG) | (c >= 2 * SEG) | (c <= r))
    fill = jnp.where(same, -1e9 / SCALE, -jnp.inf).astype(f32)

    def step(s, mem, zero, left):
        woff = pl.multiple_of((XR // 2 * s) % (RING // 2), 4)
        roff = pl.multiple_of((SEG // 2 * s + QOFF // 2) % (RING // 2), SEG // 2)
        arow = pl.multiple_of(SEG * s, SEG)
        acc = [None] * NT
        ym, ps, ol, part, rest = {}, {}, {}, {}, {}
        HK = D // 2
        tiles = [_unpk(jnp.concatenate(
            [hx_v[k, pl.ds(s * (XR // 2), XR // 2), :] | zero, mem[k]], axis=0))
            for k in range(NT)]
        mem_new = []

        def lhs(lo, hi):
            return jnp.concatenate(tiles[lo // 128:hi // 128], axis=1)

        def qkv_lo(h, t):
            part[(t, h)] = _dot(lhs(0, HK), w_slab(2 * t + h // 16, h % 16, 0, HK))

        def proj(t, h):
            ch, l = 2 * t + h // 16, h % 16
            if (t, h) in part:
                y = _dot(lhs(HK, D), w_slab(ch, l, HK, D)) + part.pop((t, h))
            else:
                y = _dot(lhs(0, D), w_slab(ch, l))
            rg, ix = ring_of(ch, l)
            rg[ix, pl.ds(woff, XR // 2), :] = _pk(y[0:XR])
            ym[(t, h)] = y[XR:XR + MEM]

        def get(t, p):
            rg, i0 = ring_of(2 * t + p // 8, (2 * p) % 16)
            mm = jnp.concatenate([ym.pop((t, 2 * p)), ym.pop((t, 2 * p + 1))], axis=0)
            return _unpk(jnp.concatenate(
                [rg[i0, pl.ds(roff, SEG // 2), :], rg[i0 + 1, pl.ds(roff, SEG // 2), :], _pk(mm)],
                axis=0))

        def sm(p):
            sc = lax.dot_general(get(0, p), get(1, p), (((1,), (1,)), ((), ())),
                                 preferred_element_type=f32)
            sc = jnp.where(mask, sc, fill)
            e = jnp.exp2((sc - jnp.max(sc, axis=-1, keepdims=True)) * (SCALE * LOG2E))
            ps[p] = (e * pl.reciprocal(jnp.sum(e, axis=-1, keepdims=True), approx=True)
                     ).astype(bf16)

        def pv(p):
            o = _dot(ps.pop(p), get(2, p))
            for j in range(2):
                h = 2 * p + j
                ox = o[SEG * j:SEG * (j + 1)]
                om = o[2 * SEG + MEM * j:2 * SEG + MEM * (j + 1)]
                if left is None:
                    ol[h] = jnp.concatenate([ox[0:XR], om], axis=0).astype(bf16)
                    rest[h] = ox[XR:SEG]
                else:
                    ol[h] = jnp.concatenate([ox, left[h], om], axis=0).astype(bf16)

        def wo(n, h0, h1):
            for h in range(h0, h1):
                y = _dot(ol[h], wo_v[h * DH:(h + 1) * DH, tile(n)])
                acc[n] = y if acc[n] is None else y + acc[n]
            if h1 == H:
                if left is None:
                    a_v[pl.ds(arow, XR), tile(n)] = acc[n][0:XR].astype(bf16)
                else:
                    a_v[pl.ds(arow, SEG), tile(n)] = acc[n][0:SEG].astype(bf16)
                    a_v[pl.ds(arow - (SEG - XR), SEG - XR), tile(n)] = (
                        acc[n][SEG:2 * SEG - XR].astype(bf16))
                mem_new.append(_pk(acc[n][-MEM:]))

        HE, DS, DP, DV = CFG['he'], CFG['ds'], CFG['dp'], CFG['dv']
        seq = []
        for p in range(NPAIR + DV):
            if p < NPAIR:
                seq += [(t, 2 * p + j) for t, j in CFG['qk']]
            if p - DV >= 0:
                seq += [(2, 2 * (p - DV)), (2, 2 * (p - DV) + 1)]
        events = {}
        for p in range(NPAIR):
            at = max(seq.index((t, 2 * p + j)) for t in range(2) for j in range(2)) + DS
            events.setdefault(at, []).append((sm, p))
            events.setdefault(at + DP, []).append((pv, p))
        for t, h in seq[:CFG['nlo']]:
            qkv_lo(h, t)
        WU = HE // 8
        for i in range(len(seq) + NT * WU):
            if i < len(seq):
                proj(*seq[i])
            else:
                u = i - len(seq)
                wo(u // WU, (u % WU) * 8, (u % WU + 1) * 8)
            for fn, p in events.pop(i, []):
                fn(p)
        assert not events
        for n in range(NT):
            wo(n, HE, H)
        return mem_new, rest

    def steps(i, carry):
        zero = zero_s[0].astype(u32)
        mem = [mem_v[:, tile(k)] for k in range(NT)]
        mem, rest = step(2 * i, mem, zero, None)
        mem, _ = step(2 * i + 1, mem, zero, rest)
        for k in range(NT):
            mem_v[:, tile(k)] = mem[k]
        return carry
    if CFG['step']:
        lax.fori_loop(0, NSEG // 2, steps, 0)

    if not CFG['b']:
        cp = pltpu.make_async_copy(a_v.at[pl.ds(0, S)], out_hbm, sem_out)
        cp.start()
        cp.wait()
        return

    mod1_cp.wait()
    for cp in (w1_cp, w2_cp, w3_cp, w4_cp):
        cp.wait()
    mod_compute(wmod_v, range(4 * NT), 2 * NT)

    def p0(tok, w):
        rows = pl.ds(tok, RC)
        xa = x_v[rows, :].astype(f32) + mod(2) * a_v[rows, :].astype(f32)
        hb = _ln(xa) * (1.0 + mod(4)) + mod(3)
        xa_v[w:w + RC, :] = xa
        hb_v[w:w + RC, :] = hb
        return _pk(_ln(hb))

    y0 = p0(0, 0)
    for k in range(BM // RC):
        y1_v[k * 8:(k + 1) * 8, :] = p0(SH + k * RC, SH + k * RC)
    for n in range(NT):
        g_v[n, 0:8, :] = jnp.zeros((8, 128), f32)
        g_v[n, 8:8 + SH, :] = _gelu(_dot(_unpk(y0), w1_v[:, tile(n)]))

    HM = BM // 2
    shift = (-1, 1, -2, 2)

    def blk(j, c):
        r0 = pl.multiple_of(j * BM, BM)
        nxt = pl.multiple_of(jnp.minimum(j + 1, NB - 1) * BM + SH, SH)
        more = j < NB - 1

        def w1_half(hf):
            for n in range(NT):
                g = _gelu(_dot(_unpk(y1_v[hf * 32:(hf + 1) * 32, :]), w1_v[:, tile(n)]))
                w0 = 8 + SH + hf * HM
                if hf == 0:
                    g_v[n, w0:w0 + HM, :] = g
                else:
                    g_v[n, w0:w0 + HM - SH, :] = g[0:HM - SH]
                    g_v[n, w0 + HM - SH:w0 + HM, :] = jnp.where(more, g[HM - SH:HM], 0.0)

        def w2_half(hf):
            for n in range(NT):
                w0 = 8 + hf * HM + shift[n // 2]
                z_v[hf * 32:(hf + 1) * 32, tile(n)] = _pk(g_v[n, w0:w0 + HM, :])
            for n in range(NT):
                x1_v[hf * HM:(hf + 1) * HM, tile(n)] = (
                    _dot(_unpk(z_v[hf * 32:(hf + 1) * 32, :]), w2_v[:, tile(n)])
                    + hb_v[hf * HM:(hf + 1) * HM, tile(n)])

        def p1_half(hf):
            for k in range(hf * HM // RC, (hf + 1) * HM // RC):
                x1 = x1_v[k * RC:(k + 1) * RC, :]
                y2_v[k * 8:(k + 1) * 8, :] = _pk(_ln(x1))
                base_v[k * RC:(k + 1) * RC, :] = xa_v[k * RC:(k + 1) * RC, :] + mod(5) * x1

        def w3(f, lo, hi, after=None):
            u_v[lo:hi, tile(f)] = _pk(_gelu(
                _dot(_unpk(_tie(y2_v[lo:hi, :], after)), w3_v[:, tile(f)])))

        w1_half(0)
        w1_half(1)
        w2_half(0)
        w2_half(1)
        p1_half(0)
        for f in range(CFG['nf']):
            w3(f, 0, 32)
        p1_half(1)
        for f in range(CFG['nf']):
            w3(f, 32, 64)
        for n in range(NT):
            g_v[n, 0:8 + SH, :] = g_v[n, BM:BM + 8 + SH, :]
        xa_v[0:SH, :] = xa_v[BM:BM + SH, :]
        hb_v[0:SH, :] = hb_v[BM:BM + SH, :]
        for f in range(CFG['nf'], NF):
            w3(f, 0, 64)
        for n in range(NT):
            y = p0(nxt + n * RC, SH + n * RC)
            y1_v[n * 8:(n + 1) * 8, :] = y
            gb = mod_v[0:1, 5 * D + n * 128:5 * D + (n + 1) * 128]
            u = _unpk(_tie(u_v[...], y, 0, CFG['p0k']))
            a_v[pl.ds(r0, BM), tile(n)] = (
                base_v[:, tile(n)] + gb * _dot(u, w4_v[:, tile(n)])).astype(bf16)
            if n + 1 in CFG['ow'][1:]:
                lo = CFG['ow'][CFG['ow'].index(n + 1) - 1]
                cols = pl.ds(lo * 128, (n + 1 - lo) * 128)
                pltpu.make_async_copy(a_v.at[pl.ds(r0, BM), cols], out_hbm.at[pl.ds(r0, BM), cols],
                                      sem_out).start()
        return c
    lax.fori_loop(0, NB, blk, 0)
    pltpu.make_async_copy(a_v.at[pl.ds(0, S)], out_hbm, sem_out).wait()


@functools.partial(jax.jit, static_argnames=("A_seg_len",))
def pallas_adaLN_cond__memory_aug_recurrent_mem_tr__mixer_s_mlp__prompt_kernel(
    A_x: jax.Array,
    A_mem0: jax.Array,
    A_Wq: jax.Array,
    A_Wk: jax.Array,
    A_Wv: jax.Array,
    A_Wo: jax.Array,
    A_seg_len,
    B_x: jax.Array,
    B_w1: jax.Array,
    B_w2: jax.Array,
    B_w3: jax.Array,
    B_w4: jax.Array,
    c: jax.Array,
    w_mod: jax.Array,
):
    assert A_seg_len == SEG and A_x.shape == (1, S, D) and A_Wq.shape == (D, H, DH)
    any_spec = pl.BlockSpec(memory_space=pl.ANY)
    out = pl.pallas_call(
        _kernel,
        out_shape=jax.ShapeDtypeStruct((S, D), bf16),
        in_specs=[any_spec] * 12,
        out_specs=any_spec,
        scratch_shapes=[
            pltpu.VMEM((1, D), bf16),
            pltpu.VMEM((S + SH, D), bf16),
            pltpu.VMEM((S + SH, D), bf16),
            pltpu.VMEM((D // KP, PRE // 2, KP), u32),
            pltpu.VMEM((MEM // 2, D), u32),
            pltpu.VMEM((MEM, D), bf16),
            pltpu.VMEM((8, 6 * D), f32),
            pltpu.VMEM((D, 4 * D + PADL), bf16),
            pltpu.VMEM((96 * PITCH, 128), u32),
            pltpu.VMEM((H * DH, D + PADL), bf16),
            pltpu.VMEM((D, D + PADL), bf16),
            pltpu.VMEM((D, D + PADL), bf16),
            pltpu.VMEM((D, F + PADL), bf16),
            pltpu.VMEM((F, D + PADL), bf16),
            pltpu.VMEM((NT, BM + 32, 128), f32),
            pltpu.VMEM((BM + SH, D), f32),
            pltpu.VMEM((BM + SH, D), f32),
            pltpu.VMEM((BM, D), f32),
            pltpu.VMEM((BM, D), f32),
            pltpu.VMEM((BM // 2, D), u32),
            pltpu.VMEM((BM // 2, D), u32),
            pltpu.VMEM((BM // 2, D), u32),
            pltpu.VMEM((BM // 2, F), u32),
            pltpu.VMEM((2, D, 16, DH), bf16),
            pltpu.VMEM((PRE, D), f32),
            pltpu.VMEM((NT, HR, 128), u32),
            pltpu.VMEM((H, PRE, DH), f32),
        ] + [pltpu.VMEM((12, RING // 2, DH), u32)] * 8 + [
            pltpu.SMEM((1,), jnp.int32),
            pltpu.SemaphoreType.DMA((2,)),
            pltpu.SemaphoreType.DMA((4,)),
            pltpu.SemaphoreType.DMA((2, 4)),
            pltpu.SemaphoreType.DMA((2, 4)),
            pltpu.SemaphoreType.DMA((6,)),
            pltpu.SemaphoreType.DMA(()),
        ],
        compiler_params=pltpu.CompilerParams(vmem_limit_bytes=120 * 1024 * 1024),
    )(A_x.reshape(S, D), A_mem0.reshape(MEM, D), A_Wq, A_Wk, A_Wv, A_Wo.reshape(H * DH, D),
      B_w1, B_w2, B_w3, B_w4, c, w_mod)
    return out.reshape(1, S, D)
```

```python
import functools

import jax
import jax.numpy as jnp
from jax import lax
import jax.experimental.pallas as pl
import jax.experimental.pallas.tpu as pltpu

bf16, f32, u32 = jnp.bfloat16, jnp.float32, jnp.uint32

S, D, H, DH, MEM, SEG, F = 2048, 1024, 32, 128, 8, 32, 3584
NSEG = S // SEG
XR = 24
PRE = S - XR * NSEG
RING = 576
QOFF = RING - PRE
PITCH = 520
NT = D // 128
NF = F // 128
BM = 128
NB = S // BM
NPAIR = H // 2
HR = (S - PRE) // 2
PADL = 128
SH = 16
KP = 256
MJ = 512
RC = 16
EPS = 1e-5
LOG2E = 1.4426950408889634
SCALE = DH ** -0.5
CFG = dict(pre=True, step=True, b=True, nlo=6, he=24, mh=28, md=9, mw=512, ds=5, dp=10, dv=0, qk=((0, 0), (1, 0), (0, 1), (1, 1)), ow=(0, 7, 8), nf=7, p0k=24)


def _ln(x):
    m = jnp.mean(x, axis=-1, keepdims=True)
    xc = x - m
    v = jnp.mean(xc * xc, axis=-1, keepdims=True)
    return xc * lax.rsqrt(v + EPS)


def _gelu(x):
    return jax.nn.gelu(x, approximate=True)


def _dot(a, b):
    return jnp.dot(a, b, preferred_element_type=f32)


def _pk(x):
    return pltpu.bitcast(x.astype(bf16), u32)


def _unpk(x):
    return pltpu.bitcast(x, bf16)


def _tie(w, after, r=0, k=0):
    if after is None:
        return w
    m = functools.reduce(lambda a, b: a & b,
                         [after[:, i * 128:(i + 1) * 128] for i in range(after.shape[1] // 128)])
    mf = pltpu.bitcast(m, f32)
    z = jnp.where(mf * mf < 0.0, jnp.uint32(1), jnp.uint32(0))
    row = w[r:r + 8]
    parts = [row[:, :k * 128], row[:, k * 128:(k + 1) * 128] | z, row[:, (k + 1) * 128:]]
    row = jnp.concatenate([p for p in parts if p.shape[1]], axis=1)
    parts = [w[:r], row, w[r + 8:]]
    return jnp.concatenate([p for p in parts if p.shape[0]], axis=0)


def _kernel(x_hbm, mem0_hbm, wq_hbm, wk_hbm, wv_hbm, wo_hbm, w1_hbm, w2_hbm, w3_hbm, w4_hbm,
            c_hbm, wmod_hbm, out_hbm,
            c_v, x_v, a_v, h0_v, mem_v, mem0_v, mod_v, modr_v, cb_v, wm_v, w_v, wo_v,
            w1_v, w2_v, w3_v, w4_v,
            g_v, xa_v, hb_v, base_v, x1_v, y1_v, z_v, y2_v, u_v,
            stage, xh_v, hx_v, acc_v,
            r0_, r1_, r2_, r3_, r4_, r5_, r6_, r7_,
            zero_s, sem_small, sem_x, sem_stage, sem_mod, sem_w, sem_out):
    wqkv_hbm = (wq_hbm, wk_hbm, wv_hbm)
    rings = (r0_, r1_, r2_, r3_, r4_, r5_, r6_, r7_)

    c_cp = pltpu.make_async_copy(c_hbm, c_v, sem_small.at[0])
    mem0_cp = pltpu.make_async_copy(mem0_hbm, mem0_v, sem_small.at[1])

    def x_cp(q):
        rows = pl.ds(q * PRE if isinstance(q, int) else pl.multiple_of(q * PRE, PRE), PRE)
        return pltpu.make_async_copy(x_hbm.at[rows], x_v.at[rows], sem_x.at[q])

    def w_cp(src, dst, k):
        return pltpu.make_async_copy(src, dst.at[:, pl.ds(0, src.shape[1])], sem_w.at[k])

    wo_cp, w1_cp, w2_cp, w3_cp, w4_cp = (
        w_cp(a, b, k) for k, (a, b) in enumerate(
            ((wo_hbm, wo_v), (w1_hbm, w1_v), (w2_hbm, w2_v), (w3_hbm, w3_v), (w4_hbm, w4_v))))

    def mod0_cp(j, k):
        return pltpu.make_async_copy(wmod_hbm.at[:, pl.ds(j * D + k * KP, KP)],
                                     wm_v.at[k, :, pl.ds(j * KP, KP)], sem_mod.at[j, k])

    def mod1_cp(q):
        col = 2 * D + q * MJ
        col = col if isinstance(q, int) else pl.multiple_of(col, MJ)
        return pltpu.make_async_copy(wmod_hbm.at[:, pl.ds(col, MJ)], wm_v.at[4 + q],
                                     sem_mod.at[q >> 2, q & 3])

    def stage_cp(t, hh, piece):
        d0 = piece * KP if isinstance(piece, int) else pl.multiple_of(piece * KP, KP)
        return pltpu.make_async_copy(
            wqkv_hbm[t].at[pl.ds(d0, KP), pl.ds(hh * 16, 16), :],
            stage.at[hh, pl.ds(d0, KP)], sem_stage.at[hh, piece])

    def tile(n):
        return slice(n * 128, (n + 1) * 128)

    def silu_c():
        cf = c_v[...].astype(f32)
        return (cf * jax.nn.sigmoid(cf)).astype(bf16)

    def mod(k, lo=0, hi=D):
        return mod_v[0:1, k * D + lo:k * D + hi]

    def repack(hh, ch, p0, n):
        for u in range(n):
            p = p0 + u
            a = pltpu.bitcast(stage[hh, 2 * p], u32)
            b = pltpu.bitcast(stage[hh, 2 * p + 1], u32)
            ev = (a & jnp.uint32(0xFFFF)) | (b << 16)
            od = (a >> 16) | (b & jnp.uint32(0xFFFF0000))
            w_v[pl.ds(ch * (16 * PITCH) + p, 8, stride=PITCH), :] = ev
            w_v[pl.ds(ch * (16 * PITCH) + 8 * PITCH + p, 8, stride=PITCH), :] = od

    def w_slab(ch, l, lo=0, hi=D):
        base = (ch * 16 + (l % 2) * 8 + l // 2) * PITCH + lo // 2
        return _unpk(w_v[base:base + (hi - lo) // 2, :])

    def ring_of(ch, l):
        return rings[l // 2], ch * 2 + l % 2

    c_cp.start()
    mem0_cp.start()
    x_cp(0).start()
    stage_cp(0, 0, 0).start()
    zero_s[0] = 0
    x_v[S:S + SH, :] = jnp.zeros((SH, D), bf16)
    a_v[S:S + SH, :] = jnp.zeros((SH, D), bf16)
    mod_v[:, 0:2 * D] = jnp.zeros((8, 2 * D), f32)
    mod0_cp(0, 0).start()
    mod0_cp(1, 0).start()
    c_cp.wait()
    mem0_cp.wait()
    mem_v[...] = pltpu.bitcast(mem0_v[...], u32)
    cb_v[...] = jnp.transpose(jnp.broadcast_to(silu_c().astype(f32), (128, D)))
    x_cp(0).wait()
    stage_cp(0, 1, 0).start()

    def xhat_body(i, c):
        r0 = pl.multiple_of(i * 64, 64)
        for u in range(4):
            rows = pl.ds(r0 + RC * u, RC)
            xh_v[rows, :] = _ln(x_v[rows, :].astype(f32))
        return c
    lax.fori_loop(0, PRE // 64, xhat_body, 0)

    stage_cp(0, 0, 0).wait()

    def first_repack(i, c):
        repack(0, 0, i * 16, 16)
        return c
    lax.fori_loop(0, KP // 32, first_repack, 0)

    NPC = D // KP
    assert NPC == 4

    def pre_body(i, c):
        t, k = i >> 2, i & 3
        fresh = jnp.logical_and(i > 0, i < 3 * NPC - 1)
        i1 = jnp.where(fresh, i + 1, i)
        t1, k1 = i1 >> 2, i1 & 3

        for kk in range(NPC):
            @pl.when(i == kk)
            def _():
                mod0_cp(0, kk).wait()
                mod0_cp(1, kk).wait()
                if kk == 1:
                    stage_cp(0, 0, 1).wait()
                    repack(0, 0, KP // 2, KP // 2)
                sc = jnp.broadcast_to(silu_c(), (8, D))
                for n in range(MJ // 128):
                    col = (n // 2) * D + kk * KP + (n % 2) * 128
                    mod_v[:, col:col + 128] = _dot(sc, wm_v[kk, :, tile(n)])
                cols = slice(kk * KP, (kk + 1) * KP)
                sa = mod_v[0:1, kk * KP:(kk + 1) * KP]
                ca = mod_v[0:1, D + kk * KP:D + (kk + 1) * KP]
                for q in range(PRE // 64):
                    h0_v[kk, q * 32:(q + 1) * 32, :] = _pk(
                        xh_v[q * 64:(q + 1) * 64, cols] * (1.0 + ca) + sa)
                if kk == 0:
                    stage_cp(0, 0, 1).start()
                if kk + 1 < NPC:
                    mod0_cp(0, kk + 1).start()
                    mod0_cp(1, kk + 1).start()
                stage_cp((kk + 1) // NPC, 1, (kk + 1) % NPC).start()
                stage_cp((kk + 2) // NPC, 0, (kk + 2) % NPC).start()
                if kk == 1:
                    x_cp(1).start()
                if kk == 2:
                    mod1_cp(0).start()
                if kk == 3:
                    stage_cp(1, 1, 1).start()
                    stage_cp(1, 0, 2).start()

        stage_cp(0, 1, k).wait()

        @pl.when(fresh)
        def _():
            stage_cp(0, 0, k1).wait()

        @pl.when(i >= NPC)
        def _():
            mod1_cp(i - NPC).wait()

        @pl.when(jnp.logical_and(i & 1 == 0, jnp.logical_and(i >= 4, i <= 8)))
        def _():
            x_cp((i - 2) >> 1).wait()

        z0 = pl.multiple_of(zero_s[0], 64)
        w0 = pl.multiple_of(t * (32 * PITCH) + k * (KP // 2), 32)
        xrow = jnp.where(i >= NPC, PRE + (i - NPC) * 192, 0)
        hrow = jnp.maximum(i - NPC, 0) * 96
        done = {}
        nd = 0
        macc = None
        for h in range(H):
            hh, l = h // 16, h % 16
            w = _unpk(w_v[pl.ds(w0 + (hh * 16 + (l % 2) * 8 + l // 2) * PITCH, KP // 2), :])
            for rb in range(PRE // BM):
                lhs = _tie(h0_v[k, rb * 64:(rb + 1) * 64, :], done.pop(nd, None))
                rows = pl.ds(z0 + rb * BM, BM)
                y = _dot(_unpk(lhs), w) + jnp.where(k > 0, acc_v[h, rows, :], 0.0)
                acc_v[h, rows, :] = y
                rings[l // 2][t * 4 + hh * 2 + l % 2,
                              QOFF // 2 + rb * 64:QOFF // 2 + (rb + 1) * 64, :] = _pk(y)
                nd += 1
            if l < 15:
                n = 9 if l < 8 else 8
                p0_ = l * 9 if l < 8 else 72 + (l - 8) * 8
                if hh == 0:
                    repack(1, 2 * t + 1 + zero_s[0], k * (KP // 2) + p0_, n)
                else:
                    repack(0, 2 * t1, k1 * (KP // 2) + p0_, n)
            if h < CFG['mh']:
                g0, g1 = (h * 128) // CFG['mh'], ((h + 1) * 128) // CFG['mh']
                for g in range(g0, g1):
                    cb = cb_v[pl.ds(z0 + g * 8, 8), :]
                    wmg = wm_v[i, g * 8:(g + 1) * 8, :].astype(f32)
                    pr = wmg * jnp.concatenate([cb] * (MJ // 128), axis=1)
                    macc = pr if macc is None else macc + pr
                done[nd + CFG['md']] = pltpu.bitcast(macc[:, 0:CFG['mw']], u32)
                if h == CFG['mh'] - 1:
                    modr_v[jnp.where(i >= NPC, i - NPC, 2 * NPC)] = macc
            if h % 2 == 1 and h < 24:
                q = h // 2
                xs = x_v[pl.ds(pl.multiple_of(xrow + q * RC, RC), RC), :].astype(f32)
                hx = _pk(_ln(xs) * (1.0 + mod(1)) + mod(0))
                done[nd + 12] = hx
                for n in range(NT):
                    hx_v[n, pl.ds(pl.multiple_of(hrow + q * 8, 8), 8), :] = hx[:, tile(n)]
        @pl.when(i == 3)
        def _():
            mod1_cp(1).start()

        @pl.when(jnp.logical_or(i == 4, i == 5))
        def _():
            x_cp(i - 2).start()

        for tt in range(1, 3):
            @pl.when(jnp.logical_and(i >= 3, (i + 3) >> 2 == tt))
            def _():
                stage_cp(tt, 1, (i + 3) & 3).start()

            @pl.when(jnp.logical_and(i >= 3, t + 1 == tt))
            def _():
                stage_cp(tt, 0, k).start()

        @pl.when(jnp.logical_and(i >= 3, i <= 8))
        def _():
            mod1_cp(i - 1).start()

        @pl.when(i == 8)
        def _():
            wo_cp.start()
        return c
    if CFG['pre']:
        lax.fori_loop(0, 3 * NPC, pre_body, 0)

    for cp in (w1_cp, w2_cp, w3_cp, w4_cp):
        cp.start()
    for q in range(2 * NPC):
        mod_v[:, 2 * D + q * MJ:2 * D + (q + 1) * MJ] = jnp.broadcast_to(
            jnp.sum(modr_v[q], axis=0, keepdims=True), (8, MJ))
    wo_cp.wait()

    L2 = 2 * (SEG + MEM)
    r = lax.broadcasted_iota(jnp.int32, (L2, L2), 0)
    c = lax.broadcasted_iota(jnp.int32, (L2, L2), 1)
    r1 = ((r >= SEG) & (r < 2 * SEG)) | (r >= 2 * SEG + MEM)
    c1 = ((c >= SEG) & (c < 2 * SEG)) | (c >= 2 * SEG + MEM)
    same = r1 == c1
    mask = same & ((r >= 2 * SEG) | (c >= 2 * SEG) | (c <= r))
    fill = jnp.where(same, -1e9 / SCALE, -jnp.inf).astype(f32)

    def step(s, mem, zero, left):
        woff = pl.multiple_of((XR // 2 * s) % (RING // 2), 4)
        roff = pl.multiple_of((SEG // 2 * s + QOFF // 2) % (RING // 2), SEG // 2)
        arow = pl.multiple_of(SEG * s, SEG)
        acc = [None] * NT
        ym, ps, ol, part, rest = {}, {}, {}, {}, {}
        HK = D // 2
        tiles = [_unpk(jnp.concatenate(
            [hx_v[k, pl.ds(s * (XR // 2), XR // 2), :] | zero, mem[k]], axis=0))
            for k in range(NT)]
        mem_new = []

        def lhs(lo, hi):
            return jnp.concatenate(tiles[lo // 128:hi // 128], axis=1)

        def qkv_lo(h, t):
            part[(t, h)] = _dot(lhs(0, HK), w_slab(2 * t + h // 16, h % 16, 0, HK))

        def proj(t, h):
            ch, l = 2 * t + h // 16, h % 16
            if (t, h) in part:
                y = _dot(lhs(HK, D), w_slab(ch, l, HK, D)) + part.pop((t, h))
            else:
                y = _dot(lhs(0, D), w_slab(ch, l))
            rg, ix = ring_of(ch, l)
            rg[ix, pl.ds(woff, XR // 2), :] = _pk(y[0:XR])
            ym[(t, h)] = y[XR:XR + MEM]

        def get(t, p):
            rg, i0 = ring_of(2 * t + p // 8, (2 * p) % 16)
            mm = jnp.concatenate([ym.pop((t, 2 * p)), ym.pop((t, 2 * p + 1))], axis=0)
            return _unpk(jnp.concatenate(
                [rg[i0, pl.ds(roff, SEG // 2), :], rg[i0 + 1, pl.ds(roff, SEG // 2), :], _pk(mm)],
                axis=0))

        def sm(p):
            sc = lax.dot_general(get(0, p), get(1, p), (((1,), (1,)), ((), ())),
                                 preferred_element_type=f32)
            sc = jnp.where(mask, sc, fill)
            e = jnp.exp2((sc - jnp.max(sc, axis=-1, keepdims=True)) * (SCALE * LOG2E))
            ps[p] = (e * pl.reciprocal(jnp.sum(e, axis=-1, keepdims=True), approx=True)
                     ).astype(bf16)

        def pv(p):
            o = _dot(ps.pop(p), get(2, p))
            for j in range(2):
                h = 2 * p + j
                ox = o[SEG * j:SEG * (j + 1)]
                om = o[2 * SEG + MEM * j:2 * SEG + MEM * (j + 1)]
                if left is None:
                    ol[h] = jnp.concatenate([ox[0:XR], om], axis=0).astype(bf16)
                    rest[h] = ox[XR:SEG]
                else:
                    ol[h] = jnp.concatenate([ox, left[h], om], axis=0).astype(bf16)

        def wo(n, h0, h1):
            for h in range(h0, h1):
                y = _dot(ol[h], wo_v[h * DH:(h + 1) * DH, tile(n)])
                acc[n] = y if acc[n] is None else y + acc[n]
            if h1 == H:
                if left is None:
                    a_v[pl.ds(arow, XR), tile(n)] = acc[n][0:XR].astype(bf16)
                else:
                    a_v[pl.ds(arow, SEG), tile(n)] = acc[n][0:SEG].astype(bf16)
                    a_v[pl.ds(arow - (SEG - XR), SEG - XR), tile(n)] = (
                        acc[n][SEG:2 * SEG - XR].astype(bf16))
                mem_new.append(_pk(acc[n][-MEM:]))

        HE, DS, DP, DV = CFG['he'], CFG['ds'], CFG['dp'], CFG['dv']
        seq = []
        for p in range(NPAIR + DV):
            if p < NPAIR:
                seq += [(t, 2 * p + j) for t, j in CFG['qk']]
            if p - DV >= 0:
                seq += [(2, 2 * (p - DV)), (2, 2 * (p - DV) + 1)]
        events = {}
        for p in range(NPAIR):
            at = max(seq.index((t, 2 * p + j)) for t in range(2) for j in range(2)) + DS
            events.setdefault(at, []).append((sm, p))
            events.setdefault(at + DP, []).append((pv, p))
        for t, h in seq[:CFG['nlo']]:
            qkv_lo(h, t)
        WU = HE // 8
        for i in range(len(seq) + NT * WU):
            if i < len(seq):
                proj(*seq[i])
            else:
                u = i - len(seq)
                wo(u // WU, (u % WU) * 8, (u % WU + 1) * 8)
            for fn, p in events.pop(i, []):
                fn(p)
        assert not events
        for n in range(NT):
            wo(n, HE, H)
        return mem_new, rest

    def steps(i, carry):
        zero = zero_s[0].astype(u32)
        mem = [mem_v[:, tile(k)] for k in range(NT)]
        mem, rest = step(2 * i, mem, zero, None)
        mem, _ = step(2 * i + 1, mem, zero, rest)
        for k in range(NT):
            mem_v[:, tile(k)] = mem[k]
        return carry
    if CFG['step']:
        lax.fori_loop(0, NSEG // 2, steps, 0)

    if not CFG['b']:
        cp = pltpu.make_async_copy(a_v.at[pl.ds(0, S)], out_hbm, sem_out)
        cp.start()
        cp.wait()
        return

    for cp in (w1_cp, w2_cp, w3_cp, w4_cp):
        cp.wait()

    def p0(tok, w):
        rows = pl.ds(tok, RC)
        xa = x_v[rows, :].astype(f32) + mod(2) * a_v[rows, :].astype(f32)
        hb = _ln(xa) * (1.0 + mod(4)) + mod(3)
        xa_v[w:w + RC, :] = xa
        hb_v[w:w + RC, :] = hb
        return _pk(_ln(hb))

    y0 = p0(0, 0)
    for k in range(BM // RC):
        y1_v[k * 8:(k + 1) * 8, :] = p0(SH + k * RC, SH + k * RC)
    for n in range(NT):
        g_v[n, 0:8, :] = jnp.zeros((8, 128), f32)
        g_v[n, 8:8 + SH, :] = _gelu(_dot(_unpk(y0), w1_v[:, tile(n)]))

    HM = BM // 2
    shift = (-1, 1, -2, 2)

    def blk(j, c):
        r0 = pl.multiple_of(j * BM, BM)
        nxt = pl.multiple_of(jnp.minimum(j + 1, NB - 1) * BM + SH, SH)
        more = j < NB - 1

        def w1_half(hf):
            for n in range(NT):
                g = _gelu(_dot(_unpk(y1_v[hf * 32:(hf + 1) * 32, :]), w1_v[:, tile(n)]))
                w0 = 8 + SH + hf * HM
                if hf == 0:
                    g_v[n, w0:w0 + HM, :] = g
                else:
                    g_v[n, w0:w0 + HM - SH, :] = g[0:HM - SH]
                    g_v[n, w0 + HM - SH:w0 + HM, :] = jnp.where(more, g[HM - SH:HM], 0.0)

        def w2_half(hf):
            for n in range(NT):
                w0 = 8 + hf * HM + shift[n // 2]
                z_v[hf * 32:(hf + 1) * 32, tile(n)] = _pk(g_v[n, w0:w0 + HM, :])
            for n in range(NT):
                x1_v[hf * HM:(hf + 1) * HM, tile(n)] = (
                    _dot(_unpk(z_v[hf * 32:(hf + 1) * 32, :]), w2_v[:, tile(n)])
                    + hb_v[hf * HM:(hf + 1) * HM, tile(n)])

        def p1_half(hf):
            for k in range(hf * HM // RC, (hf + 1) * HM // RC):
                x1 = x1_v[k * RC:(k + 1) * RC, :]
                y2_v[k * 8:(k + 1) * 8, :] = _pk(_ln(x1))
                base_v[k * RC:(k + 1) * RC, :] = xa_v[k * RC:(k + 1) * RC, :] + mod(5) * x1

        def w3(f, lo, hi, after=None):
            u_v[lo:hi, tile(f)] = _pk(_gelu(
                _dot(_unpk(_tie(y2_v[lo:hi, :], after)), w3_v[:, tile(f)])))

        w1_half(0)
        w1_half(1)
        w2_half(0)
        w2_half(1)
        p1_half(0)
        for f in range(CFG['nf']):
            w3(f, 0, 32)
        p1_half(1)
        for f in range(CFG['nf']):
            w3(f, 32, 64)
        for n in range(NT):
            g_v[n, 0:8 + SH, :] = g_v[n, BM:BM + 8 + SH, :]
        xa_v[0:SH, :] = xa_v[BM:BM + SH, :]
        hb_v[0:SH, :] = hb_v[BM:BM + SH, :]
        for f in range(CFG['nf'], NF):
            w3(f, 0, 64)
        for n in range(NT):
            y = p0(nxt + n * RC, SH + n * RC)
            y1_v[n * 8:(n + 1) * 8, :] = y
            gb = mod(5, n * 128, (n + 1) * 128)
            u = _unpk(_tie(u_v[...], y, 0, CFG['p0k']))
            a_v[pl.ds(r0, BM), tile(n)] = (
                base_v[:, tile(n)] + gb * _dot(u, w4_v[:, tile(n)])).astype(bf16)
            if n + 1 in CFG['ow'][1:]:
                lo = CFG['ow'][CFG['ow'].index(n + 1) - 1]
                cols = pl.ds(lo * 128, (n + 1 - lo) * 128)
                pltpu.make_async_copy(a_v.at[pl.ds(r0, BM), cols], out_hbm.at[pl.ds(r0, BM), cols],
                                      sem_out).start()
        return c
    lax.fori_loop(0, NB, blk, 0)
    pltpu.make_async_copy(a_v.at[pl.ds(0, S)], out_hbm, sem_out).wait()


@functools.partial(jax.jit, static_argnames=("A_seg_len",))
def pallas_adaLN_cond__memory_aug_recurrent_mem_tr__mixer_s_mlp__prompt_kernel(
    A_x: jax.Array,
    A_mem0: jax.Array,
    A_Wq: jax.Array,
    A_Wk: jax.Array,
    A_Wv: jax.Array,
    A_Wo: jax.Array,
    A_seg_len,
    B_x: jax.Array,
    B_w1: jax.Array,
    B_w2: jax.Array,
    B_w3: jax.Array,
    B_w4: jax.Array,
    c: jax.Array,
    w_mod: jax.Array,
):
    assert A_seg_len == SEG and A_x.shape == (1, S, D) and A_Wq.shape == (D, H, DH)
    any_spec = pl.BlockSpec(memory_space=pl.ANY)
    out = pl.pallas_call(
        _kernel,
        out_shape=jax.ShapeDtypeStruct((S, D), bf16),
        in_specs=[any_spec] * 12,
        out_specs=any_spec,
        scratch_shapes=[
            pltpu.VMEM((1, D), bf16),
            pltpu.VMEM((S + SH, D), bf16),
            pltpu.VMEM((S + SH, D), bf16),
            pltpu.VMEM((D // KP, PRE // 2, KP), u32),
            pltpu.VMEM((MEM // 2, D), u32),
            pltpu.VMEM((MEM, D), bf16),
            pltpu.VMEM((8, 6 * D), f32),
            pltpu.VMEM((9, 8, MJ), f32),
            pltpu.VMEM((D, 128), f32),
            pltpu.VMEM((12, D, MJ), bf16),
            pltpu.VMEM((96 * PITCH, 128), u32),
            pltpu.VMEM((H * DH, D + PADL), bf16),
            pltpu.VMEM((D, D + PADL), bf16),
            pltpu.VMEM((D, D + PADL), bf16),
            pltpu.VMEM((D, F + PADL), bf16),
            pltpu.VMEM((F, D + PADL), bf16),
            pltpu.VMEM((NT, BM + 32, 128), f32),
            pltpu.VMEM((BM + SH, D), f32),
            pltpu.VMEM((BM + SH, D), f32),
            pltpu.VMEM((BM, D), f32),
            pltpu.VMEM((BM, D), f32),
            pltpu.VMEM((BM // 2, D), u32),
            pltpu.VMEM((BM // 2, D), u32),
            pltpu.VMEM((BM // 2, D), u32),
            pltpu.VMEM((BM // 2, F), u32),
            pltpu.VMEM((2, D, 16, DH), bf16),
            pltpu.VMEM((PRE, D), f32),
            pltpu.VMEM((NT, HR, 128), u32),
            pltpu.VMEM((H, PRE, DH), f32),
        ] + [pltpu.VMEM((12, RING // 2, DH), u32)] * 8 + [
            pltpu.SMEM((1,), jnp.int32),
            pltpu.SemaphoreType.DMA((2,)),
            pltpu.SemaphoreType.DMA((4,)),
            pltpu.SemaphoreType.DMA((2, 4)),
            pltpu.SemaphoreType.DMA((2, 4)),
            pltpu.SemaphoreType.DMA((5,)),
            pltpu.SemaphoreType.DMA(()),
        ],
        compiler_params=pltpu.CompilerParams(vmem_limit_bytes=120 * 1024 * 1024),
    )(A_x.reshape(S, D), A_mem0.reshape(MEM, D), A_Wq, A_Wk, A_Wv, A_Wo.reshape(H * DH, D),
      B_w1, B_w2, B_w3, B_w4, c, w_mod)
    return out.reshape(1, S, D)
```

```python
import functools

import jax
import jax.numpy as jnp
from jax import lax
import jax.experimental.pallas as pl
import jax.experimental.pallas.tpu as pltpu

bf16, f32, u32 = jnp.bfloat16, jnp.float32, jnp.uint32

S, D, H, DH, MEM, SEG, F = 2048, 1024, 32, 128, 8, 32, 3584
NSEG = S // SEG
XR = 24
PRE = S - XR * NSEG
RING = 576
QOFF = RING - PRE
EP = RING // 2
PITCH = 520
NT = D // 128
NF = F // 128
BM = 128
NB = S // BM
NPAIR = H // 2
HR = 32 * (NSEG // 2)
PADL = 128
SH = 16
KP = 256
MJ = 512
RC = 16
EPS = 1e-5
LOG2E = 1.4426950408889634
SCALE = DH ** -0.5
CFG = dict(pre=True, step=True, b=True, nlo=6, he=16, mh=28, md=9, mw=512, ds=5, dp=10, dv=0, qk=((0, 0), (1, 0), (0, 1), (1, 1)), ow=(0, 7, 8), nf=7, p0k=24)


def _ln(x):
    m = jnp.mean(x, axis=-1, keepdims=True)
    xc = x - m
    v = jnp.mean(xc * xc, axis=-1, keepdims=True)
    return xc * lax.rsqrt(v + EPS)


def _gelu(x):
    return jax.nn.gelu(x, approximate=True)


def _dot(a, b):
    return jnp.dot(a, b, preferred_element_type=f32)


def _pk(x):
    return pltpu.bitcast(x.astype(bf16), u32)


def _unpk(x):
    return pltpu.bitcast(x, bf16)


def _tie(w, after, r=0, k=0):
    if after is None:
        return w
    m = functools.reduce(lambda a, b: a & b,
                         [after[:, i * 128:(i + 1) * 128] for i in range(after.shape[1] // 128)])
    mf = pltpu.bitcast(m, f32)
    z = jnp.where(mf * mf < 0.0, jnp.uint32(1), jnp.uint32(0))
    row = w[r:r + 8]
    parts = [row[:, :k * 128], row[:, k * 128:(k + 1) * 128] | z, row[:, (k + 1) * 128:]]
    row = jnp.concatenate([p for p in parts if p.shape[1]], axis=1)
    parts = [w[:r], row, w[r + 8:]]
    return jnp.concatenate([p for p in parts if p.shape[0]], axis=0)


def _kernel(x_hbm, mem0_hbm, wq_hbm, wk_hbm, wv_hbm, wo_hbm, w1_hbm, w2_hbm, w3_hbm, w4_hbm,
            c_hbm, wmod_hbm, out_hbm,
            c_v, x_v, a_v, h0_v, mem_v, mem0_v, mod_v, modr_v, cb_v, sc_v, wm_v, w_v, wo_v,
            w1_v, w2_v, w3_v, w4_v,
            g_v, xa_v, hb_v, base_v, x1_v, y1_v, z_v, y2_v, u_v,
            stage, xh_v, hx_v, acc_v,
            r0_, r1_, r2_, r3_, r4_, r5_, r6_, r7_,
            zero_s, sem_small, sem_x, sem_stage, sem_mod, sem_w, sem_out):
    wqkv_hbm = (wq_hbm, wk_hbm, wv_hbm)
    rings = (r0_, r1_, r2_, r3_, r4_, r5_, r6_, r7_)

    c_cp = pltpu.make_async_copy(c_hbm, c_v.at[:, pl.ds(0, D)], sem_small.at[0])
    mem0_cp = pltpu.make_async_copy(mem0_hbm, mem0_v, sem_small.at[1])

    def x_cp(q):
        rows = pl.ds(q * PRE if isinstance(q, int) else pl.multiple_of(q * PRE, PRE), PRE)
        return pltpu.make_async_copy(x_hbm.at[rows], x_v.at[rows], sem_x.at[q])

    def w_cp(src, dst, k):
        return pltpu.make_async_copy(src, dst.at[:, pl.ds(0, src.shape[1])], sem_w.at[k])

    wo_cp, w1_cp, w2_cp, w3_cp, w4_cp = (
        w_cp(a, b, k) for k, (a, b) in enumerate(
            ((wo_hbm, wo_v), (w1_hbm, w1_v), (w2_hbm, w2_v), (w3_hbm, w3_v), (w4_hbm, w4_v))))

    def mod0_cp(j, k):
        return pltpu.make_async_copy(wmod_hbm.at[:, pl.ds(j * D + k * KP, KP)],
                                     wm_v.at[k, :, pl.ds(j * KP, KP)], sem_mod.at[j, k])

    def mod1_cp(q):
        col = 2 * D + q * MJ
        col = col if isinstance(q, int) else pl.multiple_of(col, MJ)
        return pltpu.make_async_copy(wmod_hbm.at[:, pl.ds(col, MJ)], wm_v.at[(4 + q) & 7],
                                     sem_mod.at[q >> 2, q & 3])

    def stage_cp(t, hh, piece):
        d0 = piece * KP if isinstance(piece, int) else pl.multiple_of(piece * KP, KP)
        return pltpu.make_async_copy(
            wqkv_hbm[t].at[pl.ds(d0, KP), pl.ds(hh * 16, 16), :],
            stage.at[hh, pl.ds(d0, KP)], sem_stage.at[hh, piece])

    def tile(n):
        return slice(n * 128, (n + 1) * 128)

    def silu_c():
        cf = c_v[:, 0:D].astype(f32)
        return (cf * jax.nn.sigmoid(cf)).astype(bf16)

    def mod(k, lo=0, hi=D):
        return mod_v[0:1, k * D + lo:k * D + hi]

    def repack(hh, ch, p0, n):
        both = None
        for u in range(n):
            p = p0 + u
            a = pltpu.bitcast(stage[hh, 2 * p], u32)
            b = pltpu.bitcast(stage[hh, 2 * p + 1], u32)
            ev = (a & jnp.uint32(0xFFFF)) | (b << 16)
            od = (a >> 16) | (b & jnp.uint32(0xFFFF0000))
            w_v[pl.ds(ch * (16 * PITCH) + p, 8, stride=PITCH), :] = ev
            w_v[pl.ds(ch * (16 * PITCH) + 8 * PITCH + p, 8, stride=PITCH), :] = od
            both = ev & od if both is None else both & ev & od
        return both

    def w_slab(ch, l, lo=0, hi=D):
        base = (ch * 16 + (l % 2) * 8 + l // 2) * PITCH + lo // 2
        return _unpk(w_v[base:base + (hi - lo) // 2, :])

    def ring_of(ch, l):
        return rings[l // 2], (ch * 2 + l % 2) * EP

    c_cp.start()
    mem0_cp.start()
    x_cp(0).start()
    stage_cp(0, 0, 0).start()
    zero_s[0] = 0
    x_v[S:S + SH, :] = jnp.zeros((SH, D), bf16)
    a_v[S:S + SH, :] = jnp.zeros((SH, D), bf16)
    mod_v[:, 0:2 * D] = jnp.zeros((8, 2 * D), f32)
    mod0_cp(0, 0).start()
    mod0_cp(1, 0).start()
    c_cp.wait()
    mem0_cp.wait()
    mem_v[...] = pltpu.bitcast(mem0_v[...], u32)
    cb_v[...] = jnp.transpose(jnp.broadcast_to(silu_c().astype(f32), (128, D)))
    sc_v[...] = _pk(jnp.broadcast_to(silu_c().astype(f32), (16, D)))
    x_cp(0).wait()
    stage_cp(0, 1, 0).start()

    def xhat_body(i, c):
        r0 = pl.multiple_of(i * 64, 64)
        for u in range(4):
            rows = pl.ds(r0 + RC * u, RC)
            xh_v[rows, :] = _ln(x_v[rows, :].astype(f32))
        return c
    lax.fori_loop(0, PRE // 64, xhat_body, 0)

    stage_cp(0, 0, 0).wait()

    def first_repack(i, c):
        repack(0, 0, i * 16, 16)
        return c
    lax.fori_loop(0, KP // 32, first_repack, 0)

    NPC = D // KP
    assert NPC == 4

    def pre_body(i, c):
        t, k = i >> 2, i & 3
        fresh = jnp.logical_and(i > 0, i < 3 * NPC - 1)
        i1 = jnp.where(fresh, i + 1, i)
        t1, k1 = i1 >> 2, i1 & 3

        for kk in range(NPC):
            @pl.when(i == kk)
            def _():
                mod0_cp(0, kk).wait()
                mod0_cp(1, kk).wait()
                if kk == 1:
                    stage_cp(0, 0, 1).wait()
                for e in range(KP // 128):
                    m = []
                    for j in range(2):
                        m.append(_dot(_unpk(sc_v[...]), wm_v[kk, :, tile(2 * j + e)])[0:8])
                        col = j * D + kk * KP + e * 128
                        mod_v[:, col:col + 128] = m[j]
                    cols = slice(kk * KP + e * 128, kk * KP + (e + 1) * 128)
                    for q in range(PRE // 64):
                        ca = m[1]
                        if kk == 1:
                            rp = repack(0, 0, KP // 2 + (e * 8 + q) * 8, 8)
                            ca = pltpu.bitcast(_tie(pltpu.bitcast(ca, u32), rp), f32)
                        h0_v[kk, q * 32:(q + 1) * 32, tile(e)] = _pk(
                            xh_v[q * 64:(q + 1) * 64, cols] * (1.0 + ca[0:1]) + m[0][0:1])
                if kk == 0:
                    stage_cp(0, 0, 1).start()
                if kk + 1 < NPC:
                    mod0_cp(0, kk + 1).start()
                    mod0_cp(1, kk + 1).start()
                stage_cp((kk + 1) // NPC, 1, (kk + 1) % NPC).start()
                stage_cp((kk + 2) // NPC, 0, (kk + 2) % NPC).start()
                if kk == 1:
                    x_cp(1).start()
                if kk == 2:
                    mod1_cp(0).start()
                if kk == 3:
                    stage_cp(1, 1, 1).start()
                    stage_cp(1, 0, 2).start()

        stage_cp(0, 1, k).wait()

        @pl.when(fresh)
        def _():
            stage_cp(0, 0, k1).wait()

        @pl.when(i >= NPC)
        def _():
            mod1_cp(i - NPC).wait()

        @pl.when(jnp.logical_and(i & 1 == 0, jnp.logical_and(i >= 4, i <= 8)))
        def _():
            x_cp((i - 2) >> 1).wait()

        z0 = pl.multiple_of(zero_s[0], 64)
        w0 = pl.multiple_of(t * (32 * PITCH) + k * (KP // 2), 32)
        xrow = jnp.where(i >= NPC, PRE + (i - NPC) * 192, 0)
        hrow = pl.multiple_of(jnp.maximum(i - NPC, 0) * 128, 128)
        done = {}
        nd = 0
        macc = None
        for h in range(H):
            hh, l = h // 16, h % 16
            w = _unpk(w_v[pl.ds(w0 + (hh * 16 + (l % 2) * 8 + l // 2) * PITCH, KP // 2), :])
            q0 = pl.multiple_of(t * (4 * EP), 32) + ring_of(hh, l)[1] + QOFF // 2
            for rb in range(PRE // BM):
                lhs = _tie(h0_v[k, rb * 64:(rb + 1) * 64, :], done.pop(nd, None))
                rows = pl.ds(z0 + rb * BM, BM)
                y = _dot(_unpk(lhs), w) + jnp.where(k > 0, acc_v[h, rows, :], 0.0)
                acc_v[h, rows, :] = y
                rings[l // 2][pl.ds(q0 + rb * 64, 64), :] = _pk(y)
                nd += 1
            if l < 15:
                n = 9 if l < 8 else 8
                p0_ = l * 9 if l < 8 else 72 + (l - 8) * 8
                if hh == 0:
                    repack(1, 2 * t + 1 + zero_s[0], k * (KP // 2) + p0_, n)
                else:
                    repack(0, 2 * t1, k1 * (KP // 2) + p0_, n)
            if h < CFG['mh']:
                g0, g1 = (h * 128) // CFG['mh'], ((h + 1) * 128) // CFG['mh']
                for g in range(g0, g1):
                    cb = cb_v[pl.ds(z0 + g * 8, 8), :]
                    wmg = wm_v[i & 7, g * 8:(g + 1) * 8, :].astype(f32)
                    pr = wmg * jnp.concatenate([cb] * (MJ // 128), axis=1)
                    macc = pr if macc is None else macc + pr
                done[nd + CFG['md']] = pltpu.bitcast(macc[:, 0:CFG['mw']], u32)
                if h == CFG['mh'] - 1:
                    modr_v[jnp.where(i >= NPC, i - NPC, 2 * NPC)] = macc
            if h % 2 == 1 and h < 24:
                q = h // 2
                xs = x_v[pl.ds(pl.multiple_of(xrow + q * RC, RC), RC), :].astype(f32)
                hx = _pk(_ln(xs) * (1.0 + mod(1)) + mod(0))
                done[nd + 12] = hx
                for n in range(NT):
                    hx_v[n, pl.ds(hrow + (q // 3) * 32 + (q % 3) * 8, 8), :] = hx[:, tile(n)]
        @pl.when(i == 3)
        def _():
            mod1_cp(1).start()

        @pl.when(jnp.logical_or(i == 4, i == 5))
        def _():
            x_cp(i - 2).start()

        for tt in range(1, 3):
            @pl.when(jnp.logical_and(i >= 3, (i + 3) >> 2 == tt))
            def _():
                stage_cp(tt, 1, (i + 3) & 3).start()

            @pl.when(jnp.logical_and(i >= 3, t + 1 == tt))
            def _():
                stage_cp(tt, 0, k).start()

        @pl.when(jnp.logical_and(i >= 3, i <= 8))
        def _():
            mod1_cp(i - 1).start()

        @pl.when(i == 8)
        def _():
            wo_cp.start()
        return c
    if CFG['pre']:
        lax.fori_loop(0, 3 * NPC, pre_body, 0)

    for cp in (w1_cp, w2_cp, w3_cp, w4_cp):
        cp.start()
    for q in range(2 * NPC):
        mod_v[:, 2 * D + q * MJ:2 * D + (q + 1) * MJ] = jnp.broadcast_to(
            jnp.sum(modr_v[q], axis=0, keepdims=True), (8, MJ))
    wo_cp.wait()

    L2 = 2 * (SEG + MEM)
    r = lax.broadcasted_iota(jnp.int32, (L2, L2), 0)
    c = lax.broadcasted_iota(jnp.int32, (L2, L2), 1)
    r1 = ((r >= SEG) & (r < 2 * SEG)) | (r >= 2 * SEG + MEM)
    c1 = ((c >= SEG) & (c < 2 * SEG)) | (c >= 2 * SEG + MEM)
    same = r1 == c1
    mask = same & ((r >= 2 * SEG) | (c >= 2 * SEG) | (c <= r))
    fill = jnp.where(same, -1e9 / SCALE, -jnp.inf).astype(f32)

    def step(i, mem, zero, left):
        j = 0 if left is None else 1
        woff = pl.multiple_of((XR * i) % EP, 8) + j * (XR // 2)
        roff = pl.multiple_of((SEG * i + QOFF // 2) % EP, SEG) + j * (SEG // 2)
        arow = pl.multiple_of(2 * SEG * i, 2 * SEG) + j * SEG
        hrow = pl.multiple_of(32 * i, 32) + j * (XR // 2)
        acc = [None] * NT
        ym, ps, ol, part, rest = {}, {}, {}, {}, {}
        HK = D // 2
        tiles = [_unpk(jnp.concatenate(
            [hx_v[k, pl.ds(hrow, XR // 2), :] | zero, mem[k]], axis=0))
            for k in range(NT)]
        mem_new = []

        def lhs(lo, hi):
            return jnp.concatenate(tiles[lo // 128:hi // 128], axis=1)

        def qkv_lo(h, t):
            part[(t, h)] = _dot(lhs(0, HK), w_slab(2 * t + h // 16, h % 16, 0, HK))

        def proj(t, h):
            ch, l = 2 * t + h // 16, h % 16
            if (t, h) in part:
                y = _dot(lhs(HK, D), w_slab(ch, l, HK, D)) + part.pop((t, h))
            else:
                y = _dot(lhs(0, D), w_slab(ch, l))
            rg, ix = ring_of(ch, l)
            rg[pl.ds(ix + woff, XR // 2), :] = _pk(y[0:XR])
            ym[(t, h)] = y[XR:XR + MEM]

        def get(t, p):
            rg, i0 = ring_of(2 * t + p // 8, (2 * p) % 16)
            _, i1 = ring_of(2 * t + p // 8, (2 * p) % 16 + 1)
            mm = jnp.concatenate([ym.pop((t, 2 * p)), ym.pop((t, 2 * p + 1))], axis=0)
            return _unpk(jnp.concatenate(
                [rg[pl.ds(i0 + roff, SEG // 2), :], rg[pl.ds(i1 + roff, SEG // 2), :], _pk(mm)],
                axis=0))

        def sm(p):
            sc = lax.dot_general(get(0, p), get(1, p), (((1,), (1,)), ((), ())),
                                 preferred_element_type=f32)
            sc = jnp.where(mask, sc, fill)
            e = jnp.exp2((sc - jnp.max(sc, axis=-1, keepdims=True)) * (SCALE * LOG2E))
            ps[p] = (e * pl.reciprocal(jnp.sum(e, axis=-1, keepdims=True), approx=True)
                     ).astype(bf16)

        def pv(p):
            o = _dot(ps.pop(p), get(2, p))
            for b in range(2):
                h = 2 * p + b
                ox = o[SEG * b:SEG * (b + 1)]
                om = o[2 * SEG + MEM * b:2 * SEG + MEM * (b + 1)]
                if left is None:
                    ol[h] = jnp.concatenate([ox[0:XR], om], axis=0).astype(bf16)
                    rest[h] = ox[XR:SEG]
                else:
                    ol[h] = jnp.concatenate([ox, left[h], om], axis=0).astype(bf16)

        def wo(n, h0, h1):
            for h in range(h0, h1):
                y = _dot(ol[h], wo_v[h * DH:(h + 1) * DH, tile(n)])
                acc[n] = y if acc[n] is None else y + acc[n]
            if h1 == H:
                if left is None:
                    a_v[pl.ds(arow, XR), tile(n)] = acc[n][0:XR].astype(bf16)
                else:
                    a_v[pl.ds(arow, SEG), tile(n)] = acc[n][0:SEG].astype(bf16)
                    a_v[pl.ds(arow - (SEG - XR), SEG - XR), tile(n)] = (
                        acc[n][SEG:2 * SEG - XR].astype(bf16))
                mem_new.append(_pk(acc[n][-MEM:]))

        HE, DS, DP, DV = CFG['he'], CFG['ds'], CFG['dp'], CFG['dv']
        seq = []
        for p in range(NPAIR + DV):
            if p < NPAIR:
                seq += [(t, 2 * p + j) for t, j in CFG['qk']]
            if p - DV >= 0:
                seq += [(2, 2 * (p - DV)), (2, 2 * (p - DV) + 1)]
        events = {}
        for p in range(NPAIR):
            at = max(seq.index((t, 2 * p + j)) for t in range(2) for j in range(2)) + DS
            events.setdefault(at, []).append((sm, p))
            events.setdefault(at + DP, []).append((pv, p))
        for t, h in seq[:CFG['nlo']]:
            qkv_lo(h, t)
        WU = HE // 8
        for d in range(len(seq) + NT * WU):
            if d < len(seq):
                proj(*seq[d])
            else:
                u = d - len(seq)
                wo(u // WU, (u % WU) * 8, (u % WU + 1) * 8)
            for fn, p in events.pop(d, []):
                fn(p)
        assert not events
        for n in range(NT):
            wo(n, HE, H)
        return mem_new, rest

    def steps(i, carry):
        zero = zero_s[0].astype(u32)
        mem = [mem_v[:, tile(k)] for k in range(NT)]
        mem, rest = step(i, mem, zero, None)
        mem, _ = step(i, mem, zero, rest)
        for k in range(NT):
            mem_v[:, tile(k)] = mem[k]
        return carry
    if CFG['step']:
        lax.fori_loop(0, NSEG // 2, steps, 0)

    if not CFG['b']:
        cp = pltpu.make_async_copy(a_v.at[pl.ds(0, S)], out_hbm, sem_out)
        cp.start()
        cp.wait()
        return

    for cp in (w1_cp, w2_cp, w3_cp, w4_cp):
        cp.wait()

    def p0(tok, w):
        rows = pl.ds(tok, RC)
        xa = x_v[rows, :].astype(f32) + mod(2) * a_v[rows, :].astype(f32)
        hb = _ln(xa) * (1.0 + mod(4)) + mod(3)
        xa_v[w:w + RC, :] = xa
        hb_v[w:w + RC, :] = hb
        return _pk(_ln(hb))

    y0 = p0(0, 0)
    for k in range(BM // RC):
        y1_v[k * 8:(k + 1) * 8, :] = p0(SH + k * RC, SH + k * RC)
    for n in range(NT):
        g_v[n, 0:8, :] = jnp.zeros((8, 128), f32)
        g_v[n, 8:8 + SH, :] = _gelu(_dot(_unpk(y0), w1_v[:, tile(n)]))

    HM = BM // 2
    shift = (-1, 1, -2, 2)

    def blk(j, c):
        r0 = pl.multiple_of(j * BM, BM)
        nxt = pl.multiple_of(jnp.minimum(j + 1, NB - 1) * BM + SH, SH)
        more = j < NB - 1

        def w1_half(hf):
            for n in range(NT):
                g = _gelu(_dot(_unpk(y1_v[hf * 32:(hf + 1) * 32, :]), w1_v[:, tile(n)]))
                w0 = 8 + SH + hf * HM
                if hf == 0:
                    g_v[n, w0:w0 + HM, :] = g
                else:
                    g_v[n, w0:w0 + HM - SH, :] = g[0:HM - SH]
                    g_v[n, w0 + HM - SH:w0 + HM, :] = jnp.where(more, g[HM - SH:HM], 0.0)

        def w2_half(hf):
            for n in range(NT):
                w0 = 8 + hf * HM + shift[n // 2]
                z_v[hf * 32:(hf + 1) * 32, tile(n)] = _pk(g_v[n, w0:w0 + HM, :])
            for n in range(NT):
                x1_v[hf * HM:(hf + 1) * HM, tile(n)] = (
                    _dot(_unpk(z_v[hf * 32:(hf + 1) * 32, :]), w2_v[:, tile(n)])
                    + hb_v[hf * HM:(hf + 1) * HM, tile(n)])

        def p1_half(hf):
            for k in range(hf * HM // RC, (hf + 1) * HM // RC):
                x1 = x1_v[k * RC:(k + 1) * RC, :]
                y2_v[k * 8:(k + 1) * 8, :] = _pk(_ln(x1))
                base_v[k * RC:(k + 1) * RC, :] = xa_v[k * RC:(k + 1) * RC, :] + mod(5) * x1

        def w3(f, lo, hi, after=None):
            u_v[lo:hi, tile(f)] = _pk(_gelu(
                _dot(_unpk(_tie(y2_v[lo:hi, :], after)), w3_v[:, tile(f)])))

        w1_half(0)
        w1_half(1)
        w2_half(0)
        w2_half(1)
        p1_half(0)
        for f in range(CFG['nf']):
            w3(f, 0, 32)
        p1_half(1)
        for f in range(CFG['nf']):
            w3(f, 32, 64)
        for n in range(NT):
            g_v[n, 0:8 + SH, :] = g_v[n, BM:BM + 8 + SH, :]
        xa_v[0:SH, :] = xa_v[BM:BM + SH, :]
        hb_v[0:SH, :] = hb_v[BM:BM + SH, :]
        for f in range(CFG['nf'], NF):
            w3(f, 0, 64)
        for n in range(NT):
            y = p0(nxt + n * RC, SH + n * RC)
            y1_v[n * 8:(n + 1) * 8, :] = y
            gb = mod(5, n * 128, (n + 1) * 128)
            u = _unpk(_tie(u_v[...], y, 0, CFG['p0k']))
            a_v[pl.ds(r0, BM), tile(n)] = (
                base_v[:, tile(n)] + gb * _dot(u, w4_v[:, tile(n)])).astype(bf16)
            if n + 1 in CFG['ow'][1:]:
                lo = CFG['ow'][CFG['ow'].index(n + 1) - 1]
                cols = pl.ds(lo * 128, (n + 1 - lo) * 128)
                pltpu.make_async_copy(a_v.at[pl.ds(r0, BM), cols], out_hbm.at[pl.ds(r0, BM), cols],
                                      sem_out).start()
        return c
    lax.fori_loop(0, NB, blk, 0)
    pltpu.make_async_copy(a_v.at[pl.ds(0, S)], out_hbm, sem_out).wait()


@functools.partial(jax.jit, static_argnames=("A_seg_len",))
def pallas_adaLN_cond__memory_aug_recurrent_mem_tr__mixer_s_mlp__prompt_kernel(
    A_x: jax.Array,
    A_mem0: jax.Array,
    A_Wq: jax.Array,
    A_Wk: jax.Array,
    A_Wv: jax.Array,
    A_Wo: jax.Array,
    A_seg_len,
    B_x: jax.Array,
    B_w1: jax.Array,
    B_w2: jax.Array,
    B_w3: jax.Array,
    B_w4: jax.Array,
    c: jax.Array,
    w_mod: jax.Array,
):
    assert A_seg_len == SEG and A_x.shape == (1, S, D) and A_Wq.shape == (D, H, DH)
    any_spec = pl.BlockSpec(memory_space=pl.ANY)
    out = pl.pallas_call(
        _kernel,
        out_shape=jax.ShapeDtypeStruct((S, D), bf16),
        in_specs=[any_spec] * 12,
        out_specs=any_spec,
        scratch_shapes=[
            pltpu.VMEM((1, 3 * D), bf16),
            pltpu.VMEM((S + SH, D), bf16),
            pltpu.VMEM((S + SH, D), bf16),
            pltpu.VMEM((D // KP, PRE // 2, KP), u32),
            pltpu.VMEM((MEM // 2, D), u32),
            pltpu.VMEM((MEM, D), bf16),
            pltpu.VMEM((8, 6 * D), f32),
            pltpu.VMEM((9, 8, MJ), f32),
            pltpu.VMEM((D, 128), f32),
            pltpu.VMEM((8, D), u32),
            pltpu.VMEM((8, D, MJ), bf16),
            pltpu.VMEM((96 * PITCH + 544, 128), u32),
            pltpu.VMEM((H * DH, D + PADL), bf16),
            pltpu.VMEM((D, D + PADL), bf16),
            pltpu.VMEM((D, D + PADL), bf16),
            pltpu.VMEM((D, F + PADL), bf16),
            pltpu.VMEM((F, D + PADL), bf16),
            pltpu.VMEM((NT, BM + 32, 128), f32),
            pltpu.VMEM((BM + SH, D), f32),
            pltpu.VMEM((BM + SH, D), f32),
            pltpu.VMEM((BM, D), f32),
            pltpu.VMEM((BM, D), f32),
            pltpu.VMEM((BM // 2, D), u32),
            pltpu.VMEM((BM // 2, D), u32),
            pltpu.VMEM((BM // 2, D), u32),
            pltpu.VMEM((BM // 2, F), u32),
            pltpu.VMEM((2, D, 16, DH), bf16),
            pltpu.VMEM((PRE, D), f32),
            pltpu.VMEM((NT, HR, 128), u32),
            pltpu.VMEM((H, PRE, DH), f32),
        ] + [pltpu.VMEM((12 * EP, DH), u32)] * 8 + [
            pltpu.SMEM((1,), jnp.int32),
            pltpu.SemaphoreType.DMA((2,)),
            pltpu.SemaphoreType.DMA((4,)),
            pltpu.SemaphoreType.DMA((2, 4)),
            pltpu.SemaphoreType.DMA((2, 4)),
            pltpu.SemaphoreType.DMA((5,)),
            pltpu.SemaphoreType.DMA(()),
        ],
        compiler_params=pltpu.CompilerParams(vmem_limit_bytes=120 * 1024 * 1024),
    )(A_x.reshape(S, D), A_mem0.reshape(MEM, D), A_Wq, A_Wk, A_Wv, A_Wo.reshape(H * DH, D),
      B_w1, B_w2, B_w3, B_w4, c, w_mod)
    return out.reshape(1, S, D)
```

```python
import functools

import jax
import jax.numpy as jnp
from jax import lax
import jax.experimental.pallas as pl
import jax.experimental.pallas.tpu as pltpu

bf16, f32, u32 = jnp.bfloat16, jnp.float32, jnp.uint32

S, D, H, DH, MEM, SEG, F = 2048, 1024, 32, 128, 8, 32, 3584
NSEG = S // SEG
XR = 24
PRE = S - XR * NSEG
RING = 576
QOFF = RING - PRE
EP = RING // 2
PITCH = 520
NT = D // 128
NF = F // 128
BM = 128
NB = S // BM
NPAIR = H // 2
HR = 32 * (NSEG // 2)
PADL = 128
SH = 16
KP = 256
MJ = 512
RC = 16
EPS = 1e-5
LOG2E = 1.4426950408889634
SCALE = DH ** -0.5
CFG = dict(pre=True, step=True, b=True, nlo=6, he=16, orz=1, z0=0, first=0, pa=1, ld=16, mh=28, md=9, mw=512, ds=5, dp=10, dv=0, qk=((0, 0), (1, 0), (0, 1), (1, 1)), ow=(0, 7, 8), nf=7, p0k=16)


def _ln(x):
    m = jnp.mean(x, axis=-1, keepdims=True)
    xc = x - m
    v = jnp.mean(xc * xc, axis=-1, keepdims=True)
    return xc * lax.rsqrt(v + EPS)


def _gelu(x):
    return jax.nn.gelu(x, approximate=True)


def _dot(a, b):
    return jnp.dot(a, b, preferred_element_type=f32)


def _pk(x):
    return pltpu.bitcast(x.astype(bf16), u32)


def _unpk(x):
    return pltpu.bitcast(x, bf16)


def _tie(w, after, r=0, k=0):
    if after is None:
        return w
    m = functools.reduce(lambda a, b: a & b,
                         [after[:, i * 128:(i + 1) * 128] for i in range(after.shape[1] // 128)])
    mf = pltpu.bitcast(m, f32)
    z = jnp.where(mf * mf < 0.0, jnp.uint32(1), jnp.uint32(0))
    row = w[r:r + 8]
    parts = [row[:, :k * 128], row[:, k * 128:(k + 1) * 128] | z, row[:, (k + 1) * 128:]]
    row = jnp.concatenate([p for p in parts if p.shape[1]], axis=1)
    parts = [w[:r], row, w[r + 8:]]
    return jnp.concatenate([p for p in parts if p.shape[0]], axis=0)


def _kernel(x_hbm, mem0_hbm, wq_hbm, wk_hbm, wv_hbm, wo_hbm, w1_hbm, w2_hbm, w3_hbm, w4_hbm,
            c_hbm, wmod_hbm, out_hbm,
            c_v, x_v, a_v, h0_v, mem_v, mem0_v, mod_v, modr_v, cb_v, sc_v, wm_v, w_v, wo_v,
            w1_v, w2_v, w3_v, w4_v,
            g_v, xa_v, hb_v, base_v, x1_v, y1_v, z_v, y2_v, u_v,
            stage, xh_v, hx_v, acc_v,
            r0_, r1_, r2_, r3_, r4_, r5_, r6_, r7_,
            zero_s, sem_x, sem_stage, sem_mod, sem_w, sem_out):
    wqkv_hbm = (wq_hbm, wk_hbm, wv_hbm)
    rings = (r0_, r1_, r2_, r3_, r4_, r5_, r6_, r7_)

    c_cp = pltpu.make_async_copy(c_hbm, c_v.at[:, pl.ds(0, D)], sem_w.at[0])
    mem0_cp = pltpu.make_async_copy(mem0_hbm, mem0_v, sem_w.at[1])

    def x_cp(q):
        rows = pl.ds(q * PRE if isinstance(q, int) else pl.multiple_of(q * PRE, PRE), PRE)
        return pltpu.make_async_copy(x_hbm.at[rows], x_v.at[rows], sem_x.at[q & 1])

    def w_cp(src, dst, k):
        return pltpu.make_async_copy(src, dst.at[:, pl.ds(0, src.shape[1])], sem_w.at[k])

    wo_cp, w1_cp, w2_cp, w3_cp, w4_cp = (
        w_cp(a, b, k) for k, (a, b) in enumerate(
            ((wo_hbm, wo_v), (w1_hbm, w1_v), (w2_hbm, w2_v), (w3_hbm, w3_v), (w4_hbm, w4_v))))

    def mod0_cp(j, k):
        return pltpu.make_async_copy(wmod_hbm.at[:, pl.ds(j * D + k * KP, KP)],
                                     wm_v.at[k, :, pl.ds(j * KP, KP)], sem_mod.at[k])

    def mod1_cp(q):
        col = 2 * D + q * MJ
        col = col if isinstance(q, int) else pl.multiple_of(col, MJ)
        return pltpu.make_async_copy(wmod_hbm.at[:, pl.ds(col, MJ)], wm_v.at[(4 + q) & 7],
                                     sem_mod.at[q & 3])

    def stage_cp(t, hh, piece):
        d0 = piece * KP if isinstance(piece, int) else pl.multiple_of(piece * KP, KP)
        return pltpu.make_async_copy(
            wqkv_hbm[t].at[pl.ds(d0, KP), pl.ds(hh * 16, 16), :],
            stage.at[hh, pl.ds(d0, KP)], sem_stage.at[hh, piece])

    def tile(n):
        return slice(n * 128, (n + 1) * 128)

    def silu_c():
        cf = c_v[:, 0:D].astype(f32)
        return (cf * jax.nn.sigmoid(cf)).astype(bf16)

    def mod(k, lo=0, hi=D):
        return mod_v[0:1, k * D + lo:k * D + hi]

    def repack(hh, ch, p0, n):
        both = None
        for u in range(n):
            p = p0 + u
            a = pltpu.bitcast(stage[hh, 2 * p], u32)
            b = pltpu.bitcast(stage[hh, 2 * p + 1], u32)
            ev = (a & jnp.uint32(0xFFFF)) | (b << 16)
            od = (a >> 16) | (b & jnp.uint32(0xFFFF0000))
            w_v[pl.ds(ch * (16 * PITCH) + p, 8, stride=PITCH), :] = ev
            w_v[pl.ds(ch * (16 * PITCH) + 8 * PITCH + p, 8, stride=PITCH), :] = od
            both = ev & od if both is None else both & ev & od
        return both

    def w_slab(ch, l, lo=0, hi=D):
        base = (ch * 16 + (l % 2) * 8 + l // 2) * PITCH + lo // 2
        return _unpk(w_v[base:base + (hi - lo) // 2, :])

    def ring_of(ch, l):
        return rings[l // 2], (ch * 2 + l % 2) * EP

    c_cp.start()
    mem0_cp.start()
    x_cp(0).start()
    stage_cp(0, 0, 0).start()
    zero_s[0] = 0
    x_v[S:S + SH, :] = jnp.zeros((SH, D), bf16)
    a_v[S:S + SH, :] = jnp.zeros((SH, D), bf16)
    mod_v[:, 0:2 * D] = jnp.zeros((8, 2 * D), f32)
    mod0_cp(0, 0).start()
    mod0_cp(1, 0).start()
    c_cp.wait()
    mem0_cp.wait()
    mem_v[...] = pltpu.bitcast(mem0_v[...], u32)
    cb_v[...] = jnp.transpose(jnp.broadcast_to(silu_c().astype(f32), (128, D)))
    sc_v[...] = _pk(jnp.broadcast_to(silu_c().astype(f32), (16, D)))
    x_cp(0).wait()
    stage_cp(0, 1, 0).start()

    def xhat_body(i, c):
        r0 = pl.multiple_of(i * 64, 64)
        for u in range(4):
            rows = pl.ds(r0 + RC * u, RC)
            xh_v[rows, :] = _ln(x_v[rows, :].astype(f32))
        return c
    lax.fori_loop(0, PRE // 64, xhat_body, 0)

    stage_cp(0, 0, 0).wait()

    def first_repack(i, c):
        repack(0, 0, i * 16, 16)
        return c
    lax.fori_loop(0, KP // 32, first_repack, 0)

    NPC = D // KP
    assert NPC == 4

    def pre_body(i, c):
        t, k = i >> 2, i & 3
        fresh = jnp.logical_and(i > 0, i < 3 * NPC - 1)
        i1 = jnp.where(fresh, i + 1, i)
        t1, k1 = i1 >> 2, i1 & 3

        @pl.when(i < NPC)
        def _():
            for kk in range(NPC):
                @pl.when(i == kk)
                def _():
                    mod0_cp(0, kk).wait()
                    mod0_cp(1, kk).wait()
                    if kk == 1:
                        stage_cp(0, 0, 1).wait()
                    for e in range(KP // 128):
                        m = []
                        for j in range(2):
                            m.append(_dot(_unpk(sc_v[...]), wm_v[kk, :, tile(2 * j + e)])[0:8])
                            col = j * D + kk * KP + e * 128
                            mod_v[:, col:col + 128] = m[j]
                        cols = slice(kk * KP + e * 128, kk * KP + (e + 1) * 128)
                        for q in range(PRE // 64):
                            ca = m[1]
                            if kk == 1:
                                rp = repack(0, 0, KP // 2 + (e * 8 + q) * 8, 8)
                                ca = pltpu.bitcast(_tie(pltpu.bitcast(ca, u32), rp), f32)
                            h0_v[kk, q * 32:(q + 1) * 32, tile(e)] = _pk(
                                xh_v[q * 64:(q + 1) * 64, cols] * (1.0 + ca[0:1]) + m[0][0:1])
                    if kk == 0:
                        stage_cp(0, 0, 1).start()
                    if kk + 1 < NPC:
                        mod0_cp(0, kk + 1).start()
                        mod0_cp(1, kk + 1).start()
                    stage_cp((kk + 1) // NPC, 1, (kk + 1) % NPC).start()
                    stage_cp((kk + 2) // NPC, 0, (kk + 2) % NPC).start()
                    if kk == 1:
                        x_cp(1).start()
                    if kk == 2:
                        mod1_cp(0).start()
                    if kk == 3:
                        stage_cp(1, 1, 1).start()
                        stage_cp(1, 0, 2).start()

        stage_cp(0, 1, k).wait()

        @pl.when(fresh)
        def _():
            stage_cp(0, 0, k1).wait()

        @pl.when(i >= NPC)
        def _():
            mod1_cp(i - NPC).wait()

        @pl.when(jnp.logical_and(i & 1 == 0, jnp.logical_and(i >= 4, i <= 8)))
        def _():
            x_cp((i - 2) >> 1).wait()

        z0 = pl.multiple_of(zero_s[0], 64) if CFG['z0'] else 0
        w0 = pl.multiple_of(t * (32 * PITCH) + k * (KP // 2), 32)
        xrow = jnp.where(i >= NPC, PRE + (i - NPC) * 192, 0)
        hrow = pl.multiple_of(jnp.maximum(i - NPC, 0) * 128, 128)
        done = {}
        nd = 0
        macc = None
        for h in range(H):
            hh, l = h // 16, h % 16
            w = _unpk(w_v[pl.ds(w0 + (hh * 16 + (l % 2) * 8 + l // 2) * PITCH, KP // 2), :])
            q0 = pl.multiple_of(t * (4 * EP), 32) + ring_of(hh, l)[1] + QOFF // 2
            for rb in range(PRE // BM):
                lhs = _tie(h0_v[k, rb * 64:(rb + 1) * 64, :], done.pop(nd, None))
                rows = pl.ds(z0 + rb * BM, BM)
                y = _dot(_unpk(lhs), w) + jnp.where(k > 0, acc_v[h, rows, :], 0.0)
                acc_v[h, rows, :] = y
                rings[l // 2][pl.ds(q0 + rb * 64, 64), :] = _pk(y)
                nd += 1
            if l < 15:
                n = 9 if l < 8 else 8
                p0_ = l * 9 if l < 8 else 72 + (l - 8) * 8
                if hh == 0:
                    repack(1, 2 * t + 1 + zero_s[0], k * (KP // 2) + p0_, n)
                else:
                    repack(0, 2 * t1, k1 * (KP // 2) + p0_, n)
            if h < CFG['mh']:
                g0, g1 = (h * 128) // CFG['mh'], ((h + 1) * 128) // CFG['mh']
                for g in range(g0, g1):
                    cb = cb_v[pl.ds(z0 + g * 8, 8), :]
                    wmg = wm_v[i & 7, g * 8:(g + 1) * 8, :].astype(f32)
                    pr = wmg * jnp.concatenate([cb] * (MJ // 128), axis=1)
                    macc = pr if macc is None else macc + pr
                done[nd + CFG['md']] = pltpu.bitcast(macc[:, 0:CFG['mw']], u32)
                if h == CFG['mh'] - 1:
                    modr_v[jnp.where(i >= NPC, i - NPC, 2 * NPC)] = macc
            if h % 2 == 1 and h < 24:
                q = h // 2
                xs = x_v[pl.ds(pl.multiple_of(xrow + q * RC, RC), RC), :].astype(f32)
                hx = _pk(_ln(xs) * (1.0 + mod(1)) + mod(0))
                done[nd + CFG['ld']] = hx
                for n in range(NT):
                    hx_v[n, pl.ds(hrow + (q // 3) * 32 + (q % 3) * 8, 8), :] = hx[:, tile(n)]
        @pl.when(i == 3)
        def _():
            mod1_cp(1).start()

        @pl.when(jnp.logical_or(i == 4, i == 5))
        def _():
            x_cp(i - 2).start()

        for tt in range(1, 3):
            @pl.when(jnp.logical_and(i >= 3, (i + 3) >> 2 == tt))
            def _():
                stage_cp(tt, 1, (i + 3) & 3).start()

            @pl.when(jnp.logical_and(i >= 3, t + 1 == tt))
            def _():
                stage_cp(tt, 0, k).start()

        @pl.when(jnp.logical_and(i >= 3, i <= 8))
        def _():
            mod1_cp(i - 1).start()

        @pl.when(i == 8)
        def _():
            wo_cp.start()
        return c
    if CFG['pre']:
        lax.fori_loop(0, 3 * NPC, pre_body, 0)

    for cp in (w1_cp, w2_cp, w3_cp, w4_cp):
        cp.start()
    for q in range(2 * NPC):
        mod_v[:, 2 * D + q * MJ:2 * D + (q + 1) * MJ] = jnp.broadcast_to(
            jnp.sum(modr_v[q], axis=0, keepdims=True), (8, MJ))
    wo_cp.wait()

    L2 = 2 * (SEG + MEM)
    r = lax.broadcasted_iota(jnp.int32, (L2, L2), 0)
    c = lax.broadcasted_iota(jnp.int32, (L2, L2), 1)
    r1 = ((r >= SEG) & (r < 2 * SEG)) | (r >= 2 * SEG + MEM)
    c1 = ((c >= SEG) & (c < 2 * SEG)) | (c >= 2 * SEG + MEM)
    same = r1 == c1
    mask = same & ((r >= 2 * SEG) | (c >= 2 * SEG) | (c <= r))
    fill = jnp.where(same, -1e9 / SCALE, -jnp.inf).astype(f32)

    def step(i, mem, zero, left):
        j = 0 if left is None else 1
        woff = pl.multiple_of((XR * i) % EP, 8) + j * (XR // 2)
        roff = pl.multiple_of((SEG * i + QOFF // 2) % EP, SEG) + j * (SEG // 2)
        arow = pl.multiple_of(2 * SEG * i, 2 * SEG) + j * SEG
        hrow = pl.multiple_of(32 * i, 32) + j * (XR // 2)
        acc = [None] * NT
        ym, ps, ol, part, rest = {}, {}, {}, {}, {}
        HK = D // 2
        tiles = [_unpk(jnp.concatenate(
            [(hx_v[k, pl.ds(hrow, XR // 2), :] | zero) if CFG['orz'] else hx_v[k, pl.ds(hrow, XR // 2), :], mem[k]], axis=0))
            for k in range(NT)]
        mem_new = []

        def lhs(lo, hi):
            return jnp.concatenate(tiles[lo // 128:hi // 128], axis=1)

        def qkv_lo(h, t):
            part[(t, h)] = _dot(lhs(0, HK), w_slab(2 * t + h // 16, h % 16, 0, HK))

        def proj(t, h):
            ch, l = 2 * t + h // 16, h % 16
            if (t, h) in part:
                y = _dot(lhs(HK, D), w_slab(ch, l, HK, D)) + part.pop((t, h))
            else:
                y = _dot(lhs(0, D), w_slab(ch, l))
            rg, ix = ring_of(ch, l)
            rg[pl.ds(ix + woff, XR // 2), :] = _pk(y[0:XR])
            ym[(t, h)] = y[XR:XR + MEM]

        def get(t, p):
            rg, i0 = ring_of(2 * t + p // 8, (2 * p) % 16)
            _, i1 = ring_of(2 * t + p // 8, (2 * p) % 16 + 1)
            mm = jnp.concatenate([ym.pop((t, 2 * p)), ym.pop((t, 2 * p + 1))], axis=0)
            return _unpk(jnp.concatenate(
                [rg[pl.ds(i0 + roff, SEG // 2), :], rg[pl.ds(i1 + roff, SEG // 2), :], _pk(mm)],
                axis=0))

        def sm(p):
            sc = lax.dot_general(get(0, p), get(1, p), (((1,), (1,)), ((), ())),
                                 preferred_element_type=f32)
            sc = jnp.where(mask, sc, fill)
            e = jnp.exp2((sc - jnp.max(sc, axis=-1, keepdims=True)) * (SCALE * LOG2E))
            ps[p] = (e * pl.reciprocal(jnp.sum(e, axis=-1, keepdims=True), approx=True)
                     ).astype(bf16)

        def pv(p):
            o = _dot(ps.pop(p), get(2, p))
            for b in range(2):
                h = 2 * p + b
                ox = o[SEG * b:SEG * (b + 1)]
                om = o[2 * SEG + MEM * b:2 * SEG + MEM * (b + 1)]
                if left is None:
                    ol[h] = jnp.concatenate([ox[0:XR], om], axis=0).astype(bf16)
                    rest[h] = ox[XR:SEG]
                else:
                    ol[h] = jnp.concatenate([ox, left[h], om], axis=0).astype(bf16)

        def wo(n, h0, h1):
            for h in range(h0, h1):
                y = _dot(ol[h], wo_v[h * DH:(h + 1) * DH, tile(n)])
                acc[n] = y if acc[n] is None else y + acc[n]
            if h1 == H:
                if left is None:
                    a_v[pl.ds(arow, XR), tile(n)] = acc[n][0:XR].astype(bf16)
                else:
                    a_v[pl.ds(arow, SEG), tile(n)] = acc[n][0:SEG].astype(bf16)
                    a_v[pl.ds(arow - (SEG - XR), SEG - XR), tile(n)] = (
                        acc[n][SEG:2 * SEG - XR].astype(bf16))
                mem_new.append(_pk(acc[n][-MEM:]))

        g = lambda k: CFG.get(k + str(j), CFG[k])
        HE, DS, DP, DV = g('he'), g('ds'), g('dp'), g('dv')
        seq = []
        for p in range(NPAIR + DV):
            if p < NPAIR:
                seq += [(t, 2 * p + b) for t, b in g('qk')]
            if p - DV >= 0:
                seq += [(2, 2 * (p - DV)), (2, 2 * (p - DV) + 1)]
        events = {}
        for p in range(NPAIR):
            at = max(seq.index((t, 2 * p + b)) for t in range(2) for b in range(2)) + DS
            at += g('first') if p == 0 else 0
            events.setdefault(at, []).append((sm, p))
            events.setdefault(at + DP, []).append((pv, p))
        for t, h in seq[:g('nlo')]:
            qkv_lo(h, t)
        WU = HE // 8
        for d in range(len(seq) + NT * WU):
            if d < len(seq):
                proj(*seq[d])
            else:
                u = d - len(seq)
                wo(u // WU, (u % WU) * 8, (u % WU + 1) * 8)
            for fn, p in events.pop(d, []):
                fn(p)
        assert not events
        for n in range(NT):
            wo(n, HE, H)
        return mem_new, rest

    def steps(i, carry):
        zero = zero_s[0].astype(u32)
        mem = [mem_v[:, tile(k)] for k in range(NT)]
        mem, rest = step(i, mem, zero, None)
        mem, _ = step(i, mem, zero, rest)
        for k in range(NT):
            mem_v[:, tile(k)] = mem[k]
        return carry
    if CFG['step']:
        lax.fori_loop(0, NSEG // 2, steps, 0)

    if not CFG['b']:
        cp = pltpu.make_async_copy(a_v.at[pl.ds(0, S)], out_hbm, sem_out)
        cp.start()
        cp.wait()
        return

    for cp in (w1_cp, w2_cp, w3_cp, w4_cp):
        cp.wait()

    def p0(tok, w):
        rows = pl.ds(tok, RC)
        xa = x_v[rows, :].astype(f32) + mod(2) * a_v[rows, :].astype(f32)
        hb = _ln(xa) * (1.0 + mod(4)) + mod(3)
        xa_v[w:w + RC, :] = xa
        hb_v[w:w + RC, :] = hb
        return _pk(_ln(hb))

    y0 = p0(0, 0)
    for k in range(BM // RC):
        y1_v[k * 8:(k + 1) * 8, :] = p0(SH + k * RC, SH + k * RC)
    for n in range(NT):
        g_v[n, 0:8, :] = jnp.zeros((8, 128), f32)
        g_v[n, 8:8 + SH, :] = _gelu(_dot(_unpk(y0), w1_v[:, tile(n)]))

    HM = BM // 2
    shift = (-1, 1, -2, 2)

    def blk(j, c):
        r0 = pl.multiple_of(j * BM, BM)
        nxt = pl.multiple_of(jnp.minimum(j + 1, NB - 1) * BM + SH, SH)
        more = j < NB - 1

        def w1_half(hf):
            for n in range(NT):
                g = _gelu(_dot(_unpk(y1_v[hf * 32:(hf + 1) * 32, :]), w1_v[:, tile(n)]))
                w0 = 8 + SH + hf * HM
                if hf == 0:
                    g_v[n, w0:w0 + HM, :] = g
                else:
                    g_v[n, w0:w0 + HM - SH, :] = g[0:HM - SH]
                    g_v[n, w0 + HM - SH:w0 + HM, :] = jnp.where(more, g[HM - SH:HM], 0.0)

        def w2_half(hf):
            for n in range(NT):
                w0 = 8 + hf * HM + shift[n // 2]
                z_v[hf * 32:(hf + 1) * 32, tile(n)] = _pk(g_v[n, w0:w0 + HM, :])
            for n in range(NT):
                x1_v[hf * HM:(hf + 1) * HM, tile(n)] = (
                    _dot(_unpk(z_v[hf * 32:(hf + 1) * 32, :]), w2_v[:, tile(n)])
                    + hb_v[hf * HM:(hf + 1) * HM, tile(n)])

        def p1_half(hf):
            for k in range(hf * HM // RC, (hf + 1) * HM // RC):
                x1 = x1_v[k * RC:(k + 1) * RC, :]
                y2_v[k * 8:(k + 1) * 8, :] = _pk(_ln(x1))
                base_v[k * RC:(k + 1) * RC, :] = xa_v[k * RC:(k + 1) * RC, :] + mod(5) * x1

        def w3(f, lo, hi, after=None):
            u_v[lo:hi, tile(f)] = _pk(_gelu(
                _dot(_unpk(_tie(y2_v[lo:hi, :], after)), w3_v[:, tile(f)])))

        w1_half(0)
        w1_half(1)
        w2_half(0)
        w2_half(1)
        p1_half(0)
        for f in range(CFG['nf']):
            w3(f, 0, 32)
        p1_half(1)
        for f in range(CFG['nf']):
            w3(f, 32, 64)
        for n in range(NT):
            g_v[n, 0:8 + SH, :] = g_v[n, BM:BM + 8 + SH, :]
        xa_v[0:SH, :] = xa_v[BM:BM + SH, :]
        hb_v[0:SH, :] = hb_v[BM:BM + SH, :]
        for f in range(CFG['nf'], NF):
            w3(f, 0, 64)
        ys = {}

        def prep(k):
            if k < BM // RC:
                ys[k] = p0(nxt + k * RC, SH + k * RC)
                y1_v[k * 8:(k + 1) * 8, :] = ys[k]

        for k in range(CFG['pa']):
            prep(k)
        for n in range(NT):
            prep(n + CFG['pa'])
            gb = mod(5, n * 128, (n + 1) * 128)
            u = _unpk(_tie(u_v[...], ys.pop(n), 0, CFG['p0k']))
            a_v[pl.ds(r0, BM), tile(n)] = (
                base_v[:, tile(n)] + gb * _dot(u, w4_v[:, tile(n)])).astype(bf16)
            if n + 1 in CFG['ow'][1:]:
                lo = CFG['ow'][CFG['ow'].index(n + 1) - 1]
                cols = pl.ds(lo * 128, (n + 1 - lo) * 128)
                pltpu.make_async_copy(a_v.at[pl.ds(r0, BM), cols], out_hbm.at[pl.ds(r0, BM), cols],
                                      sem_out).start()
        return c
    lax.fori_loop(0, NB, blk, 0)
    pltpu.make_async_copy(a_v.at[pl.ds(0, S)], out_hbm, sem_out).wait()


@functools.partial(jax.jit, static_argnames=("A_seg_len",))
def pallas_adaLN_cond__memory_aug_recurrent_mem_tr__mixer_s_mlp__prompt_kernel(
    A_x: jax.Array,
    A_mem0: jax.Array,
    A_Wq: jax.Array,
    A_Wk: jax.Array,
    A_Wv: jax.Array,
    A_Wo: jax.Array,
    A_seg_len,
    B_x: jax.Array,
    B_w1: jax.Array,
    B_w2: jax.Array,
    B_w3: jax.Array,
    B_w4: jax.Array,
    c: jax.Array,
    w_mod: jax.Array,
):
    assert A_seg_len == SEG and A_x.shape == (1, S, D) and A_Wq.shape == (D, H, DH)
    any_spec = pl.BlockSpec(memory_space=pl.ANY)
    out = pl.pallas_call(
        _kernel,
        out_shape=jax.ShapeDtypeStruct((S, D), bf16),
        in_specs=[any_spec] * 12,
        out_specs=any_spec,
        scratch_shapes=[
            pltpu.VMEM((1, 3 * D), bf16),
            pltpu.VMEM((S + SH, D), bf16),
            pltpu.VMEM((S + SH, D), bf16),
            pltpu.VMEM((D // KP, PRE // 2, KP), u32),
            pltpu.VMEM((MEM // 2, D), u32),
            pltpu.VMEM((MEM, D), bf16),
            pltpu.VMEM((8, 6 * D), f32),
            pltpu.VMEM((9, 8, MJ), f32),
            pltpu.VMEM((D, 128), f32),
            pltpu.VMEM((8, D), u32),
            pltpu.VMEM((8, D, MJ), bf16),
            pltpu.VMEM((96 * PITCH + 544, 128), u32),
            pltpu.VMEM((H * DH, D + PADL), bf16),
            pltpu.VMEM((D, D + PADL), bf16),
            pltpu.VMEM((D, D + PADL), bf16),
            pltpu.VMEM((D, F + PADL), bf16),
            pltpu.VMEM((F, D + PADL), bf16),
            pltpu.VMEM((NT, BM + 32, 128), f32),
            pltpu.VMEM((BM + SH, D), f32),
            pltpu.VMEM((BM + SH, D), f32),
            pltpu.VMEM((BM, D), f32),
            pltpu.VMEM((BM, D), f32),
            pltpu.VMEM((BM // 2, D), u32),
            pltpu.VMEM((BM // 2, D), u32),
            pltpu.VMEM((BM // 2, D), u32),
            pltpu.VMEM((BM // 2, F), u32),
            pltpu.VMEM((2, D, 16, DH), bf16),
            pltpu.VMEM((PRE, D), f32),
            pltpu.VMEM((NT, HR, 128), u32),
            pltpu.VMEM((H, PRE, DH), f32),
        ] + [pltpu.VMEM((12 * EP, DH), u32)] * 8 + [
            pltpu.SMEM((1,), jnp.int32),
            pltpu.SemaphoreType.DMA((2,)),
            pltpu.SemaphoreType.DMA((2, 4)),
            pltpu.SemaphoreType.DMA((4,)),
            pltpu.SemaphoreType.DMA((5,)),
            pltpu.SemaphoreType.DMA(()),
        ],
        compiler_params=pltpu.CompilerParams(vmem_limit_bytes=120 * 1024 * 1024),
    )(A_x.reshape(S, D), A_mem0.reshape(MEM, D), A_Wq, A_Wk, A_Wv, A_Wo.reshape(H * DH, D),
      B_w1, B_w2, B_w3, B_w4, c, w_mod)
    return out.reshape(1, S, D)
```

```python
import functools

import jax
import jax.numpy as jnp
from jax import lax
import jax.experimental.pallas as pl
import jax.experimental.pallas.tpu as pltpu

bf16, f32, u32 = jnp.bfloat16, jnp.float32, jnp.uint32

S, D, H, DH, MEM, SEG, F = 2048, 1024, 32, 128, 8, 32, 3584
NSEG = S // SEG
XR = 24
PRE = S - XR * NSEG
RING = 576
QOFF = RING - PRE
EP = RING // 2
PITCH = 520
NT = D // 128
NF = F // 128
BM = 128
NB = S // BM
NPAIR = H // 2
HR = 32 * (NSEG // 2)
PADL = 128
SH = 16
KP = 256
MJ = 512
RC = 16
EPS = 1e-5
LOG2E = 1.4426950408889634
SCALE = DH ** -0.5
CFG = dict(pre=True, step=True, b=True, nlo=6, he=16, orz=1, z0=0, first=0, hp=1, hn=4, pa=1, ld=16, mh=28, md=9, mw=512, ds=5, dp=10, dv=0, qk=((0, 0), (1, 0), (0, 1), (1, 1)), ow=(0, 7, 8), nf=7, p0k=16)


def _ln(x):
    m = jnp.mean(x, axis=-1, keepdims=True)
    xc = x - m
    v = jnp.mean(xc * xc, axis=-1, keepdims=True)
    return xc * lax.rsqrt(v + EPS)


def _gelu(x):
    return jax.nn.gelu(x, approximate=True)


def _dot(a, b):
    return jnp.dot(a, b, preferred_element_type=f32)


def _pk(x):
    return pltpu.bitcast(x.astype(bf16), u32)


def _unpk(x):
    return pltpu.bitcast(x, bf16)


def _tie(w, after, r=0, k=0):
    if after is None:
        return w
    m = functools.reduce(lambda a, b: a & b,
                         [after[:, i * 128:(i + 1) * 128] for i in range(after.shape[1] // 128)])
    mf = pltpu.bitcast(m, f32)
    z = jnp.where(mf * mf < 0.0, jnp.uint32(1), jnp.uint32(0))
    row = w[r:r + 8]
    parts = [row[:, :k * 128], row[:, k * 128:(k + 1) * 128] | z, row[:, (k + 1) * 128:]]
    row = jnp.concatenate([p for p in parts if p.shape[1]], axis=1)
    parts = [w[:r], row, w[r + 8:]]
    return jnp.concatenate([p for p in parts if p.shape[0]], axis=0)


def _kernel(x_hbm, mem0_hbm, wq_hbm, wk_hbm, wv_hbm, wo_hbm, w1_hbm, w2_hbm, w3_hbm, w4_hbm,
            c_hbm, wmod_hbm, out_hbm,
            c_v, x_v, a_v, h0_v, mem_v, mem0_v, mod_v, modr_v, cb_v, sc_v, wm_v, w_v, wo_v,
            w1_v, w2_v, w3_v, w4_v,
            g_v, xa_v, hb_v, base_v, x1_v, y1_v, z_v, y2_v, u_v,
            stage, xh_v, hx_v, acc_v,
            r0_, r1_, r2_, r3_, r4_, r5_, r6_, r7_,
            zero_s, sem_x, sem_stage, sem_mod, sem_w, sem_out):
    wqkv_hbm = (wq_hbm, wk_hbm, wv_hbm)
    rings = (r0_, r1_, r2_, r3_, r4_, r5_, r6_, r7_)

    c_cp = pltpu.make_async_copy(c_hbm, c_v.at[:, pl.ds(0, D)], sem_w.at[0])
    mem0_cp = pltpu.make_async_copy(mem0_hbm, mem0_v, sem_w.at[1])

    def x_cp(q):
        rows = pl.ds(q * PRE if isinstance(q, int) else pl.multiple_of(q * PRE, PRE), PRE)
        return pltpu.make_async_copy(x_hbm.at[rows], x_v.at[rows], sem_x.at[q & 1])

    def w_cp(src, dst, k):
        return pltpu.make_async_copy(src, dst.at[:, pl.ds(0, src.shape[1])], sem_w.at[k])

    wo_cp, w1_cp, w2_cp, w3_cp, w4_cp = (
        w_cp(a, b, k) for k, (a, b) in enumerate(
            ((wo_hbm, wo_v), (w1_hbm, w1_v), (w2_hbm, w2_v), (w3_hbm, w3_v), (w4_hbm, w4_v))))

    def mod0_cp(j, k):
        return pltpu.make_async_copy(wmod_hbm.at[:, pl.ds(j * D + k * KP, KP)],
                                     wm_v.at[k, :, pl.ds(j * KP, KP)], sem_mod.at[k])

    def mod1_cp(q):
        col = 2 * D + q * MJ
        col = col if isinstance(q, int) else pl.multiple_of(col, MJ)
        return pltpu.make_async_copy(wmod_hbm.at[:, pl.ds(col, MJ)], wm_v.at[(4 + q) & 7],
                                     sem_mod.at[q & 3])

    def stage_cp(t, hh, piece):
        d0 = piece * KP if isinstance(piece, int) else pl.multiple_of(piece * KP, KP)
        return pltpu.make_async_copy(
            wqkv_hbm[t].at[pl.ds(d0, KP), pl.ds(hh * 16, 16), :],
            stage.at[hh, pl.ds(d0, KP)], sem_stage.at[hh, piece])

    def tile(n):
        return slice(n * 128, (n + 1) * 128)

    def silu_c():
        cf = c_v[:, 0:D].astype(f32)
        return (cf * jax.nn.sigmoid(cf)).astype(bf16)

    def mod(k, lo=0, hi=D):
        return mod_v[0:1, k * D + lo:k * D + hi]

    def repack(hh, ch, p0, n):
        both = None
        for u in range(n):
            p = p0 + u
            a = pltpu.bitcast(stage[hh, 2 * p], u32)
            b = pltpu.bitcast(stage[hh, 2 * p + 1], u32)
            ev = (a & jnp.uint32(0xFFFF)) | (b << 16)
            od = (a >> 16) | (b & jnp.uint32(0xFFFF0000))
            w_v[pl.ds(ch * (16 * PITCH) + p, 8, stride=PITCH), :] = ev
            w_v[pl.ds(ch * (16 * PITCH) + 8 * PITCH + p, 8, stride=PITCH), :] = od
            both = ev & od if both is None else both & ev & od
        return both

    def w_slab(ch, l, lo=0, hi=D):
        base = (ch * 16 + (l % 2) * 8 + l // 2) * PITCH + lo // 2
        return _unpk(w_v[base:base + (hi - lo) // 2, :])

    def ring_of(ch, l):
        return rings[l // 2], (ch * 2 + l % 2) * EP

    c_cp.start()
    mem0_cp.start()
    x_cp(0).start()
    stage_cp(0, 0, 0).start()
    zero_s[0] = 0
    x_v[S:S + SH, :] = jnp.zeros((SH, D), bf16)
    a_v[S:S + SH, :] = jnp.zeros((SH, D), bf16)
    mod_v[:, 0:2 * D] = jnp.zeros((8, 2 * D), f32)
    mod0_cp(0, 0).start()
    mod0_cp(1, 0).start()
    c_cp.wait()
    mem0_cp.wait()
    mem_v[...] = pltpu.bitcast(mem0_v[...], u32)
    cb_v[...] = jnp.transpose(jnp.broadcast_to(silu_c().astype(f32), (128, D)))
    sc_v[...] = _pk(jnp.broadcast_to(silu_c().astype(f32), (16, D)))
    x_cp(0).wait()
    stage_cp(0, 1, 0).start()

    def xhat_body(i, c):
        r0 = pl.multiple_of(i * 64, 64)
        for u in range(4):
            rows = pl.ds(r0 + RC * u, RC)
            xh_v[rows, :] = _ln(x_v[rows, :].astype(f32))
        return c
    lax.fori_loop(0, PRE // 64, xhat_body, 0)

    stage_cp(0, 0, 0).wait()

    def first_repack(i, c):
        repack(0, 0, i * 16, 16)
        return c
    lax.fori_loop(0, KP // 32, first_repack, 0)

    NPC = D // KP
    assert NPC == 4

    def pre_body(i, c):
        t, k = i >> 2, i & 3
        fresh = jnp.logical_and(i > 0, i < 3 * NPC - 1)
        i1 = jnp.where(fresh, i + 1, i)
        t1, k1 = i1 >> 2, i1 & 3

        @pl.when(i < NPC)
        def _():
            for kk in range(NPC):
                @pl.when(i == kk)
                def _():
                    mod0_cp(0, kk).wait()
                    mod0_cp(1, kk).wait()
                    if kk == 1:
                        stage_cp(0, 0, 1).wait()
                    for e in range(KP // 128):
                        m = []
                        for j in range(2):
                            m.append(_dot(_unpk(sc_v[...]), wm_v[kk, :, tile(2 * j + e)])[0:8])
                            col = j * D + kk * KP + e * 128
                            mod_v[:, col:col + 128] = m[j]
                        cols = slice(kk * KP + e * 128, kk * KP + (e + 1) * 128)
                        for q in range(PRE // 64):
                            ca = m[1]
                            if kk == 1:
                                rp = repack(0, 0, KP // 2 + (e * 8 + q) * 8, 8)
                                ca = pltpu.bitcast(_tie(pltpu.bitcast(ca, u32), rp), f32)
                            h0_v[kk, q * 32:(q + 1) * 32, tile(e)] = _pk(
                                xh_v[q * 64:(q + 1) * 64, cols] * (1.0 + ca[0:1]) + m[0][0:1])
                    if kk == 0:
                        stage_cp(0, 0, 1).start()
                    if kk + 1 < NPC:
                        mod0_cp(0, kk + 1).start()
                        mod0_cp(1, kk + 1).start()
                    stage_cp((kk + 1) // NPC, 1, (kk + 1) % NPC).start()
                    stage_cp((kk + 2) // NPC, 0, (kk + 2) % NPC).start()
                    if kk == 1:
                        x_cp(1).start()
                    if kk == 2:
                        mod1_cp(0).start()
                    if kk == 3:
                        stage_cp(1, 1, 1).start()
                        stage_cp(1, 0, 2).start()

        stage_cp(0, 1, k).wait()

        @pl.when(fresh)
        def _():
            stage_cp(0, 0, k1).wait()

        @pl.when(i >= NPC)
        def _():
            mod1_cp(i - NPC).wait()

        @pl.when(jnp.logical_and(i & 1 == 0, jnp.logical_and(i >= 4, i <= 8)))
        def _():
            x_cp((i - 2) >> 1).wait()

        z0 = pl.multiple_of(zero_s[0], 64) if CFG['z0'] else 0
        w0 = pl.multiple_of(t * (32 * PITCH) + k * (KP // 2), 32)
        xrow = jnp.where(i >= NPC, PRE + (i - NPC) * 192, 0)
        hrow = pl.multiple_of(jnp.maximum(i - NPC, 0) * 128, 128)
        done = {}
        nd = 0
        macc = None
        for h in range(H):
            hh, l = h // 16, h % 16
            w = _unpk(w_v[pl.ds(w0 + (hh * 16 + (l % 2) * 8 + l // 2) * PITCH, KP // 2), :])
            q0 = pl.multiple_of(t * (4 * EP), 32) + ring_of(hh, l)[1] + QOFF // 2
            for rb in range(PRE // BM):
                lhs = _tie(h0_v[k, rb * 64:(rb + 1) * 64, :], done.pop(nd, None))
                rows = pl.ds(z0 + rb * BM, BM)
                y = _dot(_unpk(lhs), w) + jnp.where(k > 0, acc_v[h, rows, :], 0.0)
                acc_v[h, rows, :] = y
                rings[l // 2][pl.ds(q0 + rb * 64, 64), :] = _pk(y)
                nd += 1
            if l < 15:
                n = 9 if l < 8 else 8
                p0_ = l * 9 if l < 8 else 72 + (l - 8) * 8
                if hh == 0:
                    repack(1, 2 * t + 1 + zero_s[0], k * (KP // 2) + p0_, n)
                else:
                    repack(0, 2 * t1, k1 * (KP // 2) + p0_, n)
            if h < CFG['mh']:
                g0, g1 = (h * 128) // CFG['mh'], ((h + 1) * 128) // CFG['mh']
                for g in range(g0, g1):
                    cb = cb_v[pl.ds(z0 + g * 8, 8), :]
                    wmg = wm_v[i & 7, g * 8:(g + 1) * 8, :].astype(f32)
                    pr = wmg * jnp.concatenate([cb] * (MJ // 128), axis=1)
                    macc = pr if macc is None else macc + pr
                done[nd + CFG['md']] = pltpu.bitcast(macc[:, 0:CFG['mw']], u32)
                if h == CFG['mh'] - 1:
                    modr_v[jnp.where(i >= NPC, i - NPC, 2 * NPC)] = macc
            if h % 2 == 1 and h < 24:
                q = h // 2
                xs = x_v[pl.ds(pl.multiple_of(xrow + q * RC, RC), RC), :].astype(f32)
                hx = _pk(_ln(xs) * (1.0 + mod(1)) + mod(0))
                done[nd + CFG['ld']] = hx
                for n in range(NT):
                    hx_v[n, pl.ds(hrow + (q // 3) * 32 + (q % 3) * 8, 8), :] = hx[:, tile(n)]
        @pl.when(i == 3)
        def _():
            mod1_cp(1).start()

        @pl.when(jnp.logical_or(i == 4, i == 5))
        def _():
            x_cp(i - 2).start()

        for tt in range(1, 3):
            @pl.when(jnp.logical_and(i >= 3, (i + 3) >> 2 == tt))
            def _():
                stage_cp(tt, 1, (i + 3) & 3).start()

            @pl.when(jnp.logical_and(i >= 3, t + 1 == tt))
            def _():
                stage_cp(tt, 0, k).start()

        @pl.when(jnp.logical_and(i >= 3, i <= 8))
        def _():
            mod1_cp(i - 1).start()

        @pl.when(i == 8)
        def _():
            wo_cp.start()
        return c
    if CFG['pre']:
        lax.fori_loop(0, 3 * NPC, pre_body, 0)

    for cp in (w1_cp, w2_cp, w3_cp, w4_cp):
        cp.start()
    for q in range(2 * NPC):
        mod_v[:, 2 * D + q * MJ:2 * D + (q + 1) * MJ] = jnp.broadcast_to(
            jnp.sum(modr_v[q], axis=0, keepdims=True), (8, MJ))
    wo_cp.wait()

    L2 = 2 * (SEG + MEM)
    r = lax.broadcasted_iota(jnp.int32, (L2, L2), 0)
    c = lax.broadcasted_iota(jnp.int32, (L2, L2), 1)
    r1 = ((r >= SEG) & (r < 2 * SEG)) | (r >= 2 * SEG + MEM)
    c1 = ((c >= SEG) & (c < 2 * SEG)) | (c >= 2 * SEG + MEM)
    same = r1 == c1
    mask = same & ((r >= 2 * SEG) | (c >= 2 * SEG) | (c <= r))
    fill = jnp.where(same, -1e9 / SCALE, -jnp.inf).astype(f32)

    def p0(tok, w):
        rows = pl.ds(tok, RC)
        xa = x_v[rows, :].astype(f32) + mod(2) * a_v[rows, :].astype(f32)
        hb = _ln(xa) * (1.0 + mod(4)) + mod(3)
        xa_v[pl.ds(w, RC), :] = xa
        hb_v[pl.ds(w, RC), :] = hb
        y = _pk(_ln(hb))
        y1_v[pl.ds(w // 2 if isinstance(w, int) else pl.multiple_of(w >> 1, 8), RC // 2), :] = y
        return y

    def step(i, mem, zero, left):
        j = 0 if left is None else 1
        woff = pl.multiple_of((XR * i) % EP, 8) + j * (XR // 2)
        roff = pl.multiple_of((SEG * i + QOFF // 2) % EP, SEG) + j * (SEG // 2)
        arow = pl.multiple_of(2 * SEG * i, 2 * SEG) + j * SEG
        hrow = pl.multiple_of(32 * i, 32) + j * (XR // 2)
        acc = [None] * NT
        ym, ps, ol, part, rest = {}, {}, {}, {}, {}
        HK = D // 2
        tiles = [_unpk(jnp.concatenate(
            [(hx_v[k, pl.ds(hrow, XR // 2), :] | zero) if CFG['orz'] else hx_v[k, pl.ds(hrow, XR // 2), :], mem[k]], axis=0))
            for k in range(NT)]
        mem_new = []

        def lhs(lo, hi):
            return jnp.concatenate(tiles[lo // 128:hi // 128], axis=1)

        def qkv_lo(h, t):
            part[(t, h)] = _dot(lhs(0, HK), w_slab(2 * t + h // 16, h % 16, 0, HK))

        def proj(t, h):
            ch, l = 2 * t + h // 16, h % 16
            if (t, h) in part:
                y = _dot(lhs(HK, D), w_slab(ch, l, HK, D)) + part.pop((t, h))
            else:
                y = _dot(lhs(0, D), w_slab(ch, l))
            rg, ix = ring_of(ch, l)
            rg[pl.ds(ix + woff, XR // 2), :] = _pk(y[0:XR])
            ym[(t, h)] = y[XR:XR + MEM]

        def get(t, p):
            rg, i0 = ring_of(2 * t + p // 8, (2 * p) % 16)
            _, i1 = ring_of(2 * t + p // 8, (2 * p) % 16 + 1)
            mm = jnp.concatenate([ym.pop((t, 2 * p)), ym.pop((t, 2 * p + 1))], axis=0)
            return _unpk(jnp.concatenate(
                [rg[pl.ds(i0 + roff, SEG // 2), :], rg[pl.ds(i1 + roff, SEG // 2), :], _pk(mm)],
                axis=0))

        def sm(p):
            sc = lax.dot_general(get(0, p), get(1, p), (((1,), (1,)), ((), ())),
                                 preferred_element_type=f32)
            sc = jnp.where(mask, sc, fill)
            e = jnp.exp2((sc - jnp.max(sc, axis=-1, keepdims=True)) * (SCALE * LOG2E))
            ps[p] = (e * pl.reciprocal(jnp.sum(e, axis=-1, keepdims=True), approx=True)
                     ).astype(bf16)

        def pv(p):
            o = _dot(ps.pop(p), get(2, p))
            for b in range(2):
                h = 2 * p + b
                ox = o[SEG * b:SEG * (b + 1)]
                om = o[2 * SEG + MEM * b:2 * SEG + MEM * (b + 1)]
                if left is None:
                    ol[h] = jnp.concatenate([ox[0:XR], om], axis=0).astype(bf16)
                    rest[h] = ox[XR:SEG]
                else:
                    ol[h] = jnp.concatenate([ox, left[h], om], axis=0).astype(bf16)

        def wo(n, h0, h1, after=None):
            for h in range(h0, h1):
                o = ol[h]
                if after is not None and h == h0:
                    o = _unpk(_tie(pltpu.bitcast(o, u32), after))
                y = _dot(o, wo_v[h * DH:(h + 1) * DH, tile(n)])
                acc[n] = y if acc[n] is None else y + acc[n]
            if h1 == H:
                if left is None:
                    a_v[pl.ds(arow, XR), tile(n)] = acc[n][0:XR].astype(bf16)
                else:
                    a_v[pl.ds(arow, SEG), tile(n)] = acc[n][0:SEG].astype(bf16)
                    a_v[pl.ds(arow - (SEG - XR), SEG - XR), tile(n)] = (
                        acc[n][SEG:2 * SEG - XR].astype(bf16))
                mem_new.append(_pk(acc[n][-MEM:]))

        g = lambda k: CFG.get(k + str(j), CFG[k])
        HE, DS, DP, DV = g('he'), g('ds'), g('dp'), g('dv')
        seq = []
        for p in range(NPAIR + DV):
            if p < NPAIR:
                seq += [(t, 2 * p + b) for t, b in g('qk')]
            if p - DV >= 0:
                seq += [(2, 2 * (p - DV)), (2, 2 * (p - DV) + 1)]
        events = {}
        for p in range(NPAIR):
            at = max(seq.index((t, 2 * p + b)) for t in range(2) for b in range(2)) + DS
            at += g('first') if p == 0 else 0
            events.setdefault(at, []).append((sm, p))
            events.setdefault(at + DP, []).append((pv, p))
        for t, h in seq[:g('nlo')]:
            qkv_lo(h, t)
        WU = HE // 8
        for d in range(len(seq) + NT * WU):
            if d < len(seq):
                proj(*seq[d])
            else:
                u = d - len(seq)
                wo(u // WU, (u % WU) * 8, (u % WU + 1) * 8)
            for fn, p in events.pop(d, []):
                fn(p)
        assert not events
        side = None
        if j == 1 and CFG['hp']:
            tok = pl.multiple_of(jnp.clip(i - 22, 0, BM // RC) * RC, RC)
            side = p0(tok, tok)
        for n in range(NT):
            wo(n, HE, H, side if n == CFG['hn'] else None)
        return mem_new, rest

    def steps(i, carry):
        zero = zero_s[0].astype(u32)
        mem = [mem_v[:, tile(k)] for k in range(NT)]
        mem, rest = step(i, mem, zero, None)
        mem, _ = step(i, mem, zero, rest)
        for k in range(NT):
            mem_v[:, tile(k)] = mem[k]
        return carry
    if CFG['step']:
        lax.fori_loop(0, NSEG // 2, steps, 0)

    if not CFG['b']:
        cp = pltpu.make_async_copy(a_v.at[pl.ds(0, S)], out_hbm, sem_out)
        cp.start()
        cp.wait()
        return

    for cp in (w1_cp, w2_cp, w3_cp, w4_cp):
        cp.wait()

    if not CFG['hp']:
        for k in range(BM // RC + 1):
            p0(k * RC, k * RC)
    for n in range(NT):
        g_v[n, 0:8, :] = jnp.zeros((8, 128), f32)
        g_v[n, 8:8 + SH, :] = _gelu(_dot(_unpk(y1_v[0:SH // 2, :]), w1_v[:, tile(n)]))

    HM = BM // 2
    shift = (-1, 1, -2, 2)

    def blk(j, c):
        r0 = pl.multiple_of(j * BM, BM)
        nxt = pl.multiple_of(jnp.minimum(j + 1, NB - 1) * BM + SH, SH)
        more = j < NB - 1

        def w1_half(hf):
            for n in range(NT):
                g = _gelu(_dot(_unpk(y1_v[8 + hf * 32:8 + (hf + 1) * 32, :]), w1_v[:, tile(n)]))
                w0 = 8 + SH + hf * HM
                if hf == 0:
                    g_v[n, w0:w0 + HM, :] = g
                else:
                    g_v[n, w0:w0 + HM - SH, :] = g[0:HM - SH]
                    g_v[n, w0 + HM - SH:w0 + HM, :] = jnp.where(more, g[HM - SH:HM], 0.0)

        def w2_half(hf):
            for n in range(NT):
                w0 = 8 + hf * HM + shift[n // 2]
                z_v[hf * 32:(hf + 1) * 32, tile(n)] = _pk(g_v[n, w0:w0 + HM, :])
            for n in range(NT):
                x1_v[hf * HM:(hf + 1) * HM, tile(n)] = (
                    _dot(_unpk(z_v[hf * 32:(hf + 1) * 32, :]), w2_v[:, tile(n)])
                    + hb_v[hf * HM:(hf + 1) * HM, tile(n)])

        def p1_half(hf):
            for k in range(hf * HM // RC, (hf + 1) * HM // RC):
                x1 = x1_v[k * RC:(k + 1) * RC, :]
                y2_v[k * 8:(k + 1) * 8, :] = _pk(_ln(x1))
                base_v[k * RC:(k + 1) * RC, :] = xa_v[k * RC:(k + 1) * RC, :] + mod(5) * x1

        def w3(f, lo, hi, after=None):
            u_v[lo:hi, tile(f)] = _pk(_gelu(
                _dot(_unpk(_tie(y2_v[lo:hi, :], after)), w3_v[:, tile(f)])))

        w1_half(0)
        w1_half(1)
        w2_half(0)
        w2_half(1)
        p1_half(0)
        for f in range(CFG['nf']):
            w3(f, 0, 32)
        p1_half(1)
        for f in range(CFG['nf']):
            w3(f, 32, 64)
        for n in range(NT):
            g_v[n, 0:8 + SH, :] = g_v[n, BM:BM + 8 + SH, :]
        xa_v[0:SH, :] = xa_v[BM:BM + SH, :]
        hb_v[0:SH, :] = hb_v[BM:BM + SH, :]
        for f in range(CFG['nf'], NF):
            w3(f, 0, 64)
        ys = {}

        def prep(k):
            if k < BM // RC:
                ys[k] = p0(nxt + k * RC, SH + k * RC)

        for k in range(CFG['pa']):
            prep(k)
        for n in range(NT):
            prep(n + CFG['pa'])
            gb = mod(5, n * 128, (n + 1) * 128)
            u = _unpk(_tie(u_v[...], ys.pop(n), 0, CFG['p0k']))
            a_v[pl.ds(r0, BM), tile(n)] = (
                base_v[:, tile(n)] + gb * _dot(u, w4_v[:, tile(n)])).astype(bf16)
            if n + 1 in CFG['ow'][1:]:
                lo = CFG['ow'][CFG['ow'].index(n + 1) - 1]
                cols = pl.ds(lo * 128, (n + 1 - lo) * 128)
                pltpu.make_async_copy(a_v.at[pl.ds(r0, BM), cols], out_hbm.at[pl.ds(r0, BM), cols],
                                      sem_out).start()
        return c
    lax.fori_loop(0, NB, blk, 0)
    pltpu.make_async_copy(a_v.at[pl.ds(0, S)], out_hbm, sem_out).wait()


@functools.partial(jax.jit, static_argnames=("A_seg_len",))
def pallas_adaLN_cond__memory_aug_recurrent_mem_tr__mixer_s_mlp__prompt_kernel(
    A_x: jax.Array,
    A_mem0: jax.Array,
    A_Wq: jax.Array,
    A_Wk: jax.Array,
    A_Wv: jax.Array,
    A_Wo: jax.Array,
    A_seg_len,
    B_x: jax.Array,
    B_w1: jax.Array,
    B_w2: jax.Array,
    B_w3: jax.Array,
    B_w4: jax.Array,
    c: jax.Array,
    w_mod: jax.Array,
):
    assert A_seg_len == SEG and A_x.shape == (1, S, D) and A_Wq.shape == (D, H, DH)
    any_spec = pl.BlockSpec(memory_space=pl.ANY)
    out = pl.pallas_call(
        _kernel,
        out_shape=jax.ShapeDtypeStruct((S, D), bf16),
        in_specs=[any_spec] * 12,
        out_specs=any_spec,
        scratch_shapes=[
            pltpu.VMEM((1, 3 * D), bf16),
            pltpu.VMEM((S + SH, D), bf16),
            pltpu.VMEM((S + SH, D), bf16),
            pltpu.VMEM((D // KP, PRE // 2, KP), u32),
            pltpu.VMEM((MEM // 2, D), u32),
            pltpu.VMEM((MEM, D), bf16),
            pltpu.VMEM((8, 6 * D), f32),
            pltpu.VMEM((9, 8, MJ), f32),
            pltpu.VMEM((D, 128), f32),
            pltpu.VMEM((8, D), u32),
            pltpu.VMEM((8, D, MJ), bf16),
            pltpu.VMEM((96 * PITCH + 544, 128), u32),
            pltpu.VMEM((H * DH, D + PADL), bf16),
            pltpu.VMEM((D, D + PADL), bf16),
            pltpu.VMEM((D, D + PADL), bf16),
            pltpu.VMEM((D, F + PADL), bf16),
            pltpu.VMEM((F, D + PADL), bf16),
            pltpu.VMEM((NT, BM + 32, 128), f32),
            pltpu.VMEM((BM + SH, D), f32),
            pltpu.VMEM((BM + SH, D), f32),
            pltpu.VMEM((BM, D), f32),
            pltpu.VMEM((BM, D), f32),
            pltpu.VMEM(((BM + SH) // 2, D), u32),
            pltpu.VMEM((BM // 2, D), u32),
            pltpu.VMEM((BM // 2, D), u32),
            pltpu.VMEM((BM // 2, F), u32),
            pltpu.VMEM((2, D, 16, DH), bf16),
            pltpu.VMEM((PRE, D), f32),
            pltpu.VMEM((NT, HR, 128), u32),
            pltpu.VMEM((H, PRE, DH), f32),
        ] + [pltpu.VMEM((12 * EP, DH), u32)] * 8 + [
            pltpu.SMEM((1,), jnp.int32),
            pltpu.SemaphoreType.DMA((2,)),
            pltpu.SemaphoreType.DMA((2, 4)),
            pltpu.SemaphoreType.DMA((4,)),
            pltpu.SemaphoreType.DMA((5,)),
            pltpu.SemaphoreType.DMA(()),
        ],
        compiler_params=pltpu.CompilerParams(vmem_limit_bytes=120 * 1024 * 1024),
    )(A_x.reshape(S, D), A_mem0.reshape(MEM, D), A_Wq, A_Wk, A_Wv, A_Wo.reshape(H * DH, D),
      B_w1, B_w2, B_w3, B_w4, c, w_mod)
    return out.reshape(1, S, D)
```

```python
import functools

import jax
import jax.numpy as jnp
from jax import lax
import jax.experimental.pallas as pl
import jax.experimental.pallas.tpu as pltpu

bf16, f32, u32 = jnp.bfloat16, jnp.float32, jnp.uint32

S, D, H, DH, MEM, SEG, F = 2048, 1024, 32, 128, 8, 32, 3584
NSEG = S // SEG
XR = 24
PRE = S - XR * NSEG
RING = 576
QOFF = RING - PRE
EP = RING // 2
PITCH = 520
NT = D // 128
NF = F // 128
BM = 128
NB = S // BM
NPAIR = H // 2
PADL = 128
SH = 16
KP = 256
MJ = 512
RC = 16
EPS = 1e-5
LOG2E = 1.4426950408889634
SCALE = DH ** -0.5
CFG = dict(pre=True, step=True, b=True, nlo=6, he=16, first=0, pa=1, m0=16, m1=30, ru=(6, 9, 12), pu=15, ds=5, dp=10, dv=0, qk=((0, 0), (1, 0), (0, 1), (1, 1)), ow=(0, 7, 8), nf=7, p0k=16)


def _ln(x):
    m = jnp.mean(x, axis=-1, keepdims=True)
    xc = x - m
    v = jnp.mean(xc * xc, axis=-1, keepdims=True)
    return xc * lax.rsqrt(v + EPS)


def _gelu(x):
    return jax.nn.gelu(x, approximate=True)


def _dot(a, b):
    return jnp.dot(a, b, preferred_element_type=f32)


def _pk(x):
    return pltpu.bitcast(x.astype(bf16), u32)


def _unpk(x):
    return pltpu.bitcast(x, bf16)


def _tie(w, after, r=0, k=0):
    if after is None:
        return w
    m = functools.reduce(lambda a, b: a & b,
                         [after[:, i * 128:(i + 1) * 128] for i in range(after.shape[1] // 128)])
    mf = pltpu.bitcast(m, f32)
    z = jnp.where(mf * mf < 0.0, jnp.uint32(1), jnp.uint32(0))
    row = w[r:r + 8]
    parts = [row[:, :k * 128], row[:, k * 128:(k + 1) * 128] | z, row[:, (k + 1) * 128:]]
    row = jnp.concatenate([p for p in parts if p.shape[1]], axis=1)
    parts = [w[:r], row, w[r + 8:]]
    return jnp.concatenate([p for p in parts if p.shape[0]], axis=0)


def _kernel(x_hbm, mem0_hbm, wq_hbm, wk_hbm, wv_hbm, wo_hbm, w1_hbm, w2_hbm, w3_hbm, w4_hbm,
            c_hbm, wmod_hbm, out_hbm,
            c_v, x_v, a_v, h0_v, mem_v, mem0_v, mod_v, modr_v, cb_v, sc_v, wm_v, w_v, wo_v,
            w1_v, w2_v, w3_v, w4_v,
            g_v, xa_v, hb_v, base_v, x1_v, y1_v, z_v, y2_v, u_v,
            stage, xh_v, hx_v, acc_v,
            r0_, r1_, r2_, r3_, r4_, r5_, r6_, r7_,
            zero_s, sem_x, sem_stage, sem_mod, sem_w, sem_out):
    wqkv_hbm = (wq_hbm, wk_hbm, wv_hbm)
    rings = (r0_, r1_, r2_, r3_, r4_, r5_, r6_, r7_)

    c_cp = pltpu.make_async_copy(c_hbm, c_v.at[:, pl.ds(0, D)], sem_w.at[0])
    mem0_cp = pltpu.make_async_copy(mem0_hbm, mem0_v, sem_w.at[1])

    def x_cp(q):
        rows = pl.ds(q * PRE if isinstance(q, int) else pl.multiple_of(q * PRE, PRE), PRE)
        return pltpu.make_async_copy(x_hbm.at[rows], x_v.at[rows], sem_x.at[q & 1])

    def w_cp(src, dst, k):
        return pltpu.make_async_copy(src, dst.at[:, pl.ds(0, src.shape[1])], sem_w.at[k])

    wo_cp, w1_cp, w2_cp, w3_cp, w4_cp = (
        w_cp(a, b, k) for k, (a, b) in enumerate(
            ((wo_hbm, wo_v), (w1_hbm, w1_v), (w2_hbm, w2_v), (w3_hbm, w3_v), (w4_hbm, w4_v))))

    def mod0_cp(j, k):
        return pltpu.make_async_copy(wmod_hbm.at[:, pl.ds(j * D + k * KP, KP)],
                                     wm_v.at[k, :, pl.ds(j * KP, KP)], sem_mod.at[k])

    def mod1_cp(q):
        col = 2 * D + q * MJ
        col = col if isinstance(q, int) else pl.multiple_of(col, MJ)
        return pltpu.make_async_copy(wmod_hbm.at[:, pl.ds(col, MJ)], wm_v.at[(4 + q) & 7],
                                     sem_mod.at[q & 3])

    def stage_cp(t, hh, piece):
        d0 = piece * KP if isinstance(piece, int) else pl.multiple_of(piece * KP, KP)
        return pltpu.make_async_copy(
            wqkv_hbm[t].at[pl.ds(d0, KP), pl.ds(hh * 16, 16), :],
            stage.at[hh, pl.ds(d0, KP)], sem_stage.at[hh, piece])

    def tile(n):
        return slice(n * 128, (n + 1) * 128)

    def silu_c():
        cf = c_v[:, 0:D].astype(f32)
        return (cf * jax.nn.sigmoid(cf)).astype(bf16)

    def mod(k, lo=0, hi=D):
        return mod_v[0:1, k * D + lo:k * D + hi]

    def ride(tok, q):
        xs = x_v[pl.ds(tok, RC), :].astype(f32)
        hx = _pk(_ln(xs) * (1.0 + mod(1)) + mod(0))
        for n in range(NT):
            hx_v[n, q * 8:(q + 1) * 8, :] = hx[:, tile(n)]
        return hx

    def repack(hh, ch, p0, n):
        both = None
        for u in range(n):
            p = p0 + u
            a = pltpu.bitcast(stage[hh, 2 * p], u32)
            b = pltpu.bitcast(stage[hh, 2 * p + 1], u32)
            ev = (a & jnp.uint32(0xFFFF)) | (b << 16)
            od = (a >> 16) | (b & jnp.uint32(0xFFFF0000))
            w_v[pl.ds(ch * (16 * PITCH) + p, 8, stride=PITCH), :] = ev
            w_v[pl.ds(ch * (16 * PITCH) + 8 * PITCH + p, 8, stride=PITCH), :] = od
            both = ev & od if both is None else both & ev & od
        return both

    def w_slab(ch, l, lo=0, hi=D):
        base = (ch * 16 + (l % 2) * 8 + l // 2) * PITCH + lo // 2
        return _unpk(w_v[base:base + (hi - lo) // 2, :])

    def ring_of(ch, l):
        return rings[l // 2], (ch * 2 + l % 2) * EP

    c_cp.start()
    mem0_cp.start()
    x_cp(0).start()
    stage_cp(0, 0, 0).start()
    zero_s[0] = 0
    x_v[S:S + SH, :] = jnp.zeros((SH, D), bf16)
    a_v[S:S + SH, :] = jnp.zeros((SH, D), bf16)
    mod_v[...] = jnp.zeros(mod_v.shape, f32)
    modr_v[...] = jnp.zeros(modr_v.shape, f32)
    mod0_cp(0, 0).start()
    mod0_cp(1, 0).start()
    c_cp.wait()
    mem0_cp.wait()
    mem_v[...] = pltpu.bitcast(mem0_v[...], u32)
    cb_v[...] = jnp.transpose(jnp.broadcast_to(silu_c().astype(f32), (128, D)))
    sc_v[...] = _pk(jnp.broadcast_to(silu_c().astype(f32), (16, D)))
    x_cp(0).wait()
    stage_cp(0, 1, 0).start()

    def xhat_body(i, c):
        r0 = pl.multiple_of(i * 64, 64)
        for u in range(4):
            rows = pl.ds(r0 + RC * u, RC)
            xh_v[rows, :] = _ln(x_v[rows, :].astype(f32))
        return c
    lax.fori_loop(0, PRE // 64, xhat_body, 0)

    stage_cp(0, 0, 0).wait()

    def first_repack(i, c):
        repack(0, 0, i * 16, 16)
        return c
    lax.fori_loop(0, KP // 32, first_repack, 0)

    NPC = D // KP
    assert NPC == 4

    def pre_body(i, c):
        t, k = i >> 2, i & 3
        fresh = jnp.logical_and(i > 0, i < 3 * NPC - 1)
        i1 = jnp.where(fresh, i + 1, i)
        t1, k1 = i1 >> 2, i1 & 3

        @pl.when(i < NPC)
        def _():
            for kk in range(NPC):
                @pl.when(i == kk)
                def _():
                    mod0_cp(0, kk).wait()
                    mod0_cp(1, kk).wait()
                    if kk == 1:
                        stage_cp(0, 0, 1).wait()
                    if kk == 3:
                        x_cp(1).wait()
                    for e in range(KP // 128):
                        m = []
                        for j in range(2):
                            m.append(_dot(_unpk(sc_v[...]), wm_v[kk, :, tile(2 * j + e)])[0:8])
                            col = j * D + kk * KP + e * 128
                            mod_v[:, col:col + 128] = m[j]
                        cols = slice(kk * KP + e * 128, kk * KP + (e + 1) * 128)
                        for q in range(PRE // 64):
                            ca = m[1]
                            if kk == 1:
                                rp = repack(0, 0, KP // 2 + (e * 8 + q) * 8, 8)
                                ca = pltpu.bitcast(_tie(pltpu.bitcast(ca, u32), rp), f32)
                            h0_v[kk, q * 32:(q + 1) * 32, tile(e)] = _pk(
                                xh_v[q * 64:(q + 1) * 64, cols] * (1.0 + ca[0:1]) + m[0][0:1])
                    if kk == 0:
                        stage_cp(0, 0, 1).start()
                    if kk + 1 < NPC:
                        mod0_cp(0, kk + 1).start()
                        mod0_cp(1, kk + 1).start()
                    stage_cp((kk + 1) // NPC, 1, (kk + 1) % NPC).start()
                    stage_cp((kk + 2) // NPC, 0, (kk + 2) % NPC).start()
                    if kk == 1:
                        x_cp(1).start()
                    if kk == 2:
                        mod1_cp(0).start()
                    if kk == 3:
                        stage_cp(1, 1, 1).start()
                        stage_cp(1, 0, 2).start()

        stage_cp(0, 1, k).wait()

        @pl.when(fresh)
        def _():
            stage_cp(0, 0, k1).wait()

        w0 = pl.multiple_of(t * (32 * PITCH) + k * (KP // 2), 32)
        xrow = pl.multiple_of(jnp.where(i >= NPC - 1, PRE, 0), PRE)
        done = {}
        nd = 0
        for h in range(H):
            hh, l = h // 16, h % 16
            w = _unpk(w_v[pl.ds(w0 + (hh * 16 + (l % 2) * 8 + l // 2) * PITCH, KP // 2), :])
            q0 = pl.multiple_of(t * (4 * EP), 32) + ring_of(hh, l)[1] + QOFF // 2
            for rb in range(PRE // BM):
                lhs = _tie(h0_v[k, rb * 64:(rb + 1) * 64, :], done.pop(nd, None))
                rows = slice(rb * BM, (rb + 1) * BM)
                y = _dot(_unpk(lhs), w) + jnp.where(k > 0, acc_v[h, rows, :], 0.0)
                acc_v[h, rows, :] = y
                rings[l // 2][pl.ds(q0 + rb * 64, 64), :] = _pk(y)
                nd += 1
            if l < 15:
                n = 9 if l < 8 else 8
                p0_ = l * 9 if l < 8 else 72 + (l - 8) * 8
                if hh == 0:
                    repack(1, 2 * t + 1 + zero_s[0], k * (KP // 2) + p0_, n)
                else:
                    repack(0, 2 * t1, k1 * (KP // 2) + p0_, n)
            if h % 4 == 1 and h < 12:
                done[nd + 16] = ride(xrow + (h // 4) * RC, h // 4)
        @pl.when(i == 3)
        def _():
            mod1_cp(1).start()

        @pl.when(jnp.logical_or(i == 4, i == 5))
        def _():
            x_cp(i - 2).start()

        for tt in range(1, 3):
            @pl.when(jnp.logical_and(i >= 3, (i + 3) >> 2 == tt))
            def _():
                stage_cp(tt, 1, (i + 3) & 3).start()

            @pl.when(jnp.logical_and(i >= 3, t + 1 == tt))
            def _():
                stage_cp(tt, 0, k).start()

        @pl.when(jnp.logical_and(i >= 3, i <= 8))
        def _():
            mod1_cp(i - 1).start()

        @pl.when(i == 8)
        def _():
            wo_cp.start()
        return c
    if CFG['pre']:
        lax.fori_loop(0, 3 * NPC, pre_body, 0)

    for cp in (w1_cp, w2_cp, w3_cp, w4_cp):
        cp.start()
    for q in range(2 * NPC):
        mod1_cp(q).wait()
    x_cp(2).wait()
    x_cp(3).wait()
    wo_cp.wait()

    L2 = 2 * (SEG + MEM)
    r = lax.broadcasted_iota(jnp.int32, (L2, L2), 0)
    c = lax.broadcasted_iota(jnp.int32, (L2, L2), 1)
    r1 = ((r >= SEG) & (r < 2 * SEG)) | (r >= 2 * SEG + MEM)
    c1 = ((c >= SEG) & (c < 2 * SEG)) | (c >= 2 * SEG + MEM)
    same = r1 == c1
    mask = same & ((r >= 2 * SEG) | (c >= 2 * SEG) | (c <= r))
    fill = jnp.where(same, -1e9 / SCALE, -jnp.inf).astype(f32)

    def p0(tok, w):
        rows = pl.ds(tok, RC)
        xa = x_v[rows, :].astype(f32) + mod(2) * a_v[rows, :].astype(f32)
        hb = _ln(xa) * (1.0 + mod(4)) + mod(3)
        xa_v[pl.ds(w, RC), :] = xa
        hb_v[pl.ds(w, RC), :] = hb
        y = _pk(_ln(hb))
        y1_v[pl.ds(w // 2 if isinstance(w, int) else pl.multiple_of(w >> 1, 8), RC // 2), :] = y
        return y

    def step(i, mem, zero, left):
        j = 0 if left is None else 1
        woff = pl.multiple_of((XR * i) % EP, 8) + j * (XR // 2)
        roff = pl.multiple_of((SEG * i + QOFF // 2) % EP, SEG) + j * (SEG // 2)
        arow = pl.multiple_of(2 * SEG * i, 2 * SEG) + j * SEG
        acc = [None] * NT
        ym, ps, ol, part, rest = {}, {}, {}, {}, {}
        HK = D // 2
        tiles = [_unpk(jnp.concatenate(
            [hx_v[k, j * (XR // 2):(j + 1) * (XR // 2), :] | zero, mem[k]], axis=0))
            for k in range(NT)]
        mem_new = []

        def lhs(lo, hi):
            return jnp.concatenate(tiles[lo // 128:hi // 128], axis=1)

        def qkv_lo(h, t):
            part[(t, h)] = _dot(lhs(0, HK), w_slab(2 * t + h // 16, h % 16, 0, HK))

        def proj(t, h):
            ch, l = 2 * t + h // 16, h % 16
            if (t, h) in part:
                y = _dot(lhs(HK, D), w_slab(ch, l, HK, D)) + part.pop((t, h))
            else:
                y = _dot(lhs(0, D), w_slab(ch, l))
            rg, ix = ring_of(ch, l)
            rg[pl.ds(ix + woff, XR // 2), :] = _pk(y[0:XR])
            ym[(t, h)] = y[XR:XR + MEM]

        def get(t, p):
            rg, i0 = ring_of(2 * t + p // 8, (2 * p) % 16)
            _, i1 = ring_of(2 * t + p // 8, (2 * p) % 16 + 1)
            mm = jnp.concatenate([ym.pop((t, 2 * p)), ym.pop((t, 2 * p + 1))], axis=0)
            return _unpk(jnp.concatenate(
                [rg[pl.ds(i0 + roff, SEG // 2), :], rg[pl.ds(i1 + roff, SEG // 2), :], _pk(mm)],
                axis=0))

        def sm(p):
            sc = lax.dot_general(get(0, p), get(1, p), (((1,), (1,)), ((), ())),
                                 preferred_element_type=f32)
            sc = jnp.where(mask, sc, fill)
            e = jnp.exp2((sc - jnp.max(sc, axis=-1, keepdims=True)) * (SCALE * LOG2E))
            ps[p] = (e * pl.reciprocal(jnp.sum(e, axis=-1, keepdims=True), approx=True)
                     ).astype(bf16)

        def pv(p):
            o = _dot(ps.pop(p), get(2, p))
            for b in range(2):
                h = 2 * p + b
                ox = o[SEG * b:SEG * (b + 1)]
                om = o[2 * SEG + MEM * b:2 * SEG + MEM * (b + 1)]
                if left is None:
                    ol[h] = jnp.concatenate([ox[0:XR], om], axis=0).astype(bf16)
                    rest[h] = ox[XR:SEG]
                else:
                    ol[h] = jnp.concatenate([ox, left[h], om], axis=0).astype(bf16)

        def wo(n, h0, h1, after=None):
            for h in range(h0, h1):
                o = ol[h]
                if after is not None and h == h0:
                    o = _unpk(_tie(pltpu.bitcast(o, u32), after))
                y = _dot(o, wo_v[h * DH:(h + 1) * DH, tile(n)])
                acc[n] = y if acc[n] is None else y + acc[n]
            if h1 == H:
                if left is None:
                    a_v[pl.ds(arow, XR), tile(n)] = acc[n][0:XR].astype(bf16)
                else:
                    a_v[pl.ds(arow, SEG), tile(n)] = acc[n][0:SEG].astype(bf16)
                    a_v[pl.ds(arow - (SEG - XR), SEG - XR), tile(n)] = (
                        acc[n][SEG:2 * SEG - XR].astype(bf16))
                mem_new.append(_pk(acc[n][-MEM:]))

        g = lambda k: CFG.get(k + str(j), CFG[k])
        HE, DS, DP, DV = g('he'), g('ds'), g('dp'), g('dv')
        seq = []
        for p in range(NPAIR + DV):
            if p < NPAIR:
                seq += [(t, 2 * p + b) for t, b in g('qk')]
            if p - DV >= 0:
                seq += [(2, 2 * (p - DV)), (2, 2 * (p - DV) + 1)]
        events = {}
        for p in range(NPAIR):
            at = max(seq.index((t, 2 * p + b)) for t in range(2) for b in range(2)) + DS
            at += g('first') if p == 0 else 0
            events.setdefault(at, []).append((sm, p))
            events.setdefault(at + DP, []).append((pv, p))
        for t, h in seq[:g('nlo')]:
            qkv_lo(h, t)
        side = {}
        if j == 1:
            macc = None
            for u in range(CFG['m0'], CFG['m1']):
                n_u = CFG['m1'] - CFG['m0']
                for g in range((u - CFG['m0']) * 128 // n_u, (u + 1 - CFG['m0']) * 128 // n_u):
                    wmg = wm_v[(i + 4) & 7, g * 8:(g + 1) * 8, :].astype(f32)
                    pr = wmg * jnp.concatenate([cb_v[g * 8:(g + 1) * 8, :]] * (MJ // 128), axis=1)
                    macc = pr if macc is None else macc + pr
                side[u] = pltpu.bitcast(macc, u32)
            modr_v[i & 7] = jnp.broadcast_to(jnp.sum(macc, axis=0, keepdims=True), (8, MJ))
            nx = pl.multiple_of(PRE + 2 * XR * jnp.minimum(i + 1, NSEG // 2 - 1), RC)
            for q in range(2 * XR // RC):
                side[CFG['ru'][q]] = ride(nx + q * RC, q)
            tok = pl.multiple_of(jnp.clip(i - 22, 0, BM // RC) * RC, RC)
            side[CFG['pu']] = p0(tok, tok)
            for q in range(2 * NPC):
                mod_v[:, 2 * D + q * MJ:2 * D + (q + 1) * MJ] = modr_v[q]
        WU = HE // 8
        for d in range(len(seq) + NT * WU):
            if d < len(seq):
                proj(*seq[d])
            else:
                u = d - len(seq)
                wo(u // WU, (u % WU) * 8, (u % WU + 1) * 8, side.pop(u, None))
            for fn, p in events.pop(d, []):
                fn(p)
        assert not events
        u = NT * WU
        for n in range(NT):
            for h0 in range(HE, H, 8):
                wo(n, h0, h0 + 8, side.pop(u, None))
                u += 1
        assert not side
        return mem_new, rest

    def steps(i, carry):
        zero = zero_s[0].astype(u32)
        mem = [mem_v[:, tile(k)] for k in range(NT)]
        mem, rest = step(i, mem, zero, None)
        mem, _ = step(i, mem, zero, rest)
        for k in range(NT):
            mem_v[:, tile(k)] = mem[k]
        return carry
    if CFG['step']:
        lax.fori_loop(0, NSEG // 2, steps, 0)

    if not CFG['b']:
        cp = pltpu.make_async_copy(a_v.at[pl.ds(0, S)], out_hbm, sem_out)
        cp.start()
        cp.wait()
        return

    for cp in (w1_cp, w2_cp, w3_cp, w4_cp):
        cp.wait()

    for n in range(NT):
        g_v[n, 0:8, :] = jnp.zeros((8, 128), f32)
        g_v[n, 8:8 + SH, :] = _gelu(_dot(_unpk(y1_v[0:SH // 2, :]), w1_v[:, tile(n)]))

    HM = BM // 2
    shift = (-1, 1, -2, 2)

    def blk(j, c):
        r0 = pl.multiple_of(j * BM, BM)
        nxt = pl.multiple_of(jnp.minimum(j + 1, NB - 1) * BM + SH, SH)
        more = j < NB - 1

        def w1_half(hf):
            for n in range(NT):
                g = _gelu(_dot(_unpk(y1_v[8 + hf * 32:8 + (hf + 1) * 32, :]), w1_v[:, tile(n)]))
                w0 = 8 + SH + hf * HM
                if hf == 0:
                    g_v[n, w0:w0 + HM, :] = g
                else:
                    g_v[n, w0:w0 + HM - SH, :] = g[0:HM - SH]
                    g_v[n, w0 + HM - SH:w0 + HM, :] = jnp.where(more, g[HM - SH:HM], 0.0)

        def w2_half(hf):
            for n in range(NT):
                w0 = 8 + hf * HM + shift[n // 2]
                z_v[hf * 32:(hf + 1) * 32, tile(n)] = _pk(g_v[n, w0:w0 + HM, :])
            for n in range(NT):
                x1_v[hf * HM:(hf + 1) * HM, tile(n)] = (
                    _dot(_unpk(z_v[hf * 32:(hf + 1) * 32, :]), w2_v[:, tile(n)])
                    + hb_v[hf * HM:(hf + 1) * HM, tile(n)])

        def p1_half(hf):
            for k in range(hf * HM // RC, (hf + 1) * HM // RC):
                x1 = x1_v[k * RC:(k + 1) * RC, :]
                y2_v[k * 8:(k + 1) * 8, :] = _pk(_ln(x1))
                base_v[k * RC:(k + 1) * RC, :] = xa_v[k * RC:(k + 1) * RC, :] + mod(5) * x1

        def w3(f, lo, hi, after=None):
            u_v[lo:hi, tile(f)] = _pk(_gelu(
                _dot(_unpk(_tie(y2_v[lo:hi, :], after)), w3_v[:, tile(f)])))

        w1_half(0)
        w1_half(1)
        w2_half(0)
        w2_half(1)
        p1_half(0)
        for f in range(CFG['nf']):
            w3(f, 0, 32)
        p1_half(1)
        for f in range(CFG['nf']):
            w3(f, 32, 64)
        for n in range(NT):
            g_v[n, 0:8 + SH, :] = g_v[n, BM:BM + 8 + SH, :]
        xa_v[0:SH, :] = xa_v[BM:BM + SH, :]
        hb_v[0:SH, :] = hb_v[BM:BM + SH, :]
        for f in range(CFG['nf'], NF):
            w3(f, 0, 64)
        ys = {}

        def prep(k):
            if k < BM // RC:
                ys[k] = p0(nxt + k * RC, SH + k * RC)

        for k in range(CFG['pa']):
            prep(k)
        for n in range(NT):
            prep(n + CFG['pa'])
            gb = mod(5, n * 128, (n + 1) * 128)
            u = _unpk(_tie(u_v[...], ys.pop(n), 0, CFG['p0k']))
            a_v[pl.ds(r0, BM), tile(n)] = (
                base_v[:, tile(n)] + gb * _dot(u, w4_v[:, tile(n)])).astype(bf16)
            if n + 1 in CFG['ow'][1:]:
                lo = CFG['ow'][CFG['ow'].index(n + 1) - 1]
                cols = pl.ds(lo * 128, (n + 1 - lo) * 128)
                pltpu.make_async_copy(a_v.at[pl.ds(r0, BM), cols], out_hbm.at[pl.ds(r0, BM), cols],
                                      sem_out).start()
        return c
    lax.fori_loop(0, NB, blk, 0)
    pltpu.make_async_copy(a_v.at[pl.ds(0, S)], out_hbm, sem_out).wait()


@functools.partial(jax.jit, static_argnames=("A_seg_len",))
def pallas_adaLN_cond__memory_aug_recurrent_mem_tr__mixer_s_mlp__prompt_kernel(
    A_x: jax.Array,
    A_mem0: jax.Array,
    A_Wq: jax.Array,
    A_Wk: jax.Array,
    A_Wv: jax.Array,
    A_Wo: jax.Array,
    A_seg_len,
    B_x: jax.Array,
    B_w1: jax.Array,
    B_w2: jax.Array,
    B_w3: jax.Array,
    B_w4: jax.Array,
    c: jax.Array,
    w_mod: jax.Array,
):
    assert A_seg_len == SEG and A_x.shape == (1, S, D) and A_Wq.shape == (D, H, DH)
    any_spec = pl.BlockSpec(memory_space=pl.ANY)
    out = pl.pallas_call(
        _kernel,
        out_shape=jax.ShapeDtypeStruct((S, D), bf16),
        in_specs=[any_spec] * 12,
        out_specs=any_spec,
        scratch_shapes=[
            pltpu.VMEM((1, 3 * D), bf16),
            pltpu.VMEM((S + SH, D), bf16),
            pltpu.VMEM((S + SH, D), bf16),
            pltpu.VMEM((D // KP, PRE // 2, KP), u32),
            pltpu.VMEM((MEM // 2, D), u32),
            pltpu.VMEM((MEM, D), bf16),
            pltpu.VMEM((8, 6 * D), f32),
            pltpu.VMEM((8, 8, MJ), f32),
            pltpu.VMEM((D, 128), f32),
            pltpu.VMEM((8, D), u32),
            pltpu.VMEM((8, D, MJ), bf16),
            pltpu.VMEM((96 * PITCH + 544, 128), u32),
            pltpu.VMEM((H * DH, D + PADL), bf16),
            pltpu.VMEM((D, D + PADL), bf16),
            pltpu.VMEM((D, D + PADL), bf16),
            pltpu.VMEM((D, F + PADL), bf16),
            pltpu.VMEM((F, D + PADL), bf16),
            pltpu.VMEM((NT, BM + 32, 128), f32),
            pltpu.VMEM((BM + SH, D), f32),
            pltpu.VMEM((BM + SH, D), f32),
            pltpu.VMEM((BM, D), f32),
            pltpu.VMEM((BM, D), f32),
            pltpu.VMEM(((BM + SH) // 2, D), u32),
            pltpu.VMEM((BM // 2, D), u32),
            pltpu.VMEM((BM // 2, D), u32),
            pltpu.VMEM((BM // 2, F), u32),
            pltpu.VMEM((2, D, 16, DH), bf16),
            pltpu.VMEM((PRE, D), f32),
            pltpu.VMEM((NT, 32, 128), u32),
            pltpu.VMEM((H, PRE, DH), f32),
        ] + [pltpu.VMEM((12 * EP, DH), u32)] * 8 + [
            pltpu.SMEM((1,), jnp.int32),
            pltpu.SemaphoreType.DMA((2,)),
            pltpu.SemaphoreType.DMA((2, 4)),
            pltpu.SemaphoreType.DMA((4,)),
            pltpu.SemaphoreType.DMA((5,)),
            pltpu.SemaphoreType.DMA(()),
        ],
        compiler_params=pltpu.CompilerParams(vmem_limit_bytes=120 * 1024 * 1024),
    )(A_x.reshape(S, D), A_mem0.reshape(MEM, D), A_Wq, A_Wk, A_Wv, A_Wo.reshape(H * DH, D),
      B_w1, B_w2, B_w3, B_w4, c, w_mod)
    return out.reshape(1, S, D)
```

```python
import functools

import jax
import jax.numpy as jnp
from jax import lax
import jax.experimental.pallas as pl
import jax.experimental.pallas.tpu as pltpu

bf16, f32, u32 = jnp.bfloat16, jnp.float32, jnp.uint32

S, D, H, DH, MEM, SEG, F = 2048, 1024, 32, 128, 8, 32, 3584
NSEG = S // SEG
XR = 24
PRE = S - XR * NSEG
RING = 576
QOFF = RING - PRE
EP = RING // 2
PITCH = 520
NT = D // 128
NF = F // 128
BM = 128
NB = S // BM
NPAIR = H // 2
PADL = 128
SH = 16
KP = 256
MJ = 512
RC = 16
DS, DP = 5, 10
NLO = 6
HE = 16
NSPLIT = 7
EPS = 1e-5
LOG2E = 1.4426950408889634
SCALE = DH ** -0.5


def _ln(x):
    m = jnp.mean(x, axis=-1, keepdims=True)
    xc = x - m
    v = jnp.mean(xc * xc, axis=-1, keepdims=True)
    return xc * lax.rsqrt(v + EPS)


def _gelu(x):
    return jax.nn.gelu(x, approximate=True)


def _dot(a, b):
    return jnp.dot(a, b, preferred_element_type=f32)


def _pk(x):
    return pltpu.bitcast(x.astype(bf16), u32)


def _unpk(x):
    return pltpu.bitcast(x, bf16)


def _tie(w, after, k=0):
    if after is None:
        return w
    m = functools.reduce(lambda a, b: a & b,
                         [after[:, i * 128:(i + 1) * 128] for i in range(after.shape[1] // 128)])
    mf = pltpu.bitcast(m, f32)
    z = jnp.where(mf * mf < 0.0, jnp.uint32(1), jnp.uint32(0))
    parts = [w[0:8, k * 128:(k + 1) * 128] | z]
    if k > 0:
        parts.insert(0, w[0:8, :k * 128])
    if (k + 1) * 128 < w.shape[1]:
        parts.append(w[0:8, (k + 1) * 128:])
    row = jnp.concatenate(parts, axis=1)
    return jnp.concatenate([row, w[8:]], axis=0) if w.shape[0] > 8 else row


def _kernel(*refs):
    zero_s = refs[-6]
    zero_s[0] = 0

    def once(i, c):
        _kernel_body(*refs)
        return c
    lax.fori_loop(0, 1 + zero_s[0], once, 0)


def _kernel_body(x_hbm, mem0_hbm, wq_hbm, wk_hbm, wv_hbm, wo_hbm, w1_hbm, w2_hbm, w3_hbm, w4_hbm,
            c_hbm, wmod_hbm, out_hbm,
            c_v, x_v, a_v, h0_v, mem_v, mem0_v, mod_v, modr_v, cb_v, sc_v, wm_v, w_v, wo_v,
            w1_v, w2_v, w3_v, w4_v,
            g_v, xa_v, hb_v, base_v, x1_v, y1_v, z_v, y2_v, u_v,
            stage, xh_v, hx_v, acc_v,
            r0_, r1_, r2_, r3_, r4_, r5_, r6_, r7_,
            zero_s, sem_x, sem_stage, sem_mod, sem_w, sem_out):
    wqkv_hbm = (wq_hbm, wk_hbm, wv_hbm)
    rings = (r0_, r1_, r2_, r3_, r4_, r5_, r6_, r7_)

    c_cp = pltpu.make_async_copy(c_hbm, c_v.at[:, pl.ds(0, D)], sem_w.at[0])
    mem0_cp = pltpu.make_async_copy(mem0_hbm, mem0_v, sem_w.at[1])

    def x_cp(q):
        rows = pl.ds(q * PRE if isinstance(q, int) else pl.multiple_of(q * PRE, PRE), PRE)
        return pltpu.make_async_copy(x_hbm.at[rows], x_v.at[rows], sem_x.at[q & 1])

    def w_cp(src, dst, k):
        return pltpu.make_async_copy(src, dst.at[:, pl.ds(0, src.shape[1])], sem_w.at[k])

    wo_cp, w1_cp, w2_cp, w3_cp, w4_cp = (
        w_cp(a, b, k) for k, (a, b) in enumerate(
            ((wo_hbm, wo_v), (w1_hbm, w1_v), (w2_hbm, w2_v), (w3_hbm, w3_v), (w4_hbm, w4_v))))

    def mod0_cp(j, k):
        return pltpu.make_async_copy(wmod_hbm.at[:, pl.ds(j * D + k * KP, KP)],
                                     wm_v.at[k, :, pl.ds(j * KP, KP)], sem_mod.at[k])

    def mod1_cp(q):
        col = 2 * D + q * MJ
        col = col if isinstance(q, int) else pl.multiple_of(col, MJ)
        return pltpu.make_async_copy(wmod_hbm.at[:, pl.ds(col, MJ)], wm_v.at[(4 + q) & 7],
                                     sem_mod.at[q & 3])

    def stage_cp(t, hh, piece):
        d0 = piece * KP if isinstance(piece, int) else pl.multiple_of(piece * KP, KP)
        return pltpu.make_async_copy(
            wqkv_hbm[t].at[pl.ds(d0, KP), pl.ds(hh * 16, 16), :],
            stage.at[hh, pl.ds(d0, KP)], sem_stage.at[hh, piece])

    def tile(n):
        return slice(n * 128, (n + 1) * 128)

    def silu_c():
        cf = c_v[:, 0:D].astype(f32)
        return (cf * jax.nn.sigmoid(cf)).astype(bf16)

    def mod(k, lo=0, hi=D):
        return mod_v[0:1, k * D + lo:k * D + hi]

    def ride(tok, q):
        xs = x_v[pl.ds(tok, RC), :].astype(f32)
        hx = _pk(_ln(xs) * (1.0 + mod(1)) + mod(0))
        for n in range(NT):
            hx_v[n, q * 8:(q + 1) * 8, :] = hx[:, tile(n)]
        return hx

    def repack(hh, ch, p0, n):
        both = None
        for u in range(n):
            p = p0 + u
            a = pltpu.bitcast(stage[hh, 2 * p], u32)
            b = pltpu.bitcast(stage[hh, 2 * p + 1], u32)
            ev = (a & jnp.uint32(0xFFFF)) | (b << 16)
            od = (a >> 16) | (b & jnp.uint32(0xFFFF0000))
            w_v[pl.ds(ch * (16 * PITCH) + p, 8, stride=PITCH), :] = ev
            w_v[pl.ds(ch * (16 * PITCH) + 8 * PITCH + p, 8, stride=PITCH), :] = od
            both = ev & od if both is None else both & ev & od
        return both

    def w_slab(ch, l, lo=0, hi=D):
        base = (ch * 16 + (l % 2) * 8 + l // 2) * PITCH + lo // 2
        return _unpk(w_v[base:base + (hi - lo) // 2, :])

    def ring_of(ch, l):
        return rings[l // 2], (ch * 2 + l % 2) * EP

    x_cp(0).start()
    c_cp.start()
    mem0_cp.start()
    stage_cp(0, 0, 0).start()
    mod0_cp(0, 0).start()
    mod0_cp(1, 0).start()
    x_v[S:S + SH, :] = jnp.zeros((SH, D), bf16)
    a_v[S:S + SH, :] = jnp.zeros((SH, D), bf16)
    mod_v[...] = jnp.zeros(mod_v.shape, f32)
    modr_v[...] = jnp.zeros(modr_v.shape, f32)
    x_cp(0).wait()
    stage_cp(0, 1, 0).start()

    def xhat_body(i, c):
        r0 = pl.multiple_of(i * 64, 64)
        for u in range(4):
            rows = pl.ds(r0 + RC * u, RC)
            xh_v[rows, :] = _ln(x_v[rows, :].astype(f32))
        return c
    lax.fori_loop(0, PRE // 64, xhat_body, 0)

    c_cp.wait()
    mem0_cp.wait()
    mem_v[...] = pltpu.bitcast(mem0_v[...], u32)
    sc_v[...] = _pk(jnp.broadcast_to(silu_c().astype(f32), (16, D)))
    cb_v[...] = jnp.transpose(jnp.broadcast_to(silu_c().astype(f32), (128, D)))
    stage_cp(0, 0, 0).wait()

    def first_repack(i, c):
        repack(0, 0, i * 16, 16)
        return c
    lax.fori_loop(0, KP // 32, first_repack, 0)

    NPC = D // KP
    assert NPC == 4

    def pre_body(i, c):
        t, k = i >> 2, i & 3
        fresh = jnp.logical_and(i > 0, i < 3 * NPC - 1)
        i1 = jnp.where(fresh, i + 1, i)
        t1, k1 = i1 >> 2, i1 & 3

        @pl.when(i < NPC)
        def _():
            for kk in range(NPC):
                @pl.when(i == kk)
                def _():
                    mod0_cp(0, kk).wait()
                    mod0_cp(1, kk).wait()
                    if kk == 1:
                        stage_cp(0, 0, 1).wait()
                    if kk == 3:
                        x_cp(1).wait()
                    for e in range(KP // 128):
                        m = []
                        for j in range(2):
                            m.append(_dot(_unpk(sc_v[...]), wm_v[kk, :, tile(2 * j + e)])[0:8])
                            col = j * D + kk * KP + e * 128
                            mod_v[:, col:col + 128] = m[j]
                        cols = slice(kk * KP + e * 128, kk * KP + (e + 1) * 128)
                        for q in range(PRE // 64):
                            ca = m[1]
                            if kk == 1:
                                rp = repack(0, 0, KP // 2 + (e * 8 + q) * 8, 8)
                                ca = pltpu.bitcast(_tie(pltpu.bitcast(ca, u32), rp), f32)
                            h0_v[kk, q * 32:(q + 1) * 32, tile(e)] = _pk(
                                xh_v[q * 64:(q + 1) * 64, cols] * (1.0 + ca[0:1]) + m[0][0:1])
                    if kk == 0:
                        stage_cp(0, 0, 1).start()
                    if kk + 1 < NPC:
                        mod0_cp(0, kk + 1).start()
                        mod0_cp(1, kk + 1).start()
                    stage_cp((kk + 1) // NPC, 1, (kk + 1) % NPC).start()
                    stage_cp((kk + 2) // NPC, 0, (kk + 2) % NPC).start()
                    if kk == 1:
                        x_cp(1).start()
                    if kk == 2:
                        mod1_cp(0).start()
                    if kk == 3:
                        stage_cp(1, 1, 1).start()
                        stage_cp(1, 0, 2).start()

        stage_cp(0, 1, k).wait()

        @pl.when(fresh)
        def _():
            stage_cp(0, 0, k1).wait()

        w0 = pl.multiple_of(t * (32 * PITCH) + k * (KP // 2), 32)
        xrow = pl.multiple_of(jnp.where(i >= NPC - 1, PRE, 0), PRE)
        done = {}
        nd = 0
        for h in range(H):
            hh, l = h // 16, h % 16
            w = _unpk(w_v[pl.ds(w0 + (hh * 16 + (l % 2) * 8 + l // 2) * PITCH, KP // 2), :])
            q0 = pl.multiple_of(t * (4 * EP), 32) + ring_of(hh, l)[1] + QOFF // 2
            for rb in range(PRE // BM):
                lhs = _tie(h0_v[k, rb * 64:(rb + 1) * 64, :], done.pop(nd, None))
                rows = slice(rb * BM, (rb + 1) * BM)
                y = _dot(_unpk(lhs), w) + jnp.where(k > 0, acc_v[h, rows, :], 0.0)
                acc_v[h, rows, :] = y
                rings[l // 2][pl.ds(q0 + rb * 64, 64), :] = _pk(y)
                nd += 1
            if l < 15:
                n = 9 if l < 8 else 8
                p0_ = l * 9 if l < 8 else 72 + (l - 8) * 8
                if hh == 0:
                    repack(1, 2 * t + 1 + zero_s[0], k * (KP // 2) + p0_, n)
                else:
                    repack(0, 2 * t1, k1 * (KP // 2) + p0_, n)
            if h % 4 == 1 and h < 12:
                done[nd + 16] = ride(xrow + (h // 4) * RC, h // 4)
        @pl.when(i == 3)
        def _():
            mod1_cp(1).start()

        @pl.when(jnp.logical_or(i == 4, i == 5))
        def _():
            x_cp(i - 2).start()

        for tt in range(1, 3):
            @pl.when(jnp.logical_and(i >= 3, (i + 3) >> 2 == tt))
            def _():
                stage_cp(tt, 1, (i + 3) & 3).start()

            @pl.when(jnp.logical_and(i >= 3, t + 1 == tt))
            def _():
                stage_cp(tt, 0, k).start()

        @pl.when(jnp.logical_and(i >= 3, i <= 8))
        def _():
            mod1_cp(i - 1).start()

        @pl.when(i == 8)
        def _():
            wo_cp.start()
        return c
    lax.fori_loop(0, 3 * NPC, pre_body, 0)

    for cp in (w1_cp, w2_cp, w3_cp, w4_cp):
        cp.start()
    for q in range(2 * NPC):
        mod1_cp(q).wait()
    x_cp(2).wait()
    x_cp(3).wait()
    wo_cp.wait()

    L2 = 2 * (SEG + MEM)
    r = lax.broadcasted_iota(jnp.int32, (L2, L2), 0)
    c = lax.broadcasted_iota(jnp.int32, (L2, L2), 1)
    r1 = ((r >= SEG) & (r < 2 * SEG)) | (r >= 2 * SEG + MEM)
    c1 = ((c >= SEG) & (c < 2 * SEG)) | (c >= 2 * SEG + MEM)
    same = r1 == c1
    mask = same & ((r >= 2 * SEG) | (c >= 2 * SEG) | (c <= r))
    fill = jnp.where(same, -1e9 / SCALE, -jnp.inf).astype(f32)

    def p0(tok, w):
        rows = pl.ds(tok, RC)
        xa = x_v[rows, :].astype(f32) + mod(2) * a_v[rows, :].astype(f32)
        hb = _ln(xa) * (1.0 + mod(4)) + mod(3)
        xa_v[pl.ds(w, RC), :] = xa
        hb_v[pl.ds(w, RC), :] = hb
        y = _pk(_ln(hb))
        y1_v[pl.ds(w // 2 if isinstance(w, int) else pl.multiple_of(w >> 1, 8), RC // 2), :] = y
        return y

    def step(i, mem, zero, left):
        j = 0 if left is None else 1
        woff = pl.multiple_of((XR * i) % EP, 8) + j * (XR // 2)
        roff = pl.multiple_of((SEG * i + QOFF // 2) % EP, SEG) + j * (SEG // 2)
        arow = pl.multiple_of(2 * SEG * i, 2 * SEG) + j * SEG
        acc = [None] * NT
        ym, ps, ol, part, rest = {}, {}, {}, {}, {}
        HK = D // 2
        tiles = [_unpk(jnp.concatenate(
            [hx_v[k, j * (XR // 2):(j + 1) * (XR // 2), :] | zero, mem[k]], axis=0))
            for k in range(NT)]
        mem_new = []

        def lhs(lo, hi):
            return jnp.concatenate(tiles[lo // 128:hi // 128], axis=1)

        def qkv_lo(h, t):
            part[(t, h)] = _dot(lhs(0, HK), w_slab(2 * t + h // 16, h % 16, 0, HK))

        def proj(t, h):
            ch, l = 2 * t + h // 16, h % 16
            if (t, h) in part:
                y = _dot(lhs(HK, D), w_slab(ch, l, HK, D)) + part.pop((t, h))
            else:
                y = _dot(lhs(0, D), w_slab(ch, l))
            rg, ix = ring_of(ch, l)
            rg[pl.ds(ix + woff, XR // 2), :] = _pk(y[0:XR])
            ym[(t, h)] = y[XR:XR + MEM]

        def get(t, p):
            rg, i0 = ring_of(2 * t + p // 8, (2 * p) % 16)
            _, i1 = ring_of(2 * t + p // 8, (2 * p) % 16 + 1)
            mm = jnp.concatenate([ym.pop((t, 2 * p)), ym.pop((t, 2 * p + 1))], axis=0)
            return _unpk(jnp.concatenate(
                [rg[pl.ds(i0 + roff, SEG // 2), :], rg[pl.ds(i1 + roff, SEG // 2), :], _pk(mm)],
                axis=0))

        def sm(p):
            sc = lax.dot_general(get(0, p), get(1, p), (((1,), (1,)), ((), ())),
                                 preferred_element_type=f32)
            sc = jnp.where(mask, sc, fill)
            e = jnp.exp2((sc - jnp.max(sc, axis=-1, keepdims=True)) * (SCALE * LOG2E))
            ps[p] = (e * pl.reciprocal(jnp.sum(e, axis=-1, keepdims=True), approx=True)
                     ).astype(bf16)

        def pv(p):
            o = _dot(ps.pop(p), get(2, p))
            for b in range(2):
                h = 2 * p + b
                ox = o[SEG * b:SEG * (b + 1)]
                om = o[2 * SEG + MEM * b:2 * SEG + MEM * (b + 1)]
                if left is None:
                    ol[h] = jnp.concatenate([ox[0:XR], om], axis=0).astype(bf16)
                    rest[h] = ox[XR:SEG]
                else:
                    ol[h] = jnp.concatenate([ox, left[h], om], axis=0).astype(bf16)

        def wo(n, h0, h1, after=None):
            for h in range(h0, h1):
                o = ol[h]
                if after is not None and h == h0:
                    o = _unpk(_tie(pltpu.bitcast(o, u32), after))
                y = _dot(o, wo_v[h * DH:(h + 1) * DH, tile(n)])
                acc[n] = y if acc[n] is None else y + acc[n]
            if h1 == H:
                if left is None:
                    a_v[pl.ds(arow, XR), tile(n)] = acc[n][0:XR].astype(bf16)
                else:
                    a_v[pl.ds(arow, SEG), tile(n)] = acc[n][0:SEG].astype(bf16)
                    a_v[pl.ds(arow - (SEG - XR), SEG - XR), tile(n)] = (
                        acc[n][SEG:2 * SEG - XR].astype(bf16))
                mem_new.append(_pk(acc[n][-MEM:]))

        seq = []
        for p in range(NPAIR):
            seq += [(0, 2 * p), (1, 2 * p), (0, 2 * p + 1), (1, 2 * p + 1),
                    (2, 2 * p), (2, 2 * p + 1)]
        events = {}
        for p in range(NPAIR):
            at = seq.index((1, 2 * p + 1)) + DS
            events.setdefault(at, []).append((sm, p))
            events.setdefault(at + DP, []).append((pv, p))
        for t, h in seq[:NLO]:
            qkv_lo(h, t)
        side = {}
        if j == 1:
            macc = None
            for u in range(14):
                for g in range(u * 128 // 14, (u + 1) * 128 // 14):
                    wmg = wm_v[(i + 4) & 7, g * 8:(g + 1) * 8, :].astype(f32)
                    pr = wmg * jnp.concatenate([cb_v[g * 8:(g + 1) * 8, :]] * (MJ // 128), axis=1)
                    macc = pr if macc is None else macc + pr
                side[16 + u] = pltpu.bitcast(macc, u32)
            modr_v[i & 7] = jnp.broadcast_to(jnp.sum(macc, axis=0, keepdims=True), (8, MJ))
            nx = pl.multiple_of(PRE + 2 * XR * jnp.minimum(i + 1, NSEG // 2 - 1), RC)
            for q in range(2 * XR // RC):
                side[6 + 3 * q] = ride(nx + q * RC, q)
            tok = pl.multiple_of(jnp.clip(i - 22, 0, BM // RC) * RC, RC)
            side[15] = p0(tok, tok)
            for q in range(2 * NPC):
                mod_v[:, 2 * D + q * MJ:2 * D + (q + 1) * MJ] = modr_v[q]
        WU = HE // 8
        for d in range(len(seq) + NT * WU):
            if d < len(seq):
                proj(*seq[d])
            else:
                u = d - len(seq)
                wo(u // WU, (u % WU) * 8, (u % WU + 1) * 8, side.pop(u, None))
            for fn, p in events.pop(d, []):
                fn(p)
        assert not events
        u = NT * WU
        for n in range(NT):
            for h0 in range(HE, H, 8):
                wo(n, h0, h0 + 8, side.pop(u, None))
                u += 1
        assert not side
        return mem_new, rest

    def steps(i, carry):
        zero = zero_s[0].astype(u32)
        mem = [mem_v[:, tile(k)] for k in range(NT)]
        mem, rest = step(i, mem, zero, None)
        mem, _ = step(i, mem, zero, rest)
        for k in range(NT):
            mem_v[:, tile(k)] = mem[k]
        return carry
    lax.fori_loop(0, NSEG // 2, steps, 0)

    for cp in (w1_cp, w2_cp, w3_cp, w4_cp):
        cp.wait()

    for n in range(NT):
        g_v[n, 0:8, :] = jnp.zeros((8, 128), f32)
        g_v[n, 8:8 + SH, :] = _gelu(_dot(_unpk(y1_v[0:SH // 2, :]), w1_v[:, tile(n)]))

    HM = BM // 2
    shift = (-1, 1, -2, 2)

    def blk(j, c):
        r0 = pl.multiple_of(j * BM, BM)
        nxt = pl.multiple_of(jnp.minimum(j + 1, NB - 1) * BM + SH, SH)
        more = j < NB - 1

        def w1_half(hf):
            for n in range(NT):
                g = _gelu(_dot(_unpk(y1_v[8 + hf * 32:8 + (hf + 1) * 32, :]), w1_v[:, tile(n)]))
                w0 = 8 + SH + hf * HM
                if hf == 0:
                    g_v[n, w0:w0 + HM, :] = g
                else:
                    g_v[n, w0:w0 + HM - SH, :] = g[0:HM - SH]
                    g_v[n, w0 + HM - SH:w0 + HM, :] = jnp.where(more, g[HM - SH:HM], 0.0)

        def w2_half(hf):
            for n in range(NT):
                w0 = 8 + hf * HM + shift[n // 2]
                z_v[hf * 32:(hf + 1) * 32, tile(n)] = _pk(g_v[n, w0:w0 + HM, :])
            for n in range(NT):
                x1_v[hf * HM:(hf + 1) * HM, tile(n)] = (
                    _dot(_unpk(z_v[hf * 32:(hf + 1) * 32, :]), w2_v[:, tile(n)])
                    + hb_v[hf * HM:(hf + 1) * HM, tile(n)])

        def p1_half(hf):
            for k in range(hf * HM // RC, (hf + 1) * HM // RC):
                x1 = x1_v[k * RC:(k + 1) * RC, :]
                y2_v[k * 8:(k + 1) * 8, :] = _pk(_ln(x1))
                base_v[k * RC:(k + 1) * RC, :] = xa_v[k * RC:(k + 1) * RC, :] + mod(5) * x1

        def w3(f, lo, hi):
            u_v[lo:hi, tile(f)] = _pk(_gelu(_dot(_unpk(y2_v[lo:hi, :]), w3_v[:, tile(f)])))

        w1_half(0)
        w1_half(1)
        w2_half(0)
        w2_half(1)
        p1_half(0)
        for f in range(NSPLIT):
            w3(f, 0, 32)
        p1_half(1)
        for f in range(NSPLIT):
            w3(f, 32, 64)
        for n in range(NT):
            g_v[n, 0:8 + SH, :] = g_v[n, BM:BM + 8 + SH, :]
        xa_v[0:SH, :] = xa_v[BM:BM + SH, :]
        hb_v[0:SH, :] = hb_v[BM:BM + SH, :]
        for f in range(NSPLIT, NF):
            w3(f, 0, 64)
        ys = {}

        def prep(k):
            if k < BM // RC:
                ys[k] = p0(nxt + k * RC, SH + k * RC)

        prep(0)
        for n in range(NT):
            prep(n + 1)
            gb = mod(5, n * 128, (n + 1) * 128)
            u = _unpk(_tie(u_v[...], ys.pop(n), 16))
            a_v[pl.ds(r0, BM), tile(n)] = (
                base_v[:, tile(n)] + gb * _dot(u, w4_v[:, tile(n)])).astype(bf16)
            if n >= NT - 2:
                cols = pl.ds(0, (NT - 1) * 128) if n == NT - 2 else pl.ds(n * 128, 128)
                pltpu.make_async_copy(a_v.at[pl.ds(r0, BM), cols], out_hbm.at[pl.ds(r0, BM), cols],
                                      sem_out).start()
        return c
    lax.fori_loop(0, NB, blk, 0)
    pltpu.make_async_copy(a_v.at[pl.ds(0, S)], out_hbm, sem_out).wait()


@functools.partial(jax.jit, static_argnames=("A_seg_len",))
def pallas_adaLN_cond__memory_aug_recurrent_mem_tr__mixer_s_mlp__prompt_kernel(
    A_x: jax.Array,
    A_mem0: jax.Array,
    A_Wq: jax.Array,
    A_Wk: jax.Array,
    A_Wv: jax.Array,
    A_Wo: jax.Array,
    A_seg_len,
    B_x: jax.Array,
    B_w1: jax.Array,
    B_w2: jax.Array,
    B_w3: jax.Array,
    B_w4: jax.Array,
    c: jax.Array,
    w_mod: jax.Array,
):
    assert A_seg_len == SEG and A_x.shape == (1, S, D) and A_Wq.shape == (D, H, DH)
    any_spec = pl.BlockSpec(memory_space=pl.ANY)
    out = pl.pallas_call(
        _kernel,
        out_shape=jax.ShapeDtypeStruct((S, D), bf16),
        in_specs=[any_spec] * 12,
        out_specs=any_spec,
        scratch_shapes=[
            pltpu.VMEM((1, 3 * D), bf16),
            pltpu.VMEM((S + SH, D), bf16),
            pltpu.VMEM((S + SH, D), bf16),
            pltpu.VMEM((D // KP, PRE // 2, KP), u32),
            pltpu.VMEM((MEM // 2, D), u32),
            pltpu.VMEM((MEM, D), bf16),
            pltpu.VMEM((8, 6 * D), f32),
            pltpu.VMEM((8, 8, MJ), f32),
            pltpu.VMEM((D, 128), f32),
            pltpu.VMEM((8, D), u32),
            pltpu.VMEM((8, D, MJ), bf16),
            pltpu.VMEM((96 * PITCH + 544, 128), u32),
            pltpu.VMEM((H * DH, D + PADL), bf16),
            pltpu.VMEM((D, D + PADL), bf16),
            pltpu.VMEM((D, D + PADL), bf16),
            pltpu.VMEM((D, F + PADL), bf16),
            pltpu.VMEM((F, D + PADL), bf16),
            pltpu.VMEM((NT, BM + 32, 128), f32),
            pltpu.VMEM((BM + SH, D), f32),
            pltpu.VMEM((BM + SH, D), f32),
            pltpu.VMEM((BM, D), f32),
            pltpu.VMEM((BM, D), f32),
            pltpu.VMEM(((BM + SH) // 2, D), u32),
            pltpu.VMEM((BM // 2, D), u32),
            pltpu.VMEM((BM // 2, D), u32),
            pltpu.VMEM((BM // 2, F), u32),
            pltpu.VMEM((2, D, 16, DH), bf16),
            pltpu.VMEM((PRE, D), f32),
            pltpu.VMEM((NT, 32, 128), u32),
            pltpu.VMEM((H, PRE, DH), f32),
        ] + [pltpu.VMEM((12 * EP, DH), u32)] * 8 + [
            pltpu.SMEM((1,), jnp.int32),
            pltpu.SemaphoreType.DMA((2,)),
            pltpu.SemaphoreType.DMA((2, 4)),
            pltpu.SemaphoreType.DMA((4,)),
            pltpu.SemaphoreType.DMA((5,)),
            pltpu.SemaphoreType.DMA(()),
        ],
        compiler_params=pltpu.CompilerParams(vmem_limit_bytes=120 * 1024 * 1024),
    )(A_x.reshape(S, D), A_mem0.reshape(MEM, D), A_Wq, A_Wk, A_Wv, A_Wo.reshape(H * DH, D),
      B_w1, B_w2, B_w3, B_w4, c, w_mod)
    return out.reshape(1, S, D)
```

```python
import functools

import jax
import jax.numpy as jnp
from jax import lax
import jax.experimental.pallas as pl
import jax.experimental.pallas.tpu as pltpu

bf16, f32, u32 = jnp.bfloat16, jnp.float32, jnp.uint32

S, D, H, DH, MEM, SEG, F = 2048, 1024, 32, 128, 8, 32, 3584
NSEG = S // SEG
XR = 24
PRE = S - XR * NSEG
RING = 576
QOFF = RING - PRE
EP = RING // 2
PITCH = 520
NT = D // 128
NF = F // 128
BM = 128
NB = S // BM
NPAIR = H // 2
PADL = 128
SH = 16
KP = 256
MJ = 512
RC = 16
DS, DP = 5, 10
NLO = 6
HE = 16
NSPLIT = 7
EPS = 1e-5
LOG2E = 1.4426950408889634
SCALE = DH ** -0.5


def _ln(x):
    m = jnp.mean(x, axis=-1, keepdims=True)
    xc = x - m
    v = jnp.mean(xc * xc, axis=-1, keepdims=True)
    return xc * lax.rsqrt(v + EPS)


def _gelu(x):
    return jax.nn.gelu(x, approximate=True)


def _dot(a, b):
    return jnp.dot(a, b, preferred_element_type=f32)


def _pk(x):
    return pltpu.bitcast(x.astype(bf16), u32)


def _unpk(x):
    return pltpu.bitcast(x, bf16)


def _tie(w, after, k=0):
    if after is None:
        return w
    m = functools.reduce(lambda a, b: a & b,
                         [after[:, i * 128:(i + 1) * 128] for i in range(after.shape[1] // 128)])
    mf = pltpu.bitcast(m, f32)
    z = jnp.where(mf * mf < 0.0, jnp.uint32(1), jnp.uint32(0))
    parts = [w[0:8, k * 128:(k + 1) * 128] | z]
    if k > 0:
        parts.insert(0, w[0:8, :k * 128])
    if (k + 1) * 128 < w.shape[1]:
        parts.append(w[0:8, (k + 1) * 128:])
    row = jnp.concatenate(parts, axis=1)
    return jnp.concatenate([row, w[8:]], axis=0) if w.shape[0] > 8 else row


def _kernel(*refs):
    zero_s = refs[-6]
    zero_s[0] = 0

    def once(i, c):
        _kernel_body(*refs)
        return c
    lax.fori_loop(0, 1 + zero_s[0], once, 0)


def _kernel_body(x_hbm, mem0_hbm, wq_hbm, wk_hbm, wv_hbm, wo_hbm, w1_hbm, w2_hbm, w3_hbm, w4_hbm,
            c_hbm, wmod_hbm, out_hbm,
            c_v, x_v, a_v, h0_v, mem_v, mem0_v, mod_v, modr_v, cb_v, sc_v, wm_v, w_v, wo_v,
            w1_v, w2_v, w3_v, w4_v,
            g_v, xa_v, hb_v, base_v, x1_v, y1_v, z_v, y2_v, u_v,
            stage, xh_v, hx_v, acc_v,
            r0_, r1_, r2_, r3_, r4_, r5_, r6_, r7_,
            zero_s, sem_x, sem_stage, sem_mod, sem_w, sem_out):
    wqkv_hbm = (wq_hbm, wk_hbm, wv_hbm)
    rings = (r0_, r1_, r2_, r3_, r4_, r5_, r6_, r7_)

    c_cp = pltpu.make_async_copy(c_hbm, c_v.at[:, pl.ds(0, D)], sem_w.at[0])
    mem0_cp = pltpu.make_async_copy(mem0_hbm, mem0_v, sem_w.at[1])

    def x_cp(q):
        rows = pl.ds(q * PRE if isinstance(q, int) else pl.multiple_of(q * PRE, PRE), PRE)
        return pltpu.make_async_copy(x_hbm.at[rows], x_v.at[rows], sem_x.at[q & 1])

    def w_cp(src, dst, k):
        return pltpu.make_async_copy(src, dst.at[:, pl.ds(0, src.shape[1])], sem_w.at[k])

    wo_cp, w1_cp, w2_cp, w3_cp, w4_cp = (
        w_cp(a, b, k) for k, (a, b) in enumerate(
            ((wo_hbm, wo_v), (w1_hbm, w1_v), (w2_hbm, w2_v), (w3_hbm, w3_v), (w4_hbm, w4_v))))

    def mod0_cp(j, k):
        return pltpu.make_async_copy(wmod_hbm.at[:, pl.ds(j * D + k * KP, KP)],
                                     wm_v.at[k, :, pl.ds(j * KP, KP)], sem_mod.at[k])

    def mod1_cp(q):
        col = 2 * D + q * MJ
        col = col if isinstance(q, int) else pl.multiple_of(col, MJ)
        return pltpu.make_async_copy(wmod_hbm.at[:, pl.ds(col, MJ)], wm_v.at[(4 + q) & 7],
                                     sem_mod.at[q & 3])

    def stage_cp(t, hh, piece):
        d0 = piece * KP if isinstance(piece, int) else pl.multiple_of(piece * KP, KP)
        return pltpu.make_async_copy(
            wqkv_hbm[t].at[pl.ds(d0, KP), pl.ds(hh * 16, 16), :],
            stage.at[hh, pl.ds(d0, KP)], sem_stage.at[hh, piece])

    def tile(n):
        return slice(n * 128, (n + 1) * 128)

    def silu_c():
        cf = c_v[:, 0:D].astype(f32)
        return (cf * jax.nn.sigmoid(cf)).astype(bf16)

    def mod(k, lo=0, hi=D):
        return mod_v[0:1, k * D + lo:k * D + hi]

    def ride(tok, q):
        xs = x_v[pl.ds(tok, RC), :].astype(f32)
        hx = _pk(_ln(xs) * (1.0 + mod(1)) + mod(0))
        for n in range(NT):
            hx_v[n, q * 8:(q + 1) * 8, :] = hx[:, tile(n)]
        return hx

    def repack(hh, ch, p0, n):
        for u in range(n):
            p = p0 + u
            a = pltpu.bitcast(stage[hh, 2 * p], u32)
            b = pltpu.bitcast(stage[hh, 2 * p + 1], u32)
            ev = (a & jnp.uint32(0xFFFF)) | (b << 16)
            od = (a >> 16) | (b & jnp.uint32(0xFFFF0000))
            w_v[pl.ds(ch * (16 * PITCH) + p, 8, stride=PITCH), :] = ev
            w_v[pl.ds(ch * (16 * PITCH) + 8 * PITCH + p, 8, stride=PITCH), :] = od

    def w_slab(ch, l, lo=0, hi=D):
        base = (ch * 16 + (l % 2) * 8 + l // 2) * PITCH + lo // 2
        return _unpk(w_v[base:base + (hi - lo) // 2, :])

    def ring_of(ch, l):
        return rings[l // 2], (ch * 2 + l % 2) * EP

    x_cp(0).start()
    c_cp.start()
    mem0_cp.start()
    stage_cp(0, 0, 0).start()
    mod0_cp(0, 0).start()
    mod0_cp(1, 0).start()
    x_v[S:S + SH, :] = jnp.zeros((SH, D), bf16)
    a_v[S:S + SH, :] = jnp.zeros((SH, D), bf16)
    mod_v[...] = jnp.zeros(mod_v.shape, f32)
    modr_v[...] = jnp.zeros(modr_v.shape, f32)
    x_cp(0).wait()
    stage_cp(0, 1, 0).start()

    def xhat_body(i, c):
        r0 = pl.multiple_of(i * 64, 64)
        for u in range(4):
            rows = pl.ds(r0 + RC * u, RC)
            xh_v[rows, :] = _ln(x_v[rows, :].astype(f32))
        return c
    lax.fori_loop(0, PRE // 64, xhat_body, 0)

    c_cp.wait()
    mem0_cp.wait()
    mem_v[...] = pltpu.bitcast(mem0_v[...], u32)
    sc_v[...] = _pk(jnp.broadcast_to(silu_c().astype(f32), (16, D)))
    cb_v[...] = jnp.transpose(jnp.broadcast_to(silu_c().astype(f32), (128, D)))
    stage_cp(0, 0, 0).wait()

    def first_repack(i, c):
        repack(0, 0, i * 16, 16)
        return c
    lax.fori_loop(0, KP // 32, first_repack, 0)

    NPC = D // KP
    assert NPC == 4

    def modulate(kk):
        mod0_cp(0, kk).wait()
        mod0_cp(1, kk).wait()
        if kk == 3:
            x_cp(1).wait()
        for e in range(KP // 128):
            m = []
            for j in range(2):
                m.append(_dot(_unpk(sc_v[...]), wm_v[kk, :, tile(2 * j + e)])[0:8])
                col = j * D + kk * KP + e * 128
                mod_v[:, col:col + 128] = m[j]
            cols = slice(kk * KP + e * 128, kk * KP + (e + 1) * 128)
            for q in range(PRE // 64):
                h0_v[kk, q * 32:(q + 1) * 32, tile(e)] = _pk(
                    xh_v[q * 64:(q + 1) * 64, cols] * (1.0 + m[1][0:1]) + m[0][0:1])
        if kk == 0:
            stage_cp(0, 0, 1).start()
        if kk + 1 < NPC:
            mod0_cp(0, kk + 1).start()
            mod0_cp(1, kk + 1).start()
        stage_cp((kk + 1) // NPC, 1, (kk + 1) % NPC).start()
        stage_cp((kk + 2) // NPC, 0, (kk + 2) % NPC).start()
        if kk == 1:
            x_cp(1).start()
        if kk == 2:
            mod1_cp(0).start()
        if kk == 3:
            stage_cp(1, 1, 1).start()
            stage_cp(1, 0, 2).start()

    def first_heads(h0, h1, side):
        for h in range(h0, h1):
            w = w_slab(h // 16, h % 16, 0, KP)
            for rb in range(PRE // BM):
                acc_v[h, rb * BM:(rb + 1) * BM, :] = _dot(
                    _unpk(h0_v[0, rb * 64:(rb + 1) * 64, :]), w)
            if side is not None and h < h1 - 1:
                lo, hi = (h - h0) * 128 // (h1 - h0 - 1), (h + 1 - h0) * 128 // (h1 - h0 - 1)
                side(lo, hi - lo)

    modulate(0)
    first_heads(0, 8, None)
    stage_cp(0, 1, 0).wait()
    first_heads(8, 16, lambda p, n: repack(1, 1 + zero_s[0], p, n))
    stage_cp(0, 0, 1).wait()
    first_heads(16, 32, lambda p, n: repack(0, zero_s[0], KP // 2 + p, n))

    def pre_body(i, c):
        t, k = i >> 2, i & 3
        fresh = i < 3 * NPC - 1
        i1 = jnp.where(fresh, i + 1, i)
        t1, k1 = i1 >> 2, i1 & 3

        @pl.when(i < NPC)
        def _():
            for kk in range(1, NPC):
                pl.when(i == kk)(functools.partial(modulate, kk))

        stage_cp(0, 1, k).wait()

        @pl.when(fresh)
        def _():
            stage_cp(0, 0, k1).wait()

        w0 = pl.multiple_of(t * (32 * PITCH) + k * (KP // 2), 32)
        xrow = pl.multiple_of(jnp.where(i >= NPC - 1, PRE, 0), PRE)
        done = {}
        nd = 0
        for h in range(H):
            hh, l = h // 16, h % 16
            w = _unpk(w_v[pl.ds(w0 + (hh * 16 + (l % 2) * 8 + l // 2) * PITCH, KP // 2), :])
            q0 = pl.multiple_of(t * (4 * EP), 32) + ring_of(hh, l)[1] + QOFF // 2
            for rb in range(PRE // BM):
                lhs = _tie(h0_v[k, rb * 64:(rb + 1) * 64, :], done.pop(nd, None))
                rows = slice(rb * BM, (rb + 1) * BM)
                y = _dot(_unpk(lhs), w) + jnp.where(k > 0, acc_v[h, rows, :], 0.0)
                acc_v[h, rows, :] = y
                rings[l // 2][pl.ds(q0 + rb * 64, 64), :] = _pk(y)
                nd += 1
            if l < 15:
                n = 9 if l < 8 else 8
                p0_ = l * 9 if l < 8 else 72 + (l - 8) * 8
                if hh == 0:
                    repack(1, 2 * t + 1 + zero_s[0], k * (KP // 2) + p0_, n)
                else:
                    repack(0, 2 * t1, k1 * (KP // 2) + p0_, n)
            if h % 4 == 1 and h < 12:
                done[nd + 16] = ride(xrow + (h // 4) * RC, h // 4)
        @pl.when(i == 3)
        def _():
            mod1_cp(1).start()

        @pl.when(jnp.logical_or(i == 4, i == 5))
        def _():
            x_cp(i - 2).start()

        for tt in range(1, 3):
            @pl.when(jnp.logical_and(i >= 3, (i + 3) >> 2 == tt))
            def _():
                stage_cp(tt, 1, (i + 3) & 3).start()

            @pl.when(jnp.logical_and(i >= 3, t + 1 == tt))
            def _():
                stage_cp(tt, 0, k).start()

        @pl.when(jnp.logical_and(i >= 3, i <= 8))
        def _():
            mod1_cp(i - 1).start()

        @pl.when(i == 8)
        def _():
            wo_cp.start()
        return c
    lax.fori_loop(1, 3 * NPC, pre_body, 0)

    for cp in (w1_cp, w2_cp, w3_cp, w4_cp):
        cp.start()
    for q in range(2 * NPC):
        mod1_cp(q).wait()
    x_cp(2).wait()
    x_cp(3).wait()
    wo_cp.wait()

    L2 = 2 * (SEG + MEM)
    r = lax.broadcasted_iota(jnp.int32, (L2, L2), 0)
    c = lax.broadcasted_iota(jnp.int32, (L2, L2), 1)
    r1 = ((r >= SEG) & (r < 2 * SEG)) | (r >= 2 * SEG + MEM)
    c1 = ((c >= SEG) & (c < 2 * SEG)) | (c >= 2 * SEG + MEM)
    same = r1 == c1
    mask = same & ((r >= 2 * SEG) | (c >= 2 * SEG) | (c <= r))
    fill = jnp.where(same, -1e9 / SCALE, -jnp.inf).astype(f32)

    def p0(tok, w):
        rows = pl.ds(tok, RC)
        xa = x_v[rows, :].astype(f32) + mod(2) * a_v[rows, :].astype(f32)
        hb = _ln(xa) * (1.0 + mod(4)) + mod(3)
        xa_v[pl.ds(w, RC), :] = xa
        hb_v[pl.ds(w, RC), :] = hb
        y = _pk(_ln(hb))
        y1_v[pl.ds(w // 2 if isinstance(w, int) else pl.multiple_of(w >> 1, 8), RC // 2), :] = y
        return y

    def step(i, mem, zero, left):
        j = 0 if left is None else 1
        woff = pl.multiple_of((XR * i) % EP, 8) + j * (XR // 2)
        roff = pl.multiple_of((SEG * i + QOFF // 2) % EP, SEG) + j * (SEG // 2)
        arow = pl.multiple_of(2 * SEG * i, 2 * SEG) + j * SEG
        acc = [None] * NT
        ym, ps, ol, part, rest = {}, {}, {}, {}, {}
        HK = D // 2
        tiles = [_unpk(jnp.concatenate(
            [hx_v[k, j * (XR // 2):(j + 1) * (XR // 2), :] | zero, mem[k]], axis=0))
            for k in range(NT)]
        mem_new = []

        def lhs(lo, hi):
            return jnp.concatenate(tiles[lo // 128:hi // 128], axis=1)

        def qkv_lo(h, t):
            part[(t, h)] = _dot(lhs(0, HK), w_slab(2 * t + h // 16, h % 16, 0, HK))

        def proj(t, h):
            ch, l = 2 * t + h // 16, h % 16
            if (t, h) in part:
                y = _dot(lhs(HK, D), w_slab(ch, l, HK, D)) + part.pop((t, h))
            else:
                y = _dot(lhs(0, D), w_slab(ch, l))
            rg, ix = ring_of(ch, l)
            rg[pl.ds(ix + woff, XR // 2), :] = _pk(y[0:XR])
            ym[(t, h)] = y[XR:XR + MEM]

        def get(t, p):
            rg, i0 = ring_of(2 * t + p // 8, (2 * p) % 16)
            _, i1 = ring_of(2 * t + p // 8, (2 * p) % 16 + 1)
            mm = jnp.concatenate([ym.pop((t, 2 * p)), ym.pop((t, 2 * p + 1))], axis=0)
            return _unpk(jnp.concatenate(
                [rg[pl.ds(i0 + roff, SEG // 2), :], rg[pl.ds(i1 + roff, SEG // 2), :], _pk(mm)],
                axis=0))

        def sm(p):
            sc = lax.dot_general(get(0, p), get(1, p), (((1,), (1,)), ((), ())),
                                 preferred_element_type=f32)
            sc = jnp.where(mask, sc, fill)
            e = jnp.exp2((sc - jnp.max(sc, axis=-1, keepdims=True)) * (SCALE * LOG2E))
            ps[p] = (e * pl.reciprocal(jnp.sum(e, axis=-1, keepdims=True), approx=True)
                     ).astype(bf16)

        def pv(p):
            o = _dot(ps.pop(p), get(2, p))
            for b in range(2):
                h = 2 * p + b
                ox = o[SEG * b:SEG * (b + 1)]
                om = o[2 * SEG + MEM * b:2 * SEG + MEM * (b + 1)]
                if left is None:
                    ol[h] = jnp.concatenate([ox[0:XR], om], axis=0).astype(bf16)
                    rest[h] = ox[XR:SEG]
                else:
                    ol[h] = jnp.concatenate([ox, left[h], om], axis=0).astype(bf16)

        def wo(n, h0, h1, after=None):
            for h in range(h0, h1):
                o = ol[h]
                if after is not None and h == h0:
                    o = _unpk(_tie(pltpu.bitcast(o, u32), after))
                y = _dot(o, wo_v[h * DH:(h + 1) * DH, tile(n)])
                acc[n] = y if acc[n] is None else y + acc[n]
            if h1 == H:
                if left is None:
                    a_v[pl.ds(arow, XR), tile(n)] = acc[n][0:XR].astype(bf16)
                else:
                    a_v[pl.ds(arow, SEG), tile(n)] = acc[n][0:SEG].astype(bf16)
                    a_v[pl.ds(arow - (SEG - XR), SEG - XR), tile(n)] = (
                        acc[n][SEG:2 * SEG - XR].astype(bf16))
                mem_new.append(_pk(acc[n][-MEM:]))

        seq = []
        for p in range(NPAIR):
            seq += [(0, 2 * p), (1, 2 * p), (0, 2 * p + 1), (1, 2 * p + 1),
                    (2, 2 * p), (2, 2 * p + 1)]
        events = {}
        for p in range(NPAIR):
            at = seq.index((1, 2 * p + 1)) + DS
            events.setdefault(at, []).append((sm, p))
            events.setdefault(at + DP, []).append((pv, p))
        for t, h in seq[:NLO]:
            qkv_lo(h, t)
        side = {}
        if j == 1:
            macc = None
            for u in range(14):
                for g in range(u * 128 // 14, (u + 1) * 128 // 14):
                    wmg = wm_v[(i + 4) & 7, g * 8:(g + 1) * 8, :].astype(f32)
                    pr = wmg * jnp.concatenate([cb_v[g * 8:(g + 1) * 8, :]] * (MJ // 128), axis=1)
                    macc = pr if macc is None else macc + pr
                side[16 + u] = pltpu.bitcast(macc, u32)
            modr_v[i & 7] = jnp.broadcast_to(jnp.sum(macc, axis=0, keepdims=True), (8, MJ))
            nx = pl.multiple_of(PRE + 2 * XR * jnp.minimum(i + 1, NSEG // 2 - 1), RC)
            for q in range(2 * XR // RC):
                side[6 + 3 * q] = ride(nx + q * RC, q)
            tok = pl.multiple_of(jnp.clip(i - 22, 0, BM // RC) * RC, RC)
            side[15] = p0(tok, tok)
            for q in range(2 * NPC):
                mod_v[:, 2 * D + q * MJ:2 * D + (q + 1) * MJ] = modr_v[q]
        WU = HE // 8
        for d in range(len(seq) + NT * WU):
            if d < len(seq):
                proj(*seq[d])
            else:
                u = d - len(seq)
                wo(u // WU, (u % WU) * 8, (u % WU + 1) * 8, side.pop(u, None))
            for fn, p in events.pop(d, []):
                fn(p)
        assert not events
        u = NT * WU
        for n in range(NT):
            for h0 in range(HE, H, 8):
                wo(n, h0, h0 + 8, side.pop(u, None))
                u += 1
        assert not side
        return mem_new, rest

    def steps(i, carry):
        zero = zero_s[0].astype(u32)
        mem = [mem_v[:, tile(k)] for k in range(NT)]
        mem, rest = step(i, mem, zero, None)
        mem, _ = step(i, mem, zero, rest)
        for k in range(NT):
            mem_v[:, tile(k)] = mem[k]
        return carry
    lax.fori_loop(0, NSEG // 2, steps, 0)

    for cp in (w1_cp, w2_cp, w3_cp, w4_cp):
        cp.wait()

    for n in range(NT):
        g_v[n, 0:8, :] = jnp.zeros((8, 128), f32)
        g_v[n, 8:8 + SH, :] = _gelu(_dot(_unpk(y1_v[0:SH // 2, :]), w1_v[:, tile(n)]))

    HM = BM // 2
    shift = (-1, 1, -2, 2)

    def blk(j, c):
        r0 = pl.multiple_of(j * BM, BM)
        nxt = pl.multiple_of(jnp.minimum(j + 1, NB - 1) * BM + SH, SH)
        more = j < NB - 1

        def w1_half(hf):
            for n in range(NT):
                g = _gelu(_dot(_unpk(y1_v[8 + hf * 32:8 + (hf + 1) * 32, :]), w1_v[:, tile(n)]))
                w0 = 8 + SH + hf * HM
                if hf == 0:
                    g_v[n, w0:w0 + HM, :] = g
                else:
                    g_v[n, w0:w0 + HM - SH, :] = g[0:HM - SH]
                    g_v[n, w0 + HM - SH:w0 + HM, :] = jnp.where(more, g[HM - SH:HM], 0.0)

        def w2_half(hf):
            for n in range(NT):
                w0 = 8 + hf * HM + shift[n // 2]
                z_v[hf * 32:(hf + 1) * 32, tile(n)] = _pk(g_v[n, w0:w0 + HM, :])
            for n in range(NT):
                x1_v[hf * HM:(hf + 1) * HM, tile(n)] = (
                    _dot(_unpk(z_v[hf * 32:(hf + 1) * 32, :]), w2_v[:, tile(n)])
                    + hb_v[hf * HM:(hf + 1) * HM, tile(n)])

        def p1_half(hf):
            for k in range(hf * HM // RC, (hf + 1) * HM // RC):
                x1 = x1_v[k * RC:(k + 1) * RC, :]
                y2_v[k * 8:(k + 1) * 8, :] = _pk(_ln(x1))
                base_v[k * RC:(k + 1) * RC, :] = xa_v[k * RC:(k + 1) * RC, :] + mod(5) * x1

        def w3(f, lo, hi):
            u_v[lo:hi, tile(f)] = _pk(_gelu(_dot(_unpk(y2_v[lo:hi, :]), w3_v[:, tile(f)])))

        w1_half(0)
        w1_half(1)
        w2_half(0)
        w2_half(1)
        p1_half(0)
        for f in range(NSPLIT):
            w3(f, 0, 32)
        p1_half(1)
        for f in range(NSPLIT):
            w3(f, 32, 64)
        for n in range(NT):
            g_v[n, 0:8 + SH, :] = g_v[n, BM:BM + 8 + SH, :]
        xa_v[0:SH, :] = xa_v[BM:BM + SH, :]
        hb_v[0:SH, :] = hb_v[BM:BM + SH, :]
        for f in range(NSPLIT, NF):
            w3(f, 0, 64)
        ys = {}

        def prep(k):
            if k < BM // RC:
                ys[k] = p0(nxt + k * RC, SH + k * RC)

        prep(0)
        for n in range(NT):
            prep(n + 1)
            gb = mod(5, n * 128, (n + 1) * 128)
            u = _unpk(_tie(u_v[...], ys.pop(n), 16))
            a_v[pl.ds(r0, BM), tile(n)] = (
                base_v[:, tile(n)] + gb * _dot(u, w4_v[:, tile(n)])).astype(bf16)
            if n >= NT - 2:
                cols = pl.ds(0, (NT - 1) * 128) if n == NT - 2 else pl.ds(n * 128, 128)
                pltpu.make_async_copy(a_v.at[pl.ds(r0, BM), cols], out_hbm.at[pl.ds(r0, BM), cols],
                                      sem_out).start()
        return c
    lax.fori_loop(0, NB, blk, 0)
    pltpu.make_async_copy(a_v.at[pl.ds(0, S)], out_hbm, sem_out).wait()


@functools.partial(jax.jit, static_argnames=("A_seg_len",))
def pallas_adaLN_cond__memory_aug_recurrent_mem_tr__mixer_s_mlp__prompt_kernel(
    A_x: jax.Array,
    A_mem0: jax.Array,
    A_Wq: jax.Array,
    A_Wk: jax.Array,
    A_Wv: jax.Array,
    A_Wo: jax.Array,
    A_seg_len,
    B_x: jax.Array,
    B_w1: jax.Array,
    B_w2: jax.Array,
    B_w3: jax.Array,
    B_w4: jax.Array,
    c: jax.Array,
    w_mod: jax.Array,
):
    assert A_seg_len == SEG and A_x.shape == (1, S, D) and A_Wq.shape == (D, H, DH)
    any_spec = pl.BlockSpec(memory_space=pl.ANY)
    out = pl.pallas_call(
        _kernel,
        out_shape=jax.ShapeDtypeStruct((S, D), bf16),
        in_specs=[any_spec] * 12,
        out_specs=any_spec,
        scratch_shapes=[
            pltpu.VMEM((1, 3 * D), bf16),
            pltpu.VMEM((S + SH, D), bf16),
            pltpu.VMEM((S + SH, D), bf16),
            pltpu.VMEM((D // KP, PRE // 2, KP), u32),
            pltpu.VMEM((MEM // 2, D), u32),
            pltpu.VMEM((MEM, D), bf16),
            pltpu.VMEM((8, 6 * D), f32),
            pltpu.VMEM((8, 8, MJ), f32),
            pltpu.VMEM((D, 128), f32),
            pltpu.VMEM((8, D), u32),
            pltpu.VMEM((8, D, MJ), bf16),
            pltpu.VMEM((96 * PITCH + 544, 128), u32),
            pltpu.VMEM((H * DH, D + PADL), bf16),
            pltpu.VMEM((D, D + PADL), bf16),
            pltpu.VMEM((D, D + PADL), bf16),
            pltpu.VMEM((D, F + PADL), bf16),
            pltpu.VMEM((F, D + PADL), bf16),
            pltpu.VMEM((NT, BM + 32, 128), f32),
            pltpu.VMEM((BM + SH, D), f32),
            pltpu.VMEM((BM + SH, D), f32),
            pltpu.VMEM((BM, D), f32),
            pltpu.VMEM((BM, D), f32),
            pltpu.VMEM(((BM + SH) // 2, D), u32),
            pltpu.VMEM((BM // 2, D), u32),
            pltpu.VMEM((BM // 2, D), u32),
            pltpu.VMEM((BM // 2, F), u32),
            pltpu.VMEM((2, D, 16, DH), bf16),
            pltpu.VMEM((PRE, D), f32),
            pltpu.VMEM((NT, 32, 128), u32),
            pltpu.VMEM((H, PRE, DH), f32),
        ] + [pltpu.VMEM((12 * EP, DH), u32)] * 8 + [
            pltpu.SMEM((1,), jnp.int32),
            pltpu.SemaphoreType.DMA((2,)),
            pltpu.SemaphoreType.DMA((2, 4)),
            pltpu.SemaphoreType.DMA((4,)),
            pltpu.SemaphoreType.DMA((5,)),
            pltpu.SemaphoreType.DMA(()),
        ],
        compiler_params=pltpu.CompilerParams(vmem_limit_bytes=120 * 1024 * 1024),
    )(A_x.reshape(S, D), A_mem0.reshape(MEM, D), A_Wq, A_Wk, A_Wv, A_Wo.reshape(H * DH, D),
      B_w1, B_w2, B_w3, B_w4, c, w_mod)
    return out.reshape(1, S, D)
```

```python
import functools

import jax
import jax.numpy as jnp
from jax import lax
import jax.experimental.pallas as pl
import jax.experimental.pallas.tpu as pltpu

bf16, f32, u32 = jnp.bfloat16, jnp.float32, jnp.uint32

S, D, H, DH, MEM, SEG, F = 2048, 1024, 32, 128, 8, 32, 3584
NSEG = S // SEG
XR = 24
PRE = S - XR * NSEG
RING = 576
QOFF = RING - PRE
EP = RING // 2
PITCH = 520
NT = D // 128
NF = F // 128
BM = 128
NB = S // BM
NPAIR = H // 2
PADL = 128
SH = 16
KP = 256
MJ = 512
RC = 16
DS, DP = 5, 10
NLO = 6
HE = 16
NSPLIT = 7
EPS = 1e-5
LOG2E = 1.4426950408889634
SCALE = DH ** -0.5


def _ln(x):
    m = jnp.mean(x, axis=-1, keepdims=True)
    xc = x - m
    v = jnp.mean(xc * xc, axis=-1, keepdims=True)
    return xc * lax.rsqrt(v + EPS)


def _gelu(x):
    return jax.nn.gelu(x, approximate=True)


def _dot(a, b):
    return jnp.dot(a, b, preferred_element_type=f32)


def _pk(x):
    return pltpu.bitcast(x.astype(bf16), u32)


def _unpk(x):
    return pltpu.bitcast(x, bf16)


def _tie(w, after, k=0):
    if after is None:
        return w
    m = functools.reduce(lambda a, b: a & b,
                         [after[:, i * 128:(i + 1) * 128] for i in range(after.shape[1] // 128)])
    mf = pltpu.bitcast(m, f32)
    z = jnp.where(mf * mf < 0.0, jnp.uint32(1), jnp.uint32(0))
    parts = [w[0:8, k * 128:(k + 1) * 128] | z]
    if k > 0:
        parts.insert(0, w[0:8, :k * 128])
    if (k + 1) * 128 < w.shape[1]:
        parts.append(w[0:8, (k + 1) * 128:])
    row = jnp.concatenate(parts, axis=1)
    return jnp.concatenate([row, w[8:]], axis=0) if w.shape[0] > 8 else row


def _kernel(*refs):
    zero_s = refs[-6]
    zero_s[0] = 0

    def once(i, c):
        _kernel_body(*refs)
        return c
    lax.fori_loop(0, 1 + zero_s[0], once, 0)


def _kernel_body(x_hbm, mem0_hbm, wq_hbm, wk_hbm, wv_hbm, wo_hbm, w1_hbm, w2_hbm, w3_hbm, w4_hbm,
            c_hbm, wmod_hbm, out_hbm,
            c_v, x_v, a_v, h0_v, mem_v, mem0_v, mod_v, modr_v, cb_v, sc_v, wm_v, w_v, wo_v,
            w1_v, w2_v, w3_v, w4_v,
            g_v, xa_v, hb_v, base_v, x1_v, y1_v, z_v, y2_v, u_v,
            stage, xh_v, hx_v, acc_v,
            r0_, r1_, r2_, r3_, r4_, r5_, r6_, r7_,
            zero_s, sem_x, sem_stage, sem_mod, sem_w, sem_out):
    wqkv_hbm = (wq_hbm, wk_hbm, wv_hbm)
    rings = (r0_, r1_, r2_, r3_, r4_, r5_, r6_, r7_)

    c_cp = pltpu.make_async_copy(c_hbm, c_v.at[:, pl.ds(0, D)], sem_w.at[0])
    mem0_cp = pltpu.make_async_copy(mem0_hbm, mem0_v, sem_w.at[1])

    def x_cp(q):
        rows = pl.ds(q * PRE if isinstance(q, int) else pl.multiple_of(q * PRE, PRE), PRE)
        return pltpu.make_async_copy(x_hbm.at[rows], x_v.at[rows], sem_x.at[q & 1])

    def w_cp(src, dst, k):
        return pltpu.make_async_copy(src, dst.at[:, pl.ds(0, src.shape[1])], sem_w.at[k])

    wo_cp, w1_cp, w2_cp, w3_cp, w4_cp = (
        w_cp(a, b, k) for k, (a, b) in enumerate(
            ((wo_hbm, wo_v), (w1_hbm, w1_v), (w2_hbm, w2_v), (w3_hbm, w3_v), (w4_hbm, w4_v))))

    def mod0_cp(j, k):
        return pltpu.make_async_copy(wmod_hbm.at[:, pl.ds(j * D + k * KP, KP)],
                                     wm_v.at[k, :, pl.ds(j * KP, KP)], sem_mod.at[k])

    def mod1_cp(q):
        col = 2 * D + q * MJ
        col = col if isinstance(q, int) else pl.multiple_of(col, MJ)
        return pltpu.make_async_copy(wmod_hbm.at[:, pl.ds(col, MJ)], wm_v.at[(4 + q) & 7],
                                     sem_mod.at[q & 3])

    def stage_cp(t, hh, piece):
        d0 = piece * KP if isinstance(piece, int) else pl.multiple_of(piece * KP, KP)
        return pltpu.make_async_copy(
            wqkv_hbm[t].at[pl.ds(d0, KP), pl.ds(hh * 16, 16), :],
            stage.at[hh, pl.ds(d0, KP)], sem_stage.at[hh, piece])

    def tile(n):
        return slice(n * 128, (n + 1) * 128)

    def silu_c():
        cf = c_v[:, 0:D].astype(f32)
        return (cf * jax.nn.sigmoid(cf)).astype(bf16)

    def mod(k, lo=0, hi=D):
        return mod_v[0:1, k * D + lo:k * D + hi]

    def ride(tok, q):
        xs = x_v[pl.ds(tok, RC), :].astype(f32)
        hx = _pk(_ln(xs) * (1.0 + mod(1)) + mod(0))
        for n in range(NT):
            hx_v[n, q * 8:(q + 1) * 8, :] = hx[:, tile(n)]
        return hx

    def repack(hh, ch, p0, n, anchor=False):
        both = None
        for u in range(n):
            p = p0 + u
            a = pltpu.bitcast(stage[hh, 2 * p], u32)
            b = pltpu.bitcast(stage[hh, 2 * p + 1], u32)
            ev = (a & jnp.uint32(0xFFFF)) | (b << 16)
            od = (a >> 16) | (b & jnp.uint32(0xFFFF0000))
            w_v[pl.ds(ch * (16 * PITCH) + p, 8, stride=PITCH), :] = ev
            w_v[pl.ds(ch * (16 * PITCH) + 8 * PITCH + p, 8, stride=PITCH), :] = od
            if anchor:
                both = ev & od if both is None else both & ev & od
        return both

    def w_slab(ch, l, lo=0, hi=D):
        base = (ch * 16 + (l % 2) * 8 + l // 2) * PITCH + lo // 2
        return _unpk(w_v[base:base + (hi - lo) // 2, :])

    def ring_of(ch, l):
        return rings[l // 2], (ch * 2 + l % 2) * EP

    x_cp(0).start()
    c_cp.start()
    mem0_cp.start()
    stage_cp(0, 0, 0).start()
    mod0_cp(0, 0).start()
    mod0_cp(1, 0).start()
    x_v[S:S + SH, :] = jnp.zeros((SH, D), bf16)
    a_v[S:S + SH, :] = jnp.zeros((SH, D), bf16)
    mod_v[...] = jnp.zeros(mod_v.shape, f32)
    modr_v[...] = jnp.zeros(modr_v.shape, f32)
    x_cp(0).wait()
    stage_cp(0, 1, 0).start()

    def xhat_body(i, c):
        r0 = pl.multiple_of(i * 64, 64)
        for u in range(4):
            rows = pl.ds(r0 + RC * u, RC)
            xh_v[rows, :] = _ln(x_v[rows, :].astype(f32))
        return c
    lax.fori_loop(0, PRE // 64, xhat_body, 0)

    c_cp.wait()
    mem0_cp.wait()
    mem_v[...] = pltpu.bitcast(mem0_v[...], u32)
    sc_v[...] = _pk(jnp.broadcast_to(silu_c().astype(f32), (16, D)))
    stage_cp(0, 0, 0).wait()

    def first_repack(i, c):
        repack(0, 0, i * 16, 16)
        return c
    lax.fori_loop(0, KP // 32, first_repack, 0)

    NPC = D // KP
    assert NPC == 4

    def modulate(kk):
        mod0_cp(0, kk).wait()
        mod0_cp(1, kk).wait()
        if kk == 2:
            stage_cp(0, 0, 2).wait()
        if kk == 3:
            x_cp(1).wait()
        for e in range(KP // 128):
            m = []
            for j in range(2):
                m.append(_dot(_unpk(sc_v[...]), wm_v[kk, :, tile(2 * j + e)])[0:8])
                col = j * D + kk * KP + e * 128
                mod_v[:, col:col + 128] = m[j]
            cols = slice(kk * KP + e * 128, kk * KP + (e + 1) * 128)
            for q in range(PRE // 64):
                ca = m[1]
                if kk == 2:
                    rp = repack(0, 0, KP + (e * 8 + q) * 8, 8, anchor=True)
                    ca = pltpu.bitcast(_tie(pltpu.bitcast(ca, u32), rp), f32)
                h0_v[kk, q * 32:(q + 1) * 32, tile(e)] = _pk(
                    xh_v[q * 64:(q + 1) * 64, cols] * (1.0 + ca[0:1]) + m[0][0:1])
        if kk == 0:
            stage_cp(0, 0, 1).start()
        if kk + 1 < NPC:
            mod0_cp(0, kk + 1).start()
            mod0_cp(1, kk + 1).start()
        stage_cp((kk + 1) // NPC, 1, (kk + 1) % NPC).start()
        if kk > 0:
            stage_cp((kk + 2) // NPC, 0, (kk + 2) % NPC).start()
        if kk == 2:
            x_cp(1).start()
        if kk == 3:
            stage_cp(1, 1, 1).start()
            stage_cp(1, 0, 2).start()

    def first_heads(h0, h1, side):
        for h in range(h0, h1):
            w = w_slab(h // 16, h % 16, 0, KP)
            for rb in range(PRE // BM):
                acc_v[h, rb * BM:(rb + 1) * BM, :] = _dot(
                    _unpk(h0_v[0, rb * 64:(rb + 1) * 64, :]), w)
            if side is not None and h < h1 - 1:
                lo, hi = (h - h0) * 128 // (h1 - h0 - 1), (h + 1 - h0) * 128 // (h1 - h0 - 1)
                side(lo, hi - lo)

    modulate(0)
    first_heads(0, 8, None)
    cb_v[...] = jnp.transpose(jnp.broadcast_to(silu_c().astype(f32), (128, D)))
    stage_cp(0, 1, 0).wait()
    first_heads(8, 16, lambda p, n: repack(1, 1 + zero_s[0], p, n))
    stage_cp(0, 0, 1).wait()
    first_heads(16, 32, lambda p, n: repack(0, zero_s[0], KP // 2 + p, n))
    stage_cp(0, 0, 2).start()

    def pre_body(i, c):
        t, k = i >> 2, i & 3
        fresh = jnp.logical_and(i > 1, i < 3 * NPC - 1)
        i1 = jnp.where(fresh, i + 1, i)
        t1, k1 = i1 >> 2, i1 & 3

        @pl.when(i < NPC)
        def _():
            for kk in range(1, NPC):
                pl.when(i == kk)(functools.partial(modulate, kk))

        stage_cp(0, 1, k).wait()

        @pl.when(fresh)
        def _():
            stage_cp(0, 0, k1).wait()

        w0 = pl.multiple_of(t * (32 * PITCH) + k * (KP // 2), 32)
        xrow = pl.multiple_of(jnp.where(i >= NPC - 1, PRE, 0), PRE)
        done = {}
        nd = 0
        for h in range(H):
            hh, l = h // 16, h % 16
            w = _unpk(w_v[pl.ds(w0 + (hh * 16 + (l % 2) * 8 + l // 2) * PITCH, KP // 2), :])
            q0 = pl.multiple_of(t * (4 * EP), 32) + ring_of(hh, l)[1] + QOFF // 2
            for rb in range(PRE // BM):
                lhs = _tie(h0_v[k, rb * 64:(rb + 1) * 64, :], done.pop(nd, None))
                rows = slice(rb * BM, (rb + 1) * BM)
                y = _dot(_unpk(lhs), w) + jnp.where(k > 0, acc_v[h, rows, :], 0.0)
                acc_v[h, rows, :] = y
                rings[l // 2][pl.ds(q0 + rb * 64, 64), :] = _pk(y)
                nd += 1
            if l < 15:
                n = 9 if l < 8 else 8
                p0_ = l * 9 if l < 8 else 72 + (l - 8) * 8
                if hh == 0:
                    repack(1, 2 * t + 1 + zero_s[0], k * (KP // 2) + p0_, n)
                else:
                    repack(0, 2 * t1, k1 * (KP // 2) + p0_, n)
            if h % 4 == 1 and h < 12:
                done[nd + 16] = ride(xrow + (h // 4) * RC, h // 4)
        @pl.when(jnp.logical_or(i == 4, i == 5))
        def _():
            x_cp(i - 2).start()

        for tt in range(1, 3):
            @pl.when(jnp.logical_and(i >= 3, (i + 3) >> 2 == tt))
            def _():
                stage_cp(tt, 1, (i + 3) & 3).start()

            @pl.when(jnp.logical_and(i >= 3, t + 1 == tt))
            def _():
                stage_cp(tt, 0, k).start()

        @pl.when(jnp.logical_and(i >= 3, i <= 10))
        def _():
            mod1_cp(i - 3).start()

        @pl.when(i == 7)
        def _():
            wo_cp.start()
        return c
    lax.fori_loop(1, 3 * NPC, pre_body, 0)

    for cp in (w1_cp, w2_cp, w3_cp, w4_cp):
        cp.start()
    for q in range(2 * NPC):
        mod1_cp(q).wait()
    x_cp(2).wait()
    x_cp(3).wait()
    wo_cp.wait()

    L2 = 2 * (SEG + MEM)
    r = lax.broadcasted_iota(jnp.int32, (L2, L2), 0)
    c = lax.broadcasted_iota(jnp.int32, (L2, L2), 1)
    r1 = ((r >= SEG) & (r < 2 * SEG)) | (r >= 2 * SEG + MEM)
    c1 = ((c >= SEG) & (c < 2 * SEG)) | (c >= 2 * SEG + MEM)
    same = r1 == c1
    mask = same & ((r >= 2 * SEG) | (c >= 2 * SEG) | (c <= r))
    fill = jnp.where(same, -1e9 / SCALE, -jnp.inf).astype(f32)

    def p0(tok, w):
        rows = pl.ds(tok, RC)
        xa = x_v[rows, :].astype(f32) + mod(2) * a_v[rows, :].astype(f32)
        hb = _ln(xa) * (1.0 + mod(4)) + mod(3)
        xa_v[pl.ds(w, RC), :] = xa
        hb_v[pl.ds(w, RC), :] = hb
        y = _pk(_ln(hb))
        y1_v[pl.ds(w // 2 if isinstance(w, int) else pl.multiple_of(w >> 1, 8), RC // 2), :] = y
        return y

    def step(i, mem, zero, left):
        j = 0 if left is None else 1
        woff = pl.multiple_of((XR * i) % EP, 8) + j * (XR // 2)
        roff = pl.multiple_of((SEG * i + QOFF // 2) % EP, SEG) + j * (SEG // 2)
        arow = pl.multiple_of(2 * SEG * i, 2 * SEG) + j * SEG
        acc = [None] * NT
        ym, ps, ol, part, rest = {}, {}, {}, {}, {}
        HK = D // 2
        tiles = [_unpk(jnp.concatenate(
            [hx_v[k, j * (XR // 2):(j + 1) * (XR // 2), :] | zero, mem[k]], axis=0))
            for k in range(NT)]
        mem_new = []

        def lhs(lo, hi):
            return jnp.concatenate(tiles[lo // 128:hi // 128], axis=1)

        def qkv_lo(h, t):
            part[(t, h)] = _dot(lhs(0, HK), w_slab(2 * t + h // 16, h % 16, 0, HK))

        def proj(t, h):
            ch, l = 2 * t + h // 16, h % 16
            if (t, h) in part:
                y = _dot(lhs(HK, D), w_slab(ch, l, HK, D)) + part.pop((t, h))
            else:
                y = _dot(lhs(0, D), w_slab(ch, l))
            rg, ix = ring_of(ch, l)
            rg[pl.ds(ix + woff, XR // 2), :] = _pk(y[0:XR])
            ym[(t, h)] = y[XR:XR + MEM]

        def get(t, p):
            rg, i0 = ring_of(2 * t + p // 8, (2 * p) % 16)
            _, i1 = ring_of(2 * t + p // 8, (2 * p) % 16 + 1)
            mm = jnp.concatenate([ym.pop((t, 2 * p)), ym.pop((t, 2 * p + 1))], axis=0)
            return _unpk(jnp.concatenate(
                [rg[pl.ds(i0 + roff, SEG // 2), :], rg[pl.ds(i1 + roff, SEG // 2), :], _pk(mm)],
                axis=0))

        def sm(p):
            sc = lax.dot_general(get(0, p), get(1, p), (((1,), (1,)), ((), ())),
                                 preferred_element_type=f32)
            sc = jnp.where(mask, sc, fill)
            e = jnp.exp2((sc - jnp.max(sc, axis=-1, keepdims=True)) * (SCALE * LOG2E))
            ps[p] = (e * pl.reciprocal(jnp.sum(e, axis=-1, keepdims=True), approx=True)
                     ).astype(bf16)

        def pv(p):
            o = _dot(ps.pop(p), get(2, p))
            for b in range(2):
                h = 2 * p + b
                ox = o[SEG * b:SEG * (b + 1)]
                om = o[2 * SEG + MEM * b:2 * SEG + MEM * (b + 1)]
                if left is None:
                    ol[h] = jnp.concatenate([ox[0:XR], om], axis=0).astype(bf16)
                    rest[h] = ox[XR:SEG]
                else:
                    ol[h] = jnp.concatenate([ox, left[h], om], axis=0).astype(bf16)

        def wo(n, h0, h1, after=None):
            for h in range(h0, h1):
                o = ol[h]
                if after is not None and h == h0:
                    o = _unpk(_tie(pltpu.bitcast(o, u32), after))
                y = _dot(o, wo_v[h * DH:(h + 1) * DH, tile(n)])
                acc[n] = y if acc[n] is None else y + acc[n]
            if h1 == H:
                if left is None:
                    a_v[pl.ds(arow, XR), tile(n)] = acc[n][0:XR].astype(bf16)
                else:
                    a_v[pl.ds(arow, SEG), tile(n)] = acc[n][0:SEG].astype(bf16)
                    a_v[pl.ds(arow - (SEG - XR), SEG - XR), tile(n)] = (
                        acc[n][SEG:2 * SEG - XR].astype(bf16))
                mem_new.append(_pk(acc[n][-MEM:]))

        seq = []
        for p in range(NPAIR):
            seq += [(0, 2 * p), (1, 2 * p), (0, 2 * p + 1), (1, 2 * p + 1),
                    (2, 2 * p), (2, 2 * p + 1)]
        events = {}
        for p in range(NPAIR):
            at = seq.index((1, 2 * p + 1)) + DS
            events.setdefault(at, []).append((sm, p))
            events.setdefault(at + DP, []).append((pv, p))
        for t, h in seq[:NLO]:
            qkv_lo(h, t)
        side = {}
        if j == 1:
            macc = None
            for u in range(14):
                for g in range(u * 128 // 14, (u + 1) * 128 // 14):
                    wmg = wm_v[(i + 4) & 7, g * 8:(g + 1) * 8, :].astype(f32)
                    pr = wmg * jnp.concatenate([cb_v[g * 8:(g + 1) * 8, :]] * (MJ // 128), axis=1)
                    macc = pr if macc is None else macc + pr
                side[16 + u] = pltpu.bitcast(macc, u32)
            modr_v[i & 7] = jnp.broadcast_to(jnp.sum(macc, axis=0, keepdims=True), (8, MJ))
            nx = pl.multiple_of(PRE + 2 * XR * jnp.minimum(i + 1, NSEG // 2 - 1), RC)
            for q in range(2 * XR // RC):
                side[6 + 3 * q] = ride(nx + q * RC, q)
            tok = pl.multiple_of(jnp.clip(i - 22, 0, BM // RC) * RC, RC)
            side[15] = p0(tok, tok)
            for q in range(2 * NPC):
                mod_v[:, 2 * D + q * MJ:2 * D + (q + 1) * MJ] = modr_v[q]
        WU = HE // 8
        for d in range(len(seq) + NT * WU):
            if d < len(seq):
                proj(*seq[d])
            else:
                u = d - len(seq)
                wo(u // WU, (u % WU) * 8, (u % WU + 1) * 8, side.pop(u, None))
            for fn, p in events.pop(d, []):
                fn(p)
        assert not events
        u = NT * WU
        for n in range(NT):
            for h0 in range(HE, H, 8):
                wo(n, h0, h0 + 8, side.pop(u, None))
                u += 1
        assert not side
        return mem_new, rest

    def steps(i, carry):
        zero = zero_s[0].astype(u32)
        mem = [mem_v[:, tile(k)] for k in range(NT)]
        mem, rest = step(i, mem, zero, None)
        mem, _ = step(i, mem, zero, rest)
        for k in range(NT):
            mem_v[:, tile(k)] = mem[k]
        return carry
    lax.fori_loop(0, NSEG // 2, steps, 0)

    for cp in (w1_cp, w2_cp, w3_cp, w4_cp):
        cp.wait()

    for n in range(NT):
        g_v[n, 0:8, :] = jnp.zeros((8, 128), f32)
        g_v[n, 8:8 + SH, :] = _gelu(_dot(_unpk(y1_v[0:SH // 2, :]), w1_v[:, tile(n)]))

    HM = BM // 2
    shift = (-1, 1, -2, 2)

    def blk(j, c):
        r0 = pl.multiple_of(j * BM, BM)
        nxt = pl.multiple_of(jnp.minimum(j + 1, NB - 1) * BM + SH, SH)
        more = j < NB - 1

        def w1_half(hf):
            for n in range(NT):
                g = _gelu(_dot(_unpk(y1_v[8 + hf * 32:8 + (hf + 1) * 32, :]), w1_v[:, tile(n)]))
                w0 = 8 + SH + hf * HM
                if hf == 0:
                    g_v[n, w0:w0 + HM, :] = g
                else:
                    g_v[n, w0:w0 + HM - SH, :] = g[0:HM - SH]
                    g_v[n, w0 + HM - SH:w0 + HM, :] = jnp.where(more, g[HM - SH:HM], 0.0)

        def w2_half(hf):
            for n in range(NT):
                w0 = 8 + hf * HM + shift[n // 2]
                z_v[hf * 32:(hf + 1) * 32, tile(n)] = _pk(g_v[n, w0:w0 + HM, :])
            for n in range(NT):
                x1_v[hf * HM:(hf + 1) * HM, tile(n)] = (
                    _dot(_unpk(z_v[hf * 32:(hf + 1) * 32, :]), w2_v[:, tile(n)])
                    + hb_v[hf * HM:(hf + 1) * HM, tile(n)])

        def p1_half(hf):
            for k in range(hf * HM // RC, (hf + 1) * HM // RC):
                x1 = x1_v[k * RC:(k + 1) * RC, :]
                y2_v[k * 8:(k + 1) * 8, :] = _pk(_ln(x1))
                base_v[k * RC:(k + 1) * RC, :] = xa_v[k * RC:(k + 1) * RC, :] + mod(5) * x1

        def w3(f, lo, hi):
            u_v[lo:hi, tile(f)] = _pk(_gelu(_dot(_unpk(y2_v[lo:hi, :]), w3_v[:, tile(f)])))

        w1_half(0)
        w1_half(1)
        w2_half(0)
        w2_half(1)
        p1_half(0)
        for f in range(NSPLIT):
            w3(f, 0, 32)
        p1_half(1)
        for f in range(NSPLIT):
            w3(f, 32, 64)
        for n in range(NT):
            g_v[n, 0:8 + SH, :] = g_v[n, BM:BM + 8 + SH, :]
        xa_v[0:SH, :] = xa_v[BM:BM + SH, :]
        hb_v[0:SH, :] = hb_v[BM:BM + SH, :]
        for f in range(NSPLIT, NF):
            w3(f, 0, 64)
        ys = {}

        def prep(k):
            if k < BM // RC:
                ys[k] = p0(nxt + k * RC, SH + k * RC)

        prep(0)
        for n in range(NT):
            prep(n + 1)
            gb = mod(5, n * 128, (n + 1) * 128)
            u = _unpk(_tie(u_v[...], ys.pop(n), 16))
            a_v[pl.ds(r0, BM), tile(n)] = (
                base_v[:, tile(n)] + gb * _dot(u, w4_v[:, tile(n)])).astype(bf16)
            if n >= NT - 2:
                cols = pl.ds(0, (NT - 1) * 128) if n == NT - 2 else pl.ds(n * 128, 128)
                pltpu.make_async_copy(a_v.at[pl.ds(r0, BM), cols], out_hbm.at[pl.ds(r0, BM), cols],
                                      sem_out).start()
        return c
    lax.fori_loop(0, NB, blk, 0)
    pltpu.make_async_copy(a_v.at[pl.ds(0, S)], out_hbm, sem_out).wait()


@functools.partial(jax.jit, static_argnames=("A_seg_len",))
def pallas_adaLN_cond__memory_aug_recurrent_mem_tr__mixer_s_mlp__prompt_kernel(
    A_x: jax.Array,
    A_mem0: jax.Array,
    A_Wq: jax.Array,
    A_Wk: jax.Array,
    A_Wv: jax.Array,
    A_Wo: jax.Array,
    A_seg_len,
    B_x: jax.Array,
    B_w1: jax.Array,
    B_w2: jax.Array,
    B_w3: jax.Array,
    B_w4: jax.Array,
    c: jax.Array,
    w_mod: jax.Array,
):
    assert A_seg_len == SEG and A_x.shape == (1, S, D) and A_Wq.shape == (D, H, DH)
    any_spec = pl.BlockSpec(memory_space=pl.ANY)
    out = pl.pallas_call(
        _kernel,
        out_shape=jax.ShapeDtypeStruct((S, D), bf16),
        in_specs=[any_spec] * 12,
        out_specs=any_spec,
        scratch_shapes=[
            pltpu.VMEM((1, 3 * D), bf16),
            pltpu.VMEM((S + SH, D), bf16),
            pltpu.VMEM((S + SH, D), bf16),
            pltpu.VMEM((D // KP, PRE // 2, KP), u32),
            pltpu.VMEM((MEM // 2, D), u32),
            pltpu.VMEM((MEM, D), bf16),
            pltpu.VMEM((8, 6 * D), f32),
            pltpu.VMEM((8, 8, MJ), f32),
            pltpu.VMEM((D, 128), f32),
            pltpu.VMEM((8, D), u32),
            pltpu.VMEM((8, D, MJ), bf16),
            pltpu.VMEM((96 * PITCH + 544, 128), u32),
            pltpu.VMEM((H * DH, D + PADL), bf16),
            pltpu.VMEM((D, D + PADL), bf16),
            pltpu.VMEM((D, D + PADL), bf16),
            pltpu.VMEM((D, F + PADL), bf16),
            pltpu.VMEM((F, D + PADL), bf16),
            pltpu.VMEM((NT, BM + 32, 128), f32),
            pltpu.VMEM((BM + SH, D), f32),
            pltpu.VMEM((BM + SH, D), f32),
            pltpu.VMEM((BM, D), f32),
            pltpu.VMEM((BM, D), f32),
            pltpu.VMEM(((BM + SH) // 2, D), u32),
            pltpu.VMEM((BM // 2, D), u32),
            pltpu.VMEM((BM // 2, D), u32),
            pltpu.VMEM((BM // 2, F), u32),
            pltpu.VMEM((2, D, 16, DH), bf16),
            pltpu.VMEM((PRE, D), f32),
            pltpu.VMEM((NT, 32, 128), u32),
            pltpu.VMEM((H, PRE, DH), f32),
        ] + [pltpu.VMEM((12 * EP, DH), u32)] * 8 + [
            pltpu.SMEM((1,), jnp.int32),
            pltpu.SemaphoreType.DMA((2,)),
            pltpu.SemaphoreType.DMA((2, 4)),
            pltpu.SemaphoreType.DMA((4,)),
            pltpu.SemaphoreType.DMA((5,)),
            pltpu.SemaphoreType.DMA(()),
        ],
        compiler_params=pltpu.CompilerParams(vmem_limit_bytes=120 * 1024 * 1024),
    )(A_x.reshape(S, D), A_mem0.reshape(MEM, D), A_Wq, A_Wk, A_Wv, A_Wo.reshape(H * DH, D),
      B_w1, B_w2, B_w3, B_w4, c, w_mod)
    return out.reshape(1, S, D)
```

```python
import functools

import jax
import jax.numpy as jnp
from jax import lax
import jax.experimental.pallas as pl
import jax.experimental.pallas.tpu as pltpu

bf16, f32, u32 = jnp.bfloat16, jnp.float32, jnp.uint32

S, D, H, DH, MEM, SEG, F = 2048, 1024, 32, 128, 8, 32, 3584
NSEG = S // SEG
XR = 24
PRE = S - XR * NSEG
RING = 576
QOFF = RING - PRE
EP = RING // 2
PITCH = 520
NT = D // 128
NF = F // 128
BM = 128
NB = S // BM
NPAIR = H // 2
PADL = 128
SH = 16
KP = 256
MJ = 512
RC = 16
DS, DP = 5, 10
NLO = 6
HE = 16
NSPLIT = 7
EPS = 1e-5
LOG2E = 1.4426950408889634
SCALE = DH ** -0.5


def _ln(x):
    m = jnp.mean(x, axis=-1, keepdims=True)
    xc = x - m
    v = jnp.mean(xc * xc, axis=-1, keepdims=True)
    return xc * lax.rsqrt(v + EPS)


def _gelu(x):
    return jax.nn.gelu(x, approximate=True)


def _dot(a, b):
    return jnp.dot(a, b, preferred_element_type=f32)


def _pk(x):
    return pltpu.bitcast(x.astype(bf16), u32)


def _unpk(x):
    return pltpu.bitcast(x, bf16)


def _tie(w, after, k=0):
    if after is None:
        return w
    m = functools.reduce(lambda a, b: a & b,
                         [after[:, i * 128:(i + 1) * 128] for i in range(after.shape[1] // 128)])
    mf = pltpu.bitcast(m, f32)
    z = jnp.where(mf * mf < 0.0, jnp.uint32(1), jnp.uint32(0))
    parts = [w[0:8, k * 128:(k + 1) * 128] | z]
    if k > 0:
        parts.insert(0, w[0:8, :k * 128])
    if (k + 1) * 128 < w.shape[1]:
        parts.append(w[0:8, (k + 1) * 128:])
    row = jnp.concatenate(parts, axis=1)
    return jnp.concatenate([row, w[8:]], axis=0) if w.shape[0] > 8 else row


def _kernel(*refs):
    zero_s = refs[-6]
    zero_s[0] = 0

    def once(i, c):
        _kernel_body(*refs)
        return c
    lax.fori_loop(0, 1 + zero_s[0], once, 0)


def _kernel_body(x_hbm, mem0_hbm, wq_hbm, wk_hbm, wv_hbm, wo_hbm, w1_hbm, w2_hbm, w3_hbm, w4_hbm,
            c_hbm, wmod_hbm, out_hbm,
            c_v, x_v, a_v, h0_v, mem_v, mem0_v, mod_v, modr_v, cb_v, sc_v, wm_v, w_v, wo_v,
            w1_v, w2_v, w3_v, w4_v,
            g_v, xa_v, hb_v, base_v, x1_v, y1_v, z_v, y2_v, u_v,
            stage, xh_v, hx_v, acc_v,
            r0_, r1_, r2_, r3_, r4_, r5_, r6_, r7_,
            zero_s, sem_x, sem_stage, sem_mod, sem_w, sem_out):
    wqkv_hbm = (wq_hbm, wk_hbm, wv_hbm)
    rings = (r0_, r1_, r2_, r3_, r4_, r5_, r6_, r7_)

    c_cp = pltpu.make_async_copy(c_hbm, c_v.at[:, pl.ds(0, D)], sem_w.at[0])
    mem0_cp = pltpu.make_async_copy(mem0_hbm, mem0_v, sem_w.at[1])

    def x_cp(q):
        rows = pl.ds(q * PRE if isinstance(q, int) else pl.multiple_of(q * PRE, PRE), PRE)
        return pltpu.make_async_copy(x_hbm.at[rows], x_v.at[rows], sem_x.at[q & 1])

    def w_cp(src, dst, k):
        return pltpu.make_async_copy(src, dst.at[:, pl.ds(0, src.shape[1])], sem_w.at[k])

    w1_cp, w2_cp, w3_cp, w4_cp = (
        w_cp(a, b, k + 1) for k, (a, b) in enumerate(
            ((w1_hbm, w1_v), (w2_hbm, w2_v), (w3_hbm, w3_v), (w4_hbm, w4_v))))

    def wo_cp(half):
        rows = pl.ds(half * (H * DH // 2), H * DH // 2)
        return w_cp(wo_hbm.at[rows], wo_v.at[rows], 0)

    def mod0_cp(j, k):
        return pltpu.make_async_copy(wmod_hbm.at[:, pl.ds(j * D + k * KP, KP)],
                                     wm_v.at[k, :, pl.ds(j * KP, KP)], sem_mod.at[k])

    def mod1_cp(q):
        col = 2 * D + q * MJ
        col = col if isinstance(q, int) else pl.multiple_of(col, MJ)
        return pltpu.make_async_copy(wmod_hbm.at[:, pl.ds(col, MJ)], wm_v.at[(4 + q) & 7],
                                     sem_mod.at[q & 3])

    def stage_cp(t, hh, piece):
        d0 = piece * KP if isinstance(piece, int) else pl.multiple_of(piece * KP, KP)
        return pltpu.make_async_copy(
            wqkv_hbm[t].at[pl.ds(d0, KP), pl.ds(hh * 16, 16), :],
            stage.at[hh, pl.ds(d0, KP)], sem_stage.at[hh, piece])

    def tile(n):
        return slice(n * 128, (n + 1) * 128)

    def silu_c():
        cf = c_v[:, 0:D].astype(f32)
        return (cf * jax.nn.sigmoid(cf)).astype(bf16)

    def mod(k, lo=0, hi=D):
        return mod_v[0:1, k * D + lo:k * D + hi]

    def ride(tok, q):
        xs = x_v[pl.ds(tok, RC), :].astype(f32)
        hx = _pk(_ln(xs) * (1.0 + mod(1)) + mod(0))
        for n in range(NT):
            hx_v[n, q * 8:(q + 1) * 8, :] = hx[:, tile(n)]
        return hx

    def repack(hh, ch, p0, n, anchor=False):
        both = None
        for u in range(n):
            p = p0 + u
            a = pltpu.bitcast(stage[hh, 2 * p], u32)
            b = pltpu.bitcast(stage[hh, 2 * p + 1], u32)
            ev = (a & jnp.uint32(0xFFFF)) | (b << 16)
            od = (a >> 16) | (b & jnp.uint32(0xFFFF0000))
            w_v[pl.ds(ch * (16 * PITCH) + p, 8, stride=PITCH), :] = ev
            w_v[pl.ds(ch * (16 * PITCH) + 8 * PITCH + p, 8, stride=PITCH), :] = od
            if anchor:
                both = ev & od if both is None else both & ev & od
        return both

    def w_slab(ch, l, lo=0, hi=D):
        base = (ch * 16 + (l % 2) * 8 + l // 2) * PITCH + lo // 2
        return _unpk(w_v[base:base + (hi - lo) // 2, :])

    def ring_of(ch, l):
        return rings[l // 2], (ch * 2 + l % 2) * EP

    x_cp(0).start()
    c_cp.start()
    mem0_cp.start()
    stage_cp(0, 0, 0).start()
    mod0_cp(0, 0).start()
    mod0_cp(1, 0).start()
    x_v[S:S + SH, :] = jnp.zeros((SH, D), bf16)
    a_v[S:S + SH, :] = jnp.zeros((SH, D), bf16)
    mod_v[...] = jnp.zeros(mod_v.shape, f32)
    modr_v[...] = jnp.zeros(modr_v.shape, f32)
    x_cp(0).wait()
    stage_cp(0, 1, 0).start()

    def xhat_body(i, c):
        r0 = pl.multiple_of(i * 64, 64)
        for u in range(4):
            rows = pl.ds(r0 + RC * u, RC)
            xh_v[rows, :] = _ln(x_v[rows, :].astype(f32))
        return c
    lax.fori_loop(0, PRE // 64, xhat_body, 0)

    c_cp.wait()
    mem0_cp.wait()
    mem_v[...] = pltpu.bitcast(mem0_v[...], u32)
    sc_v[...] = _pk(jnp.broadcast_to(silu_c().astype(f32), (16, D)))
    stage_cp(0, 0, 0).wait()

    def first_repack(i, c):
        repack(0, 0, i * 16, 16)
        return c
    lax.fori_loop(0, KP // 32, first_repack, 0)

    NPC = D // KP
    assert NPC == 4

    def modulate(kk):
        mod0_cp(0, kk).wait()
        mod0_cp(1, kk).wait()
        if kk == 2:
            stage_cp(0, 0, 2).wait()
        if kk == 3:
            x_cp(1).wait()
        if kk == 0:
            stage_cp(0, 0, 1).start()
        else:
            if kk + 1 < NPC:
                mod0_cp(0, kk + 1).start()
                mod0_cp(1, kk + 1).start()
            stage_cp((kk + 1) // NPC, 1, (kk + 1) % NPC).start()
            stage_cp((kk + 2) // NPC, 0, (kk + 2) % NPC).start()
        if kk == 2:
            x_cp(1).start()
        if kk == 3:
            stage_cp(1, 1, 1).start()
            stage_cp(1, 0, 2).start()
        for e in range(KP // 128):
            m = []
            for j in range(2):
                m.append(_dot(_unpk(sc_v[...]), wm_v[kk, :, tile(2 * j + e)])[0:8])
                col = j * D + kk * KP + e * 128
                mod_v[:, col:col + 128] = m[j]
            cols = slice(kk * KP + e * 128, kk * KP + (e + 1) * 128)
            for q in range(PRE // 64):
                ca = m[1]
                if kk == 2:
                    rp = repack(0, 0, KP + (e * 8 + q) * 8, 8, anchor=True)
                    ca = pltpu.bitcast(_tie(pltpu.bitcast(ca, u32), rp), f32)
                h0_v[kk, q * 32:(q + 1) * 32, tile(e)] = _pk(
                    xh_v[q * 64:(q + 1) * 64, cols] * (1.0 + ca[0:1]) + m[0][0:1])

    def first_heads(h0, h1, side):
        for h in range(h0, h1):
            w = w_slab(h // 16, h % 16, 0, KP)
            for rb in range(PRE // BM):
                acc_v[h, rb * BM:(rb + 1) * BM, :] = _dot(
                    _unpk(h0_v[0, rb * 64:(rb + 1) * 64, :]), w)
            if side is not None and h < h1 - 1:
                lo, hi = (h - h0) * 128 // (h1 - h0 - 1), (h + 1 - h0) * 128 // (h1 - h0 - 1)
                side(lo, hi - lo)
            if h == 25:
                stage_cp(0, 0, 2).start()

    modulate(0)
    first_heads(0, 8, None)
    cb_v[...] = jnp.transpose(jnp.broadcast_to(silu_c().astype(f32), (128, D)))
    stage_cp(0, 1, 0).wait()
    mod0_cp(0, 1).start()
    mod0_cp(1, 1).start()
    stage_cp(0, 1, 1).start()
    first_heads(8, 16, lambda p, n: repack(1, 1 + zero_s[0], p, n))
    stage_cp(0, 0, 1).wait()
    first_heads(16, 32, lambda p, n: repack(0, zero_s[0], KP // 2 + p, n))

    def pre_body(i, c):
        t, k = i >> 2, i & 3
        fresh = jnp.logical_and(i > 1, i < 3 * NPC - 1)
        i1 = jnp.where(fresh, i + 1, i)
        t1, k1 = i1 >> 2, i1 & 3

        @pl.when(i < NPC)
        def _():
            for kk in range(1, NPC):
                pl.when(i == kk)(functools.partial(modulate, kk))

        stage_cp(0, 1, k).wait()

        @pl.when(fresh)
        def _():
            stage_cp(0, 0, k1).wait()

        w0 = pl.multiple_of(t * (32 * PITCH) + k * (KP // 2), 32)
        xrow = pl.multiple_of(jnp.where(i >= NPC - 1, PRE, 0), PRE)
        done = {}
        nd = 0
        for h in range(H):
            hh, l = h // 16, h % 16
            w = _unpk(w_v[pl.ds(w0 + (hh * 16 + (l % 2) * 8 + l // 2) * PITCH, KP // 2), :])
            q0 = pl.multiple_of(t * (4 * EP), 32) + ring_of(hh, l)[1] + QOFF // 2
            for rb in range(PRE // BM):
                lhs = _tie(h0_v[k, rb * 64:(rb + 1) * 64, :], done.pop(nd, None))
                rows = slice(rb * BM, (rb + 1) * BM)
                y = _dot(_unpk(lhs), w) + jnp.where(k > 0, acc_v[h, rows, :], 0.0)
                acc_v[h, rows, :] = y
                rings[l // 2][pl.ds(q0 + rb * 64, 64), :] = _pk(y)
                nd += 1
            if l < 15:
                n = 9 if l < 8 else 8
                p0_ = l * 9 if l < 8 else 72 + (l - 8) * 8
                if hh == 0:
                    repack(1, 2 * t + 1 + zero_s[0], k * (KP // 2) + p0_, n)
                else:
                    repack(0, 2 * t1, k1 * (KP // 2) + p0_, n)
            if h % 4 == 1 and h < 12:
                done[nd + 16] = ride(xrow + (h // 4) * RC, h // 4)
        @pl.when(jnp.logical_or(i == 4, i == 5))
        def _():
            x_cp(i - 2).start()

        for tt in range(1, 3):
            @pl.when(jnp.logical_and(i >= 3, (i + 3) >> 2 == tt))
            def _():
                stage_cp(tt, 1, (i + 3) & 3).start()

            @pl.when(jnp.logical_and(i >= 3, t + 1 == tt))
            def _():
                stage_cp(tt, 0, k).start()

        @pl.when(jnp.logical_and(i >= 3, i <= 10))
        def _():
            mod1_cp(i - 3).start()

        @pl.when(i == 6)
        def _():
            wo_cp(0).start()

        @pl.when(i == 8)
        def _():
            wo_cp(1).start()
        return c
    lax.fori_loop(1, 3 * NPC, pre_body, 0)

    for cp in (w1_cp, w2_cp, w3_cp, w4_cp):
        cp.start()
    for q in range(2 * NPC):
        mod1_cp(q).wait()
    x_cp(2).wait()
    x_cp(3).wait()
    wo_cp(0).wait()
    wo_cp(1).wait()

    L2 = 2 * (SEG + MEM)
    r = lax.broadcasted_iota(jnp.int32, (L2, L2), 0)
    c = lax.broadcasted_iota(jnp.int32, (L2, L2), 1)
    r1 = ((r >= SEG) & (r < 2 * SEG)) | (r >= 2 * SEG + MEM)
    c1 = ((c >= SEG) & (c < 2 * SEG)) | (c >= 2 * SEG + MEM)
    same = r1 == c1
    mask = same & ((r >= 2 * SEG) | (c >= 2 * SEG) | (c <= r))
    fill = jnp.where(same, -1e9 / SCALE, -jnp.inf).astype(f32)

    def p0(tok, w):
        rows = pl.ds(tok, RC)
        xa = x_v[rows, :].astype(f32) + mod(2) * a_v[rows, :].astype(f32)
        hb = _ln(xa) * (1.0 + mod(4)) + mod(3)
        xa_v[pl.ds(w, RC), :] = xa
        hb_v[pl.ds(w, RC), :] = hb
        y = _pk(_ln(hb))
        y1_v[pl.ds(w // 2 if isinstance(w, int) else pl.multiple_of(w >> 1, 8), RC // 2), :] = y
        return y

    def step(i, mem, zero, left):
        j = 0 if left is None else 1
        woff = pl.multiple_of((XR * i) % EP, 8) + j * (XR // 2)
        roff = pl.multiple_of((SEG * i + QOFF // 2) % EP, SEG) + j * (SEG // 2)
        arow = pl.multiple_of(2 * SEG * i, 2 * SEG) + j * SEG
        acc = [None] * NT
        ym, ps, ol, part, rest = {}, {}, {}, {}, {}
        HK = D // 2
        tiles = [_unpk(jnp.concatenate(
            [hx_v[k, j * (XR // 2):(j + 1) * (XR // 2), :] | zero, mem[k]], axis=0))
            for k in range(NT)]
        mem_new = []

        def lhs(lo, hi):
            return jnp.concatenate(tiles[lo // 128:hi // 128], axis=1)

        def qkv_lo(h, t):
            part[(t, h)] = _dot(lhs(0, HK), w_slab(2 * t + h // 16, h % 16, 0, HK))

        def proj(t, h):
            ch, l = 2 * t + h // 16, h % 16
            if (t, h) in part:
                y = _dot(lhs(HK, D), w_slab(ch, l, HK, D)) + part.pop((t, h))
            else:
                y = _dot(lhs(0, D), w_slab(ch, l))
            rg, ix = ring_of(ch, l)
            rg[pl.ds(ix + woff, XR // 2), :] = _pk(y[0:XR])
            ym[(t, h)] = y[XR:XR + MEM]

        def get(t, p):
            rg, i0 = ring_of(2 * t + p // 8, (2 * p) % 16)
            _, i1 = ring_of(2 * t + p // 8, (2 * p) % 16 + 1)
            mm = jnp.concatenate([ym.pop((t, 2 * p)), ym.pop((t, 2 * p + 1))], axis=0)
            return _unpk(jnp.concatenate(
                [rg[pl.ds(i0 + roff, SEG // 2), :], rg[pl.ds(i1 + roff, SEG // 2), :], _pk(mm)],
                axis=0))

        def sm(p):
            sc = lax.dot_general(get(0, p), get(1, p), (((1,), (1,)), ((), ())),
                                 preferred_element_type=f32)
            sc = jnp.where(mask, sc, fill)
            e = jnp.exp2((sc - jnp.max(sc, axis=-1, keepdims=True)) * (SCALE * LOG2E))
            ps[p] = (e * pl.reciprocal(jnp.sum(e, axis=-1, keepdims=True), approx=True)
                     ).astype(bf16)

        def pv(p):
            o = _dot(ps.pop(p), get(2, p))
            for b in range(2):
                h = 2 * p + b
                ox = o[SEG * b:SEG * (b + 1)]
                om = o[2 * SEG + MEM * b:2 * SEG + MEM * (b + 1)]
                if left is None:
                    ol[h] = jnp.concatenate([ox[0:XR], om], axis=0).astype(bf16)
                    rest[h] = ox[XR:SEG]
                else:
                    ol[h] = jnp.concatenate([ox, left[h], om], axis=0).astype(bf16)

        def wo(n, h0, h1, after=None):
            for h in range(h0, h1):
                o = ol[h]
                if after is not None and h == h0:
                    o = _unpk(_tie(pltpu.bitcast(o, u32), after))
                y = _dot(o, wo_v[h * DH:(h + 1) * DH, tile(n)])
                acc[n] = y if acc[n] is None else y + acc[n]
            if h1 == H:
                if left is None:
                    a_v[pl.ds(arow, XR), tile(n)] = acc[n][0:XR].astype(bf16)
                else:
                    a_v[pl.ds(arow, SEG), tile(n)] = acc[n][0:SEG].astype(bf16)
                    a_v[pl.ds(arow - (SEG - XR), SEG - XR), tile(n)] = (
                        acc[n][SEG:2 * SEG - XR].astype(bf16))
                mem_new.append(_pk(acc[n][-MEM:]))

        seq = []
        for p in range(NPAIR):
            seq += [(0, 2 * p), (1, 2 * p), (0, 2 * p + 1), (1, 2 * p + 1),
                    (2, 2 * p), (2, 2 * p + 1)]
        events = {}
        for p in range(NPAIR):
            at = seq.index((1, 2 * p + 1)) + DS
            events.setdefault(at, []).append((sm, p))
            events.setdefault(at + DP, []).append((pv, p))
        for t, h in seq[:NLO]:
            qkv_lo(h, t)
        side = {}
        if j == 1:
            macc = None
            for u in range(14):
                for g in range(u * 128 // 14, (u + 1) * 128 // 14):
                    wmg = wm_v[(i + 4) & 7, g * 8:(g + 1) * 8, :].astype(f32)
                    pr = wmg * jnp.concatenate([cb_v[g * 8:(g + 1) * 8, :]] * (MJ // 128), axis=1)
                    macc = pr if macc is None else macc + pr
                side[16 + u] = pltpu.bitcast(macc, u32)
            modr_v[i & 7] = jnp.broadcast_to(jnp.sum(macc, axis=0, keepdims=True), (8, MJ))
            nx = pl.multiple_of(PRE + 2 * XR * jnp.minimum(i + 1, NSEG // 2 - 1), RC)
            for q in range(2 * XR // RC):
                side[6 + 3 * q] = ride(nx + q * RC, q)
            tok = pl.multiple_of(jnp.clip(i - 22, 0, BM // RC) * RC, RC)
            side[15] = p0(tok, tok)
            for q in range(2 * NPC):
                mod_v[:, 2 * D + q * MJ:2 * D + (q + 1) * MJ] = modr_v[q]
        WU = HE // 8
        for d in range(len(seq) + NT * WU):
            if d < len(seq):
                proj(*seq[d])
            else:
                u = d - len(seq)
                wo(u // WU, (u % WU) * 8, (u % WU + 1) * 8, side.pop(u, None))
            for fn, p in events.pop(d, []):
                fn(p)
        assert not events
        u = NT * WU
        for n in range(NT):
            for h0 in range(HE, H, 8):
                wo(n, h0, h0 + 8, side.pop(u, None))
                u += 1
        assert not side
        return mem_new, rest

    def steps(i, carry):
        zero = zero_s[0].astype(u32)
        mem = [mem_v[:, tile(k)] for k in range(NT)]
        mem, rest = step(i, mem, zero, None)
        mem, _ = step(i, mem, zero, rest)
        for k in range(NT):
            mem_v[:, tile(k)] = mem[k]
        return carry
    lax.fori_loop(0, NSEG // 2, steps, 0)

    for cp in (w1_cp, w2_cp, w3_cp, w4_cp):
        cp.wait()

    for n in range(NT):
        g_v[n, 0:8, :] = jnp.zeros((8, 128), f32)
        g_v[n, 8:8 + SH, :] = _gelu(_dot(_unpk(y1_v[0:SH // 2, :]), w1_v[:, tile(n)]))

    HM = BM // 2
    shift = (-1, 1, -2, 2)

    def blk(j, c):
        r0 = pl.multiple_of(j * BM, BM)
        nxt = pl.multiple_of(jnp.minimum(j + 1, NB - 1) * BM + SH, SH)
        more = j < NB - 1

        def w1_half(hf):
            for n in range(NT):
                g = _gelu(_dot(_unpk(y1_v[8 + hf * 32:8 + (hf + 1) * 32, :]), w1_v[:, tile(n)]))
                w0 = 8 + SH + hf * HM
                if hf == 0:
                    g_v[n, w0:w0 + HM, :] = g
                else:
                    g_v[n, w0:w0 + HM - SH, :] = g[0:HM - SH]
                    g_v[n, w0 + HM - SH:w0 + HM, :] = jnp.where(more, g[HM - SH:HM], 0.0)

        def w2_half(hf):
            for n in range(NT):
                w0 = 8 + hf * HM + shift[n // 2]
                z_v[hf * 32:(hf + 1) * 32, tile(n)] = _pk(g_v[n, w0:w0 + HM, :])
            for n in range(NT):
                x1_v[hf * HM:(hf + 1) * HM, tile(n)] = (
                    _dot(_unpk(z_v[hf * 32:(hf + 1) * 32, :]), w2_v[:, tile(n)])
                    + hb_v[hf * HM:(hf + 1) * HM, tile(n)])

        def p1_half(hf):
            for k in range(hf * HM // RC, (hf + 1) * HM // RC):
                x1 = x1_v[k * RC:(k + 1) * RC, :]
                y2_v[k * 8:(k + 1) * 8, :] = _pk(_ln(x1))
                base_v[k * RC:(k + 1) * RC, :] = xa_v[k * RC:(k + 1) * RC, :] + mod(5) * x1

        def w3(f, lo, hi):
            u_v[lo:hi, tile(f)] = _pk(_gelu(_dot(_unpk(y2_v[lo:hi, :]), w3_v[:, tile(f)])))

        w1_half(0)
        w1_half(1)
        w2_half(0)
        w2_half(1)
        p1_half(0)
        for f in range(NSPLIT):
            w3(f, 0, 32)
        p1_half(1)
        for f in range(NSPLIT):
            w3(f, 32, 64)
        for n in range(NT):
            g_v[n, 0:8 + SH, :] = g_v[n, BM:BM + 8 + SH, :]
        xa_v[0:SH, :] = xa_v[BM:BM + SH, :]
        hb_v[0:SH, :] = hb_v[BM:BM + SH, :]
        for f in range(NSPLIT, NF):
            w3(f, 0, 64)
        ys = {}

        def prep(k):
            if k < BM // RC:
                ys[k] = p0(nxt + k * RC, SH + k * RC)

        prep(0)
        for n in range(NT):
            prep(n + 1)
            gb = mod(5, n * 128, (n + 1) * 128)
            u = _unpk(_tie(u_v[...], ys.pop(n), 16))
            a_v[pl.ds(r0, BM), tile(n)] = (
                base_v[:, tile(n)] + gb * _dot(u, w4_v[:, tile(n)])).astype(bf16)
            if n >= NT - 2:
                cols = pl.ds(0, (NT - 1) * 128) if n == NT - 2 else pl.ds(n * 128, 128)
                pltpu.make_async_copy(a_v.at[pl.ds(r0, BM), cols], out_hbm.at[pl.ds(r0, BM), cols],
                                      sem_out).start()
        return c
    lax.fori_loop(0, NB, blk, 0)
    pltpu.make_async_copy(a_v.at[pl.ds(0, S)], out_hbm, sem_out).wait()


@functools.partial(jax.jit, static_argnames=("A_seg_len",))
def pallas_adaLN_cond__memory_aug_recurrent_mem_tr__mixer_s_mlp__prompt_kernel(
    A_x: jax.Array,
    A_mem0: jax.Array,
    A_Wq: jax.Array,
    A_Wk: jax.Array,
    A_Wv: jax.Array,
    A_Wo: jax.Array,
    A_seg_len,
    B_x: jax.Array,
    B_w1: jax.Array,
    B_w2: jax.Array,
    B_w3: jax.Array,
    B_w4: jax.Array,
    c: jax.Array,
    w_mod: jax.Array,
):
    assert A_seg_len == SEG and A_x.shape == (1, S, D) and A_Wq.shape == (D, H, DH)
    any_spec = pl.BlockSpec(memory_space=pl.ANY)
    out = pl.pallas_call(
        _kernel,
        out_shape=jax.ShapeDtypeStruct((S, D), bf16),
        in_specs=[any_spec] * 12,
        out_specs=any_spec,
        scratch_shapes=[
            pltpu.VMEM((1, 3 * D), bf16),
            pltpu.VMEM((S + SH, D), bf16),
            pltpu.VMEM((S + SH, D), bf16),
            pltpu.VMEM((D // KP, PRE // 2, KP), u32),
            pltpu.VMEM((MEM // 2, D), u32),
            pltpu.VMEM((MEM, D), bf16),
            pltpu.VMEM((8, 6 * D), f32),
            pltpu.VMEM((8, 8, MJ), f32),
            pltpu.VMEM((D, 128), f32),
            pltpu.VMEM((8, D), u32),
            pltpu.VMEM((8, D, MJ), bf16),
            pltpu.VMEM((96 * PITCH + 544, 128), u32),
            pltpu.VMEM((H * DH, D + PADL), bf16),
            pltpu.VMEM((D, D + PADL), bf16),
            pltpu.VMEM((D, D + PADL), bf16),
            pltpu.VMEM((D, F + PADL), bf16),
            pltpu.VMEM((F, D + PADL), bf16),
            pltpu.VMEM((NT, BM + 32, 128), f32),
            pltpu.VMEM((BM + SH, D), f32),
            pltpu.VMEM((BM + SH, D), f32),
            pltpu.VMEM((BM, D), f32),
            pltpu.VMEM((BM, D), f32),
            pltpu.VMEM(((BM + SH) // 2, D), u32),
            pltpu.VMEM((BM // 2, D), u32),
            pltpu.VMEM((BM // 2, D), u32),
            pltpu.VMEM((BM // 2, F), u32),
            pltpu.VMEM((2, D, 16, DH), bf16),
            pltpu.VMEM((PRE, D), f32),
            pltpu.VMEM((NT, 32, 128), u32),
            pltpu.VMEM((H, PRE, DH), f32),
        ] + [pltpu.VMEM((12 * EP, DH), u32)] * 8 + [
            pltpu.SMEM((1,), jnp.int32),
            pltpu.SemaphoreType.DMA((2,)),
            pltpu.SemaphoreType.DMA((2, 4)),
            pltpu.SemaphoreType.DMA((4,)),
            pltpu.SemaphoreType.DMA((5,)),
            pltpu.SemaphoreType.DMA(()),
        ],
        compiler_params=pltpu.CompilerParams(vmem_limit_bytes=120 * 1024 * 1024),
    )(A_x.reshape(S, D), A_mem0.reshape(MEM, D), A_Wq, A_Wk, A_Wv, A_Wo.reshape(H * DH, D),
      B_w1, B_w2, B_w3, B_w4, c, w_mod)
    return out.reshape(1, S, D)
```
